```python
import jax
import jax.numpy as jnp

def _softmax(x, axis=-1):
    return jax.nn.softmax(x, axis=axis)

def _gelu(x):
    return jax.nn.gelu(x, approximate=True)

def _silu(x):
    return jax.nn.silu(x)

def _sigmoid(x):
    return jax.nn.sigmoid(x)

def _layernorm(x, axis=-1, eps=1e-05):
    m = jnp.mean(x, axis=axis, keepdims=True)
    v = jnp.var(x, axis=axis, keepdims=True)
    return (x - m) / jnp.sqrt(v + eps)

def _scatter_add(tgt, idx, src, axis=0):
    return tgt.at[idx].add(src)

def _segment_sum(src, seg, n):
    return jax.ops.segment_sum(src, seg, n)

class _Rng:

    def __init__(self, key):
        self._k = key

    def _next(self):
        self._k, sub = jax.random.split(self._k)
        return sub

    def normal(self, shape):
        return jax.random.normal(self._next(), shape, dtype=jnp.bfloat16)

    def randint(self, lo, hi, shape):
        return jax.random.randint(self._next(), shape, lo, hi, dtype=jnp.int32)

    def uniform(self, shape, lo=0.0, hi=1.0):
        return jax.random.uniform(self._next(), shape, jnp.bfloat16, lo, hi)

    def permutation(self, n):
        return jax.random.permutation(self._next(), n)
kernel_name = 'interleave_layers__sliding_local_dilated__memory_aug_infini_attn__prompt'

def setup_inputs():
    _rng = _Rng(jax.random.key(int.from_bytes(__import__("os").urandom(4), "little")))
    _w = lambda a: (lambda t: t.astype(jnp.bfloat16) if jnp.issubdtype(t.dtype, jnp.floating) else t)(jnp.asarray(a))

    def _A_setup():
        B, S, D = (1, 2048, 1024)
        return {'x': _w((lambda *s: _rng.normal(s) * 0.05)(B, S, D)), 'wqkv': _w((lambda *s: _rng.normal(s) * 0.05)(D, 3 * D)), 'wo': _w((lambda *s: _rng.normal(s) * 0.05)(D, D))}
    _A_in = _A_setup()

    def _B_setup():
        B, S, D, H = (1, 2048, 1024, 32)
        N = 4
        L = max(1, S // N)
        sc = D ** (-0.5)
        return {'x': _w((lambda *s: _rng.normal(s) * 0.05)(B, N * L, D)), 'wq': _w((lambda *s: _rng.normal(s) * 0.05)(D, D) * sc), 'wk': _w((lambda *s: _rng.normal(s) * 0.05)(D, D) * sc), 'wv': _w((lambda *s: _rng.normal(s) * 0.05)(D, D) * sc), 'wo': _w((lambda *s: _rng.normal(s) * 0.05)(D, D) * sc), 'beta': _w((lambda *s: _rng.normal(s) * 0.05)(H))}
    _B_in = _B_setup()
    return {'A_x': _A_in['x'], 'A_wqkv': _A_in['wqkv'], 'A_wo': _A_in['wo'], 'B_x': _B_in['x'], 'B_wq': _B_in['wq'], 'B_wk': _B_in['wk'], 'B_wv': _B_in['wv'], 'B_wo': _B_in['wo'], 'B_beta': _B_in['beta']}

def reference(A_x, A_wqkv, A_wo, B_x, B_wq, B_wk, B_wv, B_wo, B_beta):

    def _A_ref(x, wqkv, wo):
        B, S, D = x.shape
        H = 32
        Dh = D // H
        W, dil = (8, 2)
        qkv = (lambda x, *d: x.transpose(*d))((x @ wqkv).reshape(B, S, 3, H, Dh), 2, 0, 3, 1, 4)
        q, k, v = (qkv[0], qkv[1], qkv[2])
        scale = Dh ** (-0.5)
        pos = jnp.arange(S)
        off = jnp.arange(W) * dil
        idx = pos[:, None] - off[None, :]
        mask = idx >= 0
        idx_c = jnp.where(mask, idx, 0).reshape(-1)
        kg = k[:, :, idx_c, :].reshape(B, H, S, W, Dh)
        vg = v[:, :, idx_c, :].reshape(B, H, S, W, Dh)
        logits = jnp.einsum('bhsd,bhswd->bhsw', q, kg) * scale
        logits = jnp.where(mask[None, None, :, :], logits, -1000000000.0)
        attn = _softmax(logits, axis=-1)
        o = jnp.einsum('bhsw,bhswd->bhsd', attn, vg)
        return (lambda x, *d: x.transpose(*d))(o, 0, 2, 1, 3).reshape(B, S, D) @ wo

    def _B_ref(x, wq, wk, wv, wo, beta):
        B, S, D = x.shape
        H = 32
        Dh = D // H
        N = 4
        L = S // N
        q = (lambda x, *d: x.transpose(*d))((x @ wq).reshape(B, S, H, Dh), 0, 2, 1, 3).reshape(B, H, N, L, Dh)
        k = (lambda x, *d: x.transpose(*d))((x @ wk).reshape(B, S, H, Dh), 0, 2, 1, 3).reshape(B, H, N, L, Dh)
        v = (lambda x, *d: x.transpose(*d))((x @ wv).reshape(B, S, H, Dh), 0, 2, 1, 3).reshape(B, H, N, L, Dh)
        phi = lambda t: jnp.where(t > 0, t + 1.0, jnp.exp(t))
        scale = Dh ** (-0.5)
        ar = jnp.arange(L)
        mask = (lambda x, dt: x.astype(dt))(ar[:, None] < ar[None, :], x.dtype) * -1000000000.0
        g = _sigmoid(beta).reshape(1, H, 1, 1)
        M = jnp.einsum('bhd,bhe->bhde', q[:, :, 0, 0, :] * 0.0, q[:, :, 0, 0, :] * 0.0)
        z = q[:, :, 0, 0, :] * 0.0
        outs = []
        for s in range(N):
            qs, ks, vs = (q[:, :, s].copy(), k[:, :, s].copy(), v[:, :, s].copy())
            logits = jnp.einsum('bhqd,bhkd->bhqk', qs, ks) * scale + mask
            p = _softmax(logits, axis=-1)
            a_dot = jnp.einsum('bhqk,bhkd->bhqd', p, vs)
            pq = phi(qs)
            num = jnp.einsum('bhld,bhde->bhle', pq, M)
            den = jnp.einsum('bhld,bhd->bhl', pq, z)[..., None] + 1e-06
            a_mem = num / den
            o = g * a_mem + (1.0 - g) * a_dot
            outs.append(o)
            pk = phi(ks)
            M = M + jnp.einsum('bhld,bhle->bhde', pk, vs)
            z = z + jnp.einsum('bhld->bhd', pk)
        o = (lambda x, *d: x.transpose(*d))(jnp.stack(outs, 2).reshape(B, H, S, Dh), 0, 2, 1, 3).reshape(B, S, D)
        return o @ wo
    x = A_x
    x = x + _A_ref(_layernorm(x, axis=-1), A_wqkv, A_wo)
    x = x + _B_ref(_layernorm(x, axis=-1), B_wq, B_wk, B_wv, B_wo, B_beta)
    x = x + _A_ref(_layernorm(x, axis=-1), A_wqkv, A_wo)
    x = x + _B_ref(_layernorm(x, axis=-1), B_wq, B_wk, B_wv, B_wo, B_beta)
    return x
```

```python
import numpy as np
import jax
import jax.numpy as jnp
from jax import lax
import jax.experimental.pallas as pl
import jax.experimental.pallas.tpu as pltpu

S, D, H, DH = 2048, 1024, 32, 32
NSEG, L = 4, 512
NT = D // 128
WIN, DIL = 8, 2
HALO = 16
RC = L // NT
MZ_ROWS = 128 + 32
LOG2E = 1.4426950408889634
QSCALE = float(DH ** -0.5 * LOG2E)
MASKVAL = float(-1e9 * LOG2E)

F32, BF16, U32 = jnp.float32, jnp.bfloat16, jnp.uint32
_NT_DIMS = (((1,), (1,)), ((), ()))


def _iota(shape, axis):
    return lax.broadcasted_iota(jnp.int32, shape, axis)


def _dot(a, b):
    return jnp.dot(a, b, preferred_element_type=F32)


def _dot_nt(a, b):
    return lax.dot_general(a, b, _NT_DIMS, preferred_element_type=F32)


def _phi(t):
    return jnp.where(t > 0, t + 1.0, jnp.exp(t))


def _tree(op, xs):
    xs = list(xs)
    while len(xs) > 1:
        xs = [op(xs[i], xs[i + 1]) if i + 1 < len(xs) else xs[i]
              for i in range(0, len(xs), 2)]
    return xs[0]


def _kernel(x_hbm, wqkv_hbm, awo_hbm, wq_hbm, wk_hbm, wv_hbm, wo_hbm, beta_ref,
            out_hbm,
            x0, x1, x2, x3, wa, wao, wtmp, wb, wbo,
            xn0, xn1, o0, o1,
            qa0, qa1, ka0, ka1, va0, va1,
            qs0, qs1, pq0, pq1, kb0, kb1, pk0, pk1, vt0, vt1,
            mz, gtab, sem_x, sem_w, sem_o):
    X = (x0, x1, x2, x3)
    XN, O = (xn0, xn1), (o0, o1)
    QA, KA, VA = (qa0, qa1), (ka0, ka1), (va0, va1)
    QS, PQ, KB, PK, VT = (qs0, qs1), (pq0, pq1), (kb0, kb1), (pk0, pk1), (vt0, vt1)

    def col(t):
        return pl.ds(t * 128, 128)

    def x_copies(s):
        return [pltpu.make_async_copy(x_hbm.at[pl.ds(s * L, L), col(t)],
                                      X[s].at[t], sem_x.at[s]) for t in range(NT)]

    def out_copies(s):
        return [pltpu.make_async_copy(X[s].at[t], out_hbm.at[pl.ds(s * L, L), col(t)],
                                      sem_o.at[s]) for t in range(NT)]

    def w_copies(src, src0, dst, dst0, k):
        return [pltpu.make_async_copy(src.at[:, col(src0 + t)], dst.at[dst0 + t],
                                      sem_w.at[k]) for t in range(NT)]

    wa_c = [w_copies(wqkv_hbm, NT * i, wa, NT * i, i) for i in range(3)]
    wao_c = w_copies(awo_hbm, 0, wao, 0, 3)
    wb_c = [w_copies(w, 0, wb, NT * i, 4 + i) for i, w in enumerate((wq_hbm, wk_hbm, wv_hbm))]
    wbo_c = w_copies(wo_hbm, 0, wbo, 0, 7)

    def start(cs):
        for c in cs:
            c.start()

    def wait(cs):
        for c in cs:
            c.wait()

    def permute_cols(base):
        rows = 64

        def body(i, c):
            r = pl.ds(pl.multiple_of(i * rows, rows), rows)
            slot = (_iota((rows // 2, 128), 1) >> 1) & 7
            v = [pltpu.bitcast(wa[base + t, r, :], U32) for t in range(NT)]
            v = [x if t == 0 else pltpu.roll(x, 2 * t, 1) for t, x in enumerate(v)]
            v = [v[(-b) % NT] for b in range(NT)]
            for bit in (1, 2, 4):
                m = (slot & bit) != 0
                v = [jnp.where(m, v[(b - bit) % NT], v[b]) for b in range(NT)]
            for b in range(NT):
                y = v[b] if b == 0 else pltpu.roll(v[b], 128 - 2 * b, 1)
                wa[base + b, r, :] = pltpu.bitcast(y, BF16)
            return c

        lax.fori_loop(0, D // rows, body, 0)

    def permute_rows():
        def body(t, c):
            wtmp[...] = pltpu.bitcast(wao[t], U32)
            for b in range(NT):
                parts = [wtmp[pl.ds(8 * u + b, 8, stride=64), :] for u in range(8)]
                wao[t, pl.ds(b * 128, 128), :] = pltpu.bitcast(
                    jnp.concatenate(parts, axis=0), BF16)
            return c

        lax.fori_loop(0, NT, body, 0)

    def lhs(ref):
        return jnp.concatenate([ref[t] for t in range(NT)], axis=1)

    def ln_stage(n, g):
        src, dst = X[n % NSEG], XN[n % 2]
        for c in range(RC // 16):
            r = pl.ds(pl.multiple_of(g * RC + c * 16, 16), 16)
            xs = [src[t, r, :].astype(F32) for t in range(NT)]
            mean = jnp.sum(_tree(jnp.add, xs), axis=1, keepdims=True) * (1.0 / D)
            xc = [x - mean for x in xs]
            var = jnp.sum(_tree(jnp.add, [x * x for x in xc]), axis=1, keepdims=True) * (1.0 / D)
            inv = lax.rsqrt(var + 1e-5)
            for t in range(NT):
                dst[t, r, :] = (xc[t] * inv).astype(BF16)

    def proj_a(n, g, which):
        p = n % 2
        y = _dot(lhs(XN[p]), wa[which * NT + g])
        if which == 0:
            QA[p][g] = y
            return
        buf = KA if which == 1 else VA
        buf[p][g, pl.ds(HALO, L), :] = y
        if n % NSEG == 0:
            buf[p][g, pl.ds(0, HALO), :] = jnp.zeros((HALO, 128), F32)
        else:
            buf[p][g, pl.ds(0, HALO), :] = buf[1 - p][g, pl.ds(L, HALO), :]

    def proj_b(n, g, which):
        p = n % 2
        y = _dot(lhs(XN[p]), wb[which * NT + g])
        if which == 0:
            QS[p][g] = (y * QSCALE).astype(BF16)
            PQ[p][g] = _phi(y).astype(BF16)
        elif which == 1:
            KB[p][g] = y.astype(BF16)
            PK[p][g] = _phi(y).astype(BF16)
        else:
            VT[p][g] = y.astype(BF16).T

    def att_a_rows(n, g, c):
        p = n % 2
        lane = _iota((8, 128), 1)
        m1, m16 = (lane & 1) == 0, (lane & 16) == 0
        outs = []
        for half in range(2):
            off = c * 16 + half * 8
            r0 = pl.multiple_of(g * RC, RC) + off
            q = [QA[p][t, pl.ds(r0, 8), :] for t in range(NT)]
            lg = []
            for w in range(WIN):
                kr = pl.ds(r0 + HALO - DIL * w, 8)
                a = _tree(jnp.add, [q[t] * KA[p][t, kr, :] for t in range(NT)])
                a = a + jnp.where(m1, pltpu.roll(a, 127, 1), pltpu.roll(a, 1, 1))
                a = a + jnp.where(m16, pltpu.roll(a, 112, 1), pltpu.roll(a, 16, 1))
                a = a * QSCALE
                if n % NSEG == 0 and off < DIL * w:
                    a = jnp.where(_iota((8, 128), 0) + r0 >= DIL * w, a, MASKVAL)
                lg.append(a)
            m = _tree(jnp.maximum, lg)
            e = [jnp.exp2(a - m) for a in lg]
            inv = 1.0 / _tree(jnp.add, e)
            e = [a * inv for a in e]
            outs.append([
                _tree(jnp.add, [e[w] * VA[p][t, pl.ds(r0 + HALO - DIL * w, 8), :]
                                for w in range(WIN)])
                for t in range(NT)])
        r = pl.ds(pl.multiple_of(g * RC + c * 16, 16), 16)
        for t in range(NT):
            O[p][t, r, :] = jnp.concatenate([outs[0][t], outs[1][t]], axis=0).astype(BF16)

    def att_b_tile(n, g, j, mem):
        p = n % 2
        nk = 128 * (j + 1)
        rows = pl.ds(128 * j, 128)
        qw = pltpu.bitcast(QS[p][g, rows, :], U32)
        head = _iota((64, 128), 1) >> 5
        qcat = jnp.concatenate(
            [pltpu.bitcast(jnp.where(head == hh, qw, jnp.uint32(0)), BF16) for hh in range(4)],
            axis=0)
        st = _dot_nt(KB[p][g, pl.ds(0, nk), :], qcat)
        causal = jnp.where(_iota((128, 128), 0) > _iota((128, 128), 1), MASKVAL, 0.0)
        r = _dot_nt(mem, PQ[p][g, rows, :])
        ot = []
        for hh in range(4):
            s = st[:, 128 * hh:128 * (hh + 1)]
            diag = s[nk - 128:] + causal
            s = diag if j == 0 else jnp.concatenate([s[:nk - 128], diag], axis=0)
            m = jnp.max(s, axis=0, keepdims=True)
            e = jnp.exp2(s - m)
            l = jnp.sum(e, axis=0, keepdims=True)
            acc = _dot(VT[p][g, pl.ds(32 * hh, 32), pl.ds(0, nk)], e.astype(BF16))
            gate = gtab[pl.ds(4 * g + hh, 1), :]
            den = r[128 + 8 * hh:136 + 8 * hh] + 1e-6
            wm = gate / den
            wm = jnp.concatenate([wm] * 4, axis=0)
            ot.append(r[32 * hh:32 * hh + 32] * wm + acc * ((1.0 - gate) / l))
        O[p][g, rows, :] = jnp.concatenate(ot, axis=0).T.astype(BF16)

    def mem_load(n, g):
        if n % NSEG == 0:
            return jnp.zeros((MZ_ROWS, 128), F32)
        return mz[g]

    def mem_update(n, g, state):
        p = n % 2
        if n % NSEG == NSEG - 1:
            return
        a = jnp.concatenate([VT[p][g], jnp.ones((32, L), BF16)], axis=0)
        row = _iota((MZ_ROWS, 128), 0)
        row_head = jnp.where(row < 128, row >> 5, (row - 128) >> 3)
        keep = row_head == (_iota((MZ_ROWS, 128), 1) >> 5)
        mz[g] = state + jnp.where(keep, _dot(a, PK[p][g]), 0.0)

    def out_stage(n, g):
        w = wao if is_a(n) else wbo
        x = X[n % NSEG]
        x[g] = (x[g].astype(F32) + _dot(lhs(O[n % 2]), w[g])).astype(BF16)

    def is_a(n):
        return (n // NSEG) % 2 == 0

    def step(n, ln=True, proj=True, att=True, out=True):
        def body(g, c):
            mm = []
            if proj:
                f = proj_a if is_a(n + 1) else proj_b
                mm += [lambda w=w: f(n + 1, g, w) for w in range(3)]
            if out:
                mm.append(lambda: out_stage(n - 1, g))
            vec = []
            if att and is_a(n):
                vec += [lambda i=i: att_a_rows(n, g, i) for i in range(RC // 16)]
            elif att:
                state = mem_load(n, g)
                mem = state.astype(BF16)
                vec += [lambda j=j: att_b_tile(n, g, j, mem) for j in range(4)]
            for i in range(max(len(mm), len(vec))):
                if i < len(mm):
                    mm[i]()
                if i < len(vec):
                    vec[i]()
            if att and not is_a(n):
                mem_update(n, g, state)
            if ln:
                ln_stage(n + 2, g)
            return c

        lax.fori_loop(0, NT, body, 0)

    start(x_copies(0))
    for cs in wa_c:
        start(cs)
    start(x_copies(1))
    start(x_copies(2))
    start(wao_c)
    start(x_copies(3))
    for cs in wb_c:
        start(cs)
    start(wbo_c)

    gate = jax.nn.sigmoid(beta_ref[...].astype(F32))
    eye = _iota((H, H), 0) == _iota((H, H), 1)
    gcol = jnp.sum(jnp.where(eye, jnp.broadcast_to(gate, (H, H)), 0.0), axis=1, keepdims=True)
    gtab[...] = jnp.broadcast_to(gcol, (H, 128))

    wait(x_copies(0))
    step(-2, proj=False, att=False, out=False)
    for i in range(3):
        wait(wa_c[i])
        permute_cols(i * NT)
    wait(x_copies(1))
    step(-1, att=False, out=False)
    wait(x_copies(2))
    step(0, out=False)
    wait(wao_c)
    permute_rows()
    wait(x_copies(3))

    def pair(it, c):
        step(1)
        step(2)

        @pl.when(it == 0)
        def _():
            for cs in wb_c:
                wait(cs)
            wait(wbo_c)

        step(3)
        step(4)
        step(5)

        @pl.when(it == 1)
        def _():
            start(out_copies(0))

        step(6)

        @pl.when(it == 0)
        def _():
            step(7)
            step(8)

        return c

    lax.fori_loop(0, 2, pair, 0)
    start(out_copies(1))
    step(15, ln=False, proj=False)
    start(out_copies(2))
    step(16, ln=False, proj=False, att=False)
    start(out_copies(3))
    for s in range(NSEG):
        wait(out_copies(s))


@jax.jit
def pallas_interleave_layers__sliding_local_dilated__memory_aug_infini_attn__prompt_kernel(
    A_x: jax.Array,
    A_wqkv: jax.Array,
    A_wo: jax.Array,
    B_x: jax.Array,
    B_wq: jax.Array,
    B_wk: jax.Array,
    B_wv: jax.Array,
    B_wo: jax.Array,
    B_beta: jax.Array,
):
    del B_x
    assert A_x.shape == (1, S, D)
    hbm = pl.BlockSpec(memory_space=pl.ANY)
    act = pltpu.VMEM((NT, L, 128), BF16)
    scratch = (
        [act] * 4
        + [pltpu.VMEM((3 * NT, D, 128), BF16), pltpu.VMEM((NT, D, 128), BF16),
           pltpu.VMEM((D // 2, 128), U32),
           pltpu.VMEM((3 * NT, D, 128), BF16), pltpu.VMEM((NT, D, 128), BF16)]
        + [act] * 4
        + [pltpu.VMEM((NT, L, 128), F32)] * 2
        + [pltpu.VMEM((NT, HALO + L, 128), F32)] * 4
        + [act] * 8
        + [pltpu.VMEM((NT, 128, L), BF16)] * 2
        + [pltpu.VMEM((NT, MZ_ROWS, 128), F32), pltpu.VMEM((H, 128), F32),
           pltpu.SemaphoreType.DMA((NSEG,)), pltpu.SemaphoreType.DMA((8,)),
           pltpu.SemaphoreType.DMA((NSEG,))]
    )
    out = pl.pallas_call(
        _kernel,
        out_shape=jax.ShapeDtypeStruct((S, D), BF16),
        in_specs=[hbm] * 7 + [pl.BlockSpec(memory_space=pltpu.VMEM)],
        out_specs=hbm,
        scratch_shapes=scratch,
        compiler_params=pltpu.CompilerParams(vmem_limit_bytes=100 * 2**20),
        name="abab_stack",
    )(A_x.reshape(S, D), A_wqkv, A_wo, B_wq, B_wk, B_wv, B_wo, B_beta.reshape(1, H))
    return out.reshape(1, S, D)
```

```python
import jax
import jax.numpy as jnp
from jax import lax
import jax.experimental.pallas as pl
import jax.experimental.pallas.tpu as pltpu

S, D, H, DH = 2048, 1024, 32, 32
NSEG, L = 4, 512
HL = L // 2
NT = D // 128
NP = NT // 2
RC = HL // NP
WIN, DIL = 8, 2
HALO = 16
MZ_ROWS = 128 + 32
LOG2E = 1.4426950408889634
QSCALE = float(DH ** -0.5 * LOG2E)
MASKVAL = float(-1e9 * LOG2E)

F32, BF16, U32 = jnp.float32, jnp.bfloat16, jnp.uint32
_NT_DIMS = (((1,), (1,)), ((), ()))


def _iota(shape, axis):
    return lax.broadcasted_iota(jnp.int32, shape, axis)


def _dot(a, b):
    return jnp.dot(a, b, preferred_element_type=F32)


def _dot_nt(a, b):
    return lax.dot_general(a, b, _NT_DIMS, preferred_element_type=F32)


def _pack(x):
    return pltpu.bitcast(x.astype(BF16), U32)


def _bf(words):
    return pltpu.bitcast(words, BF16)


def _phi(t):
    return jnp.where(t > 0, t + 1.0, jnp.exp(t))


def _tree(op, xs):
    xs = list(xs)
    while len(xs) > 1:
        xs = [op(xs[i], xs[i + 1]) if i + 1 < len(xs) else xs[i]
              for i in range(0, len(xs), 2)]
    return xs[0]


def _lhs_terms(a11, a12, a21, a22):
    return (a11 + a22, a21 + a22, a11, a22, a11 + a12, a21 - a11, a12 - a22)


def _rhs_terms(b11, b12, b21, b22):
    return (b11 + b22, b11, b12 - b22, b21 - b11, b22, b11 + b12, b21 + b22)


def _kernel(x_hbm, wqkv_hbm, awo_hbm, wq_hbm, wk_hbm, wv_hbm, wo_hbm, beta_ref,
            out_hbm,
            x0, x1, x2, x3, wraw, wtmp, wa, wao, wb,
            xn0, xn1, o0, o1,
            qa0, qa1, ka0, ka1, va0, va1,
            qs0, qs1, pq0, pq1, kb0, kb1, pk0, pk1, vt0, vt1,
            mz, gtab, zero_ref, sem_x, sem_w, sem_o):
    X = (x0, x1, x2, x3)
    XN, O = (xn0, xn1), (o0, o1)
    QA, KA, VA = (qa0, qa1), (ka0, ka1), (va0, va1)
    QS, PQ, KB, PK, VT = (qs0, qs1), (pq0, pq1), (kb0, kb1), (pk0, pk1), (vt0, vt1)

    def col(t):
        return pl.ds(t * 128, 128)

    def x_copies(s):
        return [pltpu.make_async_copy(x_hbm.at[pl.ds(s * L, L), col(t)],
                                      X[s].at[t], sem_x.at[s]) for t in range(NT)]

    def out_copies(s):
        return [pltpu.make_async_copy(X[s].at[t], out_hbm.at[pl.ds(s * L, L), col(t)],
                                      sem_o.at[s]) for t in range(NT)]

    w_src = ((wqkv_hbm, 0), (wqkv_hbm, NT), (wqkv_hbm, 2 * NT), (awo_hbm, 0),
             (wq_hbm, 0), (wk_hbm, 0), (wv_hbm, 0), (wo_hbm, 0))

    def w_copies(m):
        src, t0 = w_src[m]
        return [pltpu.make_async_copy(src.at[:, col(t0 + t)], wraw.at[m, t], sem_w.at[m])
                for t in range(NT)]

    def start(cs):
        for c in cs:
            c.start()

    def wait(cs):
        for c in cs:
            c.wait()

    def token(*vals):
        bits = [pltpu.bitcast(v[:8, :128], U32) for v in vals]
        return _tree(jnp.bitwise_or, bits) & zero_ref[...]

    def after(words, tok):
        if tok is None:
            return words
        head = words[:8] | jnp.concatenate([tok] * (words.shape[1] // 128), axis=1)
        return jnp.concatenate([head, words[8:]], axis=0) if words.shape[0] > 8 else head

    def store_rhs(dst, m, i, r, b11, b12, b21, b22):
        for k, v in enumerate(_rhs_terms(b11, b12, b21, b22)):
            dst[m, i, k, r, :] = _pack(v)

    def prep_plain(src_m, dst, m, i):
        for c in range(4):
            r0, r1 = pl.ds(128 * c, 128), pl.ds(D // 2 + 128 * c, 128)
            store_rhs(dst, m, i, pl.ds(64 * c, 64),
                      wraw[src_m, i, r0, :].astype(F32), wraw[src_m, i + NP, r0, :].astype(F32),
                      wraw[src_m, i, r1, :].astype(F32), wraw[src_m, i + NP, r1, :].astype(F32))

    def prep_a_cols(m, i):
        rows = D // 2 // NP
        slot = (_iota((rows, 128), 1) >> 1) & 7
        r0 = pl.ds(pl.multiple_of(i * rows, rows), rows)
        r1 = pl.ds(pl.multiple_of(D // 2 + i * rows, rows), rows)
        v = [jnp.concatenate([pltpu.bitcast(wraw[m, t, r0, :], U32),
                              pltpu.bitcast(wraw[m, t, r1, :], U32)], axis=0) for t in range(NT)]
        v = [x if t == 0 else pltpu.roll(x, 2 * t, 1) for t, x in enumerate(v)]
        v = [v[(-b) % NT] for b in range(NT)]
        for bit in (1, 2, 4):
            sel = (slot & bit) != 0
            v = [jnp.where(sel, v[(b - bit) % NT], v[b]) for b in range(NT)]
        v = [_bf(x if b == 0 else pltpu.roll(x, 128 - 2 * b, 1)).astype(F32)
             for b, x in enumerate(v)]
        r = pl.ds(pl.multiple_of(i * (rows // 2), rows // 2), rows // 2)
        for j in range(NP):
            store_rhs(wa, m, j, r, v[j][:rows], v[j + NP][:rows], v[j][rows:], v[j + NP][rows:])

    def prep_a_rows(i):
        for h in range(2):
            wtmp[h] = pltpu.bitcast(wraw[3, i + h * NP], U32)

        def rows(h, b):
            parts = [wtmp[h, pl.ds(8 * u + b, 8, stride=64), :] for u in range(8)]
            return _bf(jnp.concatenate(parts, axis=0)).astype(F32)

        for c in range(4):
            store_rhs(wao, 0, i, pl.ds(64 * c, 64),
                      rows(0, c), rows(1, c), rows(0, c + NP), rows(1, c + NP))

    def store_lhs(dst, t, r, a11, a12, a21, a22):
        for k, v in enumerate(_lhs_terms(a11, a12, a21, a22)):
            dst[t, k, r, :] = _pack(v)

    def products(a_ref, w_ref, m, i, emit):
        st = {}

        def prod(k, tok):
            a = jnp.concatenate([a_ref[t, k] for t in range(NP)], axis=1)
            w = jnp.concatenate(
                [after(w_ref[m, i, k, pl.ds(64 * c, 64), :], tok) for c in range(NP)], axis=0)
            return _dot(_bf(a), _bf(w))

        def p1(tok):
            st["m1"] = r = prod(0, tok)
            return r

        def p2(tok):
            st["c21"] = r = prod(1, tok)
            st["c22"] = st["m1"] - r
            return r

        def p3(tok):
            st["c12"] = r = prod(2, tok)
            st["c22"] = st["c22"] + r
            return r

        def p4(tok):
            r = prod(3, tok)
            emit(1, i, st["c21"] + r)
            st["c11"] = st["m1"] + r
            return r

        def p5(tok):
            r = prod(4, tok)
            emit(0, i + NP, st["c12"] + r)
            st["c11"] = st["c11"] - r
            return r

        def p6(tok):
            r = prod(5, tok)
            emit(1, i + NP, st["c22"] + r)
            return r

        def p7(tok):
            r = prod(6, tok)
            emit(0, i, st["c11"] + r)
            return r

        return [p1, p2, p3, p4, p5, p6, p7]

    def ln_rows(n, i, off, nr):
        src, dst = X[n % NSEG], XN[n % 2]
        base = pl.multiple_of(i * RC, RC) + off
        xs = [jnp.concatenate([src[t, pl.ds(pl.multiple_of(base + h * HL, nr), nr), :]
                               for h in range(2)], axis=0).astype(F32) for t in range(NT)]
        mean = jnp.sum(_tree(jnp.add, xs), axis=1, keepdims=True) * (1.0 / D)
        xc = [x - mean for x in xs]
        var = jnp.sum(_tree(jnp.add, [x * x for x in xc]), axis=1, keepdims=True) * (1.0 / D)
        inv = lax.rsqrt(var + 1e-5)
        y = [x * inv for x in xc]
        r = pl.ds(pl.multiple_of((i * RC + off) // 2, nr // 2), nr // 2)
        for t in range(NP):
            store_lhs(dst, t, r, y[t][:nr], y[t + NP][:nr], y[t][nr:], y[t + NP][nr:])
        return [v[u:u + 8] for v in y for u in range(0, 2 * nr, 8)]

    def proj_a(n, i, which):
        p = n % 2

        def emit(h, t, y):
            if which == 0:
                QA[p][t, pl.ds(h * HL, HL), :] = y
                return
            buf = KA if which == 1 else VA
            buf[p][t, pl.ds(HALO + h * HL, HL), :] = y
            if h == 0 and n % NSEG == 0:
                buf[p][t, pl.ds(0, HALO), :] = jnp.zeros((HALO, 128), F32)
            elif h == 0:
                buf[p][t, pl.ds(0, HALO), :] = buf[1 - p][t, pl.ds(L, HALO), :]

        return products(XN[p], wa, which, i, emit)

    def proj_b(n, i, which):
        p = n % 2

        def emit(h, t, y):
            r = pl.ds(h * HL // 2, HL // 2)
            if which == 0:
                QS[p][t, r, :] = _pack(y * QSCALE)
                PQ[p][t, r, :] = _pack(_phi(y))
            elif which == 1:
                KB[p][t, r, :] = _pack(y)
                if n % NSEG != NSEG - 1:
                    PK[p][t, r, :] = _pack(_phi(y))
            else:
                VT[p][t, :, pl.ds(h * HL, HL)] = pltpu.bitcast(y.astype(BF16).T, U32)

        return products(XN[p], wb, which, i, emit)

    def out_stage(n, i):
        x = X[n % NSEG]

        def emit(h, t, y):
            r = pl.ds(h * HL, HL)
            x[t, r, :] = (x[t, r, :].astype(F32) + y).astype(BF16)

        if is_a(n):
            return products(O[n % 2], wao, 0, i, emit)
        return products(O[n % 2], wb, 3, i, emit)

    def att_a_probs(n, i, off):
        p = n % 2
        base = pl.multiple_of(i * RC, RC) + off
        starts = [base + h * HL + 8 * u for h in range(2) for u in range(2)]
        lg = [[None] * 4 for _ in range(WIN)]
        for u, r0 in enumerate(starts):
            q = [QA[p][t, pl.ds(r0, 8), :] for t in range(NT)]
            for w in range(WIN):
                kr = pl.ds(r0 + HALO - DIL * w, 8)
                lg[w][u] = _tree(jnp.add, [q[t] * KA[p][t, kr, :] for t in range(NT)])
        a = jnp.concatenate([v for row in lg for v in row], axis=0)
        lane = _iota(a.shape, 1)
        a = a + jnp.where((lane & 1) == 0, pltpu.roll(a, 127, 1), pltpu.roll(a, 1, 1))
        a = a + jnp.where((lane & 16) == 0, pltpu.roll(a, 112, 1), pltpu.roll(a, 16, 1))
        a = a * QSCALE
        lg = [a[32 * w:32 * (w + 1)] for w in range(WIN)]
        if n % NSEG == 0 and off == 0:
            row = _iota((32, 128), 0)
            pos = jnp.where(row < 16, row + base, HL)
            lg = [v if w == 0 else jnp.where(pos >= DIL * w, v, MASKVAL)
                  for w, v in enumerate(lg)]
        m = _tree(jnp.maximum, lg)
        e = [jnp.exp2(v - m) for v in lg]
        inv = 1.0 / _tree(jnp.add, e)
        return [v * inv for v in e]

    def att_a_values(n, i, off, e):
        p = n % 2
        base = pl.multiple_of(i * RC, RC) + off
        r = pl.ds(pl.multiple_of((i * RC + off) // 2, 8), 8)
        outs = []

        def mix(t, h):
            parts = []
            for u in range(2):
                r0, k = base + h * HL + 8 * u, 16 * h + 8 * u
                parts.append(_tree(jnp.add, [
                    e[w][k:k + 8] * VA[p][t, pl.ds(r0 + HALO - DIL * w, 8), :]
                    for w in range(WIN)]))
            outs.extend(parts)
            return jnp.concatenate(parts, axis=0)

        for t in range(NP):
            store_lhs(O[p], t, r, mix(t, 0), mix(t + NP, 0), mix(t, 1), mix(t + NP, 1))
        return outs

    def att_b_scores(n, g, j, mem, tok):
        p = n % 2
        rows = pl.ds(64 * j, 64)
        qw = after(QS[p][g, rows, :], tok)
        head = _iota((64, 128), 1) >> 5
        qcat = jnp.concatenate(
            [jnp.where(head == hh, qw, jnp.uint32(0)) for hh in range(4)], axis=0)
        r = _dot_nt(mem, _bf(after(PQ[p][g, rows, :], tok)))
        st = _dot_nt(_bf(KB[p][g, pl.ds(0, 64 * (j + 1)), :]), _bf(qcat))
        return st, r

    def att_b_values(n, g, j, st, r, tok):
        p = n % 2
        nk = 128 * (j + 1)
        causal = jnp.where(_iota((128, 128), 0) > _iota((128, 128), 1), MASKVAL, 0.0)
        ot, accs = [], []
        for hh in range(4):
            s = st[:, 128 * hh:128 * (hh + 1)]
            diag = s[nk - 128:] + causal
            s = diag if j == 0 else jnp.concatenate([s[:nk - 128], diag], axis=0)
            m = jnp.max(s, axis=0, keepdims=True)
            e = jnp.exp2(s - m)
            l = jnp.sum(e, axis=0, keepdims=True)
            vt = after(VT[p][g, pl.ds(16 * hh, 16), pl.ds(0, nk)], tok)
            acc = _dot(_bf(vt), e.astype(BF16))
            accs.append(acc)
            gate = gtab[pl.ds(4 * g + hh, 1), :]
            wm = gate / (r[128 + 8 * hh:136 + 8 * hh] + 1e-6)
            wm = jnp.concatenate([wm] * 4, axis=0)
            ot.append(r[32 * hh:32 * hh + 32] * wm + acc * ((1.0 - gate) / l))
        return jnp.concatenate(ot, axis=0).T, accs

    def mem_load(n, g):
        if n % NSEG == 0:
            return jnp.zeros((MZ_ROWS, 128), F32)
        return mz[g]

    def mem_update(n, g, state):
        p = n % 2
        if n % NSEG == NSEG - 1:
            return
        a = jnp.concatenate([_bf(VT[p][g]), jnp.ones((32, L), BF16)], axis=0)
        row = _iota((MZ_ROWS, 128), 0)
        row_head = jnp.where(row < 128, row >> 5, (row - 128) >> 3)
        keep = row_head == (_iota((MZ_ROWS, 128), 1) >> 5)
        mz[g] = state + jnp.where(keep, _dot(a, _bf(PK[p][g])), 0.0)

    def is_a(n):
        return (n // NSEG) % 2 == 0

    def run(mm, count, tok):
        r = None
        for _ in range(min(count, len(mm))):
            r = mm.pop(0)(tok)
            tok = None
        return r

    def step(n, ln=True, proj=(0, 1, 2), att=True, out=True, extra=None):
        def body(i, c):
            mm = []
            for which in proj:
                mm += (proj_a if is_a(n + 1) else proj_b)(n + 1, i, which)
            if out:
                mm += out_stage(n - 1, i)
            total = len(mm)
            if extra is not None:
                extra(i)
            if att and not is_a(n):
                groups = (i, i + NP)
                state = [mem_load(n, g) for g in groups]
                pieces = [(j, h) for j in (3, 1, 2, 0) for h in range(2)]
                share = [4, 4, 3, 3, 4, 4, 2, 2] if total == 28 else [1, 1, 1, 0, 1, 1, 1, 0]
                tiles, tok = {}, None
                for k, (j, h) in enumerate(pieces):
                    st, r = att_b_scores(n, groups[h], j, state[h].astype(BF16), tok)
                    tok = token(*[st[:, 128 * hh:] for hh in range(4)])
                    if ln and k in (2, 3, 6, 7) :
                        prev = run(mm, 1, tok)
                        off = 16 * (k % 2 + 2 * (k // 6))
                        tok = token(*ln_rows(n + 2, i, off, 16))
                        prev = run(mm, share[k] - 1, tok)
                    else:
                        prev = run(mm, share[k], tok)
                    tok = None if prev is None else token(prev)
                    tiles[j, h], accs = att_b_values(n, groups[h], j, st, r, tok)
                    tok = token(*accs) if total == 28 else None
                    if k % 4 == 3:
                        store_lhs(O[n % 2], i, pl.ds(64 * j, 64), tiles[j, 0], tiles[j, 1],
                                  tiles[j + 2, 0], tiles[j + 2, 1])
                for h in range(2):
                    mem_update(n, groups[h], state[h])
                run(mm, len(mm), tok)
                return c
            tok = None
            for off in range(0, RC, 16):
                per = total // 4
                if att:
                    run(mm, per // 2, tok)
                    e = att_a_probs(n, i, off)
                    tok = token(*[v[u:u + 8] for v in e for u in range(0, 32, 8)])
                    run(mm, per // 3, tok)
                    tok = token(*att_a_values(n, i, off, e))
                    per -= per // 2 + per // 3
                if ln:
                    run(mm, per - 1, tok)
                    tok = token(*ln_rows(n + 2, i, off, 16))
                    per = 1
                run(mm, per, tok)
                tok = None
            run(mm, len(mm), tok)
            return c

        lax.fori_loop(0, NP, body, 0)

    start(x_copies(0))
    for m in range(3):
        start(w_copies(m))
    start(x_copies(1))
    start(w_copies(3))
    start(x_copies(2))
    for m in range(4, 8):
        start(w_copies(m))
    start(x_copies(3))

    zero_ref[...] = jnp.zeros((8, 128), U32)
    gate = jax.nn.sigmoid(beta_ref[...].astype(F32))
    eye = _iota((H, H), 0) == _iota((H, H), 1)
    gcol = jnp.sum(jnp.where(eye, jnp.broadcast_to(gate, (H, H)), 0.0), axis=1, keepdims=True)
    gtab[...] = jnp.broadcast_to(gcol, (H, 128))

    wait(x_copies(0))
    step(-2, proj=(), att=False, out=False)
    wait(w_copies(0))
    step(-1, ln=False, proj=(), att=False, out=False, extra=lambda i: prep_a_cols(0, i))
    wait(w_copies(1))
    step(-1, ln=False, proj=(0,), att=False, out=False, extra=lambda i: prep_a_cols(1, i))
    wait(w_copies(2))
    step(-1, ln=False, proj=(1,), att=False, out=False, extra=lambda i: prep_a_cols(2, i))
    wait(x_copies(1))
    wait(w_copies(3))
    step(-1, proj=(2,), att=False, out=False, extra=prep_a_rows)
    wait(x_copies(2))
    for m in range(4, 8):
        wait(w_copies(m))

    def prep_b(i):
        for m in range(4):
            prep_plain(4 + m, wb, m, i)

    step(0, out=False, extra=prep_b)
    wait(x_copies(3))

    def pair(it, c):
        for n in range(1, 6):
            step(n)

        @pl.when(it == 1)
        def _():
            start(out_copies(0))

        step(6)

        @pl.when(it == 0)
        def _():
            step(7)
            step(8)

        return c

    lax.fori_loop(0, 2, pair, 0)
    start(out_copies(1))
    step(15, ln=False, proj=())
    start(out_copies(2))
    step(16, ln=False, proj=(), att=False)
    start(out_copies(3))
    for s in range(NSEG):
        wait(out_copies(s))


@jax.jit
def pallas_interleave_layers__sliding_local_dilated__memory_aug_infini_attn__prompt_kernel(
    A_x: jax.Array,
    A_wqkv: jax.Array,
    A_wo: jax.Array,
    B_x: jax.Array,
    B_wq: jax.Array,
    B_wk: jax.Array,
    B_wv: jax.Array,
    B_wo: jax.Array,
    B_beta: jax.Array,
):
    del B_x
    assert A_x.shape == (1, S, D)
    hbm = pl.BlockSpec(memory_space=pl.ANY)
    scratch = (
        [pltpu.VMEM((NT, L, 128), BF16)] * 4
        + [pltpu.VMEM((8, NT, D, 128), BF16),
           pltpu.VMEM((2, D // 2, 128), U32),
           pltpu.VMEM((3, NP, 7, D // 4, 128), U32),
           pltpu.VMEM((1, NP, 7, D // 4, 128), U32),
           pltpu.VMEM((4, NP, 7, D // 4, 128), U32)]
        + [pltpu.VMEM((NP, 7, HL // 2, 128), U32)] * 4
        + [pltpu.VMEM((NT, L, 128), F32)] * 2
        + [pltpu.VMEM((NT, HALO + L, 128), F32)] * 4
        + [pltpu.VMEM((NT, L // 2, 128), U32)] * 8
        + [pltpu.VMEM((NT, 64, L), U32)] * 2
        + [pltpu.VMEM((NT, MZ_ROWS, 128), F32), pltpu.VMEM((H, 128), F32),
           pltpu.VMEM((8, 128), U32),
           pltpu.SemaphoreType.DMA((NSEG,)), pltpu.SemaphoreType.DMA((8,)),
           pltpu.SemaphoreType.DMA((NSEG,))]
    )
    out = pl.pallas_call(
        _kernel,
        out_shape=jax.ShapeDtypeStruct((S, D), BF16),
        in_specs=[hbm] * 7 + [pl.BlockSpec(memory_space=pltpu.VMEM)],
        out_specs=hbm,
        scratch_shapes=scratch,
        compiler_params=pltpu.CompilerParams(vmem_limit_bytes=110 * 2**20),
        name="abab_stack",
    )(A_x.reshape(S, D), A_wqkv, A_wo, B_wq, B_wk, B_wv, B_wo, B_beta.reshape(1, H))
    return out.reshape(1, S, D)
```

```python
import jax
import jax.numpy as jnp
from jax import lax
import jax.experimental.pallas as pl
import jax.experimental.pallas.tpu as pltpu

S, D, H, DH = 2048, 1024, 32, 32
NSEG, L = 4, 512
HL = L // 2
NT = D // 128
NP = NT // 2
RC = HL // NP
WIN, DIL = 8, 2
HALO = 16
MZ_ROWS = 128 + 32
LOG2E = 1.4426950408889634
QSCALE = float(DH ** -0.5 * LOG2E)
MASKVAL = float(-1e9 * LOG2E)

F32, BF16, U32 = jnp.float32, jnp.bfloat16, jnp.uint32
_NT_DIMS = (((1,), (1,)), ((), ()))


def _iota(shape, axis):
    return lax.broadcasted_iota(jnp.int32, shape, axis)


def _dot(a, b):
    return jnp.dot(a, b, preferred_element_type=F32)


def _dot_nt(a, b):
    return lax.dot_general(a, b, _NT_DIMS, preferred_element_type=F32)


def _pack(x):
    return pltpu.bitcast(x.astype(BF16), U32)


def _bf(words):
    return pltpu.bitcast(words, BF16)


def _phi(t):
    return jnp.where(t > 0, t + 1.0, jnp.exp(t))


def _tree(op, xs):
    xs = list(xs)
    while len(xs) > 1:
        xs = [op(xs[i], xs[i + 1]) if i + 1 < len(xs) else xs[i]
              for i in range(0, len(xs), 2)]
    return xs[0]


def _lhs_terms(a11, a12, a21, a22):
    return (a11 + a22, a21 + a22, a11, a22, a11 + a12, a21 - a11, a12 - a22)


def _rhs_terms(b11, b12, b21, b22):
    return (b11 + b22, b11, b12 - b22, b21 - b11, b22, b11 + b12, b21 + b22)


def _kernel(x_hbm, wqkv_hbm, awo_hbm, wq_hbm, wk_hbm, wv_hbm, wo_hbm, beta_ref,
            out_hbm,
            x0, x1, x2, x3, wraw, wtmp, wa, wao, wb,
            xn0, xn1, o0, o1,
            qa0, qa1, ka0, ka1, va0, va1,
            qs0, qs1, pq0, pq1, kb0, kb1, pk0, pk1, vt0, vt1,
            mz, gtab, zero_ref, sem_x, sem_w, sem_o):
    X = (x0, x1, x2, x3)
    XN, O = (xn0, xn1), (o0, o1)
    QA, KA, VA = (qa0, qa1), (ka0, ka1), (va0, va1)
    QS, PQ, KB, PK, VT = (qs0, qs1), (pq0, pq1), (kb0, kb1), (pk0, pk1), (vt0, vt1)

    def col(t):
        return pl.ds(t * 128, 128)

    def x_copies(s):
        return [pltpu.make_async_copy(x_hbm.at[pl.ds(s * L, L), col(t)],
                                      X[s].at[t], sem_x.at[s]) for t in range(NT)]

    def out_copies(s):
        return [pltpu.make_async_copy(X[s].at[t], out_hbm.at[pl.ds(s * L, L), col(t)],
                                      sem_o.at[s]) for t in range(NT)]

    w_src = ((wqkv_hbm, 0), (wqkv_hbm, NT), (wqkv_hbm, 2 * NT), (awo_hbm, 0),
             (wq_hbm, 0), (wk_hbm, 0), (wv_hbm, 0), (wo_hbm, 0))

    def w_copies(m):
        src, t0 = w_src[m]
        return [pltpu.make_async_copy(src.at[:, col(t0 + t)], wraw.at[m, t], sem_w.at[m])
                for t in range(NT)]

    def start(cs):
        for c in cs:
            c.start()

    def wait(cs):
        for c in cs:
            c.wait()

    def token(*vals):
        bits = [pltpu.bitcast(v[:8, :128], U32) for v in vals]
        return _tree(jnp.bitwise_or, bits) & zero_ref[...]

    def vregs(vals, every=1):
        return [v[u:u + 8] for v in vals for u in range(0, v.shape[0], 8)][::-1][::every]

    def after(words, toks):
        if not toks:
            return words
        slabs = []
        for k in range(words.shape[0] // 8):
            slab = words[8 * k:8 * k + 8]
            if toks.get(k) is not None:
                slab = slab | jnp.concatenate([toks[k]] * (words.shape[1] // 128), axis=1)
            slabs.append(slab)
        return jnp.concatenate(slabs, axis=0)

    def store_rhs(dst, m, i, r, b11, b12, b21, b22):
        for k, v in enumerate(_rhs_terms(b11, b12, b21, b22)):
            dst[m, i, k, r, :] = _pack(v)

    def prep_plain(src_m, dst, m, i):
        for c in range(4):
            r0, r1 = pl.ds(128 * c, 128), pl.ds(D // 2 + 128 * c, 128)
            store_rhs(dst, m, i, pl.ds(64 * c, 64),
                      wraw[src_m, i, r0, :].astype(F32), wraw[src_m, i + NP, r0, :].astype(F32),
                      wraw[src_m, i, r1, :].astype(F32), wraw[src_m, i + NP, r1, :].astype(F32))

    def prep_a_cols(m, i):
        rows = D // 2 // NP
        slot = (_iota((rows, 128), 1) >> 1) & 7
        r0 = pl.ds(pl.multiple_of(i * rows, rows), rows)
        r1 = pl.ds(pl.multiple_of(D // 2 + i * rows, rows), rows)
        v = [jnp.concatenate([pltpu.bitcast(wraw[m, t, r0, :], U32),
                              pltpu.bitcast(wraw[m, t, r1, :], U32)], axis=0) for t in range(NT)]
        v = [x if t == 0 else pltpu.roll(x, 2 * t, 1) for t, x in enumerate(v)]
        v = [v[(-b) % NT] for b in range(NT)]
        for bit in (1, 2, 4):
            sel = (slot & bit) != 0
            v = [jnp.where(sel, v[(b - bit) % NT], v[b]) for b in range(NT)]
        v = [_bf(x if b == 0 else pltpu.roll(x, 128 - 2 * b, 1)).astype(F32)
             for b, x in enumerate(v)]
        r = pl.ds(pl.multiple_of(i * (rows // 2), rows // 2), rows // 2)
        for j in range(NP):
            store_rhs(wa, m, j, r, v[j][:rows], v[j + NP][:rows], v[j][rows:], v[j + NP][rows:])

    def prep_a_rows(i):
        for h in range(2):
            wtmp[h] = pltpu.bitcast(wraw[3, i + h * NP], U32)

        def rows(h, b):
            parts = [wtmp[h, pl.ds(8 * u + b, 8, stride=64), :] for u in range(8)]
            return _bf(jnp.concatenate(parts, axis=0)).astype(F32)

        for c in range(4):
            store_rhs(wao, 0, i, pl.ds(64 * c, 64),
                      rows(0, c), rows(1, c), rows(0, c + NP), rows(1, c + NP))

    def store_lhs(dst, t, r, a11, a12, a21, a22):
        packed = [_pack(v) for v in _lhs_terms(a11, a12, a21, a22)]
        for k, v in enumerate(packed):
            dst[t, k, r, :] = v
        return packed

    def products(a_ref, w_ref, m, i, emit):
        st = {}

        def prod(k, toks):
            a = jnp.concatenate(
                [after(a_ref[t, k], toks if t == 0 else None) for t in range(NP)], axis=1)
            return _dot(_bf(a), _bf(w_ref[m, i, k]))

        def p1(tok):
            st["m1"] = r = prod(0, tok)
            return r

        def p2(tok):
            st["c21"] = r = prod(1, tok)
            st["c22"] = st["m1"] - r
            return r

        def p3(tok):
            st["c12"] = r = prod(2, tok)
            st["c22"] = st["c22"] + r
            return r

        def p4(tok):
            r = prod(3, tok)
            emit(1, i, st["c21"] + r)
            st["c11"] = st["m1"] + r
            return r

        def p5(tok):
            r = prod(4, tok)
            emit(0, i + NP, st["c12"] + r)
            st["c11"] = st["c11"] - r
            return r

        def p6(tok):
            r = prod(5, tok)
            emit(1, i + NP, st["c22"] + r)
            return r

        def p7(tok):
            r = prod(6, tok)
            emit(0, i, st["c11"] + r)
            return r

        return [p1, p2, p3, p4, p5, p6, p7]

    def ln_tasks(n, i, off, nr=16):
        src, dst = X[n % NSEG], XN[n % 2]
        base = pl.multiple_of(i * RC, RC) + off
        st = {}

        def mean():
            st["x"] = [
                jnp.concatenate([src[t, pl.ds(pl.multiple_of(base + h * HL, nr), nr), :]
                                 for h in range(2)], axis=0).astype(F32) for t in range(NT)]
            part = _tree(jnp.add, st["x"])
            st["mean"] = jnp.sum(part, axis=1, keepdims=True) * (1.0 / D)
            return vregs([part])

        def var():
            st["x"] = [x - st["mean"] for x in st["x"]]
            part = _tree(jnp.add, [x * x for x in st["x"]])
            st["var"] = jnp.sum(part, axis=1, keepdims=True) * (1.0 / D)
            return vregs([part])

        def scale():
            inv = lax.rsqrt(st["var"] + 1e-5)
            y = [x * inv for x in st["x"]]
            r = pl.ds(pl.multiple_of((i * RC + off) // 2, nr // 2), nr // 2)
            outs = []
            for t in range(NP):
                outs += store_lhs(dst, t, r, y[t][:nr], y[t + NP][:nr], y[t][nr:], y[t + NP][nr:])
            return vregs(outs)

        return [mean, var, scale]

    def proj_a(n, i, which):
        p = n % 2

        def emit(h, t, y):
            if which == 0:
                QA[p][t, pl.ds(h * HL, HL), :] = y
                return
            buf = KA if which == 1 else VA
            buf[p][t, pl.ds(HALO + h * HL, HL), :] = y
            if h == 0 and n % NSEG == 0:
                buf[p][t, pl.ds(0, HALO), :] = jnp.zeros((HALO, 128), F32)
            elif h == 0:
                buf[p][t, pl.ds(0, HALO), :] = buf[1 - p][t, pl.ds(L, HALO), :]

        return products(XN[p], wa, which, i, emit)

    def proj_b(n, i, which):
        p = n % 2

        def emit(h, t, y):
            r = pl.ds(h * HL // 2, HL // 2)
            if which == 0:
                QS[p][t, r, :] = _pack(y * QSCALE)
                PQ[p][t, r, :] = _pack(_phi(y))
            elif which == 1:
                KB[p][t, r, :] = _pack(y)
                if n % NSEG != NSEG - 1:
                    PK[p][t, r, :] = _pack(_phi(y))
            else:
                VT[p][t, :, pl.ds(h * HL, HL)] = pltpu.bitcast(y.astype(BF16).T, U32)

        return products(XN[p], wb, which, i, emit)

    def out_stage(n, i):
        x = X[n % NSEG]

        def emit(h, t, y):
            r = pl.ds(h * HL, HL)
            x[t, r, :] = (x[t, r, :].astype(F32) + y).astype(BF16)

        if is_a(n):
            return products(O[n % 2], wao, 0, i, emit)
        return products(O[n % 2], wb, 3, i, emit)

    def att_a_tasks(n, i, off):
        p = n % 2
        base = pl.multiple_of(i * RC, RC) + off
        lg = [[None] * 4 for _ in range(WIN)]
        prob = [None] * 2
        st = {}

        def scores(u):
            r0 = base + (u // 2) * HL + 8 * (u % 2)
            q = [QA[p][t, pl.ds(r0, 8), :] for t in range(NT)]
            for w in range(WIN):
                kr = pl.ds(r0 + HALO - DIL * w, 8)
                lg[w][u] = _tree(jnp.add, [q[t] * KA[p][t, kr, :] for t in range(NT)])
            return [lg[w][u] for w in range(WIN)]

        def exchange(bit):
            a = st["a"] if "a" in st else jnp.concatenate([v for row in lg for v in row], axis=0)
            low = (_iota(a.shape, 1) & bit) == 0
            st["a"] = a + jnp.where(low, pltpu.roll(a, 128 - bit, 1), pltpu.roll(a, bit, 1))
            return vregs([st["a"]], 4)

        def softmax(h):
            v = [st["a"][32 * w + 16 * h:32 * w + 16 * h + 16] * QSCALE for w in range(WIN)]
            if n % NSEG == 0 and off == 0 and h == 0:
                pos = _iota((16, 128), 0) + base
                v = [a if w == 0 else jnp.where(pos >= DIL * w, a, MASKVAL)
                     for w, a in enumerate(v)]
            m = _tree(jnp.maximum, v)
            e = [jnp.exp2(a - m) for a in v]
            inv = 1.0 / _tree(jnp.add, e)
            prob[h] = [a * inv for a in e]
            return vregs(prob[h], 2)

        def mix(t, h):
            return jnp.concatenate([
                _tree(jnp.add, [
                    prob[h][w][8 * u:8 * u + 8]
                    * VA[p][t, pl.ds(base + h * HL + 8 * u + HALO - DIL * w, 8), :]
                    for w in range(WIN)])
                for u in range(2)], axis=0)

        def values(t):
            r = pl.ds(pl.multiple_of((i * RC + off) // 2, 8), 8)
            return store_lhs(O[p], t, r, mix(t, 0), mix(t + NP, 0), mix(t, 1), mix(t + NP, 1))

        return ([lambda u=u: scores(u) for u in range(4)]
                + [lambda: exchange(1), lambda: exchange(16)]
                + [lambda h=h: softmax(h) for h in range(2)]
                + [lambda t=t: values(t) for t in range(NP)])

    def att_b_piece(n, g, j, mem, tok):
        p = n % 2
        rows = pl.ds(64 * j, 64)
        qw = after(QS[p][g, rows, :], {0: tok})
        head = _iota((64, 128), 1) >> 5
        qcat = jnp.concatenate(
            [jnp.where(head == hh, qw, jnp.uint32(0)) for hh in range(4)], axis=0)
        st = _dot_nt(_bf(KB[p][g, pl.ds(0, 64 * (j + 1)), :]), _bf(qcat))
        causal = jnp.where(_iota((128, 128), 0) > _iota((128, 128), 1), MASKVAL, 0.0)
        s = [[st[128 * c:128 * (c + 1), 128 * hh:128 * (hh + 1)] for c in range(j + 1)]
             for hh in range(4)]
        for hh in range(4):
            s[hh][j] = s[hh][j] + causal
        m = [jnp.broadcast_to(jnp.max(_tree(jnp.maximum, s[hh]), axis=0, keepdims=True), (8, 128))
             for hh in range(4)]
        e = [[] for _ in range(4)]
        part = [None] * 4

        def exp_tile(hh, c, tok):
            mh = m[hh] if tok is None else m[hh] + pltpu.bitcast(tok, F32)
            v = [jnp.exp2(s[hh][c][u:u + 8] - mh) for u in range(0, 128, 8)]
            part[hh] = _tree(jnp.add, v if part[hh] is None else v + [part[hh]])
            e[hh].append(jnp.concatenate(v, axis=0).astype(BF16))

        def finish(tok):
            r = _dot_nt(mem, _bf(after(PQ[p][g, rows, :], {0: tok})))
            ot = []
            for hh in range(4):
                vt = VT[p][g, pl.ds(16 * hh, 16), pl.ds(0, 128 * (j + 1))]
                acc = _dot(_bf(vt), jnp.concatenate(e[hh], axis=0))
                l = jnp.sum(part[hh], axis=0, keepdims=True)
                gate = gtab[pl.ds(4 * g + hh, 1), :]
                wm = gate / (r[128 + 8 * hh:136 + 8 * hh] + 1e-6)
                wm = jnp.concatenate([wm] * 4, axis=0)
                ot.append(r[32 * hh:32 * hh + 32] * wm + acc * ((1.0 - gate) / l))
            return ot

        tasks = [lambda tok, hh=hh, c=c: exp_tile(hh, c, tok)
                 for hh in range(4) for c in range(j + 1)]
        return st, tasks, finish

    def mem_load(n, g):
        if n % NSEG == 0:
            return jnp.zeros((MZ_ROWS, 128), F32)
        return mz[g]

    def mem_update(n, g, state):
        p = n % 2
        if n % NSEG == NSEG - 1:
            return
        a = jnp.concatenate([_bf(VT[p][g]), jnp.ones((32, L), BF16)], axis=0)
        row = _iota((MZ_ROWS, 128), 0)
        row_head = jnp.where(row < 128, row >> 5, (row - 128) >> 3)
        keep = row_head == (_iota((MZ_ROWS, 128), 1) >> 5)
        mz[g] = state + jnp.where(keep, _dot(a, _bf(PK[p][g])), 0.0)

    def is_a(n):
        return (n // NSEG) % 2 == 0

    def join(toks, slot, tok):
        if tok is not None:
            toks[slot] = tok if toks.get(slot) is None else toks[slot] | tok

    def run_timed(mm, tasks):
        tasks = sorted(tasks, key=lambda x: x[0])
        for k, prod in enumerate(mm):
            toks = {}
            while tasks and tasks[0][0] < 16 * (k + 1):
                time, f = tasks.pop(0)
                join(toks, time - 16 * k, token(*f()))
            prod(toks)
        for _, f in tasks:
            f()

    def body_b(n, i, mm, ln):
        groups = (i, i + NP)
        state = [mem_load(n, g) for g in groups]
        pieces = [(j, h) for j in (3, 1, 2, 0) for h in range(2)]
        full = len(mm) == 28
        share = [4, 4, 3, 3, 4, 3, 2, 2] if full else [1, 1, 1, 0, 1, 1, 0, 1]
        late = []
        if ln:
            for off in range(0, RC, 16):
                late += ln_tasks(n + 2, i, off)
        tiles, tok, done = {}, None, []
        for k, (j, h) in enumerate(pieces):
            st, exps, finish = att_b_piece(n, groups[h], j, state[h].astype(BF16), tok)
            first = token(*[st[:, 128 * hh:] for hh in range(4)])
            todo = len(exps)
            for c in range(share[k]):
                toks = {}
                if c == 0:
                    join(toks, 0, first)
                if done and c >= min(1, share[k] - 1):
                    join(toks, 8 if c else 15, token(*done.pop(0)()))
                if late:
                    join(toks, 4, token(*late.pop(0)()))
                r = mm.pop(0)(toks)
                cnt = (todo * (c + 1)) // share[k] - (todo * c) // share[k]
                for u in range(cnt):
                    exps.pop(0)(token(r[8 * ((32 * u) // cnt):]) if full else None)
                tok = token(r)
            for f in exps:
                f(None)
            ot = finish(tok)

            def post(ot=ot, j=j, h=h):
                tiles[j, h] = jnp.concatenate(ot, axis=0).T
                if j < 2 and h == 1:
                    return vregs(store_lhs(O[n % 2], i, pl.ds(64 * j, 64), tiles[j, 0], tiles[j, 1],
                                           tiles[j + 2, 0], tiles[j + 2, 1]), 4)
                return vregs([tiles[j, h]], 4)

            done.append(post)
        for h in range(2):
            mem_update(n, groups[h], state[h])
        run_timed(mm, [(16 * len(mm) - 8, f) for f in done + late])

    def step(n, ln=True, proj=(0, 1, 2), att=True, out=True, extra=None):
        def body(i, c):
            mm = []
            for which in proj:
                mm += (proj_a if is_a(n + 1) else proj_b)(n + 1, i, which)
            if out:
                mm += out_stage(n - 1, i)
            if extra is not None:
                extra(i)
            if att and not is_a(n):
                body_b(n, i, mm, ln)
                return c
            span = 16 * len(mm) / 4
            tasks = []
            for u, off in enumerate(range(0, RC, 16)):
                if att:
                    when = (.05, .10, .15, .20, .36, .52, .60, .66, .73, .80, .87, .94)
                    tasks += [(int(span * (u + w)), f)
                              for w, f in zip(when, att_a_tasks(n, i, off))]
                if ln:
                    tasks += [(int(span * (u + w)), f)
                              for w, f in zip((.26, .37, .46), ln_tasks(n + 2, i, off))]
            run_timed(mm, tasks)
            return c

        lax.fori_loop(0, NP, body, 0)

    start(x_copies(0))
    for m in range(3):
        start(w_copies(m))
    start(x_copies(1))
    start(w_copies(3))
    start(x_copies(2))
    for m in range(4, 8):
        start(w_copies(m))
    start(x_copies(3))

    zero_ref[...] = jnp.zeros((8, 128), U32)
    gate = jax.nn.sigmoid(beta_ref[...].astype(F32))
    eye = _iota((H, H), 0) == _iota((H, H), 1)
    gcol = jnp.sum(jnp.where(eye, jnp.broadcast_to(gate, (H, H)), 0.0), axis=1, keepdims=True)
    gtab[...] = jnp.broadcast_to(gcol, (H, 128))

    wait(x_copies(0))
    step(-2, proj=(), att=False, out=False)
    wait(w_copies(0))
    step(-1, ln=False, proj=(), att=False, out=False, extra=lambda i: prep_a_cols(0, i))
    wait(w_copies(1))
    step(-1, ln=False, proj=(0,), att=False, out=False, extra=lambda i: prep_a_cols(1, i))
    wait(w_copies(2))
    step(-1, ln=False, proj=(1,), att=False, out=False, extra=lambda i: prep_a_cols(2, i))
    wait(x_copies(1))
    wait(w_copies(3))
    step(-1, proj=(2,), att=False, out=False, extra=prep_a_rows)
    wait(x_copies(2))
    for m in range(4, 8):
        wait(w_copies(m))

    def prep_b(i):
        for m in range(4):
            prep_plain(4 + m, wb, m, i)

    step(0, out=False, extra=prep_b)
    wait(x_copies(3))

    def pair(it, c):
        for n in range(1, 6):
            step(n)

        @pl.when(it == 1)
        def _():
            start(out_copies(0))

        step(6)

        @pl.when(it == 0)
        def _():
            step(7)
            step(8)

        return c

    lax.fori_loop(0, 2, pair, 0)
    start(out_copies(1))
    step(15, ln=False, proj=())
    start(out_copies(2))
    step(16, ln=False, proj=(), att=False)
    start(out_copies(3))
    for s in range(NSEG):
        wait(out_copies(s))


@jax.jit
def pallas_interleave_layers__sliding_local_dilated__memory_aug_infini_attn__prompt_kernel(
    A_x: jax.Array,
    A_wqkv: jax.Array,
    A_wo: jax.Array,
    B_x: jax.Array,
    B_wq: jax.Array,
    B_wk: jax.Array,
    B_wv: jax.Array,
    B_wo: jax.Array,
    B_beta: jax.Array,
):
    del B_x
    assert A_x.shape == (1, S, D)
    hbm = pl.BlockSpec(memory_space=pl.ANY)
    scratch = (
        [pltpu.VMEM((NT, L, 128), BF16)] * 4
        + [pltpu.VMEM((8, NT, D, 128), BF16),
           pltpu.VMEM((2, D // 2, 128), U32),
           pltpu.VMEM((3, NP, 7, D // 4, 128), U32),
           pltpu.VMEM((1, NP, 7, D // 4, 128), U32),
           pltpu.VMEM((4, NP, 7, D // 4, 128), U32)]
        + [pltpu.VMEM((NP, 7, HL // 2, 128), U32)] * 4
        + [pltpu.VMEM((NT, L, 128), F32)] * 2
        + [pltpu.VMEM((NT, HALO + L, 128), F32)] * 4
        + [pltpu.VMEM((NT, L // 2, 128), U32)] * 8
        + [pltpu.VMEM((NT, 64, L), U32)] * 2
        + [pltpu.VMEM((NT, MZ_ROWS, 128), F32), pltpu.VMEM((H, 128), F32),
           pltpu.VMEM((8, 128), U32),
           pltpu.SemaphoreType.DMA((NSEG,)), pltpu.SemaphoreType.DMA((8,)),
           pltpu.SemaphoreType.DMA((NSEG,))]
    )
    out = pl.pallas_call(
        _kernel,
        out_shape=jax.ShapeDtypeStruct((S, D), BF16),
        in_specs=[hbm] * 7 + [pl.BlockSpec(memory_space=pltpu.VMEM)],
        out_specs=hbm,
        scratch_shapes=scratch,
        compiler_params=pltpu.CompilerParams(vmem_limit_bytes=110 * 2**20),
        name="abab_stack",
    )(A_x.reshape(S, D), A_wqkv, A_wo, B_wq, B_wk, B_wv, B_wo, B_beta.reshape(1, H))
    return out.reshape(1, S, D)
```

```python
import jax
import jax.numpy as jnp
from jax import lax
import jax.experimental.pallas as pl
import jax.experimental.pallas.tpu as pltpu

S, D, H, DH = 2048, 1024, 32, 32
NSEG, L = 4, 512
HL = L // 2
NT = D // 128
NP = NT // 2
RC = HL // NP
WIN, DIL = 8, 2
HALO = 16
MZ_ROWS = 128 + 32
LOG2E = 1.4426950408889634
QSCALE = float(DH ** -0.5 * LOG2E)
MASKVAL = float(-1e9 * LOG2E)

F32, BF16, U32 = jnp.float32, jnp.bfloat16, jnp.uint32
_NT_DIMS = (((1,), (1,)), ((), ()))


def _iota(shape, axis):
    return lax.broadcasted_iota(jnp.int32, shape, axis)


def _dot(a, b):
    return jnp.dot(a, b, preferred_element_type=F32)


def _dot_nt(a, b):
    return lax.dot_general(a, b, _NT_DIMS, preferred_element_type=F32)


def _pack(x):
    return pltpu.bitcast(x.astype(BF16), U32)


def _bf(words):
    return pltpu.bitcast(words, BF16)


def _phi(t):
    return jnp.where(t > 0, t + 1.0, jnp.exp(t))


def _tree(op, xs):
    xs = list(xs)
    while len(xs) > 1:
        xs = [op(xs[i], xs[i + 1]) if i + 1 < len(xs) else xs[i]
              for i in range(0, len(xs), 2)]
    return xs[0]


def _lhs_terms(a11, a12, a21, a22):
    return (a11 + a22, a21 + a22, a11, a22, a11 + a12, a21 - a11, a12 - a22)


def _rhs_terms(b11, b12, b21, b22):
    return (b11 + b22, b11, b12 - b22, b21 - b11, b22, b11 + b12, b21 + b22)


def _kernel(x_hbm, wqkv_hbm, awo_hbm, wq_hbm, wk_hbm, wv_hbm, wo_hbm, beta_ref,
            out_hbm,
            x0, x1, x2, x3, wraw, wtmp, wa, wao, wb,
            xn0, xn1, o0, o1,
            qa0, qa1, ka0, ka1, va0, va1,
            qs0, qs1, pq0, pq1, kb0, kb1, pk0, pk1, vt0, vt1,
            mz, gtab, zero_ref, sem_x, sem_w, sem_s, sem_o):
    X = (x0, x1, x2, x3)
    XN, O = (xn0, xn1), (o0, o1)
    QA, KA, VA = (qa0, qa1), (ka0, ka1), (va0, va1)
    QS, PQ, KB, PK, VT = (qs0, qs1), (pq0, pq1), (kb0, kb1), (pk0, pk1), (vt0, vt1)

    def col(t):
        return pl.ds(t * 128, 128)

    def x_copies(s):
        return [pltpu.make_async_copy(x_hbm.at[pl.ds(s * L, L), col(t)],
                                      X[s].at[t], sem_x.at[s]) for t in range(NT)]

    def out_copies(s):
        return [pltpu.make_async_copy(X[s].at[t], out_hbm.at[pl.ds(s * L, L), col(t)],
                                      sem_o.at[s]) for t in range(NT)]

    w_src = ((wqkv_hbm, 0), (wqkv_hbm, NT), (wqkv_hbm, 2 * NT), (awo_hbm, 0),
             (wq_hbm, 0), (wk_hbm, 0), (wv_hbm, 0), (wo_hbm, 0))

    def w_copies(m):
        src, t0 = w_src[m]
        return [pltpu.make_async_copy(src.at[:, col(t0 + t)], wraw.at[m, t], sem_w.at[m])
                for t in range(NT)]

    def slab_copies(m, i):
        rows = D // 2 // NP
        rs = [pl.ds(pl.multiple_of(h * (D // 2) + i * rows, rows), rows) for h in range(2)]
        return [pltpu.make_async_copy(wqkv_hbm.at[r, col(m * NT + t)], wraw.at[m, t, r],
                                      sem_s.at[m, i]) for r in rs for t in range(NT)]

    def start(cs):
        for c in cs:
            c.start()

    def wait(cs):
        for c in cs:
            c.wait()

    def token(*vals):
        bits = [pltpu.bitcast(v[:8, :128], U32) for v in vals]
        return _tree(jnp.bitwise_or, bits) & zero_ref[...]

    def vregs(vals, every=1):
        return [v[u:u + 8] for v in vals for u in range(0, v.shape[0], 8)][::-1][::every]

    def after(words, toks):
        if not toks:
            return words
        slabs = []
        for k in range(words.shape[0] // 8):
            slab = words[8 * k:8 * k + 8]
            if toks.get(k) is not None:
                slab = slab | jnp.concatenate([toks[k]] * (words.shape[1] // 128), axis=1)
            slabs.append(slab)
        return jnp.concatenate(slabs, axis=0)

    def store_rhs(dst, m, i, r, b11, b12, b21, b22):
        packed = [_pack(v) for v in _rhs_terms(b11, b12, b21, b22)]
        for k, v in enumerate(packed):
            dst[m, i, k, r, :] = v
        return vregs(packed, 2)

    def prep_plain(m, i):
        def piece(c):
            r0, r1 = pl.ds(64 * c, 64), pl.ds(D // 2 + 64 * c, 64)
            return store_rhs(
                wb, m - 4, i, pl.ds(32 * c, 32),
                wraw[m, i, r0, :].astype(F32), wraw[m, i + NP, r0, :].astype(F32),
                wraw[m, i, r1, :].astype(F32), wraw[m, i + NP, r1, :].astype(F32))

        return [lambda c=c: piece(c) for c in range(8)]

    def prep_a_cols(m, i):
        rows = 32
        st = {}

        def shear(c):
            base = i * (D // 2 // NP) + c * rows
            slot = (_iota((rows, 128), 1) >> 1) & 7
            r0 = pl.ds(pl.multiple_of(base, rows), rows)
            r1 = pl.ds(pl.multiple_of(D // 2 + base, rows), rows)
            v = [pltpu.bitcast(jnp.concatenate([wraw[m, t, r0, :], wraw[m, t, r1, :]], axis=0), U32)
                 for t in range(NT)]
            v = [x if t == 0 else pltpu.roll(x, 2 * t, 1) for t, x in enumerate(v)]
            v = [v[(-b) % NT] for b in range(NT)]
            for bit in (1, 2, 4):
                sel = (slot & bit) != 0
                v = [jnp.where(sel, v[(b - bit) % NT], v[b]) for b in range(NT)]
            st[c] = [x if b == 0 else pltpu.roll(x, 128 - 2 * b, 1) for b, x in enumerate(v)]
            return vregs(v, 2)

        def terms(c):
            v = [_bf(x).astype(F32) for x in st[c]]
            r = pl.ds(pl.multiple_of((i * (D // 2 // NP) + c * rows) // 2, rows // 2), rows // 2)
            outs = []
            for j in range(NP):
                outs += store_rhs(wa, m, j, r, v[j][:rows], v[j + NP][:rows],
                                  v[j][rows:], v[j + NP][rows:])
            return outs

        order = ((shear, 0), (shear, 1), (terms, 0), (shear, 2), (terms, 1), (shear, 3),
                 (terms, 2), (terms, 3))
        return [lambda f=f, c=c: f(c) for f, c in order]

    def prep_a_rows(i):
        def stage():
            for h in range(2):
                wtmp[h] = pltpu.bitcast(wraw[3, i + h * NP], U32)
            return [zero_ref[...]]

        def rows(h, b):
            parts = [wtmp[h, pl.ds(8 * u + b, 8, stride=64), :] for u in range(8)]
            return _bf(jnp.concatenate(parts, axis=0)).astype(F32)

        def piece(c):
            return store_rhs(wao, 0, i, pl.ds(64 * c, 64),
                             rows(0, c), rows(1, c), rows(0, c + NP), rows(1, c + NP))

        return [stage] + [lambda c=c: piece(c) for c in range(4)]

    def store_lhs(dst, t, r, a11, a12, a21, a22):
        packed = [_pack(v) for v in _lhs_terms(a11, a12, a21, a22)]
        for k, v in enumerate(packed):
            dst[t, k, r, :] = v
        return packed

    def products(a_ref, w_ref, m, i, emit):
        st = {}

        def prod(k, toks):
            a = jnp.concatenate(
                [after(a_ref[t, k], toks if t == 0 else None) for t in range(NP)], axis=1)
            return _dot(_bf(a), _bf(w_ref[m, i, k]))

        def p1(tok):
            st["m1"] = r = prod(0, tok)
            return r

        def p2(tok):
            st["c21"] = r = prod(1, tok)
            st["c22"] = st["m1"] - r
            return r

        def p3(tok):
            st["c12"] = r = prod(2, tok)
            st["c22"] = st["c22"] + r
            return r

        def p4(tok):
            r = prod(3, tok)
            emit(1, i, st["c21"] + r)
            st["c11"] = st["m1"] + r
            return r

        def p5(tok):
            r = prod(4, tok)
            emit(0, i + NP, st["c12"] + r)
            st["c11"] = st["c11"] - r
            return r

        def p6(tok):
            r = prod(5, tok)
            emit(1, i + NP, st["c22"] + r)
            return r

        def p7(tok):
            r = prod(6, tok)
            emit(0, i, st["c11"] + r)
            return r

        return [p1, p2, p3, p4, p5, p6, p7]

    def ln_tasks(n, i, off, nr=16):
        src, dst = X[n % NSEG], XN[n % 2]
        base = pl.multiple_of(i * RC, RC) + off
        st = {}

        def mean():
            st["x"] = [
                jnp.concatenate([src[t, pl.ds(pl.multiple_of(base + h * HL, nr), nr), :]
                                 for h in range(2)], axis=0).astype(F32) for t in range(NT)]
            part = _tree(jnp.add, st["x"])
            st["mean"] = jnp.sum(part, axis=1, keepdims=True) * (1.0 / D)
            return vregs([part])

        def var():
            st["x"] = [x - st["mean"] for x in st["x"]]
            part = _tree(jnp.add, [x * x for x in st["x"]])
            st["var"] = jnp.sum(part, axis=1, keepdims=True) * (1.0 / D)
            return vregs([part])

        def scale():
            inv = lax.rsqrt(st["var"] + 1e-5)
            y = [x * inv for x in st["x"]]
            r = pl.ds(pl.multiple_of((i * RC + off) // 2, nr // 2), nr // 2)
            outs = []
            for t in range(NP):
                outs += store_lhs(dst, t, r, y[t][:nr], y[t + NP][:nr], y[t][nr:], y[t + NP][nr:])
            return vregs(outs)

        return [mean, var, scale]

    def proj_a(n, i, which):
        p = n % 2

        def emit(h, t, y):
            if which == 0:
                QA[p][t, pl.ds(h * HL, HL), :] = y
                return
            buf = KA if which == 1 else VA
            buf[p][t, pl.ds(HALO + h * HL, HL), :] = y
            if h == 0 and n % NSEG == 0:
                buf[p][t, pl.ds(0, HALO), :] = jnp.zeros((HALO, 128), F32)
            elif h == 0:
                buf[p][t, pl.ds(0, HALO), :] = buf[1 - p][t, pl.ds(L, HALO), :]

        return products(XN[p], wa, which, i, emit)

    def proj_b(n, i, which):
        p = n % 2

        def emit(h, t, y):
            r = pl.ds(h * HL // 2, HL // 2)
            if which == 0:
                QS[p][t, r, :] = _pack(y * QSCALE)
                PQ[p][t, r, :] = _pack(_phi(y))
            elif which == 1:
                KB[p][t, r, :] = _pack(y)
                if n % NSEG != NSEG - 1:
                    PK[p][t, r, :] = _pack(_phi(y))
            else:
                VT[p][t, :, pl.ds(h * HL, HL)] = pltpu.bitcast(y.astype(BF16).T, U32)

        return products(XN[p], wb, which, i, emit)

    def out_stage(n, i):
        x = X[n % NSEG]

        def emit(h, t, y):
            r = pl.ds(h * HL, HL)
            x[t, r, :] = (x[t, r, :].astype(F32) + y).astype(BF16)

        if is_a(n):
            return products(O[n % 2], wao, 0, i, emit)
        return products(O[n % 2], wb, 3, i, emit)

    def att_a_tasks(n, i, off):
        p = n % 2
        base = pl.multiple_of(i * RC, RC) + off
        lg = [[None] * 4 for _ in range(WIN)]
        prob = [None] * 2
        st = {}

        def scores(u):
            r0 = base + (u // 2) * HL + 8 * (u % 2)
            q = [QA[p][t, pl.ds(r0, 8), :] for t in range(NT)]
            for w in range(WIN):
                kr = pl.ds(r0 + HALO - DIL * w, 8)
                lg[w][u] = _tree(jnp.add, [q[t] * KA[p][t, kr, :] for t in range(NT)])
            return [lg[w][u] for w in range(WIN)]

        def exchange(bit):
            a = st["a"] if "a" in st else jnp.concatenate([v for row in lg for v in row], axis=0)
            low = (_iota(a.shape, 1) & bit) == 0
            st["a"] = a + jnp.where(low, pltpu.roll(a, 128 - bit, 1), pltpu.roll(a, bit, 1))
            return vregs([st["a"]], 4)

        def softmax(h):
            v = [st["a"][32 * w + 16 * h:32 * w + 16 * h + 16] * QSCALE for w in range(WIN)]
            if n % NSEG == 0 and off == 0 and h == 0:
                pos = _iota((16, 128), 0) + base
                v = [a if w == 0 else jnp.where(pos >= DIL * w, a, MASKVAL)
                     for w, a in enumerate(v)]
            m = _tree(jnp.maximum, v)
            e = [jnp.exp2(a - m) for a in v]
            inv = 1.0 / _tree(jnp.add, e)
            prob[h] = [a * inv for a in e]
            return vregs(prob[h], 2)

        def mix(t, h):
            return jnp.concatenate([
                _tree(jnp.add, [
                    prob[h][w][8 * u:8 * u + 8]
                    * VA[p][t, pl.ds(base + h * HL + 8 * u + HALO - DIL * w, 8), :]
                    for w in range(WIN)])
                for u in range(2)], axis=0)

        def values(t):
            r = pl.ds(pl.multiple_of((i * RC + off) // 2, 8), 8)
            return store_lhs(O[p], t, r, mix(t, 0), mix(t + NP, 0), mix(t, 1), mix(t + NP, 1))

        return ([lambda u=u: scores(u) for u in range(4)]
                + [lambda: exchange(1), lambda: exchange(16)]
                + [lambda h=h: softmax(h) for h in range(2)]
                + [lambda t=t: values(t) for t in range(NP)])

    def att_b_piece(n, g, j, mem, tok):
        p = n % 2
        rows = pl.ds(64 * j, 64)
        qw = after(QS[p][g, rows, :], {0: tok})
        head = _iota((64, 128), 1) >> 5
        qcat = jnp.concatenate(
            [jnp.where(head == hh, qw, jnp.uint32(0)) for hh in range(4)], axis=0)
        st = _dot_nt(_bf(KB[p][g, pl.ds(0, 64 * (j + 1)), :]), _bf(qcat))
        causal = jnp.where(_iota((128, 128), 0) > _iota((128, 128), 1), MASKVAL, 0.0)
        s = [[st[128 * c:128 * (c + 1), 128 * hh:128 * (hh + 1)] for c in range(j + 1)]
             for hh in range(4)]
        for hh in range(4):
            s[hh][j] = s[hh][j] + causal
        m = [jnp.broadcast_to(jnp.max(_tree(jnp.maximum, s[hh]), axis=0, keepdims=True), (8, 128))
             for hh in range(4)]
        e = [[] for _ in range(4)]
        part = [None] * 4

        def exp_tile(hh, c, tok):
            mh = m[hh] if tok is None else m[hh] + pltpu.bitcast(tok, F32)
            v = [jnp.exp2(s[hh][c][u:u + 8] - mh) for u in range(0, 128, 8)]
            part[hh] = _tree(jnp.add, v if part[hh] is None else v + [part[hh]])
            e[hh].append(jnp.concatenate(v, axis=0).astype(BF16))

        def finish(tok):
            r = _dot_nt(mem, _bf(after(PQ[p][g, rows, :], {0: tok})))
            ot = []
            for hh in range(4):
                vt = VT[p][g, pl.ds(16 * hh, 16), pl.ds(0, 128 * (j + 1))]
                acc = _dot(_bf(vt), jnp.concatenate(e[hh], axis=0))
                l = jnp.sum(part[hh], axis=0, keepdims=True)
                gate = gtab[pl.ds(4 * g + hh, 1), :]
                wm = gate / (r[128 + 8 * hh:136 + 8 * hh] + 1e-6)
                wm = jnp.concatenate([wm] * 4, axis=0)
                ot.append(r[32 * hh:32 * hh + 32] * wm + acc * ((1.0 - gate) / l))
            return ot

        tasks = [lambda tok, hh=hh, c=c: exp_tile(hh, c, tok)
                 for hh in range(4) for c in range(j + 1)]
        return st, tasks, finish

    def mem_load(n, g):
        if n % NSEG == 0:
            return jnp.zeros((MZ_ROWS, 128), F32)
        return mz[g]

    def mem_update(n, g, state):
        p = n % 2
        if n % NSEG == NSEG - 1:
            return
        a = jnp.concatenate([_bf(VT[p][g]), jnp.ones((32, L), BF16)], axis=0)
        row = _iota((MZ_ROWS, 128), 0)
        row_head = jnp.where(row < 128, row >> 5, (row - 128) >> 3)
        keep = row_head == (_iota((MZ_ROWS, 128), 1) >> 5)
        mz[g] = state + jnp.where(keep, _dot(a, _bf(PK[p][g])), 0.0)

    def is_a(n):
        return (n // NSEG) % 2 == 0

    def join(toks, slot, tok):
        if tok is not None:
            toks[slot] = tok if toks.get(slot) is None else toks[slot] | tok

    def run_timed(mm, tasks):
        tasks = sorted(tasks, key=lambda x: x[0])
        for k, prod in enumerate(mm):
            toks = {}
            while tasks and tasks[0][0] < 16 * (k + 1):
                time, f = tasks.pop(0)
                join(toks, time - 16 * k, token(*f()))
            prod(toks)
        for _, f in tasks:
            f()

    def body_b(n, i, mm, ln):
        groups = (i, i + NP)
        state = [mem_load(n, g) for g in groups]
        pieces = [(j, h) for j in (3, 1, 2, 0) for h in range(2)]
        full = len(mm) == 28
        share = [4, 4, 3, 3, 4, 3, 2, 2] if full else [1, 1, 1, 0, 1, 1, 0, 1]
        late = []
        if ln:
            for off in range(0, RC, 16):
                late += ln_tasks(n + 2, i, off)
        tiles, tok, done = {}, None, []
        for k, (j, h) in enumerate(pieces):
            st, exps, finish = att_b_piece(n, groups[h], j, state[h].astype(BF16), tok)
            first = token(*[st[:, 128 * hh:] for hh in range(4)])
            todo = len(exps)
            for c in range(share[k]):
                toks = {}
                if c == 0:
                    join(toks, 0, first)
                if done and c >= min(1, share[k] - 1):
                    join(toks, 8 if c else 15, token(*done.pop(0)()))
                if late:
                    join(toks, 4, token(*late.pop(0)()))
                r = mm.pop(0)(toks)
                cnt = (todo * (c + 1)) // share[k] - (todo * c) // share[k]
                for u in range(cnt):
                    exps.pop(0)(token(r[8 * ((32 * u) // cnt):]) if full else None)
                tok = token(r)
            for f in exps:
                f(None)
            ot = finish(tok)

            def post(ot=ot, j=j, h=h):
                tiles[j, h] = jnp.concatenate(ot, axis=0).T
                if j < 2 and h == 1:
                    return vregs(store_lhs(O[n % 2], i, pl.ds(64 * j, 64), tiles[j, 0], tiles[j, 1],
                                           tiles[j + 2, 0], tiles[j + 2, 1]), 4)
                return vregs([tiles[j, h]], 4)

            done.append(post)
        for h in range(2):
            mem_update(n, groups[h], state[h])
        run_timed(mm, [(16 * len(mm) - 8, f) for f in done + late])

    def step(n, ln=True, proj=(0, 1, 2), att=True, out=True, extra=None):
        def body(i, c):
            mm = []
            for which in proj:
                mm += (proj_a if is_a(n + 1) else proj_b)(n + 1, i, which)
            if out:
                mm += out_stage(n - 1, i)
            if att and not is_a(n):
                body_b(n, i, mm, ln)
                return c
            tasks = []
            if extra is not None:
                fs = extra(i)
                tasks += [(int(16 * len(mm) * (u + 1) / len(fs)) - 1, f) for u, f in enumerate(fs)]
            span = 16 * len(mm) / 4
            for u, off in enumerate(range(0, RC, 16)):
                if att:
                    when = (.05, .10, .15, .20, .36, .52, .60, .66, .73, .80, .87, .94)
                    tasks += [(int(span * (u + w)), f)
                              for w, f in zip(when, att_a_tasks(n, i, off))]
                if ln:
                    when = (.26, .37, .46) if att else (.3, .8, 1.3)
                    tasks += [(int(span * (u + w)), f)
                              for w, f in zip(when, ln_tasks(n + 2, i, off))]
            run_timed(mm, tasks)
            return c

        lax.fori_loop(0, NP, body, 0)

    def prep_in_flight(m):
        def tasks(i):
            @pl.when(i + 2 < NP)
            def _():
                start(slab_copies(m, i + 2))

            if m < 2:
                @pl.when(i + 2 >= NP)
                def _():
                    start(slab_copies(m + 1, i + 2 - NP))

            wait(slab_copies(m, i))
            return prep_a_cols(m, i)

        return tasks

    start(x_copies(0))
    zero_ref[...] = jnp.zeros((8, 128), U32)
    gate = jax.nn.sigmoid(beta_ref[...].astype(F32))
    eye = _iota((H, H), 0) == _iota((H, H), 1)
    gcol = jnp.sum(jnp.where(eye, jnp.broadcast_to(gate, (H, H)), 0.0), axis=1, keepdims=True)
    gtab[...] = jnp.broadcast_to(gcol, (H, 128))
    start(slab_copies(0, 0))
    wait(x_copies(0))
    start(slab_copies(0, 1))
    step(-2, proj=(), att=False, out=False)
    step(-1, ln=False, proj=(), att=False, out=False, extra=prep_in_flight(0))
    step(-1, ln=False, proj=(0,), att=False, out=False, extra=prep_in_flight(1))
    start(x_copies(1))
    step(-1, ln=False, proj=(1,), att=False, out=False, extra=prep_in_flight(2))
    start(x_copies(2))
    start(w_copies(3))
    wait(x_copies(1))
    step(-1, proj=(2,), att=False, out=False)
    start(x_copies(3))
    for m in range(4, 8):
        start(w_copies(m))
    wait(x_copies(2))
    wait(w_copies(3))
    step(0, out=False, extra=prep_a_rows)
    wait(x_copies(3))
    for m in range(4, 8):
        wait(w_copies(m))
    step(1, extra=lambda i: prep_plain(4, i) + prep_plain(5, i))
    step(2, extra=lambda i: prep_plain(6, i) + prep_plain(7, i))
    for n in range(3, 14):
        step(n)
    start(out_copies(0))
    step(14, ln=False)
    start(out_copies(1))
    step(15, ln=False, proj=())
    start(out_copies(2))
    step(16, ln=False, proj=(), att=False)
    start(out_copies(3))
    for s in range(NSEG):
        wait(out_copies(s))


@jax.jit
def pallas_interleave_layers__sliding_local_dilated__memory_aug_infini_attn__prompt_kernel(
    A_x: jax.Array,
    A_wqkv: jax.Array,
    A_wo: jax.Array,
    B_x: jax.Array,
    B_wq: jax.Array,
    B_wk: jax.Array,
    B_wv: jax.Array,
    B_wo: jax.Array,
    B_beta: jax.Array,
):
    del B_x
    assert A_x.shape == (1, S, D)
    hbm = pl.BlockSpec(memory_space=pl.ANY)
    scratch = (
        [pltpu.VMEM((NT, L, 128), BF16)] * 4
        + [pltpu.VMEM((8, NT, D, 128), BF16),
           pltpu.VMEM((2, D // 2, 128), U32),
           pltpu.VMEM((3, NP, 7, D // 4, 128), U32),
           pltpu.VMEM((1, NP, 7, D // 4, 128), U32),
           pltpu.VMEM((4, NP, 7, D // 4, 128), U32)]
        + [pltpu.VMEM((NP, 7, HL // 2, 128), U32)] * 4
        + [pltpu.VMEM((NT, L, 128), F32)] * 2
        + [pltpu.VMEM((NT, HALO + L, 128), F32)] * 4
        + [pltpu.VMEM((NT, L // 2, 128), U32)] * 8
        + [pltpu.VMEM((NT, 64, L), U32)] * 2
        + [pltpu.VMEM((NT, MZ_ROWS, 128), F32), pltpu.VMEM((H, 128), F32),
           pltpu.VMEM((8, 128), U32),
           pltpu.SemaphoreType.DMA((NSEG,)), pltpu.SemaphoreType.DMA((8,)),
           pltpu.SemaphoreType.DMA((3, NP)),
           pltpu.SemaphoreType.DMA((NSEG,))]
    )
    out = pl.pallas_call(
        _kernel,
        out_shape=jax.ShapeDtypeStruct((S, D), BF16),
        in_specs=[hbm] * 7 + [pl.BlockSpec(memory_space=pltpu.VMEM)],
        out_specs=hbm,
        scratch_shapes=scratch,
        compiler_params=pltpu.CompilerParams(vmem_limit_bytes=110 * 2**20),
        name="abab_stack",
    )(A_x.reshape(S, D), A_wqkv, A_wo, B_wq, B_wk, B_wv, B_wo, B_beta.reshape(1, H))
    return out.reshape(1, S, D)
```

```python
import jax
import jax.numpy as jnp
from jax import lax
import jax.experimental.pallas as pl
import jax.experimental.pallas.tpu as pltpu

S, D, H, DH = 2048, 1024, 32, 32
NSEG, L = 4, 512
HL = L // 2
NT = D // 128
NP = NT // 2
RC = HL // NP
KC = D // 2 // NP
WIN, DIL = 8, 2
HALO = 16
MZ_ROWS = 128 + 16
LOG2E = 1.4426950408889634
QSCALE = float(DH ** -0.5 * LOG2E)
MASKVAL = float(-1e9 * LOG2E)

B_ORDER = (3, 1, 2, 0)
B_SHARE = (8, 5, 6, 4)
B_SHARE_LAST = (1, 1, 1, 1)
B_FRONT = 0.85
B_POST = (1, 12)
B_LN = (1, 4)
A_WHEN = (.07, .13, .19, .25, .41, .57, .64, .70, .77, .84, .91, .98)
A_LN_WHEN = (.03, .31, .48)

F32, BF16, U32 = jnp.float32, jnp.bfloat16, jnp.uint32
_NT_DIMS = (((1,), (1,)), ((), ()))


def _iota(shape, axis):
    return lax.broadcasted_iota(jnp.int32, shape, axis)


def _dot(a, b):
    return jnp.dot(a, b, preferred_element_type=F32)


def _dot_nt(a, b):
    return lax.dot_general(a, b, _NT_DIMS, preferred_element_type=F32)


def _rows(start, size):
    return pl.ds(start if isinstance(start, int) else pl.multiple_of(start, size), size)


def _tile(k):
    return _rows(128 * k, 128)


def _words(val):
    return pltpu.bitcast(val.astype(BF16), U32)


def _split(words):
    return jnp.concatenate(
        [pltpu.unpack_elementwise(words, index=k, packed_dtype=BF16, unpacked_dtype=F32)
         for k in range(2)], axis=0)


def _merge(val):
    half = val.shape[0] // 2
    return pltpu.pack_elementwise([val[:half], val[half:]], packed_dtype=BF16)


def _put(ref, idx, start, k, words):
    ref[(*idx, _rows(start // 2, words.shape[0]), _tile(k))] = words
    return words


def _bf(words):
    return pltpu.bitcast(words, BF16)


def _phi(t):
    return jnp.where(t > 0, t + 1.0, jnp.exp(t))


def _tree(op, xs):
    xs = list(xs)
    while len(xs) > 1:
        xs = [op(xs[i], xs[i + 1]) if i + 1 < len(xs) else xs[i]
              for i in range(0, len(xs), 2)]
    return xs[0]


def _lhs_terms(a11, a12, a21, a22):
    return (a11 + a22, a21 + a22, a11, a22, a11 + a12, a21 - a11, a12 - a22)


def _rhs_terms(b11, b12, b21, b22):
    return (b11 + b22, b11, b12 - b22, b21 - b11, b22, b11 + b12, b21 + b22)


def _kernel(x_hbm, wqkv_hbm, awo_hbm, wq_hbm, wk_hbm, wv_hbm, wo_hbm, beta_hbm,
            out_hbm,
            x0, x1, x2, x3, wraw, wraw_o, wtmp, wa, wao, wb,
            xn0, xn1, o0, o1,
            qa0, qa1, ka0, ka1, va0, va1,
            qs0, qs1, pq0, pq1, kb0, kb1, pk0, pk1, vt0, vt1,
            zs0, zs1, mz, beta_ref, gtab, zero_ref, sem_x, sem_w, sem_s, sem_o, sem_b):
    X = (x0, x1, x2, x3)
    XN, O = (xn0, xn1), (o0, o1)
    QA, KA, VA = (qa0, qa1), (ka0, ka1), (va0, va1)
    QS, PQ, KB, PK, VT = (qs0, qs1), (pq0, pq1), (kb0, kb1), (pk0, pk1), (vt0, vt1)
    ZS = (zs0, zs1)

    copy = pltpu.make_async_copy

    def x_copies(s):
        return [copy(x_hbm.at[pl.ds(s * L, L)], X[s], sem_x.at[s])]

    def out_copies(s):
        return [copy(X[s], out_hbm.at[pl.ds(s * L, L)], sem_o.at[s])]

    def out_pair_copies(i):
        s = NSEG - 1
        return [copy(X[s].at[:, _tile(t)], out_hbm.at[pl.ds(s * L, L), _tile(t)], sem_o.at[s])
                for t in (i, i + NP)]

    def wao_copies():
        return [copy(awo_hbm.at[:, _tile(t)], wraw_o.at[t], sem_w.at[4]) for t in range(NT)]

    def wb_copies(m):
        return [copy((wq_hbm, wk_hbm, wv_hbm, wo_hbm)[m], wraw.at[3 + m], sem_w.at[m])]

    def slab_copies(m, i):
        cs = [copy(wqkv_hbm.at[r, pl.ds(m * D, D)], wraw.at[m, r], sem_s.at[m, i])
              for r in (_rows(h * (D // 2) + i * KC, KC) for h in range(2))]
        if m == 0:
            cs += [copy(x_hbm.at[r], x0.at[r], sem_s.at[m, i])
                   for r in (_rows(h * HL + i * RC, RC) for h in range(2))]
        return cs

    def start(cs):
        for c in cs:
            c.start()

    def wait(cs):
        for c in cs:
            c.wait()

    def token(*vals):
        bits = [pltpu.bitcast(v[:8, :128], U32) for v in vals]
        return _tree(jnp.bitwise_or, bits) & zero_ref[...]

    def vregs(vals, every=1):
        return [v[u:u + 8] for v in vals for u in range(0, v.shape[0], 8)][::-1][::every]

    def after(words, toks):
        if not toks:
            return words
        slabs = []
        for k in range(words.shape[0] // 8):
            slab = words[8 * k:8 * k + 8]
            if toks.get(k) is not None:
                slab = slab | jnp.concatenate([toks[k]] * (words.shape[1] // 128), axis=1)
            slabs.append(slab)
        return jnp.concatenate(slabs, axis=0)

    def store_rhs(dst, m, i, r, b11, b12, b21, b22):
        terms = _rhs_terms(*[_split(b) for b in (b11, b12, b21, b22)])
        words = [{1: b11, 4: b22}[k] if k in (1, 4) else _merge(v) for k, v in enumerate(terms)]
        return vregs([_put(dst, (m, i), r, k, v) for k, v in enumerate(words)])

    def raw_words(m, r, rows, t):
        return pltpu.bitcast(wraw[m, _rows(r, rows), _tile(t)], U32)

    def prep_b(m, i):
        def piece(j, c):
            r = i * KC + 64 * c
            return store_rhs(wb, m, j, r, *[raw_words(3 + m, r + h * (D // 2), 64, j + u * NP)
                                            for h in range(2) for u in range(2)])

        return [lambda j=j, c=c: piece(j, c) for j in range(NP) for c in range(KC // 64)]

    def prep_a_cols(m, i):
        rows = 32
        st = {}

        def shear(c):
            slot = (_iota((rows, 128), 1) >> 1) & 7
            v = [jnp.concatenate([raw_words(m, i * KC + c * rows + h * (D // 2), rows, t)
                                  for h in range(2)], axis=0) for t in range(NT)]
            v = [x if t == 0 else pltpu.roll(x, 2 * t, 1) for t, x in enumerate(v)]
            v = [v[(-b) % NT] for b in range(NT)]
            for bit in (1, 2, 4):
                sel = (slot & bit) != 0
                v = [jnp.where(sel, v[(b - bit) % NT], v[b]) for b in range(NT)]
            st[c] = [x if b == 0 else pltpu.roll(x, 128 - 2 * b, 1) for b, x in enumerate(v)]
            return vregs(v, 2)

        def terms(c):
            v, half, outs = st[c], rows // 2, []
            for j in range(NP):
                outs += store_rhs(wa, m, j, i * KC + c * rows, v[j][:half], v[j + NP][:half],
                                  v[j][half:], v[j + NP][half:])
            return outs

        order = ((shear, 0), (shear, 1), (terms, 0), (shear, 2), (terms, 1), (shear, 3),
                 (terms, 2), (terms, 3))
        return [lambda f=f, c=c: f(c) for f, c in order]

    def prep_a_rows(i):
        def stage():
            for h in range(2):
                wtmp[h] = pltpu.bitcast(wraw_o[i + h * NP], U32)
            return [zero_ref[...]]

        def rows(h, b):
            parts = [wtmp[h, pl.ds(8 * u + b, 8, stride=64), :] for u in range(8)]
            return jnp.concatenate(parts, axis=0)

        def piece(c):
            return store_rhs(wao, 0, i, 128 * c,
                             rows(0, c), rows(1, c), rows(0, c + NP), rows(1, c + NP))

        return [stage] + [lambda c=c: piece(c) for c in range(4)]

    def store_lhs(dst, t, r, a11, a12, a21, a22, pack=_words):
        terms = _lhs_terms(a11, a12, a21, a22)
        return vregs([_put(dst, (t,), r, k, pack(v)) for k, v in enumerate(terms)])

    def join(toks, slot, tok):
        if tok is not None:
            toks[slot] = tok if toks.get(slot) is None else toks[slot] | tok

    def products(a_ref, w_ref, m, i, emit):
        st = {}

        def prod(k, toks, finish):
            a = jnp.concatenate(
                [after(a_ref[t, :, _tile(k)], toks if t == 0 else None) for t in range(NP)], axis=1)
            r = _dot(_bf(a), _bf(w_ref[m, i, :, _tile(k)]))
            finish(r)
            return r

        def p1(r):
            st["m1"] = r

        def p2(r):
            st["c21"], st["c22"] = r, st["m1"] - r

        def p3(r):
            st["c12"], st["c22"] = r, st["c22"] + r

        def p4(r):
            st["c11"] = st["m1"] + r
            emit(1, 0, st["c21"] + r)

        def p5(r):
            st["c11"] = st["c11"] - r
            emit(0, 1, st["c12"] + r)

        def p6(r):
            emit(1, 1, st["c22"] + r)

        def p7(r):
            emit(0, 0, st["c11"] + r)

        return [lambda toks, k=k, f=f: prod(k, toks, f)
                for k, f in enumerate((p1, p2, p3, p4, p5, p6, p7))]

    def ln_tasks(n, i, off, nr=16):
        src, dst = X[n % NSEG], XN[n % 2]
        st = {}

        def mean():
            st["x"] = [
                jnp.concatenate(
                    [_split(pltpu.bitcast(src[_rows(i * RC + off + h * HL, nr), _tile(t)], U32))
                     for h in range(2)], axis=0) for t in range(NT)]
            part = _tree(jnp.add, st["x"])
            st["mean"] = jnp.sum(part, axis=1, keepdims=True) * (1.0 / D)
            return vregs([part])

        def var():
            st["x"] = [x - st["mean"] for x in st["x"]]
            part = _tree(jnp.add, [x * x for x in st["x"]])
            st["var"] = jnp.sum(part, axis=1, keepdims=True) * (1.0 / D)
            return vregs([part])

        def scale():
            inv = lax.rsqrt(st["var"] + 1e-5)
            y = [x * inv for x in st["x"]]
            r = i * RC + off
            outs = []
            for t in range(NP):
                outs += store_lhs(dst, t, r, y[t][:nr], y[t + NP][:nr], y[t][nr:], y[t + NP][nr:],
                                  _merge)
            return outs

        return [mean, var, scale]

    def proj_a(n, i, which):
        p = n % 2

        def emit(h, c, y):
            t = i + c * NP
            if which == 0:
                QA[p][t, pl.ds(h * HL, HL), :] = y
                return
            buf = KA if which == 1 else VA
            buf[p][t, pl.ds(HALO + h * HL, HL), :] = y
            if h == 0 and n % NSEG == 0:
                buf[p][t, pl.ds(0, HALO), :] = jnp.zeros((HALO, 128), F32)
            elif h == 0:
                buf[p][t, pl.ds(0, HALO), :] = buf[1 - p][t, pl.ds(L, HALO), :]

        return products(XN[p], wa, which, i, emit)

    def proj_b(n, i, which):
        p = n % 2

        def emit(h, c, y):
            if which == 0:
                _put(QS[p], (i,), h * HL, c, _words(y * QSCALE))
                _put(PQ[p], (i,), h * HL, c, _words(_phi(y)))
            elif which == 1:
                _put(KB[p], (i,), h * HL, c, _words(y))
                if n % NSEG != NSEG - 1:
                    y = _phi(y)
                    _put(PK[p], (i,), h * HL, c, _words(y))
                    ZS[p][i + c * NP, pl.ds(8 * h, 8), :] = _tree(jnp.add, vregs([y]))
            else:
                VT[p][i + c * NP, :, pl.ds(h * HL, HL)] = pltpu.bitcast(y.astype(BF16).T, U32)

        return products(XN[p], wb, which, i, emit)

    def out_stage(n, i):
        x = X[n % NSEG]

        def emit(h, c, y):
            where = (pl.ds(h * HL, HL), _tile(i + c * NP))
            x[where] = (x[where].astype(F32) + y).astype(BF16)

        if is_a(n):
            return products(O[n % 2], wao, 0, i, emit)
        return products(O[n % 2], wb, 3, i, emit)

    def att_a_tasks(n, i, off):
        p = n % 2
        base = pl.multiple_of(i * RC, RC) + off
        lg = [[None] * 4 for _ in range(WIN)]
        prob = [None] * 2
        st = {}

        def scores(u):
            r0 = base + (u // 2) * HL + 8 * (u % 2)
            q = [QA[p][t, pl.ds(r0, 8), :] for t in range(NT)]
            for w in range(WIN):
                kr = pl.ds(r0 + HALO - DIL * w, 8)
                lg[w][u] = _tree(jnp.add, [q[t] * KA[p][t, kr, :] for t in range(NT)])
            return [lg[w][u] for w in range(WIN)]

        def exchange(bit):
            a = st["a"] if "a" in st else jnp.concatenate([v for row in lg for v in row], axis=0)
            low = (_iota(a.shape, 1) & bit) == 0
            st["a"] = a + jnp.where(low, pltpu.roll(a, 128 - bit, 1), pltpu.roll(a, bit, 1))
            return vregs([st["a"]], 4)

        def softmax(h):
            v = [st["a"][32 * w + 16 * h:32 * w + 16 * h + 16] * QSCALE for w in range(WIN)]
            if n % NSEG == 0 and off == 0 and h == 0:
                pos = _iota((16, 128), 0) + base
                v = [a if w == 0 else jnp.where(pos >= DIL * w, a, MASKVAL)
                     for w, a in enumerate(v)]
            m = _tree(jnp.maximum, v)
            e = [jnp.exp2(a - m) for a in v]
            inv = 1.0 / _tree(jnp.add, e)
            prob[h] = [a * inv for a in e]
            return vregs(prob[h], 2)

        def mix(t, h):
            return jnp.concatenate([
                _tree(jnp.add, [
                    prob[h][w][8 * u:8 * u + 8]
                    * VA[p][t, pl.ds(base + h * HL + 8 * u + HALO - DIL * w, 8), :]
                    for w in range(WIN)])
                for u in range(2)], axis=0)

        def values(t):
            return store_lhs(O[p], t, i * RC + off, mix(t, 0), mix(t + NP, 0), mix(t, 1), mix(t + NP, 1))

        return ([lambda u=u: scores(u) for u in range(4)]
                + [lambda: exchange(1), lambda: exchange(16)]
                + [lambda h=h: softmax(h) for h in range(2)]
                + [lambda t=t: values(t) for t in range(NP)])

    def att_b_piece(n, i, j, mem, tok):
        p = n % 2
        rows = pl.ds(64 * j, 64)
        nk = 128 * j + 64
        head = _iota((32, 128), 1) >> 5
        key, lane = _iota((64, 128), 0), _iota((64, 128), 1)
        causal = [jnp.where(key > q, MASKVAL, 0.0) for q in (lane, lane ^ 64, lane & 63)]
        high = _iota((8, 128), 1) >= 64
        s, sx, late_q = [], [], []
        for h in range(2):
            qw = after(QS[p][i, rows, _tile(h)], {0: tok, 4: tok})
            early = [jnp.where(head == hh, qw[:32], jnp.uint32(0)) for hh in range(4)]
            late = [jnp.where(head == hh, qw[32:], jnp.uint32(0)) for hh in range(4)]
            late_q.append(jnp.concatenate([late[1], late[0], late[3], late[2]], axis=0))
            qcat = jnp.concatenate([early[0], late[0], late[1], early[1],
                                    early[2], late[2], late[3], early[3]], axis=0)
            st = _dot_nt(_bf(KB[p][i, pl.ds(0, nk // 2), _tile(h)]), _bf(qcat))
            for hh in range(4):
                v = st[:, 128 * hh:128 * (hh + 1)]
                s.append([v[u:u + 8] for u in range(0, nk - 64, 8)]
                         + [v[nk - 64 + u:nk - 56 + u] + causal[hh % 2][u:u + 8]
                            for u in range(0, 64, 8)])
        for h in range(2):
            st = _dot_nt(_bf(KB[p][i, pl.ds(nk // 2, 32), _tile(h)]), _bf(late_q[h]))
            for u in range(2):
                v = st[:, 128 * u:128 * (u + 1)] + causal[2]
                sx.append([v[r:r + 8] for r in range(0, 64, 8)])
        first = token(*[v[0] for v in s])
        m = []
        for u in range(4):
            mx = _tree(jnp.maximum, sx[u])
            for odd in range(2):
                a = _tree(jnp.maximum, s[2 * u + odd])
                b = jnp.maximum(a, mx)
                a = jnp.where(high, a, b) if odd else jnp.where(high, b, a)
                m.append(jnp.broadcast_to(jnp.max(a, axis=0, keepdims=True), (8, 128)))
        e = [[] for _ in range(8)]
        part = [[] for _ in range(8)]

        def exps(v, mh, tok):
            mh = mh if tok is None else mh + pltpu.bitcast(tok, F32)
            return [jnp.exp2(a - mh) for a in v]

        def exp_tile(u, c, tok):
            v = exps(s[u][16 * c:16 * (c + 1)], m[u], tok)
            part[u] = [_tree(jnp.add, part[u] + v)]
            e[u].extend(v)

        def exp_diag(u, tok):
            for odd in range(2):
                exp_tile(2 * u + odd, j, tok)
            v = exps(sx[u], jnp.where(high, m[2 * u], m[2 * u + 1]), tok)
            tot = _tree(jnp.add, v)
            for odd in range(2):
                pick = (lambda a: jnp.where(high, 0.0, a)) if odd else (lambda a: jnp.where(high, a, 0.0))
                part[2 * u + odd] = [part[2 * u + odd][0] + pick(tot)]
                e[2 * u + odd].extend(pick(a) for a in v)

        def finish(h, tok):
            g = i + h * NP
            r = _dot_nt(mem[h], _bf(after(PQ[p][i, rows, _tile(h)], {0: tok})))
            ot = []
            for hh in range(4):
                u = 4 * h + hh
                vt = after(VT[p][g, pl.ds(16 * hh, 16), pl.ds(0, 128 * (j + 1))], {0: tok})
                acc = _dot(_bf(vt), jnp.concatenate(e[u], axis=0).astype(BF16))
                l = jnp.sum(part[u][0], axis=0, keepdims=True)
                gate = gtab[pl.ds(4 * g + hh, 1), :]
                acc = acc * ((1.0 - gate) / l)
                if hh % 2:
                    acc = pltpu.roll(acc, 64, 1)
                wm = gate / (r[128 + 4 * hh:129 + 4 * hh] + 1e-6)
                ot.append(r[32 * hh:32 * hh + 32] * wm + acc)
            return ot

        tasks = []
        for u in range(4):
            tasks += [lambda tok, u=2 * u + odd, c=c: exp_tile(u, c, tok)
                      for odd in range(2) for c in range(j)]
            tasks.append(lambda tok, u=u: exp_diag(u, tok))
        return first, tasks, finish

    def mem_load(n, g):
        if n % NSEG == 0:
            return jnp.zeros((MZ_ROWS, 128), F32)
        return mz[g]

    def mem_update(n, i, h, state):
        p, g = n % 2, i + h * NP
        if n % NSEG == NSEG - 1:
            return
        z = jnp.sum(ZS[p][g], axis=0, keepdims=True)
        new = jnp.concatenate([_dot(_bf(VT[p][g]), _bf(PK[p][i, :, _tile(h)])),
                               jnp.broadcast_to(z, (MZ_ROWS - 128, 128))], axis=0)
        row = _iota((MZ_ROWS, 128), 0)
        row_head = jnp.where(row < 128, row >> 5, (row - 128) >> 2)
        keep = row_head == (_iota((MZ_ROWS, 128), 1) >> 5)
        mz[g] = state + jnp.where(keep, new, 0.0)

    def is_a(n):
        return (n // NSEG) % 2 == 0

    def run_timed(mm, tasks):
        tasks = sorted(tasks, key=lambda x: x[0])
        for k, prod in enumerate(mm):
            toks = {}
            while tasks and tasks[0][0] < 16 * (k + 1):
                time, f = tasks.pop(0)
                join(toks, time - 16 * k, token(*f()))
            prod(toks)
        for _, f in tasks:
            f()

    def body_b(n, i, mm, ln):
        state = [mem_load(n, i + h * NP) for h in range(2)]
        mem = [v.astype(BF16) for v in state]
        share = B_SHARE if len(mm) == 28 else B_SHARE_LAST
        late = []
        if ln:
            for off in range(0, RC, 16):
                late += ln_tasks(n + 2, i, off)
        tiles, tok, pending, done = {}, None, None, []

        def finisher(j, finish):
            def run(tok):
                posts = []
                for h in range(2):
                    ot = finish(h, tok)

                    def post(ot=ot, h=h):
                        tiles[j, h] = jnp.concatenate(ot, axis=0).T
                        return vregs([tiles[j, h]], 4)

                    posts.append(post)
                if j < 2:
                    posts.append(lambda: store_lhs(
                        O[n % 2], i, 128 * j, tiles[j, 0], tiles[j, 1],
                        tiles[j + 2, 0], tiles[j + 2, 1]))
                return posts

            return run

        for k, j in enumerate(B_ORDER):
            first, exps, finish = att_b_piece(n, i, j, mem, tok)
            done += pending(first) if pending else []
            cnt_p = share[k]
            when = [int(32 * cnt_p * B_FRONT * u / len(exps)) for u in range(len(exps))]
            for c in range(cnt_p):
                toks = {}
                if c == 0:
                    join(toks, 0, first)
                if done and c >= min(B_POST[0], cnt_p - 1):
                    join(toks, B_POST[1], token(*done.pop(0)()))
                if late and c >= B_LN[0]:
                    join(toks, B_LN[1], token(*late.pop(0)()))
                r = mm.pop(0)(toks)
                while exps and when[0] < 32 * (c + 1):
                    exps.pop(0)(token(r[8 * (when.pop(0) - 32 * c):]))
                tok = token(r)
            pending = finisher(j, finish)
        for h in range(2):
            mem_update(n, i, h, state[h])
        tok = token(mm.pop(0)(None))
        done += late + pending(tok)
        run_timed(mm, [(16 * (u + 1) + 8, f) for u, f in enumerate(done)])

    def step(n, ln=True, proj=(0, 1, 2), att=True, out=True, extra=None):
        def body(i, c):
            mm = []
            for which in proj:
                mm += (proj_a if is_a(n + 1) else proj_b)(n + 1, i, which)
            if out:
                mm += out_stage(n - 1, i)
            if att and not is_a(n):
                body_b(n, i, mm[14:21] + mm[:14] + mm[21:], ln)
                return c
            tasks = []
            if extra is not None:
                fs = extra(i)
                tasks += [(int(16 * len(mm) * (u + 1) / len(fs)) - 1, f) for u, f in enumerate(fs)]
            span = 16 * len(mm) / 4
            for u, off in enumerate(range(0, RC, 16)):
                if att:
                    tasks += [(int(span * (u + w)), f)
                              for w, f in zip(A_WHEN, att_a_tasks(n, i, off))]
                if ln:
                    when = A_LN_WHEN if att else (.3, .8, 1.3)
                    tasks += [(int(span * (u + w)), f)
                              for w, f in zip(when, ln_tasks(n + 2, i, off))]
            run_timed(mm, tasks)
            return c

        lax.fori_loop(0, NP, body, 0)

    def prep_in_flight(m):
        def tasks(i):
            @pl.when(i + 2 < NP)
            def _():
                start(slab_copies(m, i + 2))

            @pl.when(i + 2 >= NP)
            def _():
                if m < 2:
                    start(slab_copies(m + 1, i + 2 - NP))
                else:
                    pl.when(i + 2 == NP)(lambda: start(x_copies(1) + wao_copies()))

            wait(slab_copies(m, i))
            return prep_a_cols(m, i)

        return tasks

    start(slab_copies(0, 0))
    start([copy(beta_hbm, beta_ref, sem_b)])
    start(slab_copies(0, 1))
    zero_ref[...] = jnp.zeros((8, 128), U32)
    step(-2, proj=(), att=False, out=False, extra=prep_in_flight(0))
    step(-1, ln=False, proj=(0,), att=False, out=False, extra=prep_in_flight(1))
    step(-1, ln=False, proj=(1,), att=False, out=False, extra=prep_in_flight(2))
    start(x_copies(2))
    start(x_copies(3))
    wait(x_copies(1))
    wait(wao_copies())
    step(-1, proj=(2,), att=False, out=False, extra=prep_a_rows)
    for m in range(4):
        start(wb_copies(m))
    wait([copy(beta_hbm, beta_ref, sem_b)])
    gate = jax.nn.sigmoid(beta_ref[...].astype(F32))
    eye = _iota((H, H), 0) == _iota((H, H), 1)
    gcol = jnp.sum(jnp.where(eye, jnp.broadcast_to(gate, (H, H)), 0.0), axis=1, keepdims=True)
    gtab[...] = jnp.broadcast_to(gcol, (H, 128))
    wait(x_copies(2))
    step(0, out=False)
    wait(x_copies(3))
    for m in range(4):
        wait(wb_copies(m))
    step(1, extra=lambda i: prep_b(0, i) + prep_b(1, i))
    step(2, extra=lambda i: prep_b(2, i) + prep_b(3, i))
    for n in range(3, 14):
        step(n)
    start(out_copies(0))
    step(14, ln=False)
    start(out_copies(1))
    step(15, ln=False, proj=())
    start(out_copies(2))
    for i in range(NP):
        run_timed(out_stage(15, i), [])
        start(out_pair_copies(i))
    for s in range(NSEG):
        wait(out_copies(s))


@jax.jit
def pallas_interleave_layers__sliding_local_dilated__memory_aug_infini_attn__prompt_kernel(
    A_x: jax.Array,
    A_wqkv: jax.Array,
    A_wo: jax.Array,
    B_x: jax.Array,
    B_wq: jax.Array,
    B_wk: jax.Array,
    B_wv: jax.Array,
    B_wo: jax.Array,
    B_beta: jax.Array,
):
    del B_x
    assert A_x.shape == (1, S, D)
    hbm = pl.BlockSpec(memory_space=pl.ANY)
    scratch = (
        [pltpu.VMEM((L, D), BF16)] * 4
        + [pltpu.VMEM((7, D, D), BF16), pltpu.VMEM((NT, D, 128), BF16),
           pltpu.VMEM((2, D // 2, 128), U32),
           pltpu.VMEM((3, NP, D // 4, 7 * 128), U32),
           pltpu.VMEM((1, NP, D // 4, 7 * 128), U32),
           pltpu.VMEM((4, NP, D // 4, 7 * 128), U32)]
        + [pltpu.VMEM((NP, HL // 2, 7 * 128), U32)] * 4
        + [pltpu.VMEM((NT, L, 128), F32)] * 2
        + [pltpu.VMEM((NT, HALO + L, 128), F32)] * 4
        + [pltpu.VMEM((NP, L // 2, 2 * 128), U32)] * 8
        + [pltpu.VMEM((NT, 64, L), U32)] * 2
        + [pltpu.VMEM((NT, 16, 128), F32)] * 2
        + [pltpu.VMEM((NT, MZ_ROWS, 128), F32), pltpu.VMEM((1, H), BF16),
           pltpu.VMEM((H, 128), F32),
           pltpu.VMEM((8, 128), U32),
           pltpu.SemaphoreType.DMA((NSEG,)), pltpu.SemaphoreType.DMA((5,)),
           pltpu.SemaphoreType.DMA((3, NP)),
           pltpu.SemaphoreType.DMA((NSEG,)), pltpu.SemaphoreType.DMA]
    )
    out = pl.pallas_call(
        _kernel,
        out_shape=jax.ShapeDtypeStruct((S, D), BF16),
        in_specs=[hbm] * 8,
        out_specs=hbm,
        scratch_shapes=scratch,
        compiler_params=pltpu.CompilerParams(vmem_limit_bytes=110 * 2**20),
        name="abab_stack",
    )(A_x.reshape(S, D), A_wqkv, A_wo, B_wq, B_wk, B_wv, B_wo, B_beta.reshape(1, H))
    return out.reshape(1, S, D)
```

```python
import jax
import jax.numpy as jnp
from jax import lax
import jax.experimental.pallas as pl
import jax.experimental.pallas.tpu as pltpu

S, D, H, DH = 2048, 1024, 32, 32
NSEG, L = 4, 512
HL = L // 2
NT = D // 128
NP = NT // 2
RC = HL // NP
KC = D // 2 // NP
WIN, DIL = 8, 2
HALO = 16
MZ_ROWS = 128 + 16
LOG2E = 1.4426950408889634
QSCALE = float(DH ** -0.5 * LOG2E)
MASKVAL = float(-1e9 * LOG2E)

B_ORDER = (3, 1, 2, 0)
B_SHARE = (8, 5, 6, 4)
B_SHARE_LAST = (1, 1, 1, 1)
B_FRONT = 0.85
B_POST = (8, 14)
B_WAIT = 30
B_TAIL = (22, 4)
B_STORE = 32
B_UPDATE = 2
B_MATS = (2, 0, 1, 3)
UNROLL = 1
B_LN = (1, 4)
A_START = .05
A_TIMES = (.035, .09, .18, .25, .62, .04, .055)
A_LN_WHEN = (.01, .30, .47)
A_PREP_WHEN = (.28, .33, .36, .39, .44, .50, .53, .60)

F32, BF16, U32 = jnp.float32, jnp.bfloat16, jnp.uint32
_NT_DIMS = (((1,), (1,)), ((), ()))


def _iota(shape, axis):
    return lax.broadcasted_iota(jnp.int32, shape, axis)


def _dot(a, b):
    return jnp.dot(a, b, preferred_element_type=F32)


def _dot_nt(a, b):
    return lax.dot_general(a, b, _NT_DIMS, preferred_element_type=F32)


def _rows(start, size):
    return pl.ds(start if isinstance(start, int) else pl.multiple_of(start, size), size)


def _tile(k):
    return _rows(128 * k, 128)


def _words(val):
    return pltpu.bitcast(val.astype(BF16), U32)


def _split(words):
    return jnp.concatenate(
        [pltpu.unpack_elementwise(words, index=k, packed_dtype=BF16, unpacked_dtype=F32)
         for k in range(2)], axis=0)


def _merge(val):
    half = val.shape[0] // 2
    return pltpu.pack_elementwise([val[:half], val[half:]], packed_dtype=BF16)


def _put(ref, idx, start, k, words):
    ref[(*idx, _rows(start // 2, words.shape[0]), _tile(k))] = words
    return words


def _bf(words):
    return pltpu.bitcast(words, BF16)


def _phi(t):
    return jnp.where(t > 0, t + 1.0, jnp.exp(t))


def _tree(op, xs):
    xs = list(xs)
    while len(xs) > 1:
        xs = [op(xs[i], xs[i + 1]) if i + 1 < len(xs) else xs[i]
              for i in range(0, len(xs), 2)]
    return xs[0]


def _lhs_terms(a11, a12, a21, a22):
    return (a11 + a22, a21 + a22, a11, a22, a11 + a12, a21 - a11, a12 - a22)


def _rhs_terms(b11, b12, b21, b22):
    return (b11 + b22, b11, b12 - b22, b21 - b11, b22, b11 + b12, b21 + b22)


def _kernel(x_hbm, wqkv_hbm, awo_hbm, wq_hbm, wk_hbm, wv_hbm, wo_hbm, beta_hbm,
            out_hbm,
            x0, x1, x2, x3, wraw, wraw_o, wtmp, wa, wao, wb,
            xn0, xn1, o0, o1,
            qa0, qa1, ka0, ka1, va0, va1,
            qs0, qs1, pq0, pq1, kb0, kb1, pk0, pk1, vt0, vt1,
            zs0, zs1, mz, beta_ref, gtab, zero_ref, sem_x, sem_w, sem_s, sem_o, sem_b):
    X = (x0, x1, x2, x3)
    XN, O = (xn0, xn1), (o0, o1)
    QA, KA, VA = (qa0, qa1), (ka0, ka1), (va0, va1)
    QS, PQ, KB, PK, VT = (qs0, qs1), (pq0, pq1), (kb0, kb1), (pk0, pk1), (vt0, vt1)
    ZS = (zs0, zs1)

    copy = pltpu.make_async_copy

    def x_copies(s):
        return [copy(x_hbm.at[pl.ds(s * L, L)], X[s], sem_x.at[s])]

    def out_copies(s):
        return [copy(X[s], out_hbm.at[pl.ds(s * L, L)], sem_o.at[s])]

    def out_pair_copies(i):
        s = NSEG - 1
        return [copy(X[s].at[:, _tile(t)], out_hbm.at[pl.ds(s * L, L), _tile(t)], sem_o.at[s])
                for t in (i, i + NP)]

    def wao_copies():
        return [copy(awo_hbm.at[:, _tile(t)], wraw_o.at[t], sem_w.at[4]) for t in range(NT)]

    def wb_copies(m):
        return [copy((wq_hbm, wk_hbm, wv_hbm, wo_hbm)[m], wraw.at[3 + m], sem_w.at[m])]

    def slab_copies(m, i):
        cs = [copy(wqkv_hbm.at[r, pl.ds(m * D, D)], wraw.at[m, r], sem_s.at[m, i])
              for r in (_rows(h * (D // 2) + i * KC, KC) for h in range(2))]
        if m == 0:
            cs += [copy(x_hbm.at[r], x0.at[r], sem_s.at[m, i])
                   for r in (_rows(h * HL + i * RC, RC) for h in range(2))]
        return cs

    def start(cs):
        for c in cs:
            c.start()

    def wait(cs):
        for c in cs:
            c.wait()

    def token(*vals):
        bits = [pltpu.bitcast(v[:8, :128], U32) for v in vals]
        return _tree(jnp.bitwise_or, bits) & zero_ref[:8]

    def vregs(vals, every=1):
        return [v[u:u + 8] for v in vals for u in range(0, v.shape[0], 8)][::-1][::every]

    def after(words, toks):
        if not toks:
            return words
        slabs = []
        for k in range(words.shape[0] // 8):
            slab = words[8 * k:8 * k + 8]
            if toks.get(k) is not None:
                slab = slab | jnp.concatenate([toks[k]] * (words.shape[1] // 128), axis=1)
            slabs.append(slab)
        return jnp.concatenate(slabs, axis=0)

    def store_rhs(dst, m, i, r, b11, b12, b21, b22):
        terms = _rhs_terms(*[_split(b) for b in (b11, b12, b21, b22)])
        words = [{1: b11, 4: b22}[k] if k in (1, 4) else _merge(v) for k, v in enumerate(terms)]
        return vregs([_put(dst, (m, i), r, k, v) for k, v in enumerate(words)])

    def raw_words(m, r, rows, t):
        return pltpu.bitcast(wraw[m, _rows(r, rows), _tile(t)], U32)

    def prep_b(m, i):
        def piece(j, c):
            r = i * KC + 32 * c
            return store_rhs(wb, m, j, r, *[raw_words(3 + m, r + h * (D // 2), 32, j + u * NP)
                                            for h in range(2) for u in range(2)])

        return [lambda j=j, c=c: piece(j, c) for j in range(NP) for c in range(KC // 32)]

    def prep_a_cols(m, i):
        rows = 32
        st = {}

        def shear(c):
            slot = (_iota((rows, 128), 1) >> 1) & 7
            v = [jnp.concatenate([raw_words(m, i * KC + c * rows + h * (D // 2), rows, t)
                                  for h in range(2)], axis=0) for t in range(NT)]
            v = [x if t == 0 else pltpu.roll(x, 2 * t, 1) for t, x in enumerate(v)]
            v = [v[(-b) % NT] for b in range(NT)]
            for bit in (1, 2, 4):
                sel = (slot & bit) != 0
                v = [jnp.where(sel, v[(b - bit) % NT], v[b]) for b in range(NT)]
            st[c] = [x if b == 0 else pltpu.roll(x, 128 - 2 * b, 1) for b, x in enumerate(v)]
            return vregs(v, 2)

        def terms(c):
            v, half, outs = st[c], rows // 2, []
            for j in range(NP):
                outs += store_rhs(wa, m, j, i * KC + c * rows, v[j][:half], v[j + NP][:half],
                                  v[j][half:], v[j + NP][half:])
            return outs

        order = ((shear, 0), (shear, 1), (terms, 0), (shear, 2), (terms, 1), (shear, 3),
                 (terms, 2), (terms, 3))
        return [lambda f=f, c=c: f(c) for f, c in order]

    def prep_a_rows(i):
        def stage(t):
            words = [pltpu.bitcast(wraw_o[i + h * NP, _tile(t), :], U32) for h in range(2)]
            for h in range(2):
                wtmp[h, pl.ds(65 * t, 64), :] = words[h]
            return vregs(words)

        def rows(h, b, u):
            return jnp.concatenate(
                [wtmp[h, pl.ds(8 * (u + k) + b, 8, stride=65), :] for k in range(2)], axis=0)

        def piece(c, u):
            return store_rhs(wao, 0, i, 128 * c + 16 * u, rows(0, c, u), rows(1, c, u),
                             rows(0, c + NP, u), rows(1, c + NP, u))

        return ([lambda t=t: stage(t) for t in range(NT)]
                + [lambda c=c, u=u: piece(c, u) for c in range(4) for u in range(0, 8, 2)])

    def store_lhs(dst, t, r, a11, a12, a21, a22, pack=_words):
        terms = _lhs_terms(a11, a12, a21, a22)
        return vregs([_put(dst, (t,), r, k, pack(v)) for k, v in enumerate(terms)])

    def join(toks, slot, tok):
        if tok is not None:
            toks[slot] = tok if toks.get(slot) is None else toks[slot] | tok

    def products(a_ref, w_ref, m, i, emit):
        st = {}

        def prod(k, toks, finish):
            a = jnp.concatenate(
                [after(a_ref[t, :, _tile(k)], toks if t == 0 else None) for t in range(NP)], axis=1)
            r = _dot(_bf(a), _bf(w_ref[m, i, :, _tile(k)]))
            finish(r)
            return r

        def p1(r):
            st["m1"] = r

        def p2(r):
            st["c21"], st["c22"] = r, st["m1"] - r

        def p3(r):
            st["c12"], st["c22"] = r, st["c22"] + r

        def p4(r):
            st["c11"] = st["m1"] + r
            emit(1, 0, st["c21"] + r)

        def p5(r):
            st["c11"] = st["c11"] - r
            emit(0, 1, st["c12"] + r)

        def p6(r):
            emit(1, 1, st["c22"] + r)

        def p7(r):
            emit(0, 0, st["c11"] + r)

        return [lambda toks, k=k, f=f: prod(k, toks, f)
                for k, f in enumerate((p1, p2, p3, p4, p5, p6, p7))]

    def ln_tasks(n, i, off, nr=16):
        src, dst = X[n % NSEG], XN[n % 2]
        st = {}

        def mean():
            st["x"] = [
                jnp.concatenate(
                    [_split(pltpu.bitcast(src[_rows(i * RC + off + h * HL, nr), _tile(t)], U32))
                     for h in range(2)], axis=0) for t in range(NT)]
            part = _tree(jnp.add, st["x"])
            st["mean"] = jnp.sum(part, axis=1, keepdims=True) * (1.0 / D)
            return vregs([part])

        def var():
            st["x"] = [x - st["mean"] for x in st["x"]]
            part = _tree(jnp.add, [x * x for x in st["x"]])
            st["var"] = jnp.sum(part, axis=1, keepdims=True) * (1.0 / D)
            return vregs([part])

        def scale():
            inv = lax.rsqrt(st["var"] + 1e-5)
            y = [x * inv for x in st["x"]]
            r = i * RC + off
            outs = []
            for t in range(NP):
                outs += store_lhs(dst, t, r, y[t][:nr], y[t + NP][:nr], y[t][nr:], y[t + NP][nr:],
                                  _merge)
            return outs

        return [mean, var, scale]

    def proj_a(n, i, which):
        p = n % 2

        def emit(h, c, y):
            t = i + c * NP
            if which == 0:
                QA[p][t, pl.ds(h * HL, HL), :] = y
                return
            buf = KA if which == 1 else VA
            buf[p][t, pl.ds(HALO + h * HL, HL), :] = y
            if h == 0 and n % NSEG == 0:
                buf[p][t, pl.ds(0, HALO), :] = jnp.zeros((HALO, 128), F32)
            elif h == 0:
                buf[p][t, pl.ds(0, HALO), :] = buf[1 - p][t, pl.ds(L, HALO), :]

        return products(XN[p], wa, which, i, emit)

    def proj_b(n, i, which):
        p = n % 2

        def emit(h, c, y):
            if which == 0:
                _put(QS[p], (i,), h * HL, c, _words(y * QSCALE))
                _put(PQ[p], (i,), h * HL, c, _words(_phi(y)))
            elif which == 1:
                _put(KB[p], (i,), h * HL, c, _words(y))
                if n % NSEG != NSEG - 1:
                    y = _phi(y)
                    _put(PK[p], (i,), h * HL, c, _words(y))
                    ZS[p][i + c * NP, pl.ds(8 * h, 8), :] = _tree(jnp.add, vregs([y]))
            else:
                VT[p][i + c * NP, :, pl.ds(h * HL, HL)] = pltpu.bitcast(y.astype(BF16).T, U32)

        return products(XN[p], wb, which, i, emit)

    def out_stage(n, i):
        x = X[n % NSEG]

        def emit(h, c, y):
            where = (pl.ds(h * HL, HL), _tile(i + c * NP))
            x[where] = (x[where].astype(F32) + y).astype(BF16)

        if is_a(n):
            return products(O[n % 2], wao, 0, i, emit)
        return products(O[n % 2], wb, 3, i, emit)

    def att_a_tasks(n, i, off):
        p = n % 2
        base = (i * RC if isinstance(i, int) else pl.multiple_of(i * RC, RC)) + off
        starts = [base + (u // 2) * HL + 8 * (u % 2) for u in range(4)]
        lg, mixed = [[] for _ in range(4)], {}

        def scores(u, ws):
            q = [QA[p][t, pl.ds(starts[u], 8), :] for t in range(NT)]
            for w in ws:
                kr = pl.ds(starts[u] + HALO - DIL * w, 8)
                lg[u].append(_tree(jnp.add, [q[t] * KA[p][t, kr, :] for t in range(NT)]))
            return lg[u][-len(ws):]

        def exchange(u, bit):
            low = (_iota((8, 128), 1) & bit) == 0
            lg[u] = [a + jnp.where(low, pltpu.roll(a, 128 - bit, 1), pltpu.roll(a, bit, 1))
                     for a in lg[u]]
            return lg[u]

        def softmax(u):
            v = [a * QSCALE for a in lg[u]]
            if n % NSEG == 0 and off == 0 and u < 2:
                pos = _iota((8, 128), 0) + starts[u]
                v = [a if w == 0 else jnp.where(pos >= DIL * w, a, MASKVAL)
                     for w, a in enumerate(v)]
            m = _tree(jnp.maximum, v)
            e = [jnp.exp2(a - m) for a in v]
            inv = 1.0 / _tree(jnp.add, e)
            lg[u] = [a * inv for a in e]
            return lg[u]

        def mix(t, h):
            for c in range(2):
                mixed[t, h, c] = jnp.concatenate([
                    _tree(jnp.add, [
                        lg[u][w] * VA[p][t + c * NP, pl.ds(starts[u] + HALO - DIL * w, 8), :]
                        for w in range(WIN)])
                    for u in (2 * h, 2 * h + 1)], axis=0)
            return vregs([mixed[t, h, c] for c in range(2)])

        def store(t):
            return store_lhs(O[p], t, i * RC + off,
                             *[mixed[t, h, c] for h in range(2) for c in range(2)])

        d_score, lag1, lag2, lag3, t_mix, d_mix, d_store = A_TIMES
        tasks = []
        for u in range(4):
            t = A_START + d_score * (2 * u + 1)
            tasks += [(t - d_score, lambda u=u: scores(u, range(4))),
                      (t, lambda u=u: scores(u, range(4, 8))),
                      (t + lag1, lambda u=u: exchange(u, 1)),
                      (t + lag2, lambda u=u: exchange(u, 16)),
                      (t + lag3, lambda u=u: softmax(u))]
        for k in range(NP):
            t = t_mix + k * (d_mix + d_store)
            tasks += [(t, lambda k=k: mix(k, 0)), (t + d_mix, lambda k=k: mix(k, 1))]
            tasks += [(t + d_mix + d_store / 2, lambda k=k: store(k))]
        return tasks

    def att_b_piece(n, i, j, mem, tok):
        p = n % 2
        rows = pl.ds(64 * j, 64)
        nk = 128 * j + 64
        head = _iota((32, 128), 1) >> 5
        key, lane = _iota((64, 128), 0), _iota((64, 128), 1)
        causal = [jnp.where(key > q, MASKVAL, 0.0) for q in (lane, lane ^ 64, lane & 63)]
        high = _iota((8, 128), 1) >= 64
        s, sx, late_q = [], [], []
        for h in range(2):
            qw = after(QS[p][i, rows, _tile(h)], {0: tok, 4: tok})
            early = [jnp.where(head == hh, qw[:32], jnp.uint32(0)) for hh in range(4)]
            late = [jnp.where(head == hh, qw[32:], jnp.uint32(0)) for hh in range(4)]
            late_q.append(jnp.concatenate([late[1], late[0], late[3], late[2]], axis=0))
            qcat = jnp.concatenate([early[0], late[0], late[1], early[1],
                                    early[2], late[2], late[3], early[3]], axis=0)
            st = _dot_nt(_bf(KB[p][i, pl.ds(0, nk // 2), _tile(h)]), _bf(qcat))
            for hh in range(4):
                v = st[:, 128 * hh:128 * (hh + 1)]
                s.append([v[u:u + 8] for u in range(0, nk - 64, 8)]
                         + [v[nk - 64 + u:nk - 56 + u] + causal[hh % 2][u:u + 8]
                            for u in range(0, 64, 8)])
        for h in range(2):
            st = _dot_nt(_bf(KB[p][i, pl.ds(nk // 2, 32), _tile(h)]), _bf(late_q[h]))
            for u in range(2):
                v = st[:, 128 * u:128 * (u + 1)] + causal[2]
                sx.append([v[r:r + 8] for r in range(0, 64, 8)])
        first = token(*[v[0] for v in s])
        m = []
        for u in range(4):
            mx = _tree(jnp.maximum, sx[u])
            for odd in range(2):
                a = _tree(jnp.maximum, s[2 * u + odd])
                b = jnp.maximum(a, mx)
                a = jnp.where(high, a, b) if odd else jnp.where(high, b, a)
                m.append(jnp.broadcast_to(jnp.max(a, axis=0, keepdims=True), (8, 128)))
        e = [[] for _ in range(8)]
        part = [[] for _ in range(8)]

        def exps(v, mh, tok):
            mh = mh if tok is None else mh + pltpu.bitcast(tok, F32)
            return [jnp.exp2(a - mh) for a in v]

        def exp_tile(u, c, tok):
            v = exps(s[u][16 * c:16 * (c + 1)], m[u], tok)
            part[u] = [_tree(jnp.add, part[u] + v)]
            e[u].extend(v)

        def exp_diag(u, tok):
            for odd in range(2):
                exp_tile(2 * u + odd, j, tok)
            v = exps(sx[u], jnp.where(high, m[2 * u], m[2 * u + 1]), tok)
            tot = _tree(jnp.add, v)
            for odd in range(2):
                pick = (lambda a: jnp.where(high, 0.0, a)) if odd else (lambda a: jnp.where(high, a, 0.0))
                part[2 * u + odd] = [part[2 * u + odd][0] + pick(tot)]
                e[2 * u + odd].extend(pick(a) for a in v)

        def finish(h, tok):
            g = i + h * NP
            r = mem[h][:, 128 * j:128 * (j + 1)]
            ot = []
            for hh in range(4):
                u = 4 * h + hh
                vt = after(VT[p][g, pl.ds(16 * hh, 16), pl.ds(0, 128 * (j + 1))], {0: tok})
                acc = _dot(_bf(vt), jnp.concatenate(e[u], axis=0).astype(BF16))
                l = jnp.sum(part[u][0], axis=0, keepdims=True)
                gate = gtab[pl.ds(4 * g + hh, 1), :]
                acc = acc * ((1.0 - gate) / l)
                if hh % 2:
                    acc = pltpu.roll(acc, 64, 1)
                wm = gate / (r[128 + 4 * hh:129 + 4 * hh] + 1e-6)
                ot.append(r[32 * hh:32 * hh + 32] * wm + acc)
            return ot

        tasks = []
        for u in range(4):
            tasks += [lambda tok, u=2 * u + odd, c=c: exp_tile(u, c, tok)
                      for odd in range(2) for c in range(j)]
            tasks.append(lambda tok, u=u: exp_diag(u, tok))
        return first, tasks, finish

    def mem_load(n, g):
        if n % NSEG == 0:
            return jnp.zeros((MZ_ROWS, 128), F32)
        return mz[g]

    def mem_read(n, i, h, state, tok):
        pq = after(PQ[n % 2][i, :, _tile(h)], {8 * u: tok for u in range(4)})
        return _dot_nt(state.astype(BF16), _bf(pq))

    def mem_update(n, i, h, state, tok):
        p, g = n % 2, i + h * NP
        z = jnp.sum(ZS[p][g], axis=0, keepdims=True)
        new = jnp.concatenate([_dot(_bf(after(VT[p][g], {0: tok})), _bf(PK[p][i, :, _tile(h)])),
                               jnp.broadcast_to(z, (MZ_ROWS - 128, 128))], axis=0)
        row = _iota((MZ_ROWS, 128), 0)
        row_head = jnp.where(row < 128, row >> 5, (row - 128) >> 2)
        keep = row_head == (_iota((MZ_ROWS, 128), 1) >> 5)
        mz[g] = new = state + jnp.where(keep, new, 0.0)
        return new

    def is_a(n):
        return (n // NSEG) % 2 == 0

    def run_timed(mm, tasks):
        tasks = sorted(tasks, key=lambda x: x[0])
        for k, prod in enumerate(mm):
            toks = {}
            while tasks and tasks[0][0] < 16 * (k + 1):
                time, f = tasks.pop(0)
                join(toks, time - 16 * k, token(*f()))
            prod(toks)
        for _, f in tasks:
            f()

    def body_b(n, its, mm, ln):
        share = B_SHARE if len(mm) == 28 * len(its) else B_SHARE_LAST
        spare = len(mm) // len(its) - sum(share)
        late, done = [], []
        tok, pending = None, None

        def finisher(i, j, finish, tiles):
            def run(tok):
                posts = []
                for h in range(2):
                    ot = finish(h, tok)

                    def post(ot=ot, h=h):
                        tiles[j, h] = jnp.concatenate(ot, axis=0).T
                        return vregs([tiles[j, h]], 4)

                    posts.append(post)
                if (j ^ 2, 0) in tiles:
                    posts += [lambda r=r: store_lhs(
                        O[n % 2], i, 128 * (j % 2) + r,
                        *[tiles[j % 2 + u, h][r:r + B_STORE] for u in (0, 2) for h in range(2)])
                        for r in range(0, 128, B_STORE)]
                tiles[j, 0] = None
                return posts

            return run

        for i in its:
            state = [mem_load(n, i + h * NP) for h in range(2)]
            mem, tiles = [], {}
            if ln:
                for off in range(0, RC, 16):
                    late += ln_tasks(n + 2, i, off)
            for k, j in enumerate(B_ORDER):
                first, exps, finish = att_b_piece(n, i, j, mem, tok)
                done += pending(first) if pending else []
                cnt = share[k] + (0 if i is its[-1] else (spare + 3 - k) // 4)
                when = [int(32 * cnt * B_FRONT * u / len(exps)) for u in range(len(exps))]
                for c in range(cnt):
                    toks = {}
                    if c == 0:
                        join(toks, 0, first)
                    for slot in B_POST:
                        if done and 16 * c + slot >= min(B_WAIT, 16 * cnt - 4):
                            join(toks, slot, token(*done.pop(0)()))
                    if late and c >= B_LN[0]:
                        join(toks, B_LN[1], token(*late.pop(0)()))
                    r = mm.pop(0)(toks)
                    while exps and when[0] < 32 * (c + 1):
                        exps.pop(0)(token(r[8 * (when.pop(0) - 32 * c):]))
                    tok = token(r)
                    if k == 0 and c == 0:
                        mem.extend(mem_read(n, i, h, state[h], tok) for h in range(2))
                        done.append(lambda mem=mem: [v[:, 128 * u:] for v in mem for u in range(4)])
                    if k == B_UPDATE and c == 0 and n % NSEG != NSEG - 1:
                        new = [mem_update(n, i, h, state[h], tok) for h in range(2)]
                        done.append(lambda new=new: new)
                pending = finisher(i, j, finish, tiles)
        tok = token(mm.pop(0)(None))
        done += late + pending(tok)
        run_timed(mm, [(B_TAIL[0] + B_TAIL[1] * u, f) for u, f in enumerate(done)])

    def step(n, ln=True, proj=(0, 1, 2), att=True, out=True, extra=None, unroll=UNROLL):
        def body(its):
            mm = []
            for i in its:
                for which in (B_MATS if att and not is_a(n) else (0, 1, 2, 3)):
                    if which in proj:
                        mm += (proj_a if is_a(n + 1) else proj_b)(n + 1, i, which)
                    elif which == 3 and out:
                        mm += out_stage(n - 1, i)
            if att and not is_a(n):
                body_b(n, its, mm, ln)
                return
            tasks, span = [], 16 * len(mm) / (4 * len(its))
            for k, i in enumerate(its):
                if extra is not None:
                    fs = extra(i)
                    tasks += [(int(span * (4 * k + u // 8 + A_PREP_WHEN[u % 8])) if att else
                               int(4 * span * (k + (u + 1) / len(fs))) - 1, f)
                              for u, f in enumerate(fs)]
                for u, off in enumerate(range(0, RC, 16), 4 * k):
                    if att:
                        tasks += [(int(span * (u + w)), f) for w, f in att_a_tasks(n, i, off)]
                    if ln:
                        when = A_LN_WHEN if att else (.3, .8, 1.3)
                        tasks += [(int(span * (u + w)), f)
                                  for w, f in zip(when, ln_tasks(n + 2, i, off))]
            run_timed(mm, tasks)

        if unroll == NP:
            body(list(range(NP)))
        else:
            pl.loop(0, NP // unroll)(lambda i: body([unroll * i + u for u in range(unroll)]))

    def prep_in_flight(m):
        def tasks(i):
            @pl.when(i + 2 < NP)
            def _():
                start(slab_copies(m, i + 2))

            if m < 2:
                pl.when(i + 2 >= NP)(lambda: start(slab_copies(m + 1, i + 2 - NP)))
            else:
                pl.when(i == 0)(lambda: start(x_copies(1) + wao_copies()))

            wait(slab_copies(m, i))
            return prep_a_cols(m, i)

        return tasks

    start(slab_copies(0, 0))
    start([copy(beta_hbm, beta_ref.at[0], sem_b)])
    start(slab_copies(0, 1))
    zero_ref[:8] = jnp.zeros((8, 128), U32)
    step(-2, proj=(), att=False, out=False, extra=prep_in_flight(0), unroll=1)
    step(-1, ln=False, proj=(0,), att=False, out=False, extra=prep_in_flight(1), unroll=1)
    step(-1, ln=False, proj=(1,), att=False, out=False, extra=prep_in_flight(2), unroll=1)
    start(x_copies(2))
    start(x_copies(3))
    wait(x_copies(1))
    wait(wao_copies())
    step(-1, proj=(2,), att=False, out=False, extra=prep_a_rows)
    for m in range(4):
        start(wb_copies(m))
    wait([copy(beta_hbm, beta_ref.at[0], sem_b)])
    gate = jax.nn.sigmoid(beta_ref[0].astype(F32))
    eye = _iota((H, H), 0) == _iota((H, H), 1)
    gcol = jnp.sum(jnp.where(eye, jnp.broadcast_to(gate, (H, H)), 0.0), axis=1, keepdims=True)
    gtab[...] = jnp.broadcast_to(gcol, (H, 128))
    wait(x_copies(2))
    step(0, out=False)
    wait(x_copies(3))
    for m in range(4):
        wait(wb_copies(m))
    step(1, extra=lambda i: prep_b(0, i) + prep_b(1, i))
    step(2, extra=lambda i: prep_b(2, i) + prep_b(3, i))
    for n in range(3, 14):
        step(n)
    start(out_copies(0))
    step(14, ln=False)
    start(out_copies(1))
    step(15, ln=False, proj=())
    start(out_copies(2))
    for i in range(NP):
        run_timed(out_stage(15, i), [])
        start(out_pair_copies(i))
    for s in range(NSEG):
        wait(out_copies(s))


@jax.jit
def pallas_interleave_layers__sliding_local_dilated__memory_aug_infini_attn__prompt_kernel(
    A_x: jax.Array,
    A_wqkv: jax.Array,
    A_wo: jax.Array,
    B_x: jax.Array,
    B_wq: jax.Array,
    B_wk: jax.Array,
    B_wv: jax.Array,
    B_wo: jax.Array,
    B_beta: jax.Array,
):
    del B_x
    assert A_x.shape == (1, S, D)
    hbm = pl.BlockSpec(memory_space=pl.ANY)
    scratch = (
        [pltpu.VMEM((L, D), BF16)] * 4
        + [pltpu.VMEM((7, D, D), BF16), pltpu.VMEM((NT, D, 128), BF16),
           pltpu.VMEM((2, 576, 128), U32),
           pltpu.VMEM((3, NP, D // 4, 7 * 128), U32),
           pltpu.VMEM((1, NP, D // 4, 7 * 128), U32),
           pltpu.VMEM((4, NP, D // 4, 7 * 128), U32)]
        + [pltpu.VMEM((NP, HL // 2, 7 * 128), U32)] * 4
        + [pltpu.VMEM((NT, L, 128), F32)] * 2
        + [pltpu.VMEM((NT, HALO + L, 128), F32)] * 4
        + [pltpu.VMEM((NP, L // 2, 2 * 128), U32)] * 8
        + [pltpu.VMEM((NT, 64, L), U32)] * 2
        + [pltpu.VMEM((NT, 16, 128), F32)] * 2
        + [pltpu.VMEM((NT, MZ_ROWS, 128), F32), pltpu.VMEM((8, 1, H), BF16),
           pltpu.VMEM((H, 128), F32),
           pltpu.VMEM((88, 128), U32),
           pltpu.SemaphoreType.DMA((NSEG,)), pltpu.SemaphoreType.DMA((5,)),
           pltpu.SemaphoreType.DMA((3, NP)),
           pltpu.SemaphoreType.DMA((NSEG,)), pltpu.SemaphoreType.DMA]
    )
    out = pl.pallas_call(
        _kernel,
        out_shape=jax.ShapeDtypeStruct((S, D), BF16),
        in_specs=[hbm] * 8,
        out_specs=hbm,
        scratch_shapes=scratch,
        compiler_params=pltpu.CompilerParams(vmem_limit_bytes=110 * 2**20),
        name="abab_stack",
    )(A_x.reshape(S, D), A_wqkv, A_wo, B_wq, B_wk, B_wv, B_wo, B_beta.reshape(1, H))
    return out.reshape(1, S, D)
```

```python
import jax
import jax.numpy as jnp
from jax import lax
import jax.experimental.pallas as pl
import jax.experimental.pallas.tpu as pltpu

S, D, H, DH = 2048, 1024, 32, 32
NSEG, L = 4, 512
HL = L // 2
NT = D // 128
NP = NT // 2
RC = HL // NP
KC = D // 2 // NP
WIN, DIL = 8, 2
HALO = 16
MZ_ROWS = 128 + 16
LOG2E = 1.4426950408889634
QSCALE = float(DH ** -0.5 * LOG2E)
MASKVAL = float(-1e9 * LOG2E)

B_ORDER = (3, 1, 2, 0)
B_SHARE = (8, 5, 5, 5)
B_LAST = (1, 1, 1, 1, 0.811, 24, 21, 7)
B_FRONT = 0.842
B_POST = (6, 15)
B_WAIT = 29
B_TAIL = (29, 10)
B_STORE = 16
B_UPDATE = 0
B_READ = 0
A_MATS = (3, 0, 2, 1)
B_MATS = (2, 0, 1, 3)
UNROLL = 1
B_LN = (1, 3)
A_START = 0.051
A_TIMES = (0.035, 0.077, 0.18, 0.275, 0.598, 0.039, 0.055)
A_LN_WHEN = (0.023, 0.3, 0.486)
A_PREP_WHEN = (0.279, 0.33, 0.408, 0.423, 0.353, 0.5, 0.556, 0.578)

F32, BF16, U32 = jnp.float32, jnp.bfloat16, jnp.uint32
_NT_DIMS = (((1,), (1,)), ((), ()))


def _iota(shape, axis):
    return lax.broadcasted_iota(jnp.int32, shape, axis)


def _dot(a, b):
    return jnp.dot(a, b, preferred_element_type=F32)


def _dot_nt(a, b):
    return lax.dot_general(a, b, _NT_DIMS, preferred_element_type=F32)


def _rows(start, size):
    return pl.ds(start if isinstance(start, int) else pl.multiple_of(start, size), size)


def _tile(k):
    return _rows(128 * k, 128)


def _words(val):
    return pltpu.bitcast(val.astype(BF16), U32)


def _split(words):
    return jnp.concatenate(
        [pltpu.unpack_elementwise(words, index=k, packed_dtype=BF16, unpacked_dtype=F32)
         for k in range(2)], axis=0)


def _merge(val):
    half = val.shape[0] // 2
    return pltpu.pack_elementwise([val[:half], val[half:]], packed_dtype=BF16)


def _put(ref, idx, start, k, words):
    ref[(*idx, _rows(start // 2, words.shape[0]), _tile(k))] = words
    return words


def _bf(words):
    return pltpu.bitcast(words, BF16)


def _phi(t):
    return jnp.where(t > 0, t + 1.0, jnp.exp(t))


def _tree(op, xs):
    xs = list(xs)
    while len(xs) > 1:
        xs = [op(xs[i], xs[i + 1]) if i + 1 < len(xs) else xs[i]
              for i in range(0, len(xs), 2)]
    return xs[0]


def _lhs_terms(a11, a12, a21, a22):
    return (a11 + a22, a21 + a22, a11, a22, a11 + a12, a21 - a11, a12 - a22)


def _rhs_terms(b11, b12, b21, b22):
    return (b11 + b22, b11, b12 - b22, b21 - b11, b22, b11 + b12, b21 + b22)


def _kernel(x_hbm, wqkv_hbm, awo_hbm, wq_hbm, wk_hbm, wv_hbm, wo_hbm, beta_hbm,
            out_hbm,
            x0, x1, x2, x3, wraw, wraw_o, wtmp, wa, wao, wb,
            xn0, xn1, o0, o1,
            qa0, qa1, ka0, ka1, va0, va1,
            qs0, qs1, pq0, pq1, kb0, kb1, pk0, pk1, vt0, vt1,
            zs0, zs1, mz, beta_ref, gtab, zero_ref, sem_x, sem_w, sem_s, sem_o, sem_b):
    X = (x0, x1, x2, x3)
    XN, O = (xn0, xn1), (o0, o1)
    QA, KA, VA = (qa0, qa1), (ka0, ka1), (va0, va1)
    QS, PQ, KB, PK, VT = (qs0, qs1), (pq0, pq1), (kb0, kb1), (pk0, pk1), (vt0, vt1)
    ZS = (zs0, zs1)

    copy = pltpu.make_async_copy

    def x_copies(s):
        return [copy(x_hbm.at[pl.ds(s * L, L)], X[s], sem_x.at[s])]

    def out_copies(s):
        return [copy(X[s], out_hbm.at[pl.ds(s * L, L)], sem_o.at[s])]

    def out_pair_copies(i):
        s = NSEG - 1
        return [copy(X[s].at[:, _tile(t)], out_hbm.at[pl.ds(s * L, L), _tile(t)], sem_o.at[s])
                for t in (i, i + NP)]

    def wao_copies():
        return [copy(awo_hbm.at[:, _tile(t)], wraw_o.at[t], sem_w.at[4]) for t in range(NT)]

    def wb_copies(m):
        return [copy((wq_hbm, wk_hbm, wv_hbm, wo_hbm)[m], wraw.at[3 + m], sem_w.at[m])]

    def slab_copies(m, i):
        cs = [copy(wqkv_hbm.at[r, pl.ds(m * D, D)], wraw.at[m, r], sem_s.at[m, i])
              for r in (_rows(h * (D // 2) + i * KC, KC) for h in range(2))]
        if m == 0:
            cs += [copy(x_hbm.at[r], x0.at[r], sem_s.at[m, i])
                   for r in (_rows(h * HL + i * RC, RC) for h in range(2))]
        return cs

    def start(cs):
        for c in cs:
            c.start()

    def wait(cs):
        for c in cs:
            c.wait()

    def token(*vals):
        bits = [pltpu.bitcast(v[:8, :128], U32) for v in vals]
        return _tree(jnp.bitwise_or, bits) & zero_ref[:8]

    def vregs(vals, every=1):
        return [v[u:u + 8] for v in vals for u in range(0, v.shape[0], 8)][::-1][::every]

    def after(words, toks):
        if not toks:
            return words
        slabs = []
        for k in range(words.shape[0] // 8):
            slab = words[8 * k:8 * k + 8]
            if toks.get(k) is not None:
                slab = slab | jnp.concatenate([toks[k]] * (words.shape[1] // 128), axis=1)
            slabs.append(slab)
        return jnp.concatenate(slabs, axis=0)

    def store_rhs(dst, m, i, r, b11, b12, b21, b22):
        terms = _rhs_terms(*[_split(b) for b in (b11, b12, b21, b22)])
        words = [{1: b11, 4: b22}[k] if k in (1, 4) else _merge(v) for k, v in enumerate(terms)]
        return vregs([_put(dst, (m, i), r, k, v) for k, v in enumerate(words)])

    def raw_words(m, r, rows, t):
        return pltpu.bitcast(wraw[m, _rows(r, rows), _tile(t)], U32)

    def prep_b(m, i):
        def piece(j, c):
            r = i * KC + 32 * c
            return store_rhs(wb, m, j, r, *[raw_words(3 + m, r + h * (D // 2), 32, j + u * NP)
                                            for h in range(2) for u in range(2)])

        return [lambda j=j, c=c: piece(j, c) for j in range(NP) for c in range(KC // 32)]

    def prep_a_cols(m, i):
        rows = 32
        st = {}

        def rotate(c):
            v = [jnp.concatenate([raw_words(m, i * KC + c * rows + h * (D // 2), rows, t)
                                  for h in range(2)], axis=0) for t in range(NT)]
            st[c] = [x if t == 0 else pltpu.roll(x, 2 * t, 1) for t, x in enumerate(v)]
            return vregs(st[c], 4)

        def shear(c):
            slot = (_iota((rows, 128), 1) >> 1) & 7
            v = [st[c][(-b) % NT] for b in range(NT)]
            for bit in (1, 2, 4):
                sel = (slot & bit) != 0
                v = [jnp.where(sel, v[(b - bit) % NT], v[b]) for b in range(NT)]
            st[c] = [x if b == 0 else pltpu.roll(x, 128 - 2 * b, 1) for b, x in enumerate(v)]
            return vregs(v, 2)

        def terms(c):
            v, half, outs = st[c], rows // 2, []
            for j in range(NP):
                outs += store_rhs(wa, m, j, i * KC + c * rows, v[j][:half], v[j + NP][:half],
                                  v[j][half:], v[j + NP][half:])
            return outs

        order = [(f, k - lag) for k in range(6) for lag, f in enumerate((rotate, shear, terms))
                 if 0 <= k - lag < 4]
        return [lambda f=f, c=c: f(c) for f, c in order]

    def prep_a_rows(i):
        def stage(t):
            words = [pltpu.bitcast(wraw_o[i + h * NP, _tile(t), :], U32) for h in range(2)]
            for h in range(2):
                wtmp[h, pl.ds(65 * t, 64), :] = words[h]
            return vregs(words)

        def rows(h, b, u):
            return jnp.concatenate(
                [wtmp[h, pl.ds(8 * (u + k) + b, 8, stride=65), :] for k in range(2)], axis=0)

        def piece(c, u):
            return store_rhs(wao, 0, i, 128 * c + 16 * u, rows(0, c, u), rows(1, c, u),
                             rows(0, c + NP, u), rows(1, c + NP, u))

        return ([lambda t=t: stage(t) for t in range(NT)]
                + [lambda c=c, u=u: piece(c, u) for c in range(4) for u in range(0, 8, 2)])

    def store_lhs(dst, t, r, a11, a12, a21, a22, pack=_words):
        terms = _lhs_terms(a11, a12, a21, a22)
        return vregs([_put(dst, (t,), r, k, pack(v)) for k, v in enumerate(terms)])

    def join(toks, slot, tok):
        if tok is not None:
            toks[slot] = tok if toks.get(slot) is None else toks[slot] | tok

    def products(a_ref, w_ref, m, i, emit):
        st = {}

        def prod(k, toks, finish):
            a = jnp.concatenate(
                [after(a_ref[t, :, _tile(k)], toks if t == 0 else None) for t in range(NP)], axis=1)
            r = _dot(_bf(a), _bf(w_ref[m, i, :, _tile(k)]))
            finish(r)
            return r

        def p1(r):
            st["m1"] = r

        def p2(r):
            st["c21"], st["c22"] = r, st["m1"] - r

        def p3(r):
            st["c12"], st["c22"] = r, st["c22"] + r

        def p4(r):
            st["c11"] = st["m1"] + r
            emit(1, 0, st["c21"] + r)

        def p5(r):
            st["c11"] = st["c11"] - r
            emit(0, 1, st["c12"] + r)

        def p6(r):
            emit(1, 1, st["c22"] + r)

        def p7(r):
            emit(0, 0, st["c11"] + r)

        return [lambda toks, k=k, f=f: prod(k, toks, f)
                for k, f in enumerate((p1, p2, p3, p4, p5, p6, p7))]

    def ln_tasks(n, i, off, nr=16):
        src, dst = X[n % NSEG], XN[n % 2]
        st = {}

        def mean():
            st["x"] = [
                jnp.concatenate(
                    [_split(pltpu.bitcast(src[_rows(i * RC + off + h * HL, nr), _tile(t)], U32))
                     for h in range(2)], axis=0) for t in range(NT)]
            part = _tree(jnp.add, st["x"])
            st["mean"] = jnp.sum(part, axis=1, keepdims=True) * (1.0 / D)
            return vregs([part])

        def var():
            st["x"] = [x - st["mean"] for x in st["x"]]
            part = _tree(jnp.add, [x * x for x in st["x"]])
            st["var"] = jnp.sum(part, axis=1, keepdims=True) * (1.0 / D)
            return vregs([part])

        def scale():
            inv = lax.rsqrt(st["var"] + 1e-5)
            y = [x * inv for x in st["x"]]
            r = i * RC + off
            outs = []
            for t in range(NP):
                outs += store_lhs(dst, t, r, y[t][:nr], y[t + NP][:nr], y[t][nr:], y[t + NP][nr:],
                                  _merge)
            return outs

        return [mean, var, scale]

    def proj_a(n, i, which):
        p = n % 2

        def emit(h, c, y):
            t = i + c * NP
            if which == 0:
                QA[p][t, pl.ds(h * HL, HL), :] = y
                return
            buf = KA if which == 1 else VA
            buf[p][t, pl.ds(HALO + h * HL, HL), :] = y
            if h == 0 and n % NSEG == 0:
                buf[p][t, pl.ds(0, HALO), :] = jnp.zeros((HALO, 128), F32)
            elif h == 0:
                buf[p][t, pl.ds(0, HALO), :] = buf[1 - p][t, pl.ds(L, HALO), :]

        return products(XN[p], wa, which, i, emit)

    def proj_b(n, i, which):
        p = n % 2

        def emit(h, c, y):
            if which == 0:
                _put(QS[p], (i,), h * HL, c, _words(y * QSCALE))
                _put(PQ[p], (i,), h * HL, c, _words(_phi(y)))
            elif which == 1:
                _put(KB[p], (i,), h * HL, c, _words(y))
                if n % NSEG != NSEG - 1:
                    y = _phi(y)
                    _put(PK[p], (i,), h * HL, c, _words(y))
                    ZS[p][i + c * NP, pl.ds(8 * h, 8), :] = _tree(jnp.add, vregs([y]))
            else:
                VT[p][i + c * NP, :, pl.ds(h * HL, HL)] = pltpu.bitcast(y.astype(BF16).T, U32)

        return products(XN[p], wb, which, i, emit)

    def out_stage(n, i):
        x = X[n % NSEG]

        def emit(h, c, y):
            where = (pl.ds(h * HL, HL), _tile(i + c * NP))
            x[where] = (x[where].astype(F32) + y).astype(BF16)

        if is_a(n):
            return products(O[n % 2], wao, 0, i, emit)
        return products(O[n % 2], wb, 3, i, emit)

    def att_a_tasks(n, i, off):
        p = n % 2
        base = (i * RC if isinstance(i, int) else pl.multiple_of(i * RC, RC)) + off
        starts = [base + (u // 2) * HL + 8 * (u % 2) for u in range(4)]
        lg, mixed = [[] for _ in range(4)], {}

        def scores(u, ws):
            q = [QA[p][t, pl.ds(starts[u], 8), :] for t in range(NT)]
            for w in ws:
                kr = pl.ds(starts[u] + HALO - DIL * w, 8)
                lg[u].append(_tree(jnp.add, [q[t] * KA[p][t, kr, :] for t in range(NT)]))
            return lg[u][-len(ws):]

        def exchange(u, bit):
            low = (_iota((8, 128), 1) & bit) == 0
            lg[u] = [a + jnp.where(low, pltpu.roll(a, 128 - bit, 1), pltpu.roll(a, bit, 1))
                     for a in lg[u]]
            return lg[u]

        def softmax(u):
            v = [a * QSCALE for a in lg[u]]
            if n % NSEG == 0 and off == 0 and u < 2:
                pos = _iota((8, 128), 0) + starts[u]
                v = [a if w == 0 else jnp.where(pos >= DIL * w, a, MASKVAL)
                     for w, a in enumerate(v)]
            m = _tree(jnp.maximum, v)
            e = [jnp.exp2(a - m) for a in v]
            inv = 1.0 / _tree(jnp.add, e)
            lg[u] = [a * inv for a in e]
            return lg[u]

        def mix(t, h):
            for c in range(2):
                mixed[t, h, c] = jnp.concatenate([
                    _tree(jnp.add, [
                        lg[u][w] * VA[p][t + c * NP, pl.ds(starts[u] + HALO - DIL * w, 8), :]
                        for w in range(WIN)])
                    for u in (2 * h, 2 * h + 1)], axis=0)
            return vregs([mixed[t, h, c] for c in range(2)])

        def store(t):
            return store_lhs(O[p], t, i * RC + off,
                             *[mixed[t, h, c] for h in range(2) for c in range(2)])

        d_score, lag1, lag2, lag3, t_mix, d_mix, d_store = A_TIMES
        tasks = []
        for u in range(4):
            t = A_START + d_score * (2 * u + 1)
            tasks += [(t - d_score, lambda u=u: scores(u, range(4))),
                      (t, lambda u=u: scores(u, range(4, 8))),
                      (t + lag1, lambda u=u: exchange(u, 1)),
                      (t + lag2, lambda u=u: exchange(u, 16)),
                      (t + lag3, lambda u=u: softmax(u))]
        for k in range(NP):
            t = t_mix + k * (d_mix + d_store)
            tasks += [(t, lambda k=k: mix(k, 0)), (t + d_mix, lambda k=k: mix(k, 1))]
            tasks += [(t + d_mix + d_store / 2, lambda k=k: store(k))]
        return tasks

    def att_b_piece(n, i, j, mem, tok):
        p = n % 2
        rows = pl.ds(64 * j, 64)
        nk = 128 * j + 64
        head = _iota((32, 128), 1) >> 5
        key, lane = _iota((64, 128), 0), _iota((64, 128), 1)
        causal = [jnp.where(key > q, MASKVAL, 0.0) for q in (lane, lane ^ 64, lane & 63)]
        high = _iota((8, 128), 1) >= 64
        s, sx, late_q = [], [], []
        for h in range(2):
            qw = after(QS[p][i, rows, _tile(h)], {0: tok, 4: tok})
            early = [jnp.where(head == hh, qw[:32], jnp.uint32(0)) for hh in range(4)]
            late = [jnp.where(head == hh, qw[32:], jnp.uint32(0)) for hh in range(4)]
            late_q.append(jnp.concatenate([late[1], late[0], late[3], late[2]], axis=0))
            qcat = jnp.concatenate([early[0], late[0], late[1], early[1],
                                    early[2], late[2], late[3], early[3]], axis=0)
            st = _dot_nt(_bf(KB[p][i, pl.ds(0, nk // 2), _tile(h)]), _bf(qcat))
            for hh in range(4):
                v = st[:, 128 * hh:128 * (hh + 1)]
                s.append([v[u:u + 8] for u in range(0, nk - 64, 8)]
                         + [v[nk - 64 + u:nk - 56 + u] + causal[hh % 2][u:u + 8]
                            for u in range(0, 64, 8)])
        for h in range(2):
            st = _dot_nt(_bf(KB[p][i, pl.ds(nk // 2, 32), _tile(h)]), _bf(late_q[h]))
            for u in range(2):
                v = st[:, 128 * u:128 * (u + 1)] + causal[2]
                sx.append([v[r:r + 8] for r in range(0, 64, 8)])
        first = token(*[v[0] for v in s])
        m = []
        for u in range(4):
            mx = _tree(jnp.maximum, sx[u])
            for odd in range(2):
                a = _tree(jnp.maximum, s[2 * u + odd])
                b = jnp.maximum(a, mx)
                a = jnp.where(high, a, b) if odd else jnp.where(high, b, a)
                m.append(jnp.broadcast_to(jnp.max(a, axis=0, keepdims=True), (8, 128)))
        e = [[] for _ in range(8)]
        part = [[] for _ in range(8)]

        def exps(v, mh, tok):
            mh = mh if tok is None else mh + pltpu.bitcast(tok, F32)
            return [jnp.exp2(a - mh) for a in v]

        def exp_tile(u, c, tok):
            v = exps(s[u][16 * c:16 * (c + 1)], m[u], tok)
            part[u] = [_tree(jnp.add, part[u] + v)]
            e[u].extend(v)

        def exp_diag(u, tok):
            for odd in range(2):
                exp_tile(2 * u + odd, j, tok)
            v = exps(sx[u], jnp.where(high, m[2 * u], m[2 * u + 1]), tok)
            tot = _tree(jnp.add, v)
            for odd in range(2):
                pick = (lambda a: jnp.where(high, 0.0, a)) if odd else (lambda a: jnp.where(high, a, 0.0))
                part[2 * u + odd] = [part[2 * u + odd][0] + pick(tot)]
                e[2 * u + odd].extend(pick(a) for a in v)

        def finish(h, tok):
            g = i + h * NP
            ot = []
            for hh in range(4):
                u = 4 * h + hh
                vt = after(VT[p][g, pl.ds(16 * hh, 16), pl.ds(0, 128 * (j + 1))], {0: tok})
                acc = _dot(_bf(vt), jnp.concatenate(e[u], axis=0).astype(BF16))
                l = jnp.sum(part[u][0], axis=0, keepdims=True)
                gate = gtab[pl.ds(4 * g + hh, 1), :]
                acc = acc * ((1.0 - gate) / l)
                if hh % 2:
                    acc = pltpu.roll(acc, 64, 1)
                if n % NSEG:
                    r = mem[h][:, 128 * j:128 * (j + 1)]
                    den = r[128 + 4 * hh:129 + 4 * hh] + 1e-6
                    acc = acc + r[32 * hh:32 * hh + 32] * (gate / den)
                ot.append(acc)
            return ot

        tasks = []
        for u in range(4):
            tasks += [lambda tok, u=2 * u + odd, c=c: exp_tile(u, c, tok)
                      for odd in range(2) for c in range(j)]
            tasks.append(lambda tok, u=u: exp_diag(u, tok))
        return first, tasks, finish

    def mem_load(n, g):
        if n % NSEG == 0:
            return jnp.zeros((MZ_ROWS, 128), F32)
        return mz[g]

    def mem_read(n, i, h, state, tok):
        pq = after(PQ[n % 2][i, :, _tile(h)], {8 * u: tok for u in range(4)})
        return _dot_nt(state.astype(BF16), _bf(pq))

    def mem_update(n, i, h, state, tok):
        p, g = n % 2, i + h * NP
        z = jnp.sum(ZS[p][g], axis=0, keepdims=True)
        new = jnp.concatenate([_dot(_bf(after(VT[p][g], {0: tok})), _bf(PK[p][i, :, _tile(h)])),
                               jnp.broadcast_to(z, (MZ_ROWS - 128, 128))], axis=0)
        row = _iota((MZ_ROWS, 128), 0)
        row_head = jnp.where(row < 128, row >> 5, (row - 128) >> 2)
        keep = row_head == (_iota((MZ_ROWS, 128), 1) >> 5)
        mz[g] = new = state + jnp.where(keep, new, 0.0)
        return new

    def is_a(n):
        return (n // NSEG) % 2 == 0

    def run_timed(mm, tasks):
        tasks = sorted(tasks, key=lambda x: x[0])
        for k, prod in enumerate(mm):
            toks = {}
            while tasks and tasks[0][0] < 16 * (k + 1):
                time, f = tasks.pop(0)
                join(toks, time - 16 * k, token(*f()))
            prod(toks)
        for _, f in tasks:
            f()

    def body_b(n, its, mm, ln):
        full = len(mm) == 28 * len(its)
        *share, front, lag, tail, pitch = (*B_SHARE, B_FRONT, B_WAIT, *B_TAIL) if full else B_LAST
        spare = len(mm) // len(its) - sum(share)
        late, done = [], []
        tok, pending = None, None

        def finisher(i, j, finish, tiles):
            def run(tok):
                posts = []
                for h in range(2):
                    ot = finish(h, tok)

                    def post(ot=ot, h=h):
                        tiles[j, h] = jnp.concatenate(ot, axis=0).T
                        return vregs([tiles[j, h]], 4)

                    posts.append(post)
                if (j ^ 2, 0) in tiles:
                    posts += [lambda r=r: store_lhs(
                        O[n % 2], i, 128 * (j % 2) + r,
                        *[tiles[j % 2 + u, h][r:r + B_STORE] for u in (0, 2) for h in range(2)])
                        for r in range(0, 128, B_STORE)]
                tiles[j, 0] = None
                return posts

            return run

        for i in its:
            state = [mem_load(n, i + h * NP) for h in range(2)]
            mem, tiles = [], {}
            if ln:
                for off in range(0, RC, 16):
                    late += ln_tasks(n + 2, i, off)
            for k, j in enumerate(B_ORDER):
                first, exps, finish = att_b_piece(n, i, j, mem, tok)
                done += pending(first) if pending else []
                cnt = share[k] + (0 if i is its[-1] else (spare + 3 - k) // 4)
                when = [int(32 * cnt * front * u / len(exps)) for u in range(len(exps))]
                for c in range(cnt):
                    toks = {}
                    if c == 0:
                        join(toks, 0, first)
                    for slot in B_POST:
                        if done and 16 * c + slot >= min(lag, 16 * cnt - 1):
                            join(toks, slot, token(*done.pop(0)()))
                    if late and c >= B_LN[0]:
                        join(toks, B_LN[1], token(*late.pop(0)()))
                    r = mm.pop(0)(toks)
                    while exps and when[0] < 32 * (c + 1):
                        exps.pop(0)(token(r[8 * (when.pop(0) - 32 * c):]))
                    tok = token(r)
                    if k == 0 and c == B_READ and n % NSEG:
                        mem.extend(mem_read(n, i, h, state[h], tok) for h in range(2))
                        done.append(lambda mem=mem: [v[:, 128 * u:] for v in mem for u in range(4)])
                    if k == B_UPDATE and c == 0 and n % NSEG != NSEG - 1:
                        new = [mem_update(n, i, h, state[h], tok) for h in range(2)]
                        done.append(lambda new=new: new)
                pending = finisher(i, j, finish, tiles)
        tok = token(mm.pop(0)(None))
        done += late + pending(tok)
        run_timed(mm, [(tail + pitch * u, f) for u, f in enumerate(done)])

    def step(n, ln=True, proj=(0, 1, 2), att=True, out=True, extra=None, unroll=UNROLL):
        def body(its):
            mm = []
            for i in its:
                for which in (B_MATS if att and not is_a(n) else A_MATS):
                    if which in proj:
                        mm += (proj_a if is_a(n + 1) else proj_b)(n + 1, i, which)
                    elif which == 3 and out:
                        mm += out_stage(n - 1, i)
            if att and not is_a(n):
                body_b(n, its, mm, ln)
                return
            tasks, span = [], 16 * len(mm) / (4 * len(its))
            for k, i in enumerate(its):
                if extra is not None:
                    fs = extra(i)
                    tasks += [(int(span * (4 * k + u // 8 + A_PREP_WHEN[u % 8])) if att else
                               int(4 * span * (k + (u + 1) / len(fs))) - 1, f)
                              for u, f in enumerate(fs)]
                for u, off in enumerate(range(0, RC, 16), 4 * k):
                    if att:
                        tasks += [(int(span * (u + w)), f) for w, f in att_a_tasks(n, i, off)]
                    if ln:
                        when = A_LN_WHEN if att else (.3, .8, 1.3)
                        tasks += [(int(span * (u + w)), f)
                                  for w, f in zip(when, ln_tasks(n + 2, i, off))]
            run_timed(mm, tasks)

        if unroll == NP:
            body(list(range(NP)))
        else:
            pl.loop(0, NP // unroll)(lambda i: body([unroll * i + u for u in range(unroll)]))

    def prep_in_flight(m):
        def tasks(i):
            if m < 2:
                pl.when(i + 2 < NP)(lambda: start(slab_copies(m, i + 2)))
            if m == 0:
                pl.when(i + 2 >= NP)(lambda: start(slab_copies(1, i + 2 - NP)))
            elif m == 1:
                start(slab_copies(2, i))
            else:
                pl.when(i == 0)(lambda: start(x_copies(1) + wao_copies()))

            wait(slab_copies(m, i))
            return prep_a_cols(m, i)

        return tasks

    start(slab_copies(0, 0))
    start([copy(beta_hbm, beta_ref.at[0], sem_b)])
    start(slab_copies(0, 1))
    zero_ref[:8] = jnp.zeros((8, 128), U32)

    @pl.loop(0, NP)
    def _(i):
        prep = prep_in_flight(0)(i)
        ln = [ln_tasks(0, i, off) for off in range(0, RC, 16)]
        for k in range(3):
            for f in prep[4 * k:4 * k + 4] + [fs[k] for fs in ln]:
                f()

    step(-1, ln=False, proj=(0,), att=False, out=False, extra=prep_in_flight(1), unroll=1)
    step(-1, ln=False, proj=(1,), att=False, out=False, extra=prep_in_flight(2), unroll=1)
    start(x_copies(2))
    start(x_copies(3))
    wait(x_copies(1))
    wait(wao_copies())
    step(-1, proj=(2,), att=False, out=False, extra=prep_a_rows)
    for m in range(4):
        start(wb_copies(m))
    wait([copy(beta_hbm, beta_ref.at[0], sem_b)])
    gate = jax.nn.sigmoid(beta_ref[0].astype(F32))
    eye = _iota((H, H), 0) == _iota((H, H), 1)
    gcol = jnp.sum(jnp.where(eye, jnp.broadcast_to(gate, (H, H)), 0.0), axis=1, keepdims=True)
    gtab[...] = jnp.broadcast_to(gcol, (H, 128))
    wait(x_copies(2))
    step(0, out=False)
    wait(x_copies(3))
    for m in range(4):
        wait(wb_copies(m))
    step(1, extra=lambda i: prep_b(0, i) + prep_b(1, i))
    step(2, extra=lambda i: prep_b(2, i) + prep_b(3, i))
    for n in range(3, 14):
        step(n)
    start(out_copies(0))
    step(14, ln=False)
    start(out_copies(1))
    step(15, ln=False, proj=())
    start(out_copies(2))
    for i in range(NP):
        run_timed(out_stage(15, i), [])
        start(out_pair_copies(i))
    for s in range(NSEG):
        wait(out_copies(s))


@jax.jit
def pallas_interleave_layers__sliding_local_dilated__memory_aug_infini_attn__prompt_kernel(
    A_x: jax.Array,
    A_wqkv: jax.Array,
    A_wo: jax.Array,
    B_x: jax.Array,
    B_wq: jax.Array,
    B_wk: jax.Array,
    B_wv: jax.Array,
    B_wo: jax.Array,
    B_beta: jax.Array,
):
    del B_x
    assert A_x.shape == (1, S, D)
    hbm = pl.BlockSpec(memory_space=pl.ANY)
    scratch = (
        [pltpu.VMEM((L, D), BF16)] * 4
        + [pltpu.VMEM((7, D, D), BF16), pltpu.VMEM((NT, D, 128), BF16),
           pltpu.VMEM((2, 576, 128), U32),
           pltpu.VMEM((3, NP, D // 4, 7 * 128), U32),
           pltpu.VMEM((1, NP, D // 4, 7 * 128), U32),
           pltpu.VMEM((4, NP, D // 4, 7 * 128), U32)]
        + [pltpu.VMEM((NP, HL // 2, 7 * 128), U32)] * 4
        + [pltpu.VMEM((NT, L, 128), F32)] * 2
        + [pltpu.VMEM((NT, HALO + L, 128), F32)] * 4
        + [pltpu.VMEM((NP, L // 2, 2 * 128), U32)] * 8
        + [pltpu.VMEM((NT, 64, L), U32)] * 2
        + [pltpu.VMEM((NT, 16, 128), F32)] * 2
        + [pltpu.VMEM((NT, MZ_ROWS, 128), F32), pltpu.VMEM((8, 1, H), BF16),
           pltpu.VMEM((H, 128), F32),
           pltpu.VMEM((88, 128), U32),
           pltpu.SemaphoreType.DMA((NSEG,)), pltpu.SemaphoreType.DMA((5,)),
           pltpu.SemaphoreType.DMA((3, NP)),
           pltpu.SemaphoreType.DMA((NSEG,)), pltpu.SemaphoreType.DMA]
    )
    out = pl.pallas_call(
        _kernel,
        out_shape=jax.ShapeDtypeStruct((S, D), BF16),
        in_specs=[hbm] * 8,
        out_specs=hbm,
        scratch_shapes=scratch,
        compiler_params=pltpu.CompilerParams(vmem_limit_bytes=110 * 2**20),
        name="abab_stack",
    )(A_x.reshape(S, D), A_wqkv, A_wo, B_wq, B_wk, B_wv, B_wo, B_beta.reshape(1, H))
    return out.reshape(1, S, D)
```

```python
import jax
import jax.numpy as jnp
from jax import lax
import jax.experimental.pallas as pl
import jax.experimental.pallas.tpu as pltpu

S, D, H, DH = 2048, 1024, 32, 32
NSEG, L = 4, 512
HL = L // 2
NT = D // 128
NP = NT // 2
RC = HL // NP
KC = D // 2 // NP
LAST = 4 * NSEG - 1
WIN, DIL = 8, 2
HALO = 16
MZ_ROWS = 128 + 16
LOG2E = 1.4426950408889634
QSCALE = float(DH ** -0.5 * LOG2E)
MASKVAL = float(-1e9 * LOG2E)

B_ORDER = (3, 1, 2, 0)
B_SHARE = (8, 5, 5, 5)
B_LAST = (5, 2, 6, 3, 0.884, 29, 27, 4)
B_LAST2 = (4, 2, 3, 1, 0.85, 26, 27, 4)
B_FRONT = 0.842
B_POST = (6, 15)
B_WAIT = 29
B_TAIL = (29, 10)
B_STORE = 16
B_UPDATE = 0
B_READ = 0
A_MATS = (3, 0, 2, 1)
B_MATS = (2, 0, 1, 3)
UNROLL = 1
B_LN = (1, 3)
A_START = 0.051
A_TIMES = (0.035, 0.077, 0.18, 0.275, 0.598, 0.039, 0.055)
A_LN_WHEN = (0.023, 0.3, 0.486)
A_PREP_WHEN = (0.279, 0.33, 0.408, 0.423, 0.353, 0.5, 0.556, 0.578)

F32, BF16, U32 = jnp.float32, jnp.bfloat16, jnp.uint32
_NT_DIMS = (((1,), (1,)), ((), ()))


def _iota(shape, axis):
    return lax.broadcasted_iota(jnp.int32, shape, axis)


def _dot(a, b):
    return jnp.dot(a, b, preferred_element_type=F32)


def _dot_nt(a, b):
    return lax.dot_general(a, b, _NT_DIMS, preferred_element_type=F32)


def _rows(start, size):
    return pl.ds(start if isinstance(start, int) else pl.multiple_of(start, size), size)


def _tile(k):
    return _rows(128 * k, 128)


def _words(val):
    return pltpu.bitcast(val.astype(BF16), U32)


def _split(words):
    return jnp.concatenate(
        [pltpu.unpack_elementwise(words, index=k, packed_dtype=BF16, unpacked_dtype=F32)
         for k in range(2)], axis=0)


def _merge(val):
    half = val.shape[0] // 2
    return pltpu.pack_elementwise([val[:half], val[half:]], packed_dtype=BF16)


def _put(ref, idx, start, k, words):
    ref[(*idx, _rows(start // 2, words.shape[0]), _tile(k))] = words
    return words


def _bf(words):
    return pltpu.bitcast(words, BF16)


def _phi(t):
    return jnp.where(t > 0, t + 1.0, jnp.exp(t))


def _tree(op, xs):
    xs = list(xs)
    while len(xs) > 1:
        xs = [op(xs[i], xs[i + 1]) if i + 1 < len(xs) else xs[i]
              for i in range(0, len(xs), 2)]
    return xs[0]


def _lhs_terms(a11, a12, a21, a22):
    return (a11 + a22, a21 + a22, a11, a22, a11 + a12, a21 - a11, a12 - a22)


def _rhs_terms(b11, b12, b21, b22):
    return (b11 + b22, b11, b12 - b22, b21 - b11, b22, b11 + b12, b21 + b22)


def _kernel(x_hbm, wqkv_hbm, awo_hbm, wq_hbm, wk_hbm, wv_hbm, wo_hbm, beta_hbm,
            out_hbm,
            x0, x1, x2, x3, wraw, wraw_o, wtmp, waq, wak, wav, wao, wb,
            xn0, xn1, o0, o1, o2,
            qa0, qa1, ka0, ka1, va0, va1,
            qs0, qs1, pq0, pq1, kb0, kb1, pk0, pk1, vt0, vt1,
            zs0, zs1, mz, beta_ref, gtab, zero_ref, sem_x, sem_w, sem_s, sem_o, sem_b):
    X = (x0, x1, x2, x3)
    XN, wa = (xn0, xn1), (waq, wak, wav)
    O = [o2 if n == LAST else (o0, o1)[n % 2] for n in range(LAST + 1)]
    QA, KA, VA = (qa0, qa1), (ka0, ka1), (va0, va1)
    QS, PQ, KB, PK, VT = (qs0, qs1), (pq0, pq1), (kb0, kb1), (pk0, pk1), (vt0, vt1)
    ZS = (zs0, zs1)

    copy = pltpu.make_async_copy

    def x_copies(s):
        return [copy(x_hbm.at[pl.ds(s * L, L)], X[s], sem_x.at[s])]

    def out_copies(s):
        return [copy(X[s], out_hbm.at[pl.ds(s * L, L)], sem_o.at[s])]

    def out_tile_copies(t0, nt):
        cols = [pl.ds(128 * (t0 + c * NP), 128 * nt) for c in range(2)]
        return [copy(x3.at[:, c], out_hbm.at[pl.ds(S - L, L), c], sem_o.at[NSEG - 1]) for c in cols]

    def wao_copies():
        return [copy(awo_hbm.at[:, _tile(t)], wraw_o.at[t], sem_w.at[4]) for t in range(NT)]

    def wb_copies(m):
        return [copy((wq_hbm, wk_hbm, wv_hbm, wo_hbm)[m], wraw.at[3 + m], sem_w.at[m])]

    def slab_copies(m, i):
        return [copy(wqkv_hbm.at[r, _rows(m * D, D)], wraw.at[m, r], sem_s.at[m, i])
                for r in (_rows(h * (D // 2) + i * KC, KC) for h in range(2))]

    def x0_copies(i):
        return [copy(x_hbm.at[r], x0.at[r], sem_s.at[3, i])
                for r in (_rows(h * HL + i * RC, RC) for h in range(2))]

    def start(cs):
        for c in cs:
            c.start()

    def wait(cs):
        for c in cs:
            c.wait()

    def token(*vals):
        bits = [pltpu.bitcast(v[:8, :128], U32) for v in vals]
        return _tree(jnp.bitwise_or, bits) & zero_ref[:8]

    def vregs(vals, every=1):
        return [v[u:u + 8] for v in vals for u in range(0, v.shape[0], 8)][::-1][::every]

    def after(words, toks):
        if not toks:
            return words
        slabs = []
        for k in range(words.shape[0] // 8):
            slab = words[8 * k:8 * k + 8]
            if toks.get(k) is not None:
                slab = slab | jnp.concatenate([toks[k]] * (words.shape[1] // 128), axis=1)
            slabs.append(slab)
        return jnp.concatenate(slabs, axis=0)

    def store_rhs(dst, m, i, r, b11, b12, b21, b22):
        terms = _rhs_terms(*[_split(b) for b in (b11, b12, b21, b22)])
        words = [{1: b11, 4: b22}[k] if k in (1, 4) else _merge(v) for k, v in enumerate(terms)]
        return vregs([_put(dst, (m, i), r, k, v) for k, v in enumerate(words)])

    def raw_words(m, r, rows, t):
        return pltpu.bitcast(wraw[m, _rows(r, rows), _tile(t)], U32)

    def prep_b(m, i):
        def piece(j, c):
            r = i * KC + 32 * c
            return store_rhs(wb, m, j, r, *[raw_words(3 + m, r + h * (D // 2), 32, j + u * NP)
                                            for h in range(2) for u in range(2)])

        return [lambda j=j, c=c: piece(j, c) for j in range(NP) for c in range(KC // 32)]

    def prep_a_cols(m, i):
        rows = 32
        st = {}

        def rotate(c):
            v = [jnp.concatenate([raw_words(m, i * KC + c * rows + h * (D // 2), rows, t)
                                  for h in range(2)], axis=0) for t in range(NT)]
            st[c] = [x if t == 0 else pltpu.roll(x, 2 * t, 1) for t, x in enumerate(v)]
            return vregs(st[c], 4)

        def shear(c):
            slot = (_iota((rows, 128), 1) >> 1) & 7
            v = [st[c][(-b) % NT] for b in range(NT)]
            for bit in (1, 2, 4):
                sel = (slot & bit) != 0
                v = [jnp.where(sel, v[(b - bit) % NT], v[b]) for b in range(NT)]
            st[c] = [x if b == 0 else pltpu.roll(x, 128 - 2 * b, 1) for b, x in enumerate(v)]
            return vregs(v, 2)

        def terms(c):
            v, half, outs = st[c], rows // 2, []
            for j in range(NP):
                outs += store_rhs(wa[m], 0, j, i * KC + c * rows, v[j][:half], v[j + NP][:half],
                                  v[j][half:], v[j + NP][half:])
            return outs

        order = [(f, k - lag) for k in range(6) for lag, f in enumerate((rotate, shear, terms))
                 if 0 <= k - lag < 4]
        return [lambda f=f, c=c: f(c) for f, c in order]

    def prep_a_rows(i):
        def stage(t):
            words = [pltpu.bitcast(wraw_o[i + h * NP, _tile(t), :], U32) for h in range(2)]
            for h in range(2):
                wtmp[h, pl.ds(65 * t, 64), :] = words[h]
            return vregs(words)

        def rows(h, b, u):
            return jnp.concatenate(
                [wtmp[h, pl.ds(8 * (u + k) + b, 8, stride=65), :] for k in range(2)], axis=0)

        def piece(c, u):
            return store_rhs(wao, 0, i, 128 * c + 16 * u, rows(0, c, u), rows(1, c, u),
                             rows(0, c + NP, u), rows(1, c + NP, u))

        return ([lambda t=t: stage(t) for t in range(NT)]
                + [lambda c=c, u=u: piece(c, u) for c in range(4) for u in range(0, 8, 2)])

    def store_lhs(dst, t, r, a11, a12, a21, a22, pack=_words):
        terms = _lhs_terms(a11, a12, a21, a22)
        return vregs([_put(dst, (t,), r, k, pack(v)) for k, v in enumerate(terms)])

    def join(toks, slot, tok):
        if tok is not None:
            toks[slot] = tok if toks.get(slot) is None else toks[slot] | tok

    def products(a_ref, w_ref, m, i, emit, only=None):
        st = {}

        def prod(k, toks, finish):
            if only is None:
                a = jnp.concatenate([after(a_ref[t, :, _tile(k)], toks if t == 0 else None)
                                     for t in range(NP)], axis=1)
                w = w_ref[m, i, :, _tile(k)]
            else:
                a = after(a_ref[only, :, _tile(k)], toks)
                w = w_ref[m, i, _rows(64 * only, 64), _tile(k)]
            r = _dot(_bf(a), _bf(w))
            finish(r)
            return r

        def p1(r):
            st["m1"] = r

        def p2(r):
            st["c21"], st["c22"] = r, st["m1"] - r

        def p3(r):
            st["c12"], st["c22"] = r, st["c22"] + r

        def p4(r):
            st["c11"] = st["m1"] + r
            emit(1, 0, st["c21"] + r)

        def p5(r):
            st["c11"] = st["c11"] - r
            emit(0, 1, st["c12"] + r)

        def p6(r):
            emit(1, 1, st["c22"] + r)

        def p7(r):
            emit(0, 0, st["c11"] + r)

        return [lambda toks, k=k, f=f: prod(k, toks, f)
                for k, f in enumerate((p1, p2, p3, p4, p5, p6, p7))]

    def ln_tasks(n, i, off, nr=16):
        src, dst = X[n % NSEG], XN[n % 2]
        st = {}

        def mean():
            st["x"] = [
                jnp.concatenate(
                    [_split(pltpu.bitcast(src[_rows(i * RC + off + h * HL, nr), _tile(t)], U32))
                     for h in range(2)], axis=0) for t in range(NT)]
            part = _tree(jnp.add, st["x"])
            st["mean"] = jnp.sum(part, axis=1, keepdims=True) * (1.0 / D)
            return vregs([part])

        def var():
            st["x"] = [x - st["mean"] for x in st["x"]]
            part = _tree(jnp.add, [x * x for x in st["x"]])
            st["var"] = jnp.sum(part, axis=1, keepdims=True) * (1.0 / D)
            return vregs([part])

        def scale():
            inv = lax.rsqrt(st["var"] + 1e-5)
            y = [x * inv for x in st["x"]]
            r = i * RC + off
            outs = []
            for t in range(NP):
                outs += store_lhs(dst, t, r, y[t][:nr], y[t + NP][:nr], y[t][nr:], y[t + NP][nr:],
                                  _merge)
            return outs

        return [mean, var, scale]

    def proj_a(n, i, which, only=None):
        p = n % 2

        def emit(h, c, y):
            t = i + c * NP
            buf = (QA, KA, VA)[which]
            rows = pl.ds(h * HL + (HALO if which else 0), HL)
            if only:
                y = y + buf[p][t, rows, :]
            buf[p][t, rows, :] = y
            if which and h == 0 and n % NSEG == 0:
                buf[p][t, pl.ds(0, HALO), :] = jnp.zeros((HALO, 128), F32)
            elif which and h == 0:
                buf[p][t, pl.ds(0, HALO), :] = buf[1 - p][t, pl.ds(L, HALO), :]

        return products(XN[p], wa[which], 0, i, emit, only)

    def proj_b(n, i, which):
        p = n % 2

        def emit(h, c, y):
            if which == 0:
                _put(QS[p], (i,), h * HL, c, _words(y * QSCALE))
                _put(PQ[p], (i,), h * HL, c, _words(_phi(y)))
            elif which == 1:
                _put(KB[p], (i,), h * HL, c, _words(y))
                if n % NSEG != NSEG - 1:
                    y = _phi(y)
                    _put(PK[p], (i,), h * HL, c, _words(y))
                    ZS[p][i + c * NP, pl.ds(8 * h, 8), :] = _tree(jnp.add, vregs([y]))
            else:
                VT[p][i + c * NP, :, pl.ds(h * HL, HL)] = pltpu.bitcast(y.astype(BF16).T, U32)

        return products(XN[p], wb, which, i, emit)

    def out_stage(n, i):
        x = X[n % NSEG]

        def emit(h, c, y):
            where = (pl.ds(h * HL, HL), _tile(i + c * NP))
            x[where] = (x[where].astype(F32) + y).astype(BF16)

        if is_a(n):
            return products(O[n], wao, 0, i, emit)
        return products(O[n], wb, 3, i, emit)

    def att_a_tasks(n, i, off):
        p = n % 2
        base = (i * RC if isinstance(i, int) else pl.multiple_of(i * RC, RC)) + off
        starts = [base + (u // 2) * HL + 8 * (u % 2) for u in range(4)]
        lg, mixed = [[] for _ in range(4)], {}

        def scores(u, ws):
            q = [QA[p][t, pl.ds(starts[u], 8), :] for t in range(NT)]
            for w in ws:
                kr = pl.ds(starts[u] + HALO - DIL * w, 8)
                lg[u].append(_tree(jnp.add, [q[t] * KA[p][t, kr, :] for t in range(NT)]))
            return lg[u][-len(ws):]

        def exchange(u, bit):
            low = (_iota((8, 128), 1) & bit) == 0
            lg[u] = [a + jnp.where(low, pltpu.roll(a, 128 - bit, 1), pltpu.roll(a, bit, 1))
                     for a in lg[u]]
            return lg[u]

        def softmax(u):
            v = [a * QSCALE for a in lg[u]]
            if n % NSEG == 0 and off == 0 and u < 2:
                pos = _iota((8, 128), 0) + starts[u]
                v = [a if w == 0 else jnp.where(pos >= DIL * w, a, MASKVAL)
                     for w, a in enumerate(v)]
            m = _tree(jnp.maximum, v)
            e = [jnp.exp2(a - m) for a in v]
            inv = 1.0 / _tree(jnp.add, e)
            lg[u] = [a * inv for a in e]
            return lg[u]

        def mix(t, h):
            for c in range(2):
                mixed[t, h, c] = jnp.concatenate([
                    _tree(jnp.add, [
                        lg[u][w] * VA[p][t + c * NP, pl.ds(starts[u] + HALO - DIL * w, 8), :]
                        for w in range(WIN)])
                    for u in (2 * h, 2 * h + 1)], axis=0)
            return vregs([mixed[t, h, c] for c in range(2)])

        def store(t):
            return store_lhs(O[n], t, i * RC + off,
                             *[mixed[t, h, c] for h in range(2) for c in range(2)])

        d_score, lag1, lag2, lag3, t_mix, d_mix, d_store = A_TIMES
        tasks = []
        for u in range(4):
            t = A_START + d_score * (2 * u + 1)
            tasks += [(t - d_score, lambda u=u: scores(u, range(4))),
                      (t, lambda u=u: scores(u, range(4, 8))),
                      (t + lag1, lambda u=u: exchange(u, 1)),
                      (t + lag2, lambda u=u: exchange(u, 16)),
                      (t + lag3, lambda u=u: softmax(u))]
        for k in range(NP):
            t = t_mix + k * (d_mix + d_store)
            tasks += [(t, lambda k=k: mix(k, 0)), (t + d_mix, lambda k=k: mix(k, 1))]
            tasks += [(t + d_mix + d_store / 2, lambda k=k: store(k))]
        return tasks

    def att_b_piece(n, i, j, mem, tok):
        p = n % 2
        rows = pl.ds(64 * j, 64)
        nk = 128 * j + 64
        head = _iota((32, 128), 1) >> 5
        key, lane = _iota((64, 128), 0), _iota((64, 128), 1)
        causal = [jnp.where(key > q, MASKVAL, 0.0) for q in (lane, lane ^ 64, lane & 63)]
        high = _iota((8, 128), 1) >= 64
        s, sx, late_q = [], [], []
        for h in range(2):
            qw = after(QS[p][i, rows, _tile(h)], {0: tok, 4: tok})
            early = [jnp.where(head == hh, qw[:32], jnp.uint32(0)) for hh in range(4)]
            late = [jnp.where(head == hh, qw[32:], jnp.uint32(0)) for hh in range(4)]
            late_q.append(jnp.concatenate([late[1], late[0], late[3], late[2]], axis=0))
            qcat = jnp.concatenate([early[0], late[0], late[1], early[1],
                                    early[2], late[2], late[3], early[3]], axis=0)
            st = _dot_nt(_bf(KB[p][i, pl.ds(0, nk // 2), _tile(h)]), _bf(qcat))
            for hh in range(4):
                v = st[:, 128 * hh:128 * (hh + 1)]
                s.append([v[u:u + 8] for u in range(0, nk - 64, 8)]
                         + [v[nk - 64 + u:nk - 56 + u] + causal[hh % 2][u:u + 8]
                            for u in range(0, 64, 8)])
        for h in range(2):
            st = _dot_nt(_bf(KB[p][i, pl.ds(nk // 2, 32), _tile(h)]), _bf(late_q[h]))
            for u in range(2):
                v = st[:, 128 * u:128 * (u + 1)] + causal[2]
                sx.append([v[r:r + 8] for r in range(0, 64, 8)])
        first = token(*[v[0] for v in s])
        m = []
        for u in range(4):
            mx = _tree(jnp.maximum, sx[u])
            for odd in range(2):
                a = _tree(jnp.maximum, s[2 * u + odd])
                b = jnp.maximum(a, mx)
                a = jnp.where(high, a, b) if odd else jnp.where(high, b, a)
                m.append(jnp.broadcast_to(jnp.max(a, axis=0, keepdims=True), (8, 128)))
        e = [[] for _ in range(8)]
        part = [[] for _ in range(8)]

        def exps(v, mh, tok):
            mh = mh if tok is None else mh + pltpu.bitcast(tok, F32)
            return [jnp.exp2(a - mh) for a in v]

        def exp_tile(u, c, tok):
            v = exps(s[u][16 * c:16 * (c + 1)], m[u], tok)
            part[u] = [_tree(jnp.add, part[u] + v)]
            e[u].extend(v)

        def exp_diag(u, tok):
            for odd in range(2):
                exp_tile(2 * u + odd, j, tok)
            v = exps(sx[u], jnp.where(high, m[2 * u], m[2 * u + 1]), tok)
            tot = _tree(jnp.add, v)
            for odd in range(2):
                pick = (lambda a: jnp.where(high, 0.0, a)) if odd else (lambda a: jnp.where(high, a, 0.0))
                part[2 * u + odd] = [part[2 * u + odd][0] + pick(tot)]
                e[2 * u + odd].extend(pick(a) for a in v)

        def finish(h, tok):
            g = i + h * NP
            ot = []
            for hh in range(4):
                u = 4 * h + hh
                vt = after(VT[p][g, pl.ds(16 * hh, 16), pl.ds(0, 128 * (j + 1))], {0: tok})
                acc = _dot(_bf(vt), jnp.concatenate(e[u], axis=0).astype(BF16))
                l = jnp.sum(part[u][0], axis=0, keepdims=True)
                gate = gtab[pl.ds(4 * g + hh, 1), :]
                acc = acc * ((1.0 - gate) / l)
                if hh % 2:
                    acc = pltpu.roll(acc, 64, 1)
                if n % NSEG:
                    r = mem[h][:, 128 * j:128 * (j + 1)]
                    den = r[128 + 4 * hh:129 + 4 * hh] + 1e-6
                    acc = acc + r[32 * hh:32 * hh + 32] * (gate / den)
                ot.append(acc)
            return ot

        tasks = []
        for u in range(4):
            tasks += [lambda tok, u=2 * u + odd, c=c: exp_tile(u, c, tok)
                      for odd in range(2) for c in range(j)]
            tasks.append(lambda tok, u=u: exp_diag(u, tok))
        return first, tasks, finish

    def mem_load(n, g):
        if n % NSEG == 0:
            return jnp.zeros((MZ_ROWS, 128), F32)
        return mz[g]

    def mem_read(n, i, h, state, tok):
        pq = after(PQ[n % 2][i, :, _tile(h)], {8 * u: tok for u in range(4)})
        return _dot_nt(state.astype(BF16), _bf(pq))

    def mem_update(n, i, h, state, tok):
        p, g = n % 2, i + h * NP
        z = jnp.sum(ZS[p][g], axis=0, keepdims=True)
        new = jnp.concatenate([_dot(_bf(after(VT[p][g], {0: tok})), _bf(PK[p][i, :, _tile(h)])),
                               jnp.broadcast_to(z, (MZ_ROWS - 128, 128))], axis=0)
        row = _iota((MZ_ROWS, 128), 0)
        row_head = jnp.where(row < 128, row >> 5, (row - 128) >> 2)
        keep = row_head == (_iota((MZ_ROWS, 128), 1) >> 5)
        mz[g] = new = state + jnp.where(keep, new, 0.0)
        return new

    def is_a(n):
        return (n // NSEG) % 2 == 0

    def run_timed(mm, tasks):
        tasks = sorted(tasks, key=lambda x: x[0])
        for k, prod in enumerate(mm):
            toks = {}
            while tasks and tasks[0][0] < 16 * (k + 1):
                time, f = tasks.pop(0)
                join(toks, time - 16 * k, token(*f()))
            prod(toks)
        for _, f in tasks:
            f()

    def body_b(n, its, mm, ln):
        *share, front, lag, tail, pitch = {
            28: (*B_SHARE, B_FRONT, B_WAIT, *B_TAIL), 21: B_LAST, 14: B_LAST2}[len(mm) // len(its)]
        spare = len(mm) // len(its) - sum(share)
        late, done = [], []
        tok, pending = None, None

        def finisher(i, j, finish, tiles):
            def run(tok):
                posts = []
                for h in range(2):
                    ot = finish(h, tok)

                    def post(ot=ot, h=h):
                        tiles[j, h] = jnp.concatenate(ot, axis=0).T
                        return vregs([tiles[j, h]], 4)

                    posts.append(post)
                if (j ^ 2, 0) in tiles:
                    posts += [lambda r=r: store_lhs(
                        O[n], i, 128 * (j % 2) + r,
                        *[tiles[j % 2 + u, h][r:r + B_STORE] for u in (0, 2) for h in range(2)])
                        for r in range(0, 128, B_STORE)]
                tiles[j, 0] = None
                return posts

            return run

        for i in its:
            state = [mem_load(n, i + h * NP) for h in range(2)]
            mem, tiles = [], {}
            if ln:
                for off in range(0, RC, 16):
                    late += ln_tasks(n + 2, i, off)
            for k, j in enumerate(B_ORDER):
                first, exps, finish = att_b_piece(n, i, j, mem, tok)
                done += pending(first) if pending else []
                cnt = share[k] + (0 if i is its[-1] else (spare + 3 - k) // 4)
                when = [int(32 * cnt * front * u / len(exps)) for u in range(len(exps))]
                for c in range(cnt):
                    toks = {}
                    if c == 0:
                        join(toks, 0, first)
                    for slot in B_POST:
                        if done and 16 * c + slot >= min(lag, 16 * cnt - 1):
                            join(toks, slot, token(*done.pop(0)()))
                    if late and c >= B_LN[0]:
                        join(toks, B_LN[1], token(*late.pop(0)()))
                    r = mm.pop(0)(toks)
                    while exps and when[0] < 32 * (c + 1):
                        exps.pop(0)(token(r[8 * (when.pop(0) - 32 * c):]))
                    tok = token(r)
                    if k == 0 and c == B_READ and n % NSEG:
                        mem.extend(mem_read(n, i, h, state[h], tok) for h in range(2))
                        done.append(lambda mem=mem: [v[:, 128 * u:] for v in mem for u in range(4)])
                    if k == B_UPDATE and c == 0 and n % NSEG != NSEG - 1:
                        new = [mem_update(n, i, h, state[h], tok) for h in range(2)]
                        done.append(lambda new=new: new)
                pending = finisher(i, j, finish, tiles)
        tok = token(mm.pop(0)(None))
        done += late + pending(tok)
        run_timed(mm, [(tail + pitch * u, f) for u, f in enumerate(done)])

    def step(n, ln=True, proj=(0, 1, 2), att=True, out=(1,), extra=None, unroll=UNROLL):
        def body(its):
            mm = []
            for i in its:
                for which in (B_MATS if att and not is_a(n) else A_MATS):
                    if which in proj:
                        mm += (proj_a if is_a(n + 1) else proj_b)(n + 1, i, which)
                    elif which == 3:
                        for lag in out:
                            mm += out_stage(n - lag, i)
            if att and not is_a(n):
                body_b(n, its, mm, ln)
                return
            tasks, span = [], 16 * len(mm) / (4 * len(its))
            for k, i in enumerate(its):
                if extra is not None:
                    fs = extra(i)
                    tasks += [(int(span * (4 * k + u // 8 + A_PREP_WHEN[u % 8])) if att else
                               int(4 * span * (k + (u + 1) / len(fs))) - 1, f)
                              for u, f in enumerate(fs)]
                for u, off in enumerate(range(0, RC, 16), 4 * k):
                    if att:
                        tasks += [(int(span * (u + w)), f) for w, f in att_a_tasks(n, i, off)]
                    if ln:
                        when = A_LN_WHEN if att else (.3, .8, 1.3)
                        tasks += [(int(span * (u + w)), f)
                                  for w, f in zip(when, ln_tasks(n + 2, i, off))]
            run_timed(mm, tasks)

        if unroll == NP:
            body(list(range(NP)))
        else:
            pl.loop(0, NP // unroll)(lambda i: body([unroll * i + u for u in range(unroll)]))

    for i in range(NP):
        start(x0_copies(i))
    start(slab_copies(0, 0))
    start([copy(beta_hbm, beta_ref.at[0], sem_b)])
    zero_ref[:8] = jnp.zeros((8, 128), U32)

    @pl.loop(0, NP)
    def _(i):
        pl.when(i % 2 == 1)(lambda: start(slab_copies(0, (i + 1) // 2)))
        wait(x0_copies(i))
        for fs in zip(*[ln_tasks(0, i, off) for off in range(0, RC, 16)]):
            for f in fs:
                f()

    start(slab_copies(0, 3))
    wait(slab_copies(0, 0))
    for f in prep_a_cols(0, 0):
        f()

    plan = (([(1, 0)], [(0, 1)]), ([(1, 1), (1, 2)], [(0, 2), (0, 3)]),
            ([(1, 3), (2, 0)], [(1, 0), (1, 1)]), ([(2, 1), (2, 2)], [(1, 2), (1, 3)]))
    for t, (fetch, preps) in enumerate(plan):
        for mi in fetch:
            start(slab_copies(*mi))
        for mi in preps:
            wait(slab_copies(*mi))
        mm = [f for i in range(NP) for f in proj_a(0, i, 0, only=t)]
        fs = [f for group in zip(*[prep_a_cols(*mi) for mi in preps]) for f in group]
        run_timed(mm, [(16 * len(mm) * (u + 1) // (len(fs) + 1), f) for u, f in enumerate(fs)])

    def prep_wv(i):
        pl.when(i == 0)(lambda: start(x_copies(1) + wao_copies()))
        wait(slab_copies(2, i))
        return prep_a_cols(2, i)

    start(slab_copies(2, 3))
    step(-1, ln=False, proj=(1,), att=False, out=(), extra=prep_wv, unroll=1)
    start(x_copies(2))
    start(x_copies(3))
    wait(x_copies(1))
    wait(wao_copies())
    step(-1, proj=(2,), att=False, out=(), extra=prep_a_rows)
    for m in range(4):
        start(wb_copies(m))
    wait([copy(beta_hbm, beta_ref.at[0], sem_b)])
    gate = jax.nn.sigmoid(beta_ref[0].astype(F32))
    eye = _iota((H, H), 0) == _iota((H, H), 1)
    gcol = jnp.sum(jnp.where(eye, jnp.broadcast_to(gate, (H, H)), 0.0), axis=1, keepdims=True)
    gtab[...] = jnp.broadcast_to(gcol, (H, 128))
    wait(x_copies(2))
    step(0, out=())
    wait(x_copies(3))
    for m in range(4):
        wait(wb_copies(m))
    step(1, extra=lambda i: prep_b(0, i) + prep_b(1, i))
    step(2, extra=lambda i: prep_b(2, i) + prep_b(3, i))
    for n in range(3, 14):
        step(n)
    start(out_copies(0))
    step(14, ln=False, out=())
    step(15, ln=False, proj=(), out=(2, 1))
    start(out_copies(1))
    start(out_copies(2))
    for i in range(NP):
        run_timed(out_stage(LAST, i), [])
        if i >= NP - 2:
            start(out_tile_copies(0, NP - 1) if i == NP - 2 else out_tile_copies(i, 1))
    for s in range(NSEG):
        wait(out_copies(s))


@jax.jit
def pallas_interleave_layers__sliding_local_dilated__memory_aug_infini_attn__prompt_kernel(
    A_x: jax.Array,
    A_wqkv: jax.Array,
    A_wo: jax.Array,
    B_x: jax.Array,
    B_wq: jax.Array,
    B_wk: jax.Array,
    B_wv: jax.Array,
    B_wo: jax.Array,
    B_beta: jax.Array,
):
    del B_x
    assert A_x.shape == (1, S, D)
    hbm = pl.BlockSpec(memory_space=pl.ANY)
    scratch = (
        [pltpu.VMEM((L, D), BF16)] * 4
        + [pltpu.VMEM((7, D, D), BF16), pltpu.VMEM((NT, D, 128), BF16),
           pltpu.VMEM((2, 576, 128), U32),
           *[pltpu.VMEM((1, NP, D // 4, 7 * 128), U32)] * 4,
           pltpu.VMEM((4, NP, D // 4, 7 * 128), U32)]
        + [pltpu.VMEM((NP, HL // 2, 7 * 128), U32)] * 5
        + [pltpu.VMEM((NT, L, 128), F32)] * 2
        + [pltpu.VMEM((NT, HALO + L, 128), F32)] * 4
        + [pltpu.VMEM((NP, L // 2, 2 * 128), U32)] * 8
        + [pltpu.VMEM((NT, 64, L), U32)] * 2
        + [pltpu.VMEM((NT, 16, 128), F32)] * 2
        + [pltpu.VMEM((NT, MZ_ROWS, 128), F32), pltpu.VMEM((8, 1, H), BF16),
           pltpu.VMEM((H, 128), F32),
           pltpu.VMEM((88, 128), U32),
           pltpu.SemaphoreType.DMA((NSEG,)), pltpu.SemaphoreType.DMA((5,)),
           pltpu.SemaphoreType.DMA((4, NP)),
           pltpu.SemaphoreType.DMA((NSEG,)), pltpu.SemaphoreType.DMA]
    )
    out = pl.pallas_call(
        _kernel,
        out_shape=jax.ShapeDtypeStruct((S, D), BF16),
        in_specs=[hbm] * 8,
        out_specs=hbm,
        scratch_shapes=scratch,
        compiler_params=pltpu.CompilerParams(vmem_limit_bytes=110 * 2**20),
        name="abab_stack",
    )(A_x.reshape(S, D), A_wqkv, A_wo, B_wq, B_wk, B_wv, B_wo, B_beta.reshape(1, H))
    return out.reshape(1, S, D)
```

```python
import jax
import jax.numpy as jnp
from jax import lax
import jax.experimental.pallas as pl
import jax.experimental.pallas.tpu as pltpu

S, D, H, DH = 2048, 1024, 32, 32
NSEG, L = 4, 512
HL = L // 2
NT = D // 128
NP = NT // 2
RC = HL // NP
KC = D // 2 // NP
LAST = 4 * NSEG - 1
WIN, DIL = 8, 2
HALO = 16
MZ_ROWS = 128 + 16
LOG2E = 1.4426950408889634
QSCALE = float(DH ** -0.5 * LOG2E)
MASKVAL = float(-1e9 * LOG2E)

B_ORDER = (3, 1, 2, 0)
B_SHARE = (8, 5, 6, 2)
B_LAST = (3, 3, 4, 1, 0.807, 30, 32, 2)
B_LAST2 = (4, 3, 2, 1, 0.866, 28, 30, 6)
B_FRONT = 0.832
B_POST = (7, 15)
B_WAIT = 28
B_TAIL = (30, 4)
B_STORE = 16
B_UPDATE = 0
B_READ = 0
A_MATS = (3, 0, 2, 1)
B_MATS = (2, 0, 1, 3)
UNROLL = 1
B_LN = (0, 5)
A_PLAIN = (0.051, 0.035, 0.08, 0.18, 0.286, 0.598, 0.056, 0.06, 0.025, 0.3, 0.486)
A_FIRST = (0.051, 0.036, 0.1, 0.218, 0.277, 0.628, 0.039, 0.049, 0.029, 0.314, 0.486)
A_THEN_B = (0.051, 0.035, 0.077, 0.18, 0.275, 0.594, 0.039, 0.069, 0.018, 0.28, 0.486)
A_PREP_WHEN = (0.276, 0.288, 0.408, 0.423, 0.353, 0.5, 0.556, 0.578)

F32, BF16, U32 = jnp.float32, jnp.bfloat16, jnp.uint32
_NT_DIMS = (((1,), (1,)), ((), ()))


def _iota(shape, axis):
    return lax.broadcasted_iota(jnp.int32, shape, axis)


def _dot(a, b):
    return jnp.dot(a, b, preferred_element_type=F32)


def _dot_nt(a, b):
    return lax.dot_general(a, b, _NT_DIMS, preferred_element_type=F32)


def _rows(start, size):
    return pl.ds(start if isinstance(start, int) else pl.multiple_of(start, size), size)


def _tile(k):
    return _rows(128 * k, 128)


def _words(val):
    return pltpu.bitcast(val.astype(BF16), U32)


def _split(words):
    return jnp.concatenate(
        [pltpu.unpack_elementwise(words, index=k, packed_dtype=BF16, unpacked_dtype=F32)
         for k in range(2)], axis=0)


def _merge(val):
    half = val.shape[0] // 2
    return pltpu.pack_elementwise([val[:half], val[half:]], packed_dtype=BF16)


def _put(ref, idx, start, k, words):
    ref[(*idx, _rows(start // 2, words.shape[0]), _tile(k))] = words
    return words


def _bf(words):
    return pltpu.bitcast(words, BF16)


def _phi(t):
    return jnp.where(t > 0, t + 1.0, jnp.exp(t))


def _tree(op, xs):
    xs = list(xs)
    while len(xs) > 1:
        xs = [op(xs[i], xs[i + 1]) if i + 1 < len(xs) else xs[i]
              for i in range(0, len(xs), 2)]
    return xs[0]


def _lhs_terms(a11, a12, a21, a22):
    return (a11 + a22, a21 + a22, a11, a22, a11 + a12, a21 - a11, a12 - a22)


def _rhs_terms(b11, b12, b21, b22):
    return (b11 + b22, b11, b12 - b22, b21 - b11, b22, b11 + b12, b21 + b22)


def _kernel(x_hbm, wqkv_hbm, awo_hbm, wq_hbm, wk_hbm, wv_hbm, wo_hbm, beta_hbm,
            out_hbm,
            x0, x1, x2, x3, wraw, wraw_o, wtmp, waq, wak, wav, wao, wb,
            xn0, xn1, o0, o1, o2,
            qa0, qa1, ka0, ka1, va0, va1,
            qs0, qs1, pq0, pq1, kb0, kb1, pk0, pk1, vt0, vt1,
            zs0, zs1, mz, beta_ref, gtab, zero_ref, sem_x, sem_w, sem_s, sem_o, sem_b):
    X = (x0, x1, x2, x3)
    XN, wa = (xn0, xn1), (waq, wak, wav)
    O = [o2 if n == LAST else (o0, o1)[n % 2] for n in range(LAST + 1)]
    QA, KA, VA = (qa0, qa1), (ka0, ka1), (va0, va1)
    QS, PQ, KB, PK, VT = (qs0, qs1), (pq0, pq1), (kb0, kb1), (pk0, pk1), (vt0, vt1)
    ZS = (zs0, zs1)

    copy = pltpu.make_async_copy

    def x_copies(s):
        return [copy(x_hbm.at[pl.ds(s * L, L)], X[s], sem_x.at[s])]

    def out_copies(s):
        return [copy(X[s], out_hbm.at[pl.ds(s * L, L)], sem_o.at[s])]

    def out_tile_copies(t0, nt):
        cols = [pl.ds(128 * (t0 + c * NP), 128 * nt) for c in range(2)]
        return [copy(x3.at[:, c], out_hbm.at[pl.ds(S - L, L), c], sem_o.at[NSEG - 1]) for c in cols]

    def wao_copies():
        return [copy(awo_hbm.at[:, _tile(t)], wraw_o.at[t], sem_w.at[4]) for t in range(NT)]

    def wb_copies(m):
        return [copy((wq_hbm, wk_hbm, wv_hbm, wo_hbm)[m], wraw.at[3 + m], sem_w.at[m])]

    def slab_copies(m, i):
        return [copy(wqkv_hbm.at[r, _rows(m * D, D)], wraw.at[m, r], sem_s.at[m, i])
                for r in (_rows(h * (D // 2) + i * KC, KC) for h in range(2))]

    def x0_copies(i):
        return [copy(x_hbm.at[r], x0.at[r], sem_s.at[3, i])
                for r in (_rows(h * HL + i * RC, RC) for h in range(2))]

    def start(cs):
        for c in cs:
            c.start()

    def wait(cs):
        for c in cs:
            c.wait()

    def token(*vals):
        bits = [pltpu.bitcast(v[:8, :128], U32) for v in vals]
        return _tree(jnp.bitwise_or, bits) & zero_ref[:8]

    def vregs(vals, every=1):
        return [v[u:u + 8] for v in vals for u in range(0, v.shape[0], 8)][::-1][::every]

    def after(words, toks):
        if not toks:
            return words
        slabs = []
        for k in range(words.shape[0] // 8):
            slab = words[8 * k:8 * k + 8]
            if toks.get(k) is not None:
                slab = slab | jnp.concatenate([toks[k]] * (words.shape[1] // 128), axis=1)
            slabs.append(slab)
        return jnp.concatenate(slabs, axis=0)

    def store_rhs(dst, m, i, r, b11, b12, b21, b22):
        terms = _rhs_terms(*[_split(b) for b in (b11, b12, b21, b22)])
        words = [{1: b11, 4: b22}[k] if k in (1, 4) else _merge(v) for k, v in enumerate(terms)]
        return vregs([_put(dst, (m, i), r, k, v) for k, v in enumerate(words)])

    def raw_words(m, r, rows, t):
        return pltpu.bitcast(wraw[m, _rows(r, rows), _tile(t)], U32)

    def prep_b(m, i):
        def piece(j, c):
            r = i * KC + 32 * c
            return store_rhs(wb, m, j, r, *[raw_words(3 + m, r + h * (D // 2), 32, j + u * NP)
                                            for h in range(2) for u in range(2)])

        return [lambda j=j, c=c: piece(j, c) for j in range(NP) for c in range(KC // 32)]

    def prep_a_cols(m, i):
        rows = 32
        st = {}

        def rotate(c):
            v = [jnp.concatenate([raw_words(m, i * KC + c * rows + h * (D // 2), rows, t)
                                  for h in range(2)], axis=0) for t in range(NT)]
            st[c] = [x if t == 0 else pltpu.roll(x, 2 * t, 1) for t, x in enumerate(v)]
            return vregs(st[c], 4)

        def shear(c):
            slot = (_iota((rows, 128), 1) >> 1) & 7
            v = [st[c][(-b) % NT] for b in range(NT)]
            for bit in (1, 2, 4):
                sel = (slot & bit) != 0
                v = [jnp.where(sel, v[(b - bit) % NT], v[b]) for b in range(NT)]
            st[c] = [x if b == 0 else pltpu.roll(x, 128 - 2 * b, 1) for b, x in enumerate(v)]
            return vregs(v, 2)

        def terms(c):
            v, half, outs = st[c], rows // 2, []
            for j in range(NP):
                outs += store_rhs(wa[m], 0, j, i * KC + c * rows, v[j][:half], v[j + NP][:half],
                                  v[j][half:], v[j + NP][half:])
            return outs

        order = [(f, k - lag) for k in range(6) for lag, f in enumerate((rotate, shear, terms))
                 if 0 <= k - lag < 4]
        return [lambda f=f, c=c: f(c) for f, c in order]

    def prep_a_rows(i):
        def stage(t):
            words = [pltpu.bitcast(wraw_o[i + h * NP, _tile(t), :], U32) for h in range(2)]
            for h in range(2):
                wtmp[h, pl.ds(65 * t, 64), :] = words[h]
            return vregs(words)

        def rows(h, b, u):
            return jnp.concatenate(
                [wtmp[h, pl.ds(8 * (u + k) + b, 8, stride=65), :] for k in range(2)], axis=0)

        def piece(c, u):
            return store_rhs(wao, 0, i, 128 * c + 16 * u, rows(0, c, u), rows(1, c, u),
                             rows(0, c + NP, u), rows(1, c + NP, u))

        return ([lambda t=t: stage(t) for t in range(NT)]
                + [lambda c=c, u=u: piece(c, u) for c in range(4) for u in range(0, 8, 2)])

    def store_lhs(dst, t, r, a11, a12, a21, a22, pack=_words):
        terms = _lhs_terms(a11, a12, a21, a22)
        return vregs([_put(dst, (t,), r, k, pack(v)) for k, v in enumerate(terms)])

    def join(toks, slot, tok):
        if tok is not None:
            toks[slot] = tok if toks.get(slot) is None else toks[slot] | tok

    def products(a_ref, w_ref, m, i, emit, only=None):
        st = {}

        def prod(k, toks, finish):
            if only is None:
                a = jnp.concatenate([after(a_ref[t, :, _tile(k)], toks if t == 0 else None)
                                     for t in range(NP)], axis=1)
                w = w_ref[m, i, :, _tile(k)]
            else:
                a = after(a_ref[only, :, _tile(k)], toks)
                w = w_ref[m, i, _rows(64 * only, 64), _tile(k)]
            r = _dot(_bf(a), _bf(w))
            finish(r)
            return r

        def p1(r):
            st["m1"] = r

        def p2(r):
            st["c21"], st["c22"] = r, st["m1"] - r

        def p3(r):
            st["c12"], st["c22"] = r, st["c22"] + r

        def p4(r):
            st["c11"] = st["m1"] + r
            emit(1, 0, st["c21"] + r)

        def p5(r):
            st["c11"] = st["c11"] - r
            emit(0, 1, st["c12"] + r)

        def p6(r):
            emit(1, 1, st["c22"] + r)

        def p7(r):
            emit(0, 0, st["c11"] + r)

        return [lambda toks, k=k, f=f: prod(k, toks, f)
                for k, f in enumerate((p1, p2, p3, p4, p5, p6, p7))]

    def ln_tasks(n, i, off, nr=16):
        src, dst = X[n % NSEG], XN[n % 2]
        st = {}

        def mean():
            st["x"] = [
                jnp.concatenate(
                    [_split(pltpu.bitcast(src[_rows(i * RC + off + h * HL, nr), _tile(t)], U32))
                     for h in range(2)], axis=0) for t in range(NT)]
            part = _tree(jnp.add, st["x"])
            st["mean"] = jnp.sum(part, axis=1, keepdims=True) * (1.0 / D)
            return vregs([part])

        def var():
            st["x"] = [x - st["mean"] for x in st["x"]]
            part = _tree(jnp.add, [x * x for x in st["x"]])
            st["var"] = jnp.sum(part, axis=1, keepdims=True) * (1.0 / D)
            return vregs([part])

        def scale():
            inv = lax.rsqrt(st["var"] + 1e-5)
            y = [x * inv for x in st["x"]]
            r = i * RC + off
            outs = []
            for t in range(NP):
                outs += store_lhs(dst, t, r, y[t][:nr], y[t + NP][:nr], y[t][nr:], y[t + NP][nr:],
                                  _merge)
            return outs

        return [mean, var, scale]

    def proj_a(n, i, which, only=None):
        p = n % 2

        def emit(h, c, y):
            t = i + c * NP
            buf = (QA, KA, VA)[which]
            rows = pl.ds(h * HL + (HALO if which else 0), HL)
            if only:
                y = y + buf[p][t, rows, :]
            buf[p][t, rows, :] = y
            if which and h == 0 and n % NSEG == 0:
                buf[p][t, pl.ds(0, HALO), :] = jnp.zeros((HALO, 128), F32)
            elif which and h == 0:
                buf[p][t, pl.ds(0, HALO), :] = buf[1 - p][t, pl.ds(L, HALO), :]

        return products(XN[p], wa[which], 0, i, emit, only)

    def proj_b(n, i, which):
        p = n % 2

        def emit(h, c, y):
            if which == 0:
                _put(QS[p], (i,), h * HL, c, _words(y * QSCALE))
                _put(PQ[p], (i,), h * HL, c, _words(_phi(y)))
            elif which == 1:
                _put(KB[p], (i,), h * HL, c, _words(y))
                if n % NSEG != NSEG - 1:
                    y = _phi(y)
                    _put(PK[p], (i,), h * HL, c, _words(y))
                    ZS[p][i + c * NP, pl.ds(8 * h, 8), :] = _tree(jnp.add, vregs([y]))
            else:
                VT[p][i + c * NP, :, pl.ds(h * HL, HL)] = pltpu.bitcast(y.astype(BF16).T, U32)

        return products(XN[p], wb, which, i, emit)

    def out_stage(n, i):
        x = X[n % NSEG]

        def emit(h, c, y):
            where = (pl.ds(h * HL, HL), _tile(i + c * NP))
            x[where] = (x[where].astype(F32) + y).astype(BF16)

        if is_a(n):
            return products(O[n], wao, 0, i, emit)
        return products(O[n], wb, 3, i, emit)

    def att_a_tasks(n, i, off, times):
        p = n % 2
        base = (i * RC if isinstance(i, int) else pl.multiple_of(i * RC, RC)) + off
        starts = [base + (u // 2) * HL + 8 * (u % 2) for u in range(4)]
        lg, mixed = [[] for _ in range(4)], {}

        def scores(u, ws):
            q = [QA[p][t, pl.ds(starts[u], 8), :] for t in range(NT)]
            for w in ws:
                kr = pl.ds(starts[u] + HALO - DIL * w, 8)
                lg[u].append(_tree(jnp.add, [q[t] * KA[p][t, kr, :] for t in range(NT)]))
            return lg[u][-len(ws):]

        def exchange(u, bit):
            low = (_iota((8, 128), 1) & bit) == 0
            lg[u] = [a + jnp.where(low, pltpu.roll(a, 128 - bit, 1), pltpu.roll(a, bit, 1))
                     for a in lg[u]]
            return lg[u]

        def softmax(u):
            v = [a * QSCALE for a in lg[u]]
            if n % NSEG == 0 and off == 0 and u < 2:
                pos = _iota((8, 128), 0) + starts[u]
                v = [a if w == 0 else jnp.where(pos >= DIL * w, a, MASKVAL)
                     for w, a in enumerate(v)]
            m = _tree(jnp.maximum, v)
            e = [jnp.exp2(a - m) for a in v]
            inv = 1.0 / _tree(jnp.add, e)
            lg[u] = [a * inv for a in e]
            return lg[u]

        def mix(t, h):
            for c in range(2):
                mixed[t, h, c] = jnp.concatenate([
                    _tree(jnp.add, [
                        lg[u][w] * VA[p][t + c * NP, pl.ds(starts[u] + HALO - DIL * w, 8), :]
                        for w in range(WIN)])
                    for u in (2 * h, 2 * h + 1)], axis=0)
            return vregs([mixed[t, h, c] for c in range(2)])

        def store(t):
            return store_lhs(O[n], t, i * RC + off,
                             *[mixed[t, h, c] for h in range(2) for c in range(2)])

        t_score, d_score, lag1, lag2, lag3, t_mix, d_mix, d_store = times
        tasks = []
        for u in range(4):
            t = t_score + d_score * (2 * u + 1)
            tasks += [(t - d_score, lambda u=u: scores(u, range(4))),
                      (t, lambda u=u: scores(u, range(4, 8))),
                      (t + lag1, lambda u=u: exchange(u, 1)),
                      (t + lag2, lambda u=u: exchange(u, 16)),
                      (t + lag3, lambda u=u: softmax(u))]
        for k in range(NP):
            t = t_mix + k * (d_mix + d_store)
            tasks += [(t, lambda k=k: mix(k, 0)), (t + d_mix, lambda k=k: mix(k, 1))]
            tasks += [(t + d_mix + d_store / 2, lambda k=k: store(k))]
        return tasks

    def att_b_piece(n, i, j, mem, tok):
        p = n % 2
        rows = pl.ds(64 * j, 64)
        nk = 128 * j + 64
        head = _iota((32, 128), 1) >> 5
        key, lane = _iota((64, 128), 0), _iota((64, 128), 1)
        causal = [jnp.where(key > q, MASKVAL, 0.0) for q in (lane, lane ^ 64, lane & 63)]
        high = _iota((8, 128), 1) >= 64
        s, sx, late_q = [], [], []
        for h in range(2):
            qw = after(QS[p][i, rows, _tile(h)], {0: tok, 4: tok})
            early = [jnp.where(head == hh, qw[:32], jnp.uint32(0)) for hh in range(4)]
            late = [jnp.where(head == hh, qw[32:], jnp.uint32(0)) for hh in range(4)]
            late_q.append(jnp.concatenate([late[1], late[0], late[3], late[2]], axis=0))
            qcat = jnp.concatenate([early[0], late[0], late[1], early[1],
                                    early[2], late[2], late[3], early[3]], axis=0)
            st = _dot_nt(_bf(KB[p][i, pl.ds(0, nk // 2), _tile(h)]), _bf(qcat))
            for hh in range(4):
                v = st[:, 128 * hh:128 * (hh + 1)]
                s.append([v[u:u + 8] for u in range(0, nk - 64, 8)]
                         + [v[nk - 64 + u:nk - 56 + u] + causal[hh % 2][u:u + 8]
                            for u in range(0, 64, 8)])
        for h in range(2):
            st = _dot_nt(_bf(KB[p][i, pl.ds(nk // 2, 32), _tile(h)]), _bf(late_q[h]))
            for u in range(2):
                v = st[:, 128 * u:128 * (u + 1)] + causal[2]
                sx.append([v[r:r + 8] for r in range(0, 64, 8)])
        first = token(*[v[0] for v in s])
        m = []
        for u in range(4):
            mx = _tree(jnp.maximum, sx[u])
            for odd in range(2):
                a = _tree(jnp.maximum, s[2 * u + odd])
                b = jnp.maximum(a, mx)
                a = jnp.where(high, a, b) if odd else jnp.where(high, b, a)
                m.append(jnp.broadcast_to(jnp.max(a, axis=0, keepdims=True), (8, 128)))
        e = [[] for _ in range(8)]
        part = [[] for _ in range(8)]

        def exps(v, mh, tok):
            mh = mh if tok is None else mh + pltpu.bitcast(tok, F32)
            return [jnp.exp2(a - mh) for a in v]

        def exp_tile(u, c, tok):
            v = exps(s[u][16 * c:16 * (c + 1)], m[u], tok)
            part[u] = [_tree(jnp.add, part[u] + v)]
            e[u].extend(v)

        def exp_diag(u, tok):
            for odd in range(2):
                exp_tile(2 * u + odd, j, tok)
            v = exps(sx[u], jnp.where(high, m[2 * u], m[2 * u + 1]), tok)
            tot = _tree(jnp.add, v)
            for odd in range(2):
                pick = (lambda a: jnp.where(high, 0.0, a)) if odd else (lambda a: jnp.where(high, a, 0.0))
                part[2 * u + odd] = [part[2 * u + odd][0] + pick(tot)]
                e[2 * u + odd].extend(pick(a) for a in v)

        def finish(h, tok):
            g = i + h * NP
            ot = []
            for hh in range(4):
                u = 4 * h + hh
                vt = after(VT[p][g, pl.ds(16 * hh, 16), pl.ds(0, 128 * (j + 1))], {0: tok})
                acc = _dot(_bf(vt), jnp.concatenate(e[u], axis=0).astype(BF16))
                l = jnp.sum(part[u][0], axis=0, keepdims=True)
                gate = gtab[pl.ds(4 * g + hh, 1), :]
                acc = acc * ((1.0 - gate) / l)
                if hh % 2:
                    acc = pltpu.roll(acc, 64, 1)
                if n % NSEG:
                    r = mem[h][:, 128 * j:128 * (j + 1)]
                    den = r[128 + 4 * hh:129 + 4 * hh] + 1e-6
                    acc = acc + r[32 * hh:32 * hh + 32] * (gate / den)
                ot.append(acc)
            return ot

        tasks = []
        for u in range(4):
            tasks += [lambda tok, u=2 * u + odd, c=c: exp_tile(u, c, tok)
                      for odd in range(2) for c in range(j)]
            tasks.append(lambda tok, u=u: exp_diag(u, tok))
        return first, tasks, finish

    def mem_load(n, g):
        if n % NSEG == 0:
            return jnp.zeros((MZ_ROWS, 128), F32)
        return mz[g]

    def mem_read(n, i, h, state, tok):
        pq = after(PQ[n % 2][i, :, _tile(h)], {8 * u: tok for u in range(4)})
        return _dot_nt(state.astype(BF16), _bf(pq))

    def mem_update(n, i, h, state, tok):
        p, g = n % 2, i + h * NP
        z = jnp.sum(ZS[p][g], axis=0, keepdims=True)
        new = jnp.concatenate([_dot(_bf(after(VT[p][g], {0: tok})), _bf(PK[p][i, :, _tile(h)])),
                               jnp.broadcast_to(z, (MZ_ROWS - 128, 128))], axis=0)
        row = _iota((MZ_ROWS, 128), 0)
        row_head = jnp.where(row < 128, row >> 5, (row - 128) >> 2)
        keep = row_head == (_iota((MZ_ROWS, 128), 1) >> 5)
        mz[g] = new = state + jnp.where(keep, new, 0.0)
        return new

    def is_a(n):
        return (n // NSEG) % 2 == 0

    def run_timed(mm, tasks):
        tasks = sorted(tasks, key=lambda x: x[0])
        for k, prod in enumerate(mm):
            toks = {}
            while tasks and tasks[0][0] < 16 * (k + 1):
                time, f = tasks.pop(0)
                join(toks, time - 16 * k, token(*f()))
            prod(toks)
        for _, f in tasks:
            f()

    def body_b(n, its, mm, ln):
        *share, front, lag, tail, pitch = {
            28: (*B_SHARE, B_FRONT, B_WAIT, *B_TAIL), 21: B_LAST, 14: B_LAST2}[len(mm) // len(its)]
        spare = len(mm) // len(its) - sum(share)
        late, done = [], []
        tok, pending = token(mm.pop(0)(None)), None

        def finisher(i, j, finish, tiles):
            def run(tok):
                posts = []
                for h in range(2):
                    ot = finish(h, tok)

                    def post(ot=ot, h=h):
                        tiles[j, h] = jnp.concatenate(ot, axis=0).T
                        return vregs([tiles[j, h]], 4)

                    posts.append(post)
                if (j ^ 2, 0) in tiles:
                    posts += [lambda r=r: store_lhs(
                        O[n], i, 128 * (j % 2) + r,
                        *[tiles[j % 2 + u, h][r:r + B_STORE] for u in (0, 2) for h in range(2)])
                        for r in range(0, 128, B_STORE)]
                tiles[j, 0] = None
                return posts

            return run

        for i in its:
            state = [mem_load(n, i + h * NP) for h in range(2)]
            mem, tiles = [], {}
            if ln:
                for off in range(0, RC, 16):
                    late += ln_tasks(n + 2, i, off)
            for k, j in enumerate(B_ORDER):
                first, exps, finish = att_b_piece(n, i, j, mem, tok)
                done += pending(first) if pending else []
                cnt = share[k] + (0 if i is its[-1] else (spare + 3 - k) // 4)
                when = [int(32 * cnt * front * u / len(exps)) for u in range(len(exps))]
                for c in range(cnt):
                    toks = {}
                    if c == 0:
                        join(toks, 0, first)
                    for slot in B_POST:
                        if done and 16 * c + slot >= min(lag, 16 * cnt - 1):
                            join(toks, slot, token(*done.pop(0)()))
                    if late and c >= B_LN[0]:
                        join(toks, B_LN[1], token(*late.pop(0)()))
                    r = mm.pop(0)(toks)
                    while exps and when[0] < 32 * (c + 1):
                        exps.pop(0)(token(r[8 * (when.pop(0) - 32 * c):]))
                    tok = token(r)
                    if k == 0 and c == B_READ and n % NSEG:
                        mem.extend(mem_read(n, i, h, state[h], tok) for h in range(2))
                        done.append(lambda mem=mem: [v[:, 128 * u:] for v in mem for u in range(4)])
                    if k == B_UPDATE and c == 0 and n % NSEG != NSEG - 1:
                        new = [mem_update(n, i, h, state[h], tok) for h in range(2)]
                        done.append(lambda new=new: new)
                pending = finisher(i, j, finish, tiles)
        tok = token(mm.pop(0)(None))
        done += late + pending(tok)
        run_timed(mm, [(tail + pitch * u, f) for u, f in enumerate(done)])

    def step(n, ln=True, proj=(0, 1, 2), att=True, out=(1,), extra=None, unroll=UNROLL):
        def body(its):
            mm = []
            for i in its:
                for which in (B_MATS if att and not is_a(n) else A_MATS):
                    if which in proj:
                        mm += (proj_a if is_a(n + 1) else proj_b)(n + 1, i, which)
                    elif which == 3:
                        for lag in out:
                            mm += out_stage(n - lag, i)
            if att and not is_a(n):
                body_b(n, its, mm, ln)
                return
            times = A_FIRST if n == 0 else A_PLAIN if is_a(n + 1) else A_THEN_B
            tasks, span = [], 16 * len(mm) / (4 * len(its))
            for k, i in enumerate(its):
                if extra is not None:
                    fs = extra(i)
                    tasks += [(int(span * (4 * k + u // 8 + A_PREP_WHEN[u % 8])) if att else
                               int(4 * span * (k + (u + 1) / len(fs))) - 1, f)
                              for u, f in enumerate(fs)]
                for u, off in enumerate(range(0, RC, 16), 4 * k):
                    if att:
                        tasks += [(int(span * (u + w)), f) for w, f in att_a_tasks(n, i, off, times[:8])]
                    if ln:
                        when = times[8:] if att else (.3, .8, 1.3)
                        tasks += [(int(span * (u + w)), f)
                                  for w, f in zip(when, ln_tasks(n + 2, i, off))]
            run_timed(mm, tasks)

        if unroll == NP:
            body(list(range(NP)))
        else:
            pl.loop(0, NP // unroll)(lambda i: body([unroll * i + u for u in range(unroll)]))

    for i in range(NP):
        start(x0_copies(i))
    start(slab_copies(0, 0))
    start([copy(beta_hbm, beta_ref.at[0], sem_b)])
    zero_ref[:8] = jnp.zeros((8, 128), U32)

    @pl.loop(0, NP)
    def _(i):
        pl.when(i % 2 == 1)(lambda: start(slab_copies(0, (i + 1) // 2)))
        wait(x0_copies(i))
        for fs in zip(*[ln_tasks(0, i, off) for off in range(0, RC, 16)]):
            for f in fs:
                f()

    start(slab_copies(0, 3))
    wait(slab_copies(0, 0))
    for f in prep_a_cols(0, 0):
        f()

    plan = (([(1, 0)], [(0, 1)]), ([(1, 1), (1, 2)], [(0, 2), (0, 3)]),
            ([(1, 3), (2, 0)], [(1, 0), (1, 1)]), ([(2, 1), (2, 2)], [(1, 2), (1, 3)]))
    for t, (fetch, preps) in enumerate(plan):
        for mi in fetch:
            start(slab_copies(*mi))
        for mi in preps:
            wait(slab_copies(*mi))
        mm = [f for i in range(NP) for f in proj_a(0, i, 0, only=t)]
        fs = [f for group in zip(*[prep_a_cols(*mi) for mi in preps]) for f in group]
        run_timed(mm, [(16 * len(mm) * (u + 1) // (len(fs) + 1), f) for u, f in enumerate(fs)])

    def prep_wv(i):
        pl.when(i == 0)(lambda: start(x_copies(1) + wao_copies()))
        wait(slab_copies(2, i))
        return prep_a_cols(2, i)

    start(slab_copies(2, 3))
    step(-1, ln=False, proj=(1,), att=False, out=(), extra=prep_wv, unroll=1)
    start(x_copies(2))
    start(x_copies(3))
    wait(x_copies(1))
    wait(wao_copies())
    step(-1, proj=(2,), att=False, out=(), extra=prep_a_rows)
    for m in range(4):
        start(wb_copies(m))
    wait([copy(beta_hbm, beta_ref.at[0], sem_b)])
    gate = jax.nn.sigmoid(beta_ref[0].astype(F32))
    eye = _iota((H, H), 0) == _iota((H, H), 1)
    gcol = jnp.sum(jnp.where(eye, jnp.broadcast_to(gate, (H, H)), 0.0), axis=1, keepdims=True)
    gtab[...] = jnp.broadcast_to(gcol, (H, 128))
    wait(x_copies(2))
    step(0, out=())
    wait(x_copies(3))
    for m in range(4):
        wait(wb_copies(m))
    step(1, extra=lambda i: prep_b(0, i) + prep_b(1, i))
    step(2, extra=lambda i: prep_b(2, i) + prep_b(3, i))
    for n in range(3, 14):
        step(n)
    start(out_copies(0))
    step(14, ln=False, out=())
    step(15, ln=False, proj=(), out=(2, 1))
    start(out_copies(1))
    start(out_copies(2))
    for i in range(NP):
        run_timed(out_stage(LAST, i), [])
        if i >= NP - 2:
            start(out_tile_copies(0, NP - 1) if i == NP - 2 else out_tile_copies(i, 1))
    for s in range(NSEG):
        wait(out_copies(s))


@jax.jit
def pallas_interleave_layers__sliding_local_dilated__memory_aug_infini_attn__prompt_kernel(
    A_x: jax.Array,
    A_wqkv: jax.Array,
    A_wo: jax.Array,
    B_x: jax.Array,
    B_wq: jax.Array,
    B_wk: jax.Array,
    B_wv: jax.Array,
    B_wo: jax.Array,
    B_beta: jax.Array,
):
    del B_x
    assert A_x.shape == (1, S, D)
    hbm = pl.BlockSpec(memory_space=pl.ANY)
    scratch = (
        [pltpu.VMEM((L, D), BF16)] * 4
        + [pltpu.VMEM((7, D, D), BF16), pltpu.VMEM((NT, D, 128), BF16),
           pltpu.VMEM((2, 576, 128), U32),
           *[pltpu.VMEM((1, NP, D // 4, 7 * 128), U32)] * 4,
           pltpu.VMEM((4, NP, D // 4, 7 * 128), U32)]
        + [pltpu.VMEM((NP, HL // 2, 7 * 128), U32)] * 5
        + [pltpu.VMEM((NT, L, 128), F32)] * 2
        + [pltpu.VMEM((NT, HALO + L, 128), F32)] * 4
        + [pltpu.VMEM((NP, L // 2, 2 * 128), U32)] * 8
        + [pltpu.VMEM((NT, 64, L), U32)] * 2
        + [pltpu.VMEM((NT, 16, 128), F32)] * 2
        + [pltpu.VMEM((NT, MZ_ROWS, 128), F32), pltpu.VMEM((8, 1, H), BF16),
           pltpu.VMEM((H, 128), F32),
           pltpu.VMEM((88, 128), U32),
           pltpu.SemaphoreType.DMA((NSEG,)), pltpu.SemaphoreType.DMA((5,)),
           pltpu.SemaphoreType.DMA((4, NP)),
           pltpu.SemaphoreType.DMA((NSEG,)), pltpu.SemaphoreType.DMA]
    )
    out = pl.pallas_call(
        _kernel,
        out_shape=jax.ShapeDtypeStruct((S, D), BF16),
        in_specs=[hbm] * 8,
        out_specs=hbm,
        scratch_shapes=scratch,
        compiler_params=pltpu.CompilerParams(vmem_limit_bytes=110 * 2**20),
        name="abab_stack",
    )(A_x.reshape(S, D), A_wqkv, A_wo, B_wq, B_wk, B_wv, B_wo, B_beta.reshape(1, H))
    return out.reshape(1, S, D)
```

```python
import jax
import jax.numpy as jnp
from jax import lax
import jax.experimental.pallas as pl
import jax.experimental.pallas.tpu as pltpu

S, D, H, DH = 2048, 1024, 32, 32
NSEG, L = 4, 512
HL = L // 2
NT = D // 128
NP = NT // 2
RC = HL // NP
KC = D // 2 // NP
LAST = 4 * NSEG - 1
WIN, DIL = 8, 2
HALO = 16
MZ_ROWS = 128 + 16
LOG2E = 1.4426950408889634
QSCALE = float(DH ** -0.5 * LOG2E)
MASKVAL = float(-1e9 * LOG2E)

B_ORDER = (3, 1, 2, 0)
B_SHARE = (8, 5, 5, 1)
B_LAST = (3, 2, 5, 1, 0.85, 30, 31, 1)
B_LAST2 = (4, 3, 2, 1, 0.866, 29, 29, 7)
B_FRONT = 0.832
B_POST = (7, 15)
B_WAIT = 28
B_TAIL = (44, 5)
B_STORE = 16
B_UPDATE = 0
B_READ = 0
A_MATS = (3, 0, 2, 1)
B_MATS = (2, 0, 1, 3)
T_DUE = 36
UNROLL = 1
B_LN = (0, 5)
A_PLAIN = (0.051, 0.035, 0.08, 0.18, 0.286, 0.598, 0.056, 0.06, 0.025, 0.3, 0.486)
A_FIRST = (0.051, 0.036, 0.1, 0.218, 0.277, 0.628, 0.039, 0.049, 0.029, 0.314, 0.486)
A_THEN_B = (0.051, 0.035, 0.077, 0.18, 0.275, 0.594, 0.039, 0.069, 0.018, 0.28, 0.486)
A_PREP_WHEN = (0.276, 0.288, 0.408, 0.423, 0.353, 0.5, 0.556, 0.578)

F32, BF16, U32 = jnp.float32, jnp.bfloat16, jnp.uint32
_NT_DIMS = (((1,), (1,)), ((), ()))


def _iota(shape, axis):
    return lax.broadcasted_iota(jnp.int32, shape, axis)


def _dot(a, b):
    return jnp.dot(a, b, preferred_element_type=F32)


def _dot_nt(a, b):
    return lax.dot_general(a, b, _NT_DIMS, preferred_element_type=F32)


def _rows(start, size):
    return pl.ds(start if isinstance(start, int) else pl.multiple_of(start, size), size)


def _tile(k):
    return _rows(128 * k, 128)


def _words(val):
    return pltpu.bitcast(val.astype(BF16), U32)


def _split(words):
    return jnp.concatenate(
        [pltpu.unpack_elementwise(words, index=k, packed_dtype=BF16, unpacked_dtype=F32)
         for k in range(2)], axis=0)


def _merge(val):
    half = val.shape[0] // 2
    return pltpu.pack_elementwise([val[:half], val[half:]], packed_dtype=BF16)


def _put(ref, idx, start, k, words):
    ref[(*idx, _rows(start // 2, words.shape[0]), _tile(k))] = words
    return words


def _bf(words):
    return pltpu.bitcast(words, BF16)


def _phi(t):
    return jnp.where(t > 0, t + 1.0, jnp.exp(t))


def _tree(op, xs):
    xs = list(xs)
    while len(xs) > 1:
        xs = [op(xs[i], xs[i + 1]) if i + 1 < len(xs) else xs[i]
              for i in range(0, len(xs), 2)]
    return xs[0]


def _lhs_terms(a11, a12, a21, a22):
    return (a11 + a22, a21 + a22, a11, a22, a11 + a12, a21 - a11, a12 - a22)


def _rhs_terms(b11, b12, b21, b22):
    return (b11 + b22, b11, b12 - b22, b21 - b11, b22, b11 + b12, b21 + b22)


def _kernel(x_hbm, wqkv_hbm, awo_hbm, wq_hbm, wk_hbm, wv_hbm, wo_hbm, beta_hbm,
            out_hbm,
            x0, x1, x2, x3, wraw, wraw_o, wtmp, waq, wak, wav, wao, wb,
            xn0, xn1, o0, o1, o2,
            qa0, qa1, ka0, ka1, va0, va1,
            pq0, pq1, kb0, kb1, pk0, pk1, qt0, qt1, vt0, vt1,
            zs0, zs1, mz, beta_ref, gtab, zero_ref, sem_x, sem_w, sem_s, sem_o, sem_b):
    X = (x0, x1, x2, x3)
    XN, wa = (xn0, xn1), (waq, wak, wav)
    O = [o2 if n == LAST else (o0, o1)[n % 2] for n in range(LAST + 1)]
    QA, KA, VA = (qa0, qa1), (ka0, ka1), (va0, va1)
    QT, PQ, KB, PK, VT = (qt0, qt1), (pq0, pq1), (kb0, kb1), (pk0, pk1), (vt0, vt1)
    ZS = (zs0, zs1)

    copy = pltpu.make_async_copy

    def x_copies(s):
        return [copy(x_hbm.at[pl.ds(s * L, L)], X[s], sem_x.at[s])]

    def out_copies(s):
        return [copy(X[s], out_hbm.at[pl.ds(s * L, L)], sem_o.at[s])]

    def out_tile_copies(t0, nt):
        cols = [pl.ds(128 * (t0 + c * NP), 128 * nt) for c in range(2)]
        return [copy(x3.at[:, c], out_hbm.at[pl.ds(S - L, L), c], sem_o.at[NSEG - 1]) for c in cols]

    def wao_copies():
        return [copy(awo_hbm.at[:, _tile(t)], wraw_o.at[t], sem_w.at[4]) for t in range(NT)]

    def wb_copies(m):
        return [copy((wq_hbm, wk_hbm, wv_hbm, wo_hbm)[m], wraw.at[3 + m], sem_w.at[m])]

    def slab_copies(m, i):
        return [copy(wqkv_hbm.at[r, _rows(m * D, D)], wraw.at[m, r], sem_s.at[m, i])
                for r in (_rows(h * (D // 2) + i * KC, KC) for h in range(2))]

    def x0_copies(i):
        return [copy(x_hbm.at[r], x0.at[r], sem_s.at[3, i])
                for r in (_rows(h * HL + i * RC, RC) for h in range(2))]

    def start(cs):
        for c in cs:
            c.start()

    def wait(cs):
        for c in cs:
            c.wait()

    def token(*vals):
        bits = [pltpu.bitcast(v[:8, :128], U32) for v in vals]
        return _tree(jnp.bitwise_or, bits) & zero_ref[:8]

    def vregs(vals, every=1):
        return [v[u:u + 8] for v in vals for u in range(0, v.shape[0], 8)][::-1][::every]

    def after(words, toks):
        if not toks:
            return words
        slabs = []
        for k in range(words.shape[0] // 8):
            slab = words[8 * k:8 * k + 8]
            if toks.get(k) is not None:
                slab = slab | jnp.concatenate([toks[k]] * (words.shape[1] // 128), axis=1)
            slabs.append(slab)
        return jnp.concatenate(slabs, axis=0)

    def store_rhs(dst, m, i, r, b11, b12, b21, b22):
        terms = _rhs_terms(*[_split(b) for b in (b11, b12, b21, b22)])
        words = [{1: b11, 4: b22}[k] if k in (1, 4) else _merge(v) for k, v in enumerate(terms)]
        return vregs([_put(dst, (m, i), r, k, v) for k, v in enumerate(words)])

    def raw_words(m, r, rows, t):
        return pltpu.bitcast(wraw[m, _rows(r, rows), _tile(t)], U32)

    def prep_b(m, i):
        def piece(j, c):
            r = i * KC + 32 * c
            return store_rhs(wb, m, j, r, *[raw_words(3 + m, r + h * (D // 2), 32, j + u * NP)
                                            for h in range(2) for u in range(2)])

        return [lambda j=j, c=c: piece(j, c) for j in range(NP) for c in range(KC // 32)]

    def prep_a_cols(m, i):
        rows = 32
        st = {}

        def rotate(c):
            v = [jnp.concatenate([raw_words(m, i * KC + c * rows + h * (D // 2), rows, t)
                                  for h in range(2)], axis=0) for t in range(NT)]
            st[c] = [x if t == 0 else pltpu.roll(x, 2 * t, 1) for t, x in enumerate(v)]
            return vregs(st[c], 4)

        def shear(c):
            slot = (_iota((rows, 128), 1) >> 1) & 7
            v = [st[c][(-b) % NT] for b in range(NT)]
            for bit in (1, 2, 4):
                sel = (slot & bit) != 0
                v = [jnp.where(sel, v[(b - bit) % NT], v[b]) for b in range(NT)]
            st[c] = [x if b == 0 else pltpu.roll(x, 128 - 2 * b, 1) for b, x in enumerate(v)]
            return vregs(v, 2)

        def terms(c):
            v, half, outs = st[c], rows // 2, []
            for j in range(NP):
                outs += store_rhs(wa[m], 0, j, i * KC + c * rows, v[j][:half], v[j + NP][:half],
                                  v[j][half:], v[j + NP][half:])
            return outs

        order = [(f, k - lag) for k in range(6) for lag, f in enumerate((rotate, shear, terms))
                 if 0 <= k - lag < 4]
        return [lambda f=f, c=c: f(c) for f, c in order]

    def prep_a_rows(i):
        def stage(t):
            words = [pltpu.bitcast(wraw_o[i + h * NP, _tile(t), :], U32) for h in range(2)]
            for h in range(2):
                wtmp[h, pl.ds(65 * t, 64), :] = words[h]
            return vregs(words)

        def rows(h, b, u):
            return jnp.concatenate(
                [wtmp[h, pl.ds(8 * (u + k) + b, 8, stride=65), :] for k in range(2)], axis=0)

        def piece(c, u):
            return store_rhs(wao, 0, i, 128 * c + 16 * u, rows(0, c, u), rows(1, c, u),
                             rows(0, c + NP, u), rows(1, c + NP, u))

        return ([lambda t=t: stage(t) for t in range(NT)]
                + [lambda c=c, u=u: piece(c, u) for c in range(4) for u in range(0, 8, 2)])

    def store_lhs(dst, t, r, a11, a12, a21, a22, pack=_words):
        terms = _lhs_terms(a11, a12, a21, a22)
        return vregs([_put(dst, (t,), r, k, pack(v)) for k, v in enumerate(terms)])

    def join(toks, slot, tok):
        if tok is not None:
            toks[slot] = tok if toks.get(slot) is None else toks[slot] | tok

    due = []

    def products(a_ref, w_ref, m, i, emit, only=None):
        st = {}

        def prod(k, toks, finish):
            toks = dict(toks or {})
            while due and due[0][0] < 16:
                slot, vals = due.pop(0)
                join(toks, slot, token(*vals))
            for entry in due:
                entry[0] -= 16
            if only is None:
                a = jnp.concatenate([after(a_ref[t, :, _tile(k)], toks if t == 0 else None)
                                     for t in range(NP)], axis=1)
                w = w_ref[m, i, :, _tile(k)]
            else:
                a = after(a_ref[only, :, _tile(k)], toks)
                w = w_ref[m, i, _rows(64 * only, 64), _tile(k)]
            r = _dot(_bf(a), _bf(w))
            finish(r)
            return r

        def p1(r):
            st["m1"] = r

        def p2(r):
            st["c21"], st["c22"] = r, st["m1"] - r

        def p3(r):
            st["c12"], st["c22"] = r, st["c22"] + r

        def p4(r):
            st["c11"] = st["m1"] + r
            emit(1, 0, st["c21"] + r)

        def p5(r):
            st["c11"] = st["c11"] - r
            emit(0, 1, st["c12"] + r)

        def p6(r):
            emit(1, 1, st["c22"] + r)

        def p7(r):
            emit(0, 0, st["c11"] + r)

        return [lambda toks, k=k, f=f: prod(k, toks, f)
                for k, f in enumerate((p1, p2, p3, p4, p5, p6, p7))]

    def ln_tasks(n, i, off, nr=16):
        src, dst = X[n % NSEG], XN[n % 2]
        st = {}

        def mean():
            st["x"] = [
                jnp.concatenate(
                    [_split(pltpu.bitcast(src[_rows(i * RC + off + h * HL, nr), _tile(t)], U32))
                     for h in range(2)], axis=0) for t in range(NT)]
            part = _tree(jnp.add, st["x"])
            st["mean"] = jnp.sum(part, axis=1, keepdims=True) * (1.0 / D)
            return vregs([part])

        def var():
            st["x"] = [x - st["mean"] for x in st["x"]]
            part = _tree(jnp.add, [x * x for x in st["x"]])
            st["var"] = jnp.sum(part, axis=1, keepdims=True) * (1.0 / D)
            return vregs([part])

        def scale():
            inv = lax.rsqrt(st["var"] + 1e-5)
            y = [x * inv for x in st["x"]]
            r = i * RC + off
            outs = []
            for t in range(NP):
                outs += store_lhs(dst, t, r, y[t][:nr], y[t + NP][:nr], y[t][nr:], y[t + NP][nr:],
                                  _merge)
            return outs

        return [mean, var, scale]

    def proj_a(n, i, which, only=None):
        p = n % 2

        def emit(h, c, y):
            t = i + c * NP
            buf = (QA, KA, VA)[which]
            rows = pl.ds(h * HL + (HALO if which else 0), HL)
            if only:
                y = y + buf[p][t, rows, :]
            buf[p][t, rows, :] = y
            if which and h == 0 and n % NSEG == 0:
                buf[p][t, pl.ds(0, HALO), :] = jnp.zeros((HALO, 128), F32)
            elif which and h == 0:
                buf[p][t, pl.ds(0, HALO), :] = buf[1 - p][t, pl.ds(L, HALO), :]

        return products(XN[p], wa[which], 0, i, emit, only)

    def proj_b(n, i, which):
        p = n % 2

        def transposed(buf, h, c, y):
            words = pltpu.bitcast(y.astype(BF16).T, U32)
            buf[p][i + c * NP, :, pl.ds(h * HL, HL)] = words
            due.append([T_DUE, vregs([words[:, :128], words[:, 128:]], 2)])

        def emit(h, c, y):
            if which == 0:
                if n % NSEG:
                    _put(PQ[p], (i,), h * HL, c, _words(_phi(y)))
                y = y * QSCALE
                flip = jnp.concatenate([y[r ^ 96:(r ^ 96) + 32] for r in range(0, HL, 32)], axis=0)
                y = jnp.where((_iota(y.shape, 1) & 32) == 0, y, flip)
                transposed(QT, h, c, y)
            elif which == 1:
                _put(KB[p], (i,), h * HL, c, _words(y))
                if n % NSEG != NSEG - 1:
                    y = _phi(y)
                    _put(PK[p], (i,), h * HL, c, _words(y))
                    ZS[p][i + c * NP, pl.ds(8 * h, 8), :] = _tree(jnp.add, vregs([y]))
            else:
                transposed(VT, h, c, y)

        return products(XN[p], wb, which, i, emit)

    def out_stage(n, i):
        x = X[n % NSEG]

        def emit(h, c, y):
            where = (pl.ds(h * HL, HL), _tile(i + c * NP))
            x[where] = (x[where].astype(F32) + y).astype(BF16)

        if is_a(n):
            return products(O[n], wao, 0, i, emit)
        return products(O[n], wb, 3, i, emit)

    def att_a_tasks(n, i, off, times):
        p = n % 2
        base = (i * RC if isinstance(i, int) else pl.multiple_of(i * RC, RC)) + off
        starts = [base + (u // 2) * HL + 8 * (u % 2) for u in range(4)]
        lg, mixed = [[] for _ in range(4)], {}

        def scores(u, ws):
            q = [QA[p][t, pl.ds(starts[u], 8), :] for t in range(NT)]
            for w in ws:
                kr = pl.ds(starts[u] + HALO - DIL * w, 8)
                lg[u].append(_tree(jnp.add, [q[t] * KA[p][t, kr, :] for t in range(NT)]))
            return lg[u][-len(ws):]

        def exchange(u, bit):
            low = (_iota((8, 128), 1) & bit) == 0
            lg[u] = [a + jnp.where(low, pltpu.roll(a, 128 - bit, 1), pltpu.roll(a, bit, 1))
                     for a in lg[u]]
            return lg[u]

        def softmax(u):
            v = [a * QSCALE for a in lg[u]]
            if n % NSEG == 0 and off == 0 and u < 2:
                pos = _iota((8, 128), 0) + starts[u]
                v = [a if w == 0 else jnp.where(pos >= DIL * w, a, MASKVAL)
                     for w, a in enumerate(v)]
            m = _tree(jnp.maximum, v)
            e = [jnp.exp2(a - m) for a in v]
            inv = 1.0 / _tree(jnp.add, e)
            lg[u] = [a * inv for a in e]
            return lg[u]

        def mix(t, h):
            for c in range(2):
                mixed[t, h, c] = jnp.concatenate([
                    _tree(jnp.add, [
                        lg[u][w] * VA[p][t + c * NP, pl.ds(starts[u] + HALO - DIL * w, 8), :]
                        for w in range(WIN)])
                    for u in (2 * h, 2 * h + 1)], axis=0)
            return vregs([mixed[t, h, c] for c in range(2)])

        def store(t):
            return store_lhs(O[n], t, i * RC + off,
                             *[mixed[t, h, c] for h in range(2) for c in range(2)])

        t_score, d_score, lag1, lag2, lag3, t_mix, d_mix, d_store = times
        tasks = []
        for u in range(4):
            t = t_score + d_score * (2 * u + 1)
            tasks += [(t - d_score, lambda u=u: scores(u, range(4))),
                      (t, lambda u=u: scores(u, range(4, 8))),
                      (t + lag1, lambda u=u: exchange(u, 1)),
                      (t + lag2, lambda u=u: exchange(u, 16)),
                      (t + lag3, lambda u=u: softmax(u))]
        for k in range(NP):
            t = t_mix + k * (d_mix + d_store)
            tasks += [(t, lambda k=k: mix(k, 0)), (t + d_mix, lambda k=k: mix(k, 1))]
            tasks += [(t + d_mix + d_store / 2, lambda k=k: store(k))]
        return tasks

    def att_b_piece(n, i, j, mem, tok):
        p = n % 2
        nk = 128 * j + 32
        shared = ((32, 1, 3), (64, 2, 2), (96, 3, 1))
        key, lane = _iota((32, 128), 0), _iota((32, 128), 1)
        causal = [jnp.where(key > q, MASKVAL, 0.0) for q in (lane, lane ^ 96)]
        even = [_iota((8, 128), 1) >= lo for lo, _, _ in shared]

        def place(parts):
            zero = jnp.zeros((16, 128), U32)
            return jnp.concatenate([parts.get(hh, zero) for hh in range(4)], axis=0)

        q = [[after(QT[p][i + h * NP, pl.ds(16 * hh, 16), _tile(j)], {0: tok}) for hh in range(4)]
             for h in range(2)]
        s = []
        for h in range(2):
            w = jnp.concatenate([place({hh: q[h][hh]}) for hh in range(4)], axis=1)
            st = _dot(_bf(KB[p][i, pl.ds(0, nk // 2), _tile(h)]), _bf(w))
            for hh in range(4):
                v = st[:, 128 * hh:128 * (hh + 1)]
                s.append([v[u:u + 8] for u in range(0, nk - 32, 8)]
                         + [v[nk - 32 + u:nk - 24 + u] + causal[hh % 2][u:u + 8]
                            for u in range(0, 32, 8)])
        sx = [[] for _ in range(4)]
        for lo, ce, co in shared:
            ahead = jnp.where(lane >= lo, key + 32 * ce - lane, key + 32 * co - (lane ^ 96))
            mask = jnp.where(ahead > 0, MASKVAL, 0.0)
            high = _iota((16, 128), 1) >= lo
            for h in range(2):
                ke, ko = (KB[p][i, pl.ds(64 * j + 16 * c, 16), _tile(h)] for c in (ce, co))
                k = ke if ce == co else jnp.where((_iota((16, 128), 1) & 32) == 0, ke, ko)
                w = jnp.concatenate(
                    [place({hh: jnp.where(high, q[h][hh], jnp.uint32(0)),
                            hh + 1: jnp.where(high, jnp.uint32(0), q[h][hh + 1])})
                     for hh in (0, 2)], axis=1)
                st = _dot(_bf(k), _bf(w))
                for u in range(2):
                    v = st[:, 128 * u:128 * (u + 1)] + mask
                    sx[2 * h + u].append([v[r:r + 8] for r in range(0, 32, 8)])
        first = token(*[v[0] for v in s])
        m = []
        for u in range(4):
            a = [_tree(jnp.maximum, s[2 * u + odd]) for odd in range(2)]
            for sel, v in zip(even, sx[u]):
                mx = _tree(jnp.maximum, v)
                a = [jnp.where(sel, jnp.maximum(a[0], mx), a[0]),
                     jnp.where(sel, a[1], jnp.maximum(a[1], mx))]
            m += [jnp.broadcast_to(jnp.max(v, axis=0, keepdims=True), (8, 128)) for v in a]
        e = [[] for _ in range(8)]
        part = [[] for _ in range(8)]

        def exps(v, mh, tok):
            mh = mh if tok is None else mh + pltpu.bitcast(tok, F32)
            return [jnp.exp2(a - mh) for a in v]

        def collect(u, v):
            part[u] = [_tree(jnp.add, part[u] + v)]
            e[u].extend(v)

        def exp_tile(u, c, tok):
            collect(u, exps(s[u][16 * c:16 * (c + 1)], m[u], tok))

        def exp_diag(u, tok):
            for odd in range(2):
                exp_tile(2 * u + odd, j, tok)
            v = [exps(a, jnp.where(sel, m[2 * u], m[2 * u + 1]), tok) for sel, a in zip(even, sx[u])]
            collect(2 * u, [jnp.where(even[c], a, 0.0) for c in (0, 1, 2) for a in v[c]])
            collect(2 * u + 1, [jnp.where(even[c], 0.0, a) for c in (2, 1, 0) for a in v[c]])

        def finish(h, tok):
            g = i + h * NP
            ot = []
            for hh in range(4):
                u = 4 * h + hh
                vt = after(VT[p][g, pl.ds(16 * hh, 16), pl.ds(0, 128 * (j + 1))], {0: tok})
                acc = _dot(_bf(vt), jnp.concatenate(e[u], axis=0).astype(BF16))
                l = jnp.sum(part[u][0], axis=0, keepdims=True)
                gate = gtab[pl.ds(4 * g + hh, 1), :]
                acc = acc * ((1.0 - gate) / l)
                if hh % 2:
                    acc = jnp.where((lane & 32) == 0, pltpu.roll(acc, 32, 1), pltpu.roll(acc, 96, 1))
                if n % NSEG:
                    r = mem[h][:, 128 * j:128 * (j + 1)]
                    den = r[128 + 4 * hh:129 + 4 * hh] + 1e-6
                    acc = acc + r[32 * hh:32 * hh + 32] * (gate / den)
                ot.append(acc)
            return ot

        tasks = []
        for u in range(4):
            tasks += [lambda tok, u=2 * u + odd, c=c: exp_tile(u, c, tok)
                      for odd in range(2) for c in range(j)]
            tasks.append(lambda tok, u=u: exp_diag(u, tok))
        return first, tasks, finish

    def mem_load(n, g):
        if n % NSEG == 0:
            return jnp.zeros((MZ_ROWS, 128), F32)
        return mz[g]

    def mem_read(n, i, h, state, tok):
        pq = after(PQ[n % 2][i, :, _tile(h)], {8 * u: tok for u in range(4)})
        return _dot_nt(state.astype(BF16), _bf(pq))

    def mem_update(n, i, h, state, tok):
        p, g = n % 2, i + h * NP
        z = jnp.sum(ZS[p][g], axis=0, keepdims=True)
        new = jnp.concatenate([_dot(_bf(after(VT[p][g], {0: tok})), _bf(PK[p][i, :, _tile(h)])),
                               jnp.broadcast_to(z, (MZ_ROWS - 128, 128))], axis=0)
        row = _iota((MZ_ROWS, 128), 0)
        row_head = jnp.where(row < 128, row >> 5, (row - 128) >> 2)
        keep = row_head == (_iota((MZ_ROWS, 128), 1) >> 5)
        mz[g] = new = state + jnp.where(keep, new, 0.0)
        return new

    def is_a(n):
        return (n // NSEG) % 2 == 0

    def run_timed(mm, tasks):
        tasks = sorted(tasks, key=lambda x: x[0])
        for k, prod in enumerate(mm):
            toks = {}
            while tasks and tasks[0][0] < 16 * (k + 1):
                time, f = tasks.pop(0)
                join(toks, time - 16 * k, token(*f()))
            prod(toks)
        for _, f in tasks:
            f()

    def body_b(n, its, mm, ln):
        *share, front, lag, tail, pitch = {
            28: (*B_SHARE, B_FRONT, B_WAIT, *B_TAIL), 21: B_LAST, 14: B_LAST2}[len(mm) // len(its)]
        spare = len(mm) // len(its) - sum(share)
        late, done = [], []
        tok, pending = token(mm.pop(0)(None)), None

        def finisher(i, j, finish, tiles):
            def run(tok):
                posts = []
                for h in range(2):
                    ot = finish(h, tok)

                    def post(ot=ot, h=h):
                        tiles[j, h] = jnp.concatenate(ot, axis=0).T
                        return vregs([tiles[j, h]], 4)

                    posts.append(post)
                if (j ^ 2, 0) in tiles:
                    posts += [lambda r=r: store_lhs(
                        O[n], i, 128 * (j % 2) + r,
                        *[tiles[j % 2 + u, h][r:r + B_STORE] for u in (0, 2) for h in range(2)])
                        for r in range(0, 128, B_STORE)]
                tiles[j, 0] = None
                return posts

            return run

        for i in its:
            state = [mem_load(n, i + h * NP) for h in range(2)]
            mem, tiles = [], {}
            if ln:
                for off in range(0, RC, 16):
                    late += ln_tasks(n + 2, i, off)
            for k, j in enumerate(B_ORDER):
                first, exps, finish = att_b_piece(n, i, j, mem, tok)
                done += pending(first) if pending else []
                cnt = share[k] + (0 if i is its[-1] else (spare + 3 - k) // 4)
                when = [int(32 * cnt * front * u / len(exps)) for u in range(len(exps))]
                for c in range(cnt):
                    toks = {}
                    if c == 0:
                        join(toks, 0, first)
                    for slot in B_POST:
                        if done and 16 * c + slot >= min(lag, 16 * cnt - 1):
                            join(toks, slot, token(*done.pop(0)()))
                    if late and c >= B_LN[0]:
                        join(toks, B_LN[1], token(*late.pop(0)()))
                    r = mm.pop(0)(toks)
                    while exps and when[0] < 32 * (c + 1):
                        exps.pop(0)(token(r[8 * (when.pop(0) - 32 * c):]))
                    tok = token(r)
                    if k == 0 and c == B_READ and n % NSEG:
                        mem.extend(mem_read(n, i, h, state[h], tok) for h in range(2))
                        done.append(lambda mem=mem: [v[:, 128 * u:] for v in mem for u in range(4)])
                    if k == B_UPDATE and c == 0 and n % NSEG != NSEG - 1:
                        new = [mem_update(n, i, h, state[h], tok) for h in range(2)]
                        done.append(lambda new=new: new)
                pending = finisher(i, j, finish, tiles)
        tok = token(mm.pop(0)(None))
        done += late + pending(tok)
        run_timed(mm, [(tail + pitch * u, f) for u, f in enumerate(done)])

    def step(n, ln=True, proj=(0, 1, 2), att=True, out=(1,), extra=None, unroll=UNROLL):
        def body(its):
            mm = []
            due.clear()
            for i in its:
                for which in (B_MATS if att and not is_a(n) else A_MATS):
                    if which in proj:
                        mm += (proj_a if is_a(n + 1) else proj_b)(n + 1, i, which)
                    elif which == 3:
                        for lag in out:
                            mm += out_stage(n - lag, i)
            if att and not is_a(n):
                body_b(n, its, mm, ln)
                return
            times = A_FIRST if n == 0 else A_PLAIN if is_a(n + 1) else A_THEN_B
            tasks, span = [], 16 * len(mm) / (4 * len(its))
            for k, i in enumerate(its):
                if extra is not None:
                    fs = extra(i)
                    tasks += [(int(span * (4 * k + u // 8 + A_PREP_WHEN[u % 8])) if att else
                               int(4 * span * (k + (u + 1) / len(fs))) - 1, f)
                              for u, f in enumerate(fs)]
                for u, off in enumerate(range(0, RC, 16), 4 * k):
                    if att:
                        tasks += [(int(span * (u + w)), f) for w, f in att_a_tasks(n, i, off, times[:8])]
                    if ln:
                        when = times[8:] if att else (.3, .8, 1.3)
                        tasks += [(int(span * (u + w)), f)
                                  for w, f in zip(when, ln_tasks(n + 2, i, off))]
            run_timed(mm, tasks)

        if unroll == NP:
            body(list(range(NP)))
        else:
            pl.loop(0, NP // unroll)(lambda i: body([unroll * i + u for u in range(unroll)]))

    for i in range(NP):
        start(x0_copies(i))
    start(slab_copies(0, 0))
    start([copy(beta_hbm, beta_ref.at[0], sem_b)])
    zero_ref[:8] = jnp.zeros((8, 128), U32)

    @pl.loop(0, NP)
    def _(i):
        pl.when(i % 2 == 1)(lambda: start(slab_copies(0, (i + 1) // 2)))
        wait(x0_copies(i))
        for fs in zip(*[ln_tasks(0, i, off) for off in range(0, RC, 16)]):
            for f in fs:
                f()

    start(slab_copies(0, 3))
    wait(slab_copies(0, 0))
    for f in prep_a_cols(0, 0):
        f()

    plan = (([(1, 0)], [(0, 1)]), ([(1, 1), (1, 2)], [(0, 2), (0, 3)]),
            ([(1, 3), (2, 0)], [(1, 0), (1, 1)]), ([(2, 1), (2, 2)], [(1, 2), (1, 3)]))
    for t, (fetch, preps) in enumerate(plan):
        for mi in fetch:
            start(slab_copies(*mi))
        for mi in preps:
            wait(slab_copies(*mi))
        mm = [f for i in range(NP) for f in proj_a(0, i, 0, only=t)]
        fs = [f for group in zip(*[prep_a_cols(*mi) for mi in preps]) for f in group]
        run_timed(mm, [(16 * len(mm) * (u + 1) // (len(fs) + 1), f) for u, f in enumerate(fs)])

    def prep_wv(i):
        pl.when(i == 0)(lambda: start(x_copies(1) + wao_copies()))
        wait(slab_copies(2, i))
        return prep_a_cols(2, i)

    start(slab_copies(2, 3))
    step(-1, ln=False, proj=(1,), att=False, out=(), extra=prep_wv, unroll=1)
    start(x_copies(2))
    start(x_copies(3))
    wait(x_copies(1))
    wait(wao_copies())
    step(-1, proj=(2,), att=False, out=(), extra=prep_a_rows)
    for m in range(4):
        start(wb_copies(m))
    wait([copy(beta_hbm, beta_ref.at[0], sem_b)])
    gate = jax.nn.sigmoid(beta_ref[0].astype(F32))
    eye = _iota((H, H), 0) == _iota((H, H), 1)
    gcol = jnp.sum(jnp.where(eye, jnp.broadcast_to(gate, (H, H)), 0.0), axis=1, keepdims=True)
    gtab[...] = jnp.broadcast_to(gcol, (H, 128))
    wait(x_copies(2))
    step(0, out=())
    wait(x_copies(3))
    for m in range(4):
        wait(wb_copies(m))
    step(1, extra=lambda i: prep_b(0, i) + prep_b(1, i))
    step(2, extra=lambda i: prep_b(2, i) + prep_b(3, i))
    for n in range(3, 14):
        step(n)
    start(out_copies(0))
    step(14, ln=False, out=())
    step(15, ln=False, proj=(), out=(2, 1))
    start(out_copies(1))
    start(out_copies(2))
    due.clear()
    for i in range(NP):
        run_timed(out_stage(LAST, i), [])
        if i >= NP - 2:
            start(out_tile_copies(0, NP - 1) if i == NP - 2 else out_tile_copies(i, 1))
    for s in range(NSEG - 1):
        wait(out_copies(s))
    wait(out_tile_copies(0, NP - 1) + out_tile_copies(NP - 1, 1))


@jax.jit
def pallas_interleave_layers__sliding_local_dilated__memory_aug_infini_attn__prompt_kernel(
    A_x: jax.Array,
    A_wqkv: jax.Array,
    A_wo: jax.Array,
    B_x: jax.Array,
    B_wq: jax.Array,
    B_wk: jax.Array,
    B_wv: jax.Array,
    B_wo: jax.Array,
    B_beta: jax.Array,
):
    del B_x
    assert A_x.shape == (1, S, D)
    hbm = pl.BlockSpec(memory_space=pl.ANY)
    scratch = (
        [pltpu.VMEM((L, D), BF16)] * 4
        + [pltpu.VMEM((7, D, D), BF16), pltpu.VMEM((NT, D, 128), BF16),
           pltpu.VMEM((2, 576, 128), U32),
           *[pltpu.VMEM((1, NP, D // 4, 7 * 128), U32)] * 4,
           pltpu.VMEM((4, NP, D // 4, 7 * 128), U32)]
        + [pltpu.VMEM((NP, HL // 2, 7 * 128), U32)] * 5
        + [pltpu.VMEM((NT, L, 128), F32)] * 2
        + [pltpu.VMEM((NT, HALO + L, 128), F32)] * 4
        + [pltpu.VMEM((NP, L // 2, 2 * 128), U32)] * 6
        + [pltpu.VMEM((NT, 64, L), U32)] * 4
        + [pltpu.VMEM((NT, 16, 128), F32)] * 2
        + [pltpu.VMEM((NT, MZ_ROWS, 128), F32), pltpu.VMEM((8, 1, H), BF16),
           pltpu.VMEM((H, 128), F32),
           pltpu.VMEM((88, 128), U32),
           pltpu.SemaphoreType.DMA((NSEG,)), pltpu.SemaphoreType.DMA((5,)),
           pltpu.SemaphoreType.DMA((4, NP)),
           pltpu.SemaphoreType.DMA((NSEG,)), pltpu.SemaphoreType.DMA]
    )
    out = pl.pallas_call(
        _kernel,
        out_shape=jax.ShapeDtypeStruct((S, D), BF16),
        in_specs=[hbm] * 8,
        out_specs=hbm,
        scratch_shapes=scratch,
        compiler_params=pltpu.CompilerParams(vmem_limit_bytes=110 * 2**20),
        name="abab_stack",
    )(A_x.reshape(S, D), A_wqkv, A_wo, B_wq, B_wk, B_wv, B_wo, B_beta.reshape(1, H))
    return out.reshape(1, S, D)
```

```python
import jax
import jax.numpy as jnp
from jax import lax
import jax.experimental.pallas as pl
import jax.experimental.pallas.tpu as pltpu

S, D, H, DH = 2048, 1024, 32, 32
NSEG, L = 4, 512
HL = L // 2
NT = D // 128
NP = NT // 2
RC = HL // NP
KC = D // 2 // NP
LAST = 4 * NSEG - 1
WIN, DIL = 8, 2
HALO = 16
MZ_ROWS = 128 + 16
LOG2E = 1.4426950408889634
QSCALE = float(DH ** -0.5 * LOG2E)
MASKVAL = float(-1e9 * LOG2E)

A_MATS = (3, 0, 2, 1)
B_MATS = (2, 0, 1, 3)
B_SHARE = (6, 7, 6, 2)
B_FRONT = 0.729
B_WAIT = 28
B_TAIL = (44, 3)
B_LAST = (3, 2, 7, 3, 0.882, 30, 32, 1)
B_LAST2 = (4, 3, 2, 1, 0.845, 29, 28, 6)
B_POST = (6, 14)
B_LN = (4, 11)
B_STORE = 64
T_DUE = 36
A_PLAIN = (0.051, 0.047, 0.07, 0.179, 0.286, 0.632, 0.042, 0.039, 0.027, 0.3, 0.45, 0.512, 0.542, 0.57)
A_FIRST = (0.051, 0.036, 0.107, 0.22, 0.277, 0.607, 0.039, 0.047, 0.024, 0.316, 0.465, 0.5, 0.55, 0.56)
A_THEN_B = (0.055, 0.035, 0.07, 0.18, 0.27, 0.621, 0.031, 0.087, 0.062, 0.297, 0.432, 0.49, 0.53, 0.57)
A_PREP_WHEN = (0.313, 0.297, 0.373, 0.395, 0.353, 0.5, 0.556, 0.582)

F32, BF16, U32 = jnp.float32, jnp.bfloat16, jnp.uint32
_NT_DIMS = (((1,), (1,)), ((), ()))


def _iota(shape, axis):
    return lax.broadcasted_iota(jnp.int32, shape, axis)


def _dot(a, b):
    return jnp.dot(a, b, preferred_element_type=F32)


def _dot_nt(a, b):
    return lax.dot_general(a, b, _NT_DIMS, preferred_element_type=F32)


def _rows(start, size):
    return pl.ds(start if isinstance(start, int) else pl.multiple_of(start, size), size)


def _tile(k):
    return _rows(128 * k, 128)


def _words(val):
    return pltpu.bitcast(val.astype(BF16), U32)


def _put(ref, idx, start, k, words):
    ref[(*idx, _rows(start // 2, words.shape[0]), _tile(k))] = words
    return words


def _bf(words):
    return pltpu.bitcast(words, BF16)


def _phi(t):
    return jnp.where(t > 0, t + 1.0, jnp.exp(t))


def _tree(op, xs):
    xs = list(xs)
    while len(xs) > 1:
        xs = [op(xs[i], xs[i + 1]) if i + 1 < len(xs) else xs[i]
              for i in range(0, len(xs), 2)]
    return xs[0]


def _lhs_terms(a11, a12, a21, a22):
    return (a11 + a22, a21 + a22, a11, a22, a11 + a12, a21 - a11, a12 - a22)


def _rhs_terms(b11, b12, b21, b22):
    return (b11 + b22, b11, b12 - b22, b21 - b11, b22, b11 + b12, b21 + b22)


def _kernel(x_hbm, wqkv_hbm, awo_hbm, wq_hbm, wk_hbm, wv_hbm, wo_hbm, beta_hbm,
            out_hbm,
            x0, x1, x2, x3, wraw, wraw_o, wtmp, waq, wak, wav, wao, wb,
            xn0, xn1, o0, o1, o2,
            qa0, qa1, ka0, ka1, va0, va1,
            pq0, pq1, kb0, kb1, pk0, pk1, qt0, qt1, vt0, vt1,
            zs0, zs1, mz, beta_ref, gtab, zero_ref, sem_x, sem_w, sem_s, sem_o, sem_b):
    X = (x0, x1, x2, x3)
    XN, wa = (xn0, xn1), (waq, wak, wav)
    O = [o2 if n == LAST else (o0, o1)[n % 2] for n in range(LAST + 1)]
    QA, KA, VA = (qa0, qa1), (ka0, ka1), (va0, va1)
    QT, PQ, KB, PK, VT = (qt0, qt1), (pq0, pq1), (kb0, kb1), (pk0, pk1), (vt0, vt1)
    ZS = (zs0, zs1)

    copy = pltpu.make_async_copy

    def x_copies(s):
        return [copy(x_hbm.at[pl.ds(s * L, L)], X[s], sem_x.at[s])]

    def out_copies(s):
        return [copy(X[s], out_hbm.at[pl.ds(s * L, L)], sem_o.at[s])]

    def out_tile_copies(t0, nt):
        cols = [pl.ds(128 * (t0 + c * NP), 128 * nt) for c in range(2)]
        return [copy(x3.at[:, c], out_hbm.at[pl.ds(S - L, L), c], sem_o.at[NSEG - 1]) for c in cols]

    def wao_copies():
        return [copy(awo_hbm.at[:, _tile(t)], wraw_o.at[t], sem_w.at[4]) for t in range(NT)]

    def wb_copies(m):
        return [copy((wq_hbm, wk_hbm, wv_hbm, wo_hbm)[m], wraw.at[3 + m], sem_w.at[m])]

    def slab_copies(m, i):
        return [copy(wqkv_hbm.at[r, _rows(m * D, D)], wraw.at[m, r], sem_s.at[m, i])
                for r in (_rows(h * (D // 2) + i * KC, KC) for h in range(2))]

    def x0_copies(i):
        return [copy(x_hbm.at[r], x0.at[r], sem_s.at[3, i])
                for r in (_rows(h * HL + i * RC, RC) for h in range(2))]

    def start(cs):
        for c in cs:
            c.start()

    def wait(cs):
        for c in cs:
            c.wait()

    def token(*vals):
        bits = [pltpu.bitcast(v[:8, :128], U32) for v in vals]
        return _tree(jnp.bitwise_or, bits) & zero_ref[:8]

    def vregs(vals, every=1):
        return [v[u:u + 8] for v in vals for u in range(0, v.shape[0], 8)][::-1][::every]

    def after(words, toks):
        if not toks:
            return words
        slabs = []
        for k in range(words.shape[0] // 8):
            slab = words[8 * k:8 * k + 8]
            if toks.get(k) is not None:
                slab = slab | jnp.concatenate([toks[k]] * (words.shape[1] // 128), axis=1)
            slabs.append(slab)
        return jnp.concatenate(slabs, axis=0)

    def store_rhs(dst, m, i, r, b11, b12, b21, b22):
        terms = _rhs_terms(*[_bf(b).astype(F32) for b in (b11, b12, b21, b22)])
        words = [{1: b11, 4: b22}[k] if k in (1, 4) else _words(v) for k, v in enumerate(terms)]
        return vregs([_put(dst, (m, i), r, k, v) for k, v in enumerate(words)])

    def raw_words(m, r, rows, t):
        return pltpu.bitcast(wraw[m, _rows(r, rows), _tile(t)], U32)

    def prep_b(m, i):
        def piece(j, c):
            r = i * KC + 32 * c
            return store_rhs(wb, m, j, r, *[raw_words(3 + m, r + h * (D // 2), 32, j + u * NP)
                                            for h in range(2) for u in range(2)])

        return [lambda j=j, c=c: piece(j, c) for j in range(NP) for c in range(KC // 32)]

    def prep_a_cols(m, i):
        rows = 32
        st = {}

        def rotate(c):
            v = [jnp.concatenate([raw_words(m, i * KC + c * rows + h * (D // 2), rows, t)
                                  for h in range(2)], axis=0) for t in range(NT)]
            st[c] = [x if t == 0 else pltpu.roll(x, 2 * t, 1) for t, x in enumerate(v)]
            return vregs(st[c], 4)

        def shear(c):
            slot = (_iota((rows, 128), 1) >> 1) & 7
            v = [st[c][(-b) % NT] for b in range(NT)]
            for bit in (1, 2, 4):
                sel = (slot & bit) != 0
                v = [jnp.where(sel, v[(b - bit) % NT], v[b]) for b in range(NT)]
            st[c] = [x if b == 0 else pltpu.roll(x, 128 - 2 * b, 1) for b, x in enumerate(v)]
            return vregs(v, 2)

        def terms(c):
            v, half, outs = st[c], rows // 2, []
            for j in range(NP):
                outs += store_rhs(wa[m], 0, j, i * KC + c * rows, v[j][:half], v[j + NP][:half],
                                  v[j][half:], v[j + NP][half:])
            return outs

        order = [(f, k - lag) for k in range(6) for lag, f in enumerate((rotate, shear, terms))
                 if 0 <= k - lag < 4]
        return [lambda f=f, c=c: f(c) for f, c in order]

    def prep_a_rows(i):
        def stage(t):
            words = [pltpu.bitcast(wraw_o[i + h * NP, _tile(t), :], U32) for h in range(2)]
            for h in range(2):
                wtmp[h, pl.ds(65 * t, 64), :] = words[h]
            return vregs(words)

        def rows(h, b, u):
            return jnp.concatenate(
                [wtmp[h, pl.ds(8 * (u + k) + b, 8, stride=65), :] for k in range(2)], axis=0)

        def piece(c, u):
            return store_rhs(wao, 0, i, 128 * c + 16 * u, rows(0, c, u), rows(1, c, u),
                             rows(0, c + NP, u), rows(1, c + NP, u))

        return ([lambda t=t: stage(t) for t in range(NT)]
                + [lambda c=c, u=u: piece(c, u) for c in range(4) for u in range(0, 8, 2)])

    def store_lhs(dst, t, r, a11, a12, a21, a22):
        terms = _lhs_terms(a11, a12, a21, a22)
        return vregs([_put(dst, (t,), r, k, _words(v)) for k, v in enumerate(terms)])

    def join(toks, slot, tok):
        if tok is not None:
            toks[slot] = tok if toks.get(slot) is None else toks[slot] | tok

    due = []

    def products(a_ref, w_ref, m, i, emit, only=None):
        st = {}

        def prod(k, toks, finish):
            toks = dict(toks or {})
            while due and due[0][0] < 16:
                slot, vals = due.pop(0)
                join(toks, slot, token(*vals))
            for entry in due:
                entry[0] -= 16
            if only is None:
                a = jnp.concatenate([after(a_ref[t, :, _tile(k)], toks if t == 0 else None)
                                     for t in range(NP)], axis=1)
                w = w_ref[m, i, :, _tile(k)]
            else:
                a = after(a_ref[only, :, _tile(k)], toks)
                w = w_ref[m, i, _rows(64 * only, 64), _tile(k)]
            r = _dot(_bf(a), _bf(w))
            finish(r)
            return r

        def p1(r):
            st["m1"] = r

        def p2(r):
            st["c21"], st["c22"] = r, st["m1"] - r

        def p3(r):
            st["c12"], st["c22"] = r, st["c22"] + r

        def p4(r):
            st["c11"] = st["m1"] + r
            emit(1, 0, st["c21"] + r)

        def p5(r):
            st["c11"] = st["c11"] - r
            emit(0, 1, st["c12"] + r)

        def p6(r):
            emit(1, 1, st["c22"] + r)

        def p7(r):
            emit(0, 0, st["c11"] + r)

        return [lambda toks, k=k, f=f: prod(k, toks, f)
                for k, f in enumerate((p1, p2, p3, p4, p5, p6, p7))]

    def ln_tasks(n, i, off, nr=16):
        src, dst = X[n % NSEG], XN[n % 2]
        st = {}

        def mean():
            st["x"] = [
                jnp.concatenate(
                    [src[_rows(i * RC + off + h * HL, nr), _tile(t)].astype(F32)
                     for h in range(2)], axis=0) for t in range(NT)]
            part = _tree(jnp.add, st["x"])
            st["mean"] = jnp.sum(part, axis=1, keepdims=True) * (1.0 / D)
            return vregs([part])

        def var():
            st["x"] = [x - st["mean"] for x in st["x"]]
            part = _tree(jnp.add, [x * x for x in st["x"]])
            st["var"] = jnp.sum(part, axis=1, keepdims=True) * (1.0 / D)
            return vregs([part])

        def scale(t):
            if t == 0:
                st["inv"] = lax.rsqrt(st["var"] + 1e-5)
            y0, y1 = st["x"][t] * st["inv"], st["x"][t + NP] * st["inv"]
            return store_lhs(dst, t, i * RC + off, y0[:nr], y1[:nr], y0[nr:], y1[nr:])

        return [mean, var] + [lambda t=t: scale(t) for t in range(NP)]

    def proj_a(n, i, which, only=None):
        p = n % 2

        def emit(h, c, y):
            t = i + c * NP
            buf = (QA, KA, VA)[which]
            rows = pl.ds(h * HL + (HALO if which else 0), HL)
            if only:
                y = y + buf[p][t, rows, :]
            buf[p][t, rows, :] = y
            if which and h == 0 and n % NSEG == 0:
                buf[p][t, pl.ds(0, HALO), :] = jnp.zeros((HALO, 128), F32)
            elif which and h == 0:
                buf[p][t, pl.ds(0, HALO), :] = buf[1 - p][t, pl.ds(L, HALO), :]

        return products(XN[p], wa[which], 0, i, emit, only)

    def proj_b(n, i, which):
        p = n % 2

        def transposed(buf, h, c, y):
            words = pltpu.bitcast(y.astype(BF16).T, U32)
            buf[p][i + c * NP, :, pl.ds(h * HL, HL)] = words
            due.append([T_DUE, vregs([words[:, :128], words[:, 128:]], 2)])

        def emit(h, c, y):
            if which == 0:
                if n % NSEG:
                    _put(PQ[p], (i,), h * HL, c, _words(_phi(y)))
                y = y * QSCALE
                flip = jnp.concatenate([y[r ^ 96:(r ^ 96) + 32] for r in range(0, HL, 32)], axis=0)
                y = jnp.where((_iota(y.shape, 1) & 32) == 0, y, flip)
                transposed(QT, h, c, y)
            elif which == 1:
                _put(KB[p], (i,), h * HL, c, _words(y))
                if n % NSEG != NSEG - 1:
                    y = _phi(y)
                    _put(PK[p], (i,), h * HL, c, _words(y))
                    ZS[p][i + c * NP, pl.ds(8 * h, 8), :] = _tree(jnp.add, vregs([y]))
            else:
                transposed(VT, h, c, y)

        return products(XN[p], wb, which, i, emit)

    def out_stage(n, i):
        x = X[n % NSEG]

        def emit(h, c, y):
            where = (pl.ds(h * HL, HL), _tile(i + c * NP))
            x[where] = (x[where].astype(F32) + y).astype(BF16)

        if is_a(n):
            return products(O[n], wao, 0, i, emit)
        return products(O[n], wb, 3, i, emit)

    def att_a_tasks(n, i, off, times):
        p = n % 2
        base = pl.multiple_of(i * RC, RC) + off
        starts = [base + (u // 2) * HL + 8 * (u % 2) for u in range(4)]
        lg, mixed = [[] for _ in range(4)], {}

        def scores(u, ws):
            q = [QA[p][t, pl.ds(starts[u], 8), :] for t in range(NT)]
            for w in ws:
                kr = pl.ds(starts[u] + HALO - DIL * w, 8)
                lg[u].append(_tree(jnp.add, [q[t] * KA[p][t, kr, :] for t in range(NT)]))
            return lg[u][-len(ws):]

        def exchange(u, bit):
            low = (_iota((8, 128), 1) & bit) == 0
            lg[u] = [a + jnp.where(low, pltpu.roll(a, 128 - bit, 1), pltpu.roll(a, bit, 1))
                     for a in lg[u]]
            return lg[u]

        def softmax(u):
            v = [a * QSCALE for a in lg[u]]
            if n % NSEG == 0 and off == 0 and u < 2:
                pos = _iota((8, 128), 0) + starts[u]
                v = [a if w == 0 else jnp.where(pos >= DIL * w, a, MASKVAL)
                     for w, a in enumerate(v)]
            m = _tree(jnp.maximum, v)
            e = [jnp.exp2(a - m) for a in v]
            inv = 1.0 / _tree(jnp.add, e)
            lg[u] = [a * inv for a in e]
            return lg[u]

        def mix(t, h):
            for c in range(2):
                mixed[t, h, c] = jnp.concatenate([
                    _tree(jnp.add, [
                        lg[u][w] * VA[p][t + c * NP, pl.ds(starts[u] + HALO - DIL * w, 8), :]
                        for w in range(WIN)])
                    for u in (2 * h, 2 * h + 1)], axis=0)
            return vregs([mixed[t, h, c] for c in range(2)])

        def store(t):
            return store_lhs(O[n], t, i * RC + off,
                             *[mixed[t, h, c] for h in range(2) for c in range(2)])

        t_score, d_score, lag1, lag2, lag3, t_mix, d_mix, d_store = times
        tasks = []
        for u in range(4):
            t = t_score + d_score * (2 * u + 1)
            tasks += [(t - d_score, lambda u=u: scores(u, range(4))),
                      (t, lambda u=u: scores(u, range(4, 8))),
                      (t + lag1, lambda u=u: exchange(u, 1)),
                      (t + lag2, lambda u=u: exchange(u, 16)),
                      (t + lag3, lambda u=u: softmax(u))]
        for k in range(NP):
            t = t_mix + k * (d_mix + d_store)
            tasks += [(t, lambda k=k: mix(k, 0)), (t + d_mix, lambda k=k: mix(k, 1))]
            tasks += [(t + d_mix + d_store / 2, lambda k=k: store(k))]
        return tasks

    def att_b_piece(n, i, j, mem, tok):
        p = n % 2
        nk = 128 * j + 32
        shared = ((32, 1, 3), (64, 2, 2), (96, 3, 1))
        key, lane = _iota((32, 128), 0), _iota((32, 128), 1)
        causal = [jnp.where(key > q, MASKVAL, 0.0) for q in (lane, lane ^ 96)]
        even = [_iota((8, 128), 1) >= lo for lo, _, _ in shared]

        def place(parts):
            zero = jnp.zeros((16, 128), U32)
            return jnp.concatenate([parts.get(hh, zero) for hh in range(4)], axis=0)

        q = [[after(QT[p][i + h * NP, pl.ds(16 * hh, 16), _tile(j)], {0: tok}) for hh in range(4)]
             for h in range(2)]
        s = []
        for h in range(2):
            w = jnp.concatenate([place({hh: q[h][hh]}) for hh in range(4)], axis=1)
            st = _dot(_bf(KB[p][i, pl.ds(0, nk // 2), _tile(h)]), _bf(w))
            for hh in range(4):
                v = st[:, 128 * hh:128 * (hh + 1)]
                s.append([v[u:u + 8] for u in range(0, nk - 32, 8)]
                         + [v[nk - 32 + u:nk - 24 + u] + causal[hh % 2][u:u + 8]
                            for u in range(0, 32, 8)])
        sx = [[] for _ in range(4)]
        for lo, ce, co in shared:
            ahead = jnp.where(lane >= lo, key + 32 * ce - lane, key + 32 * co - (lane ^ 96))
            mask = jnp.where(ahead > 0, MASKVAL, 0.0)
            high = _iota((16, 128), 1) >= lo
            for h in range(2):
                ke, ko = (KB[p][i, pl.ds(64 * j + 16 * c, 16), _tile(h)] for c in (ce, co))
                k = ke if ce == co else jnp.where((_iota((16, 128), 1) & 32) == 0, ke, ko)
                w = jnp.concatenate(
                    [place({hh: jnp.where(high, q[h][hh], jnp.uint32(0)),
                            hh + 1: jnp.where(high, jnp.uint32(0), q[h][hh + 1])})
                     for hh in (0, 2)], axis=1)
                st = _dot(_bf(k), _bf(w))
                for u in range(2):
                    v = st[:, 128 * u:128 * (u + 1)] + mask
                    sx[2 * h + u].append([v[r:r + 8] for r in range(0, 32, 8)])
        first = token(*[v[0] for v in s])
        m = []
        for u in range(4):
            a = [_tree(jnp.maximum, s[2 * u + odd]) for odd in range(2)]
            for sel, v in zip(even, sx[u]):
                mx = _tree(jnp.maximum, v)
                a = [jnp.where(sel, jnp.maximum(a[0], mx), a[0]),
                     jnp.where(sel, a[1], jnp.maximum(a[1], mx))]
            m += [jnp.broadcast_to(jnp.max(v, axis=0, keepdims=True), (8, 128)) for v in a]
        e = [[] for _ in range(8)]
        part = [[] for _ in range(8)]

        def exps(v, mh, tok):
            mh = mh if tok is None else mh + pltpu.bitcast(tok, F32)
            return [jnp.exp2(a - mh) for a in v]

        def collect(u, v):
            part[u] = [_tree(jnp.add, part[u] + v)]
            e[u].extend(v)

        def exp_tile(u, c, tok):
            collect(u, exps(s[u][16 * c:16 * (c + 1)], m[u], tok))

        def exp_diag(u, tok):
            for odd in range(2):
                exp_tile(2 * u + odd, j, tok)
            v = [exps(a, jnp.where(sel, m[2 * u], m[2 * u + 1]), tok) for sel, a in zip(even, sx[u])]
            collect(2 * u, [jnp.where(even[c], a, 0.0) for c in (0, 1, 2) for a in v[c]])
            collect(2 * u + 1, [jnp.where(even[c], 0.0, a) for c in (2, 1, 0) for a in v[c]])

        def finish(h, tok):
            g = i + h * NP
            ot = []
            for hh in range(4):
                u = 4 * h + hh
                vt = after(VT[p][g, pl.ds(16 * hh, 16), pl.ds(0, 128 * (j + 1))], {0: tok})
                acc = _dot(_bf(vt), jnp.concatenate(e[u], axis=0).astype(BF16))
                l = jnp.sum(part[u][0], axis=0, keepdims=True)
                gate = gtab[pl.ds(4 * g + hh, 1), :]
                acc = acc * ((1.0 - gate) / l)
                if hh % 2:
                    acc = jnp.where((lane & 32) == 0, pltpu.roll(acc, 32, 1), pltpu.roll(acc, 96, 1))
                if n % NSEG:
                    r = mem[h][:, 128 * j:128 * (j + 1)]
                    den = r[128 + 4 * hh:129 + 4 * hh] + 1e-6
                    acc = acc + r[32 * hh:32 * hh + 32] * (gate / den)
                ot.append(acc)
            return ot

        tasks = []
        for u in range(4):
            tasks += [lambda tok, u=2 * u + odd, c=c: exp_tile(u, c, tok)
                      for odd in range(2) for c in range(j)]
            tasks.append(lambda tok, u=u: exp_diag(u, tok))
        return first, tasks, finish

    def mem_load(n, g):
        if n % NSEG == 0:
            return jnp.zeros((MZ_ROWS, 128), F32)
        return mz[g]

    def mem_read(n, i, h, state, tok):
        pq = after(PQ[n % 2][i, :, _tile(h)], {8 * u: tok for u in range(4)})
        return _dot_nt(state.astype(BF16), _bf(pq))

    def mem_update(n, i, h, state, tok):
        p, g = n % 2, i + h * NP
        z = jnp.sum(ZS[p][g], axis=0, keepdims=True)
        new = jnp.concatenate([_dot(_bf(after(VT[p][g], {0: tok})), _bf(PK[p][i, :, _tile(h)])),
                               jnp.broadcast_to(z, (MZ_ROWS - 128, 128))], axis=0)
        row = _iota((MZ_ROWS, 128), 0)
        row_head = jnp.where(row < 128, row >> 5, (row - 128) >> 2)
        keep = row_head == (_iota((MZ_ROWS, 128), 1) >> 5)
        mz[g] = new = state + jnp.where(keep, new, 0.0)
        return new

    def is_a(n):
        return (n // NSEG) % 2 == 0

    def run_timed(mm, tasks):
        tasks = sorted(tasks, key=lambda x: x[0])
        for k, prod in enumerate(mm):
            toks = {}
            while tasks and tasks[0][0] < 16 * (k + 1):
                time, f = tasks.pop(0)
                join(toks, time - 16 * k, token(*f()))
            prod(toks)
        for _, f in tasks:
            f()

    def body_b(n, i, mm, ln):
        *share, front, lag, tail, pitch = {
            28: (*B_SHARE, B_FRONT, B_WAIT, *B_TAIL), 21: B_LAST, 14: B_LAST2}[len(mm)]
        state = [mem_load(n, i + h * NP) for h in range(2)]
        late = [f for off in range(0, RC, 16) for f in ln_tasks(n + 2, i, off)] if ln else []
        mem, tiles, done = [], {}, []

        def values(j, finish, tok):
            posts = []
            for h in range(2):
                ot = finish(h, tok)

                def post(ot=ot, h=h):
                    tiles[j, h] = jnp.concatenate(ot, axis=0).T
                    return vregs([tiles[j, h]], 4)

                posts.append(post)
            if j < 2:
                posts += [lambda r=r: store_lhs(
                    O[n], i, 128 * j + r,
                    *[tiles[j + u, h][r:r + B_STORE] for u in (0, 2) for h in range(2)])
                    for r in range(0, 128, B_STORE)]
            return posts

        tok, pending = token(mm.pop(0)(None)), None
        for k, j in enumerate((3, 1, 2, 0)):
            first, exps, finish = att_b_piece(n, i, j, mem, tok)
            done += values(*pending, first) if pending else []
            when = [int(32 * share[k] * front * u / len(exps)) for u in range(len(exps))]
            for c in range(share[k]):
                toks = {0: first} if c == 0 else {}
                for slot in B_POST:
                    if done and 16 * c + slot >= min(lag, 16 * share[k] - 1):
                        join(toks, slot, token(*done.pop(0)()))
                for slot in B_LN[:1 if len(late) % 6 in (0, 5) else 2]:
                    if late:
                        join(toks, slot, token(*late.pop(0)()))
                r = mm.pop(0)(toks)
                while exps and when[0] < 32 * (c + 1):
                    exps.pop(0)(token(r[8 * (when.pop(0) - 32 * c):]))
                tok = token(r)
                if (k, c) == (0, 0) and n % NSEG:
                    mem.extend(mem_read(n, i, h, state[h], tok) for h in range(2))
                    done.append(lambda: [v[:, 128 * u:] for v in mem for u in range(4)])
                if (k, c) == (0, 0) and n % NSEG != NSEG - 1:
                    new = [mem_update(n, i, h, state[h], tok) for h in range(2)]
                    done.append(lambda: new)
            pending = (j, finish)
        done += late + values(*pending, token(mm.pop(0)(None)))
        run_timed(mm, [(tail + pitch * u, f) for u, f in enumerate(done)])

    def step(n, ln=True, proj=(0, 1, 2), att=True, out=(1,), extra=None):
        @pl.loop(0, NP)
        def _(i):
            mm = []
            due.clear()
            for which in (B_MATS if att and not is_a(n) else A_MATS):
                if which in proj:
                    mm += (proj_a if is_a(n + 1) else proj_b)(n + 1, i, which)
                elif which == 3:
                    mm += [f for lag in out for f in out_stage(n - lag, i)]
            if att and not is_a(n):
                body_b(n, i, mm, ln)
                return
            times = A_FIRST if n == 0 else A_PLAIN if is_a(n + 1) else A_THEN_B
            fs = extra(i) if extra else []
            tasks = [(u % 4 + A_PREP_WHEN[u // 4] if att else 4 * (u + 1) / (len(fs) + 1), f)
                     for u, f in enumerate(fs)]
            for u, off in enumerate(range(0, RC, 16)):
                if att:
                    tasks += [(u + w, f) for w, f in att_a_tasks(n, i, off, times[:8])]
                if ln:
                    when = times[8:] if att else (.2, .6, 1.0, 1.15, 1.3, 1.45)
                    tasks += [(u + w, f) for w, f in zip(when, ln_tasks(n + 2, i, off))]
            run_timed(mm, [(int(4 * len(mm) * w), f) for w, f in tasks])

    for i in range(NP):
        start(x0_copies(i))
    start(slab_copies(0, 0))
    start([copy(beta_hbm, beta_ref.at[0], sem_b)])
    zero_ref[:8] = jnp.zeros((8, 128), U32)

    @pl.loop(0, NP)
    def _(i):
        pl.when(i == 2)(lambda: start(slab_copies(0, 1)))
        wait(x0_copies(i))
        for fs in zip(*[ln_tasks(0, i, off) for off in range(0, RC, 16)]):
            for f in fs:
                f()

    start(slab_copies(0, 2))
    wait(slab_copies(0, 0))
    for f in prep_a_cols(0, 0):
        f()

    plan = (([(0, 3), (1, 0)], [(0, 1)]), ([(1, 1), (1, 2)], [(0, 2), (0, 3)]),
            ([(1, 3), (2, 0)], [(1, 0), (1, 1)]), ([(2, 1), (2, 2)], [(1, 2), (1, 3)]))
    for t, (fetch, preps) in enumerate(plan):
        for mi in fetch:
            start(slab_copies(*mi))
        for mi in preps:
            wait(slab_copies(*mi))
        mm = [f for i in range(NP) for f in proj_a(0, i, 0, only=t)]
        fs = [f for group in zip(*[prep_a_cols(*mi) for mi in preps]) for f in group]
        run_timed(mm, [(16 * len(mm) * (u + 1) // (len(fs) + 1), f) for u, f in enumerate(fs)])

    def prep_wv(i):
        pl.when(i == 0)(lambda: start(x_copies(1) + wao_copies()))
        wait(slab_copies(2, i))
        return prep_a_cols(2, i)

    start(slab_copies(2, 3))
    step(-1, ln=False, proj=(1,), att=False, out=(), extra=prep_wv)
    start(x_copies(2))
    start(x_copies(3))
    wait(x_copies(1))
    wait(wao_copies())
    step(-1, proj=(2,), att=False, out=(), extra=prep_a_rows)
    for m in range(4):
        start(wb_copies(m))
    wait([copy(beta_hbm, beta_ref.at[0], sem_b)])
    gate = jax.nn.sigmoid(beta_ref[0].astype(F32))
    eye = _iota((H, H), 0) == _iota((H, H), 1)
    gcol = jnp.sum(jnp.where(eye, jnp.broadcast_to(gate, (H, H)), 0.0), axis=1, keepdims=True)
    gtab[...] = jnp.broadcast_to(gcol, (H, 128))
    wait(x_copies(2))
    step(0, out=())
    wait(x_copies(3))
    for m in range(4):
        wait(wb_copies(m))
    step(1, extra=lambda i: prep_b(0, i) + prep_b(1, i))
    step(2, extra=lambda i: prep_b(2, i) + prep_b(3, i))
    for n in range(3, 14):
        step(n)
    start(out_copies(0))
    step(14, ln=False, out=())
    step(15, ln=False, proj=(), out=(2, 1))
    start(out_copies(1))
    start(out_copies(2))
    due.clear()
    for i in range(NP):
        run_timed(out_stage(LAST, i), [])
        if i >= NP - 2:
            start(out_tile_copies(0, NP - 1) if i == NP - 2 else out_tile_copies(i, 1))
    for s in range(NSEG - 1):
        wait(out_copies(s))
    wait(out_tile_copies(0, NP - 1) + out_tile_copies(NP - 1, 1))


@jax.jit
def pallas_interleave_layers__sliding_local_dilated__memory_aug_infini_attn__prompt_kernel(
    A_x: jax.Array,
    A_wqkv: jax.Array,
    A_wo: jax.Array,
    B_x: jax.Array,
    B_wq: jax.Array,
    B_wk: jax.Array,
    B_wv: jax.Array,
    B_wo: jax.Array,
    B_beta: jax.Array,
):
    del B_x
    assert A_x.shape == (1, S, D)
    hbm = pl.BlockSpec(memory_space=pl.ANY)
    scratch = (
        [pltpu.VMEM((L, D), BF16)] * 4
        + [pltpu.VMEM((7, D, D), BF16), pltpu.VMEM((NT, D, 128), BF16),
           pltpu.VMEM((2, 576, 128), U32),
           *[pltpu.VMEM((1, NP, D // 4, 7 * 128), U32)] * 4,
           pltpu.VMEM((4, NP, D // 4, 7 * 128), U32)]
        + [pltpu.VMEM((NP, HL // 2, 7 * 128), U32)] * 5
        + [pltpu.VMEM((NT, L, 128), F32)] * 2
        + [pltpu.VMEM((NT, HALO + L, 128), F32)] * 4
        + [pltpu.VMEM((NP, L // 2, 2 * 128), U32)] * 6
        + [pltpu.VMEM((NT, 64, L), U32)] * 4
        + [pltpu.VMEM((NT, 16, 128), F32)] * 2
        + [pltpu.VMEM((NT, MZ_ROWS, 128), F32), pltpu.VMEM((8, 1, H), BF16),
           pltpu.VMEM((H, 128), F32),
           pltpu.VMEM((88, 128), U32),
           pltpu.SemaphoreType.DMA((NSEG,)), pltpu.SemaphoreType.DMA((5,)),
           pltpu.SemaphoreType.DMA((4, NP)),
           pltpu.SemaphoreType.DMA((NSEG,)), pltpu.SemaphoreType.DMA]
    )
    out = pl.pallas_call(
        _kernel,
        out_shape=jax.ShapeDtypeStruct((S, D), BF16),
        in_specs=[hbm] * 8,
        out_specs=hbm,
        scratch_shapes=scratch,
        compiler_params=pltpu.CompilerParams(vmem_limit_bytes=110 * 2**20),
        name="abab_stack",
    )(A_x.reshape(S, D), A_wqkv, A_wo, B_wq, B_wk, B_wv, B_wo, B_beta.reshape(1, H))
    return out.reshape(1, S, D)
```

```python
import jax
import jax.numpy as jnp
from jax import lax
import jax.experimental.pallas as pl
import jax.experimental.pallas.tpu as pltpu

S, D, H, DH = 2048, 1024, 32, 32
NSEG, L = 4, 512
HL = L // 2
NT = D // 128
NP = NT // 2
RC = HL // NP
KC = D // 2 // NP
LAST = 4 * NSEG - 1
WIN, DIL = 8, 2
HALO = 16
MZ_ROWS = 128 + 16
LOG2E = 1.4426950408889634
QSCALE = float(DH ** -0.5 * LOG2E)
MASKVAL = float(-1e9 * LOG2E)

A_MATS = (3, 0, 2, 1)
B_MATS = (2, 0, 1, 3)
B_PLAIN = (7, 7, 6, 4, 0.749, 28, 42, 0, 6, 15, 4, 9)
B_FIRST = (7, 7, 6, 4, 0.749, 28, 42, 0, 6, 15, 4, 9)
B_THEN_A = (7, 7, 6, 4, 0.749, 29, 42, 0, 7, 15, 6, 7)
B_END1 = (3, 2, 9, 3, 0.902, 30, 32, 2, 6, 15, 2, 6)
B_END2 = (4, 3, 2, 1, 0.832, 29, 28, 4, 8, 15, 6, 9)
B_STORE = 64
T_DUE = 36
A_PLAIN = (0.051, 0.047, 0.07, 0.179, 0.286, 0.632, 0.042, 0.039, 0.027, 0.3, 0.45, 0.512, 0.542, 0.57)
A_FIRST = (0.051, 0.036, 0.107, 0.22, 0.277, 0.607, 0.039, 0.047, 0.024, 0.316, 0.465, 0.5, 0.55, 0.56)
A_THEN_B = (0.055, 0.035, 0.07, 0.18, 0.27, 0.621, 0.031, 0.087, 0.062, 0.297, 0.432, 0.49, 0.53, 0.57)
A_PREP_WHEN = (0.313, 0.283, 0.373, 0.395, 0.353, 0.5, 0.556, 0.582)

F32, BF16, U32 = jnp.float32, jnp.bfloat16, jnp.uint32
_NT_DIMS = (((1,), (1,)), ((), ()))


def _iota(shape, axis):
    return lax.broadcasted_iota(jnp.int32, shape, axis)


def _dot(a, b):
    return jnp.dot(a, b, preferred_element_type=F32)


def _dot_nt(a, b):
    return lax.dot_general(a, b, _NT_DIMS, preferred_element_type=F32)


def _rows(start, size):
    return pl.ds(start if isinstance(start, int) else pl.multiple_of(start, size), size)


def _tile(k):
    return _rows(128 * k, 128)


def _words(val):
    return pltpu.bitcast(val.astype(BF16), U32)


def _put(ref, idx, start, k, words):
    ref[(*idx, _rows(start // 2, words.shape[0]), _tile(k))] = words
    return words


def _bf(words):
    return pltpu.bitcast(words, BF16)


def _phi(t):
    return jnp.where(t > 0, t + 1.0, jnp.exp(t))


def _tree(op, xs):
    xs = list(xs)
    while len(xs) > 1:
        xs = [op(xs[i], xs[i + 1]) if i + 1 < len(xs) else xs[i]
              for i in range(0, len(xs), 2)]
    return xs[0]


def _lhs_terms(a11, a12, a21, a22):
    return (a11 + a22, a21 + a22, a11, a22, a11 + a12, a21 - a11, a12 - a22)


def _rhs_terms(b11, b12, b21, b22):
    return (b11 + b22, b11, b12 - b22, b21 - b11, b22, b11 + b12, b21 + b22)


def _kernel(x_hbm, wqkv_hbm, awo_hbm, wq_hbm, wk_hbm, wv_hbm, wo_hbm, beta_hbm,
            out_hbm,
            x0, x1, x2, x3, wraw, wraw_o, wtmp, waq, wak, wav, wao, wb,
            xn0, xn1, o0, o1, o2,
            qa0, qa1, ka0, ka1, va0, va1,
            pq0, pq1, kb0, kb1, pk0, pk1, qt0, qt1, vt0, vt1,
            zs0, zs1, mz, beta_ref, gtab, zero_ref, sem_x, sem_w, sem_s, sem_o, sem_b):
    X = (x0, x1, x2, x3)
    XN, wa = (xn0, xn1), (waq, wak, wav)
    O = [o2 if n == LAST else (o0, o1)[n % 2] for n in range(LAST + 1)]
    QA, KA, VA = (qa0, qa1), (ka0, ka1), (va0, va1)
    QT, PQ, KB, PK, VT = (qt0, qt1), (pq0, pq1), (kb0, kb1), (pk0, pk1), (vt0, vt1)
    ZS = (zs0, zs1)

    copy = pltpu.make_async_copy

    def x_copies(s):
        return [copy(x_hbm.at[pl.ds(s * L, L)], X[s], sem_x.at[s])]

    def out_copies(s):
        return [copy(X[s], out_hbm.at[pl.ds(s * L, L)], sem_o.at[s])]

    def out_tile_copies(t0, nt):
        cols = [pl.ds(128 * (t0 + c * NP), 128 * nt) for c in range(2)]
        return [copy(x3.at[:, c], out_hbm.at[pl.ds(S - L, L), c], sem_o.at[NSEG - 1]) for c in cols]

    def wao_copies():
        return [copy(awo_hbm.at[:, _tile(t)], wraw_o.at[t], sem_w.at[4]) for t in range(NT)]

    def wb_copies(m):
        return [copy((wq_hbm, wk_hbm, wv_hbm, wo_hbm)[m], wraw.at[3 + m], sem_w.at[m])]

    def slab_copies(m, i):
        return [copy(wqkv_hbm.at[r, _rows(m * D, D)], wraw.at[m, r], sem_s.at[m, i])
                for r in (_rows(h * (D // 2) + i * KC, KC) for h in range(2))]

    def x0_copies(i):
        return [copy(x_hbm.at[r], x0.at[r], sem_s.at[3, i])
                for r in (_rows(h * HL + i * RC, RC) for h in range(2))]

    def start(cs):
        for c in cs:
            c.start()

    def wait(cs):
        for c in cs:
            c.wait()

    def token(*vals):
        bits = [pltpu.bitcast(v[:8, :128], U32) for v in vals]
        return _tree(jnp.bitwise_or, bits) & zero_ref[:8]

    def vregs(vals, every=1):
        return [v[u:u + 8] for v in vals for u in range(0, v.shape[0], 8)][::-1][::every]

    def after(words, toks):
        if not toks:
            return words
        slabs = []
        for k in range(words.shape[0] // 8):
            slab = words[8 * k:8 * k + 8]
            if toks.get(k) is not None:
                slab = slab | jnp.concatenate([toks[k]] * (words.shape[1] // 128), axis=1)
            slabs.append(slab)
        return jnp.concatenate(slabs, axis=0)

    def store_rhs(dst, m, i, r, b11, b12, b21, b22):
        terms = _rhs_terms(*[_bf(b).astype(F32) for b in (b11, b12, b21, b22)])
        words = [{1: b11, 4: b22}[k] if k in (1, 4) else _words(v) for k, v in enumerate(terms)]
        return vregs([_put(dst, (m, i), r, k, v) for k, v in enumerate(words)])

    def raw_words(m, r, rows, t):
        return pltpu.bitcast(wraw[m, _rows(r, rows), _tile(t)], U32)

    def prep_b(m, i):
        def piece(j, c):
            r = i * KC + 32 * c
            return store_rhs(wb, m, j, r, *[raw_words(3 + m, r + h * (D // 2), 32, j + u * NP)
                                            for h in range(2) for u in range(2)])

        return [lambda j=j, c=c: piece(j, c) for j in range(NP) for c in range(KC // 32)]

    def prep_a_cols(m, i):
        rows = 32
        st = {}

        def rotate(c):
            v = [jnp.concatenate([raw_words(m, i * KC + c * rows + h * (D // 2), rows, t)
                                  for h in range(2)], axis=0) for t in range(NT)]
            st[c] = [x if t == 0 else pltpu.roll(x, 2 * t, 1) for t, x in enumerate(v)]
            return vregs(st[c], 4)

        def shear(c):
            slot = (_iota((rows, 128), 1) >> 1) & 7
            v = [st[c][(-b) % NT] for b in range(NT)]
            for bit in (1, 2, 4):
                sel = (slot & bit) != 0
                v = [jnp.where(sel, v[(b - bit) % NT], v[b]) for b in range(NT)]
            st[c] = [x if b == 0 else pltpu.roll(x, 128 - 2 * b, 1) for b, x in enumerate(v)]
            return vregs(v, 2)

        def terms(c):
            v, half, outs = st[c], rows // 2, []
            for j in range(NP):
                outs += store_rhs(wa[m], 0, j, i * KC + c * rows, v[j][:half], v[j + NP][:half],
                                  v[j][half:], v[j + NP][half:])
            return outs

        order = [(f, k - lag) for k in range(6) for lag, f in enumerate((rotate, shear, terms))
                 if 0 <= k - lag < 4]
        return [lambda f=f, c=c: f(c) for f, c in order]

    def prep_a_rows(i):
        def stage(t):
            words = [pltpu.bitcast(wraw_o[i + h * NP, _tile(t), :], U32) for h in range(2)]
            for h in range(2):
                wtmp[h, pl.ds(65 * t, 64), :] = words[h]
            return vregs(words)

        def rows(h, b, u):
            return jnp.concatenate(
                [wtmp[h, pl.ds(8 * (u + k) + b, 8, stride=65), :] for k in range(2)], axis=0)

        def piece(c, u):
            return store_rhs(wao, 0, i, 128 * c + 16 * u, rows(0, c, u), rows(1, c, u),
                             rows(0, c + NP, u), rows(1, c + NP, u))

        return ([lambda t=t: stage(t) for t in range(NT)]
                + [lambda c=c, u=u: piece(c, u) for c in range(4) for u in range(0, 8, 2)])

    def store_lhs(dst, t, r, a11, a12, a21, a22):
        terms = _lhs_terms(a11, a12, a21, a22)
        return vregs([_put(dst, (t,), r, k, _words(v)) for k, v in enumerate(terms)])

    def join(toks, slot, tok):
        if tok is not None:
            toks[slot] = tok if toks.get(slot) is None else toks[slot] | tok

    due = []

    def products(a_ref, w_ref, m, i, emit, only=None):
        st = {}

        def prod(k, toks, finish):
            toks = dict(toks or {})
            while due and due[0][0] < 16:
                slot, vals = due.pop(0)
                join(toks, slot, token(*vals))
            for entry in due:
                entry[0] -= 16
            if only is None:
                a = jnp.concatenate([after(a_ref[t, :, _tile(k)], toks if t == 0 else None)
                                     for t in range(NP)], axis=1)
                w = w_ref[m, i, :, _tile(k)]
            else:
                a = after(a_ref[only, :, _tile(k)], toks)
                w = w_ref[m, i, _rows(64 * only, 64), _tile(k)]
            r = _dot(_bf(a), _bf(w))
            finish(r)
            return r

        def p1(r):
            st["m1"] = r

        def p2(r):
            st["c21"], st["c22"] = r, st["m1"] - r

        def p3(r):
            st["c12"], st["c22"] = r, st["c22"] + r

        def p4(r):
            st["c11"] = st["m1"] + r
            emit(1, 0, st["c21"] + r)

        def p5(r):
            st["c11"] = st["c11"] - r
            emit(0, 1, st["c12"] + r)

        def p6(r):
            emit(1, 1, st["c22"] + r)

        def p7(r):
            emit(0, 0, st["c11"] + r)

        return [lambda toks, k=k, f=f: prod(k, toks, f)
                for k, f in enumerate((p1, p2, p3, p4, p5, p6, p7))]

    def ln_tasks(n, i, off, nr=16):
        src, dst = X[n % NSEG], XN[n % 2]
        st = {}

        def mean():
            st["x"] = [
                jnp.concatenate(
                    [src[_rows(i * RC + off + h * HL, nr), _tile(t)].astype(F32)
                     for h in range(2)], axis=0) for t in range(NT)]
            part = _tree(jnp.add, st["x"])
            st["mean"] = jnp.sum(part, axis=1, keepdims=True) * (1.0 / D)
            return vregs([part])

        def var():
            st["x"] = [x - st["mean"] for x in st["x"]]
            part = _tree(jnp.add, [x * x for x in st["x"]])
            st["var"] = jnp.sum(part, axis=1, keepdims=True) * (1.0 / D)
            return vregs([part])

        def scale(t):
            if t == 0:
                st["inv"] = lax.rsqrt(st["var"] + 1e-5)
            y0, y1 = st["x"][t] * st["inv"], st["x"][t + NP] * st["inv"]
            return store_lhs(dst, t, i * RC + off, y0[:nr], y1[:nr], y0[nr:], y1[nr:])

        return [mean, var] + [lambda t=t: scale(t) for t in range(NP)]

    def proj_a(n, i, which, only=None):
        p = n % 2

        def emit(h, c, y):
            t = i + c * NP
            buf = (QA, KA, VA)[which]
            rows = pl.ds(h * HL + (HALO if which else 0), HL)
            if only:
                y = y + buf[p][t, rows, :]
            buf[p][t, rows, :] = y
            if which and h == 0 and n % NSEG == 0:
                buf[p][t, pl.ds(0, HALO), :] = jnp.zeros((HALO, 128), F32)
            elif which and h == 0:
                buf[p][t, pl.ds(0, HALO), :] = buf[1 - p][t, pl.ds(L, HALO), :]

        return products(XN[p], wa[which], 0, i, emit, only)

    def proj_b(n, i, which):
        p = n % 2

        def transposed(buf, h, c, y):
            words = pltpu.bitcast(y.astype(BF16).T, U32)
            buf[p][i + c * NP, :, pl.ds(h * HL, HL)] = words
            due.append([T_DUE, vregs([words[:, :128], words[:, 128:]], 2)])

        def emit(h, c, y):
            if which == 0:
                if n % NSEG:
                    _put(PQ[p], (i,), h * HL, c, _words(_phi(y)))
                y = y * QSCALE
                flip = jnp.concatenate([y[r ^ 96:(r ^ 96) + 32] for r in range(0, HL, 32)], axis=0)
                y = jnp.where((_iota(y.shape, 1) & 32) == 0, y, flip)
                transposed(QT, h, c, y)
            elif which == 1:
                _put(KB[p], (i,), h * HL, c, _words(y))
                if n % NSEG != NSEG - 1:
                    y = _phi(y)
                    _put(PK[p], (i,), h * HL, c, _words(y))
                    ZS[p][i + c * NP, pl.ds(8 * h, 8), :] = _tree(jnp.add, vregs([y]))
            else:
                transposed(VT, h, c, y)

        return products(XN[p], wb, which, i, emit)

    def out_stage(n, i):
        x = X[n % NSEG]

        def emit(h, c, y):
            where = (pl.ds(h * HL, HL), _tile(i + c * NP))
            x[where] = (x[where].astype(F32) + y).astype(BF16)

        if is_a(n):
            return products(O[n], wao, 0, i, emit)
        return products(O[n], wb, 3, i, emit)

    def att_a_tasks(n, i, off, times):
        p = n % 2
        base = pl.multiple_of(i * RC, RC) + off
        starts = [base + (u // 2) * HL + 8 * (u % 2) for u in range(4)]
        lg, mixed = [[] for _ in range(4)], {}

        def scores(u, ws):
            q = [QA[p][t, pl.ds(starts[u], 8), :] for t in range(NT)]
            for w in ws:
                kr = pl.ds(starts[u] + HALO - DIL * w, 8)
                lg[u].append(_tree(jnp.add, [q[t] * KA[p][t, kr, :] for t in range(NT)]))
            return lg[u][-len(ws):]

        def exchange(u, bit):
            low = (_iota((8, 128), 1) & bit) == 0
            lg[u] = [a + jnp.where(low, pltpu.roll(a, 128 - bit, 1), pltpu.roll(a, bit, 1))
                     for a in lg[u]]
            return lg[u]

        def softmax(u):
            v = [a * QSCALE for a in lg[u]]
            if n % NSEG == 0 and off == 0 and u < 2:
                pos = _iota((8, 128), 0) + starts[u]
                v = [a if w == 0 else jnp.where(pos >= DIL * w, a, MASKVAL)
                     for w, a in enumerate(v)]
            m = _tree(jnp.maximum, v)
            e = [jnp.exp2(a - m) for a in v]
            inv = 1.0 / _tree(jnp.add, e)
            lg[u] = [a * inv for a in e]
            return lg[u]

        def mix(t, h):
            for c in range(2):
                mixed[t, h, c] = jnp.concatenate([
                    _tree(jnp.add, [
                        lg[u][w] * VA[p][t + c * NP, pl.ds(starts[u] + HALO - DIL * w, 8), :]
                        for w in range(WIN)])
                    for u in (2 * h, 2 * h + 1)], axis=0)
            return vregs([mixed[t, h, c] for c in range(2)])

        def store(t):
            return store_lhs(O[n], t, i * RC + off,
                             *[mixed[t, h, c] for h in range(2) for c in range(2)])

        t_score, d_score, lag1, lag2, lag3, t_mix, d_mix, d_store = times
        tasks = []
        for u in range(4):
            t = t_score + d_score * (2 * u + 1)
            tasks += [(t - d_score, lambda u=u: scores(u, range(4))),
                      (t, lambda u=u: scores(u, range(4, 8))),
                      (t + lag1, lambda u=u: exchange(u, 1)),
                      (t + lag2, lambda u=u: exchange(u, 16)),
                      (t + lag3, lambda u=u: softmax(u))]
        for k in range(NP):
            t = t_mix + k * (d_mix + d_store)
            tasks += [(t, lambda k=k: mix(k, 0)), (t + d_mix, lambda k=k: mix(k, 1))]
            tasks += [(t + d_mix + d_store / 2, lambda k=k: store(k))]
        return tasks

    def att_b_piece(n, i, j, mem, tok):
        p = n % 2
        nk = 128 * j + 32
        shared = ((32, 1, 3), (64, 2, 2), (96, 3, 1))
        key, lane = _iota((32, 128), 0), _iota((32, 128), 1)
        causal = [jnp.where(key > q, MASKVAL, 0.0) for q in (lane, lane ^ 96)]
        even = [_iota((8, 128), 1) >= lo for lo, _, _ in shared]

        def place(parts):
            zero = jnp.zeros((16, 128), U32)
            return jnp.concatenate([parts.get(hh, zero) for hh in range(4)], axis=0)

        q = [[after(QT[p][i + h * NP, pl.ds(16 * hh, 16), _tile(j)], {0: tok}) for hh in range(4)]
             for h in range(2)]
        s = []
        for h in range(2):
            w = jnp.concatenate([place({hh: q[h][hh]}) for hh in range(4)], axis=1)
            st = _dot(_bf(KB[p][i, pl.ds(0, nk // 2), _tile(h)]), _bf(w))
            for hh in range(4):
                v = st[:, 128 * hh:128 * (hh + 1)]
                s.append([v[u:u + 8] for u in range(0, nk - 32, 8)]
                         + [v[nk - 32 + u:nk - 24 + u] + causal[hh % 2][u:u + 8]
                            for u in range(0, 32, 8)])
        sx = [[] for _ in range(4)]
        for lo, ce, co in shared:
            ahead = jnp.where(lane >= lo, key + 32 * ce - lane, key + 32 * co - (lane ^ 96))
            mask = jnp.where(ahead > 0, MASKVAL, 0.0)
            high = _iota((16, 128), 1) >= lo
            for h in range(2):
                ke, ko = (KB[p][i, pl.ds(64 * j + 16 * c, 16), _tile(h)] for c in (ce, co))
                k = ke if ce == co else jnp.where((_iota((16, 128), 1) & 32) == 0, ke, ko)
                w = jnp.concatenate(
                    [place({hh: jnp.where(high, q[h][hh], jnp.uint32(0)),
                            hh + 1: jnp.where(high, jnp.uint32(0), q[h][hh + 1])})
                     for hh in (0, 2)], axis=1)
                st = _dot(_bf(k), _bf(w))
                for u in range(2):
                    v = st[:, 128 * u:128 * (u + 1)] + mask
                    sx[2 * h + u].append([v[r:r + 8] for r in range(0, 32, 8)])
        first = token(*[v[0] for v in s])
        m = []
        for u in range(4):
            a = [_tree(jnp.maximum, s[2 * u + odd]) for odd in range(2)]
            for sel, v in zip(even, sx[u]):
                mx = _tree(jnp.maximum, v)
                a = [jnp.where(sel, jnp.maximum(a[0], mx), a[0]),
                     jnp.where(sel, a[1], jnp.maximum(a[1], mx))]
            m += [jnp.broadcast_to(jnp.max(v, axis=0, keepdims=True), (8, 128)) for v in a]
        e = [[] for _ in range(8)]
        part = [[] for _ in range(8)]

        def exps(v, mh, tok):
            mh = mh if tok is None else mh + pltpu.bitcast(tok, F32)
            return [jnp.exp2(a - mh) for a in v]

        def collect(u, v):
            part[u] = [_tree(jnp.add, part[u] + v)]
            e[u].extend(v)

        def exp_tile(u, c, tok):
            collect(u, exps(s[u][16 * c:16 * (c + 1)], m[u], tok))

        def exp_diag(u, tok):
            for odd in range(2):
                exp_tile(2 * u + odd, j, tok)
            v = [exps(a, jnp.where(sel, m[2 * u], m[2 * u + 1]), tok) for sel, a in zip(even, sx[u])]
            collect(2 * u, [jnp.where(even[c], a, 0.0) for c in (0, 1, 2) for a in v[c]])
            collect(2 * u + 1, [jnp.where(even[c], 0.0, a) for c in (2, 1, 0) for a in v[c]])

        def finish(h, tok):
            g = i + h * NP
            ot = []
            for hh in range(4):
                u = 4 * h + hh
                vt = after(VT[p][g, pl.ds(16 * hh, 16), pl.ds(0, 128 * (j + 1))], {0: tok})
                acc = _dot(_bf(vt), jnp.concatenate(e[u], axis=0).astype(BF16))
                l = jnp.sum(part[u][0], axis=0, keepdims=True)
                gate = gtab[pl.ds(4 * g + hh, 1), :]
                acc = acc * ((1.0 - gate) / l)
                if hh % 2:
                    acc = jnp.where((lane & 32) == 0, pltpu.roll(acc, 32, 1), pltpu.roll(acc, 96, 1))
                if n % NSEG:
                    r = mem[h][:, 128 * j:128 * (j + 1)]
                    den = r[128 + 4 * hh:129 + 4 * hh] + 1e-6
                    acc = acc + r[32 * hh:32 * hh + 32] * (gate / den)
                ot.append(acc)
            return ot

        tasks = []
        for u in range(4):
            tasks += [lambda tok, u=2 * u + odd, c=c: exp_tile(u, c, tok)
                      for odd in range(2) for c in range(j)]
            tasks.append(lambda tok, u=u: exp_diag(u, tok))
        return first, tasks, finish

    def mem_load(n, g):
        if n % NSEG == 0:
            return jnp.zeros((MZ_ROWS, 128), F32)
        return mz[g]

    def mem_read(n, i, h, state, tok):
        pq = after(PQ[n % 2][i, :, _tile(h)], {8 * u: tok for u in range(4)})
        return _dot_nt(state.astype(BF16), _bf(pq))

    def mem_update(n, i, h, state, tok):
        p, g = n % 2, i + h * NP
        z = jnp.sum(ZS[p][g], axis=0, keepdims=True)
        new = jnp.concatenate([_dot(_bf(after(VT[p][g], {0: tok})), _bf(PK[p][i, :, _tile(h)])),
                               jnp.broadcast_to(z, (MZ_ROWS - 128, 128))], axis=0)
        row = _iota((MZ_ROWS, 128), 0)
        row_head = jnp.where(row < 128, row >> 5, (row - 128) >> 2)
        keep = row_head == (_iota((MZ_ROWS, 128), 1) >> 5)
        mz[g] = new = state + jnp.where(keep, new, 0.0)
        return new

    def is_a(n):
        return (n // NSEG) % 2 == 0

    def run_timed(mm, tasks):
        tasks = sorted(tasks, key=lambda x: x[0])
        for k, prod in enumerate(mm):
            toks = {}
            while tasks and tasks[0][0] < 16 * (k + 1):
                time, f = tasks.pop(0)
                join(toks, time - 16 * k, token(*f()))
            prod(toks)
        for _, f in tasks:
            f()

    def body_b(n, i, mm, ln):
        times = {LAST - 1: B_END1, LAST: B_END2}.get(
            n, (B_FIRST, B_PLAIN, B_PLAIN, B_THEN_A)[n % NSEG])
        share, (front, lag, tail, pitch) = times[:4], times[4:8]
        state = [mem_load(n, i + h * NP) for h in range(2)]
        late = [f for off in range(0, RC, 16) for f in ln_tasks(n + 2, i, off)] if ln else []
        mem, tiles, done = [], {}, []

        def values(j, finish, tok):
            posts = []
            for h in range(2):
                ot = finish(h, tok)

                def post(ot=ot, h=h):
                    tiles[j, h] = jnp.concatenate(ot, axis=0).T
                    return vregs([tiles[j, h]], 4)

                posts.append(post)
            if j < 2:
                posts += [lambda r=r: store_lhs(
                    O[n], i, 128 * j + r,
                    *[tiles[j + u, h][r:r + B_STORE] for u in (0, 2) for h in range(2)])
                    for r in range(0, 128, B_STORE)]
            return posts

        tok, pending = token(mm.pop(0)(None)), None
        for k, j in enumerate((3, 1, 2, 0)):
            first, exps, finish = att_b_piece(n, i, j, mem, tok)
            done += values(*pending, first) if pending else []
            when = [int(32 * share[k] * front * u / len(exps)) for u in range(len(exps))]
            for c in range(share[k]):
                toks = {0: first} if c == 0 else {}
                for slot in times[8:10]:
                    if done and 16 * c + slot >= min(lag, 16 * share[k] - 1):
                        join(toks, slot, token(*done.pop(0)()))
                for slot in times[10:11 if len(late) % 6 in (0, 5) else 12]:
                    if late:
                        join(toks, slot, token(*late.pop(0)()))
                r = mm.pop(0)(toks)
                while exps and when[0] < 32 * (c + 1):
                    exps.pop(0)(token(r[8 * (when.pop(0) - 32 * c):]))
                tok = token(r)
                if (k, c) == (0, 0) and n % NSEG:
                    mem.extend(mem_read(n, i, h, state[h], tok) for h in range(2))
                    done.append(lambda: [v[:, 128 * u:] for v in mem for u in range(4)])
                if (k, c) == (0, 0) and n % NSEG != NSEG - 1:
                    new = [mem_update(n, i, h, state[h], tok) for h in range(2)]
                    done.append(lambda: new)
            pending = (j, finish)
        done += late + values(*pending, token(mm.pop(0)(None)))
        run_timed(mm, [(tail + pitch * u, f) for u, f in enumerate(done)])

    def step(n, ln=True, proj=(0, 1, 2), att=True, out=(1,), extra=None):
        @pl.loop(0, NP)
        def _(i):
            mm = []
            due.clear()
            for which in (B_MATS if att and not is_a(n) else A_MATS):
                if which in proj:
                    mm += (proj_a if is_a(n + 1) else proj_b)(n + 1, i, which)
                elif which == 3:
                    mm += [f for lag in out for f in out_stage(n - lag, i)]
            if att and not is_a(n):
                body_b(n, i, mm, ln)
                return
            times = A_FIRST if n == 0 else A_PLAIN if is_a(n + 1) else A_THEN_B
            fs = extra(i) if extra else []
            tasks = [(u % 4 + A_PREP_WHEN[u // 4] if att else 4 * (u + 1) / (len(fs) + 1), f)
                     for u, f in enumerate(fs)]
            for u, off in enumerate(range(0, RC, 16)):
                if att:
                    tasks += [(u + w, f) for w, f in att_a_tasks(n, i, off, times[:8])]
                if ln:
                    when = times[8:] if att else (.2, .6, 1.0, 1.15, 1.3, 1.45)
                    tasks += [(u + w, f) for w, f in zip(when, ln_tasks(n + 2, i, off))]
            run_timed(mm, [(int(4 * len(mm) * w), f) for w, f in tasks])

    for i in range(NP):
        start(x0_copies(i))
    start(slab_copies(0, 0))
    start([copy(beta_hbm, beta_ref.at[0], sem_b)])
    zero_ref[:8] = jnp.zeros((8, 128), U32)

    @pl.loop(0, NP)
    def _(i):
        pl.when(i == 2)(lambda: start(slab_copies(0, 1)))
        wait(x0_copies(i))
        for fs in zip(*[ln_tasks(0, i, off) for off in range(0, RC, 16)]):
            for f in fs:
                f()

    start(slab_copies(0, 2))
    wait(slab_copies(0, 0))
    for f in prep_a_cols(0, 0):
        f()

    plan = (([(0, 3), (1, 0)], [(0, 1)]), ([(1, 1), (1, 2)], [(0, 2), (0, 3)]),
            ([(1, 3), (2, 0)], [(1, 0), (1, 1)]), ([(2, 1), (2, 2)], [(1, 2), (1, 3)]))
    for t, (fetch, preps) in enumerate(plan):
        for mi in fetch:
            start(slab_copies(*mi))
        for mi in preps:
            wait(slab_copies(*mi))
        mm = [f for i in range(NP) for f in proj_a(0, i, 0, only=t)]
        fs = [f for group in zip(*[prep_a_cols(*mi) for mi in preps]) for f in group]
        run_timed(mm, [(16 * len(mm) * (u + 1) // (len(fs) + 1), f) for u, f in enumerate(fs)])

    def prep_wv(i):
        pl.when(i == 0)(lambda: start(x_copies(1) + wao_copies()))
        wait(slab_copies(2, i))
        return prep_a_cols(2, i)

    start(slab_copies(2, 3))
    step(-1, ln=False, proj=(1,), att=False, out=(), extra=prep_wv)
    start(x_copies(2))
    start(x_copies(3))
    wait(x_copies(1))
    wait(wao_copies())
    step(-1, proj=(2,), att=False, out=(), extra=prep_a_rows)
    for m in range(4):
        start(wb_copies(m))
    wait([copy(beta_hbm, beta_ref.at[0], sem_b)])
    gate = jax.nn.sigmoid(beta_ref[0].astype(F32))
    eye = _iota((H, H), 0) == _iota((H, H), 1)
    gcol = jnp.sum(jnp.where(eye, jnp.broadcast_to(gate, (H, H)), 0.0), axis=1, keepdims=True)
    gtab[...] = jnp.broadcast_to(gcol, (H, 128))
    wait(x_copies(2))
    step(0, out=())
    wait(x_copies(3))
    for m in range(4):
        wait(wb_copies(m))
    step(1, extra=lambda i: prep_b(0, i) + prep_b(1, i))
    step(2, extra=lambda i: prep_b(2, i) + prep_b(3, i))
    for n in range(3, 14):
        step(n)
    start(out_copies(0))
    step(14, ln=False, out=())
    step(15, ln=False, proj=(), out=(2, 1))
    start(out_copies(1))
    start(out_copies(2))
    due.clear()
    for i in range(NP):
        run_timed(out_stage(LAST, i), [])
        if i >= NP - 2:
            start(out_tile_copies(0, NP - 1) if i == NP - 2 else out_tile_copies(i, 1))
    for s in range(NSEG - 1):
        wait(out_copies(s))
    wait(out_tile_copies(0, NP - 1) + out_tile_copies(NP - 1, 1))


@jax.jit
def pallas_interleave_layers__sliding_local_dilated__memory_aug_infini_attn__prompt_kernel(
    A_x: jax.Array,
    A_wqkv: jax.Array,
    A_wo: jax.Array,
    B_x: jax.Array,
    B_wq: jax.Array,
    B_wk: jax.Array,
    B_wv: jax.Array,
    B_wo: jax.Array,
    B_beta: jax.Array,
):
    del B_x
    assert A_x.shape == (1, S, D)
    hbm = pl.BlockSpec(memory_space=pl.ANY)
    scratch = (
        [pltpu.VMEM((L, D), BF16)] * 4
        + [pltpu.VMEM((7, D, D), BF16), pltpu.VMEM((NT, D, 128), BF16),
           pltpu.VMEM((2, 576, 128), U32),
           *[pltpu.VMEM((1, NP, D // 4, 7 * 128), U32)] * 4,
           pltpu.VMEM((4, NP, D // 4, 7 * 128), U32)]
        + [pltpu.VMEM((NP, HL // 2, 7 * 128), U32)] * 5
        + [pltpu.VMEM((NT, L, 128), F32)] * 2
        + [pltpu.VMEM((NT, HALO + L, 128), F32)] * 4
        + [pltpu.VMEM((NP, L // 2, 2 * 128), U32)] * 6
        + [pltpu.VMEM((NT, 64, L), U32)] * 4
        + [pltpu.VMEM((NT, 16, 128), F32)] * 2
        + [pltpu.VMEM((NT, MZ_ROWS, 128), F32), pltpu.VMEM((8, 1, H), BF16),
           pltpu.VMEM((H, 128), F32),
           pltpu.VMEM((88, 128), U32),
           pltpu.SemaphoreType.DMA((NSEG,)), pltpu.SemaphoreType.DMA((5,)),
           pltpu.SemaphoreType.DMA((4, NP)),
           pltpu.SemaphoreType.DMA((NSEG,)), pltpu.SemaphoreType.DMA]
    )
    out = pl.pallas_call(
        _kernel,
        out_shape=jax.ShapeDtypeStruct((S, D), BF16),
        in_specs=[hbm] * 8,
        out_specs=hbm,
        scratch_shapes=scratch,
        compiler_params=pltpu.CompilerParams(vmem_limit_bytes=110 * 2**20),
        name="abab_stack",
    )(A_x.reshape(S, D), A_wqkv, A_wo, B_wq, B_wk, B_wv, B_wo, B_beta.reshape(1, H))
    return out.reshape(1, S, D)
```

```python
import jax
import jax.numpy as jnp
from jax import lax
import jax.experimental.pallas as pl
import jax.experimental.pallas.tpu as pltpu

S, D, H, DH = 2048, 1024, 32, 32
NSEG, L = 4, 512
HL = L // 2
NT = D // 128
NP = NT // 2
RC = HL // NP
KC = D // 2 // NP
LAST = 4 * NSEG - 1
WIN, DIL = 8, 2
HALO = 16
MZ_ROWS = 128 + 16
LOG2E = 1.4426950408889634
QSCALE = float(DH ** -0.5 * LOG2E)
MASKVAL = float(-1e9 * LOG2E)

A_MATS = (3, 0, 2, 1)
B_MATS = (2, 0, 1, 3)
B_PLAIN = (7, 7, 6, 4, 0.749, 28, 42, 0, 6, 15, 4, 9)
B_FIRST = (7, 7, 6, 4, 0.749, 28, 42, 0, 6, 15, 4, 9)
B_THEN_A = (7, 7, 6, 4, 0.749, 29, 42, 0, 7, 15, 6, 7)
B_END1 = (3, 2, 9, 3, 0.902, 30, 32, 2, 6, 15, 2, 6)
B_END2 = (4, 3, 2, 1, 0.832, 29, 28, 4, 8, 15, 6, 9)
B_STORE = 64
T_DUE = 36
A_PLAIN = (0.051, 0.047, 0.052, 0.179, 0.297, 0.638, 0.042, 0.039, 0.027, 0.292, 0.493, 0.512, 0.542, 0.553)
A_FIRST = (0.051, 0.036, 0.1, 0.227, 0.293, 0.607, 0.039, 0.04, 0.013, 0.316, 0.446, 0.473, 0.55, 0.56)
A_THEN_B = (0.055, 0.036, 0.081, 0.18, 0.246, 0.589, 0.021, 0.076, 0.062, 0.297, 0.447, 0.493, 0.503, 0.59)
A_PREP_WHEN = (0.313, 0.283, 0.373, 0.395, 0.353, 0.5, 0.556, 0.582)

F32, BF16, U32 = jnp.float32, jnp.bfloat16, jnp.uint32
_NT_DIMS = (((1,), (1,)), ((), ()))


def _iota(shape, axis):
    return lax.broadcasted_iota(jnp.int32, shape, axis)


def _dot(a, b):
    return jnp.dot(a, b, preferred_element_type=F32)


def _dot_nt(a, b):
    return lax.dot_general(a, b, _NT_DIMS, preferred_element_type=F32)


def _rows(start, size):
    return pl.ds(start if isinstance(start, int) else pl.multiple_of(start, size), size)


def _tile(k):
    return _rows(128 * k, 128)


def _words(val):
    return pltpu.bitcast(val.astype(BF16), U32)


def _bf(words):
    return pltpu.bitcast(words, BF16)


def _phi(t):
    return jnp.where(t > 0, t + 1.0, jnp.exp(t))


def _tree(op, xs):
    xs = list(xs)
    while len(xs) > 1:
        xs = [op(xs[i], xs[i + 1]) if i + 1 < len(xs) else xs[i]
              for i in range(0, len(xs), 2)]
    return xs[0]


def _fold(reduce, val):
    return reduce(val.reshape(-1, 8, 128), axis=0)


def _lhs_terms(a11, a12, a21, a22):
    return (a11 + a22, a21 + a22, a11, a22, a11 + a12, a21 - a11, a12 - a22)


def _rhs_terms(b11, b12, b21, b22):
    return (b11 + b22, b11, b12 - b22, b21 - b11, b22, b11 + b12, b21 + b22)


def _kernel(x_hbm, wqkv_hbm, awo_hbm, wq_hbm, wk_hbm, wv_hbm, wo_hbm, beta_hbm,
            out_hbm,
            x0, x1, x2, x3, wraw, wraw_o, wtmp, waq, wak, wav, wao, wb,
            xn0, xn1, o0, o1, o2,
            qa0, qa1, ka0, ka1, va0, va1,
            pq0, pq1, kb0, kb1, pk0, pk1, qt0, qt1, vt0, vt1,
            zs0, zs1, mz, beta_ref, gtab, zero_ref, sem_x, sem_w, sem_s, sem_o, sem_b):
    X = (x0, x1, x2, x3)
    XN, wa = (xn0, xn1), (waq, wak, wav)
    O = [o2 if n == LAST else (o0, o1)[n % 2] for n in range(LAST + 1)]
    QA, KA, VA = (qa0, qa1), (ka0, ka1), (va0, va1)
    QT, PQ, KB, PK, VT = (qt0, qt1), (pq0, pq1), (kb0, kb1), (pk0, pk1), (vt0, vt1)
    ZS = (zs0, zs1)

    copy = pltpu.make_async_copy

    def x_copies(s):
        return [copy(x_hbm.at[pl.ds(s * L, L)], X[s], sem_x.at[s])]

    def out_copies(s):
        return [copy(X[s], out_hbm.at[pl.ds(s * L, L)], sem_o.at[s])]

    def out_tile_copies(t0, nt):
        cols = [pl.ds(128 * (t0 + c * NP), 128 * nt) for c in range(2)]
        return [copy(x3.at[:, c], out_hbm.at[pl.ds(S - L, L), c], sem_o.at[NSEG - 1]) for c in cols]

    def wao_copies():
        return [copy(awo_hbm.at[:, _tile(t)], wraw_o.at[t], sem_w.at[4]) for t in range(NT)]

    def wb_copies(m):
        return [copy((wq_hbm, wk_hbm, wv_hbm, wo_hbm)[m], wraw.at[3 + m], sem_w.at[m])]

    def slab_copies(m, i):
        return [copy(wqkv_hbm.at[r, _rows(m * D, D)], wraw.at[m, r], sem_s.at[m, i])
                for r in (_rows(h * (D // 2) + i * KC, KC) for h in range(2))]

    def x0_copies(i):
        return [copy(x_hbm.at[r], x0.at[r], sem_s.at[3, i])
                for r in (_rows(h * HL + i * RC, RC) for h in range(2))]

    def start(cs):
        for c in cs:
            c.start()

    def wait(cs):
        for c in cs:
            c.wait()

    def token(*vals):
        val = jnp.concatenate(vals, axis=0)
        val = _fold(jnp.max, val if val.dtype == F32 else pltpu.bitcast(val, F32))
        return pltpu.bitcast(val, U32) & zero_ref[:8]

    def slabs(val, every=1):
        return [val[u - 8:u] for u in range(val.shape[0], 0, -8 * every)]

    def after(words, toks):
        parts, done = [], 0
        for k in sorted(k for k, tok in (toks or {}).items() if tok is not None):
            tok = jnp.concatenate([toks[k]] * (words.shape[1] // 128), axis=1)
            parts += [words[done:8 * k]] * (done < 8 * k) + [words[8 * k:8 * k + 8] | tok]
            done = 8 * k + 8
        parts += [words[done:]] * (done < words.shape[0])
        return jnp.concatenate(parts, axis=0)

    def store_rhs(dst, m, i, r, b11, b12, b21, b22):
        terms = _rhs_terms(*[_bf(b).astype(F32) for b in (b11, b12, b21, b22)])
        words = [{1: b11, 4: b22}[k] if k in (1, 4) else _words(v) for k, v in enumerate(terms)]
        dst[m, i, _rows(r >> 1, b11.shape[0]), :] = jnp.concatenate(words, axis=1)
        return words

    def raw_words(m, r, tiles):
        rows = [_rows(r + h * (D // 2), 32) for h in range(2)]
        return [[pltpu.bitcast(wraw[m, rr, _tile(t)], U32) for t in tiles] for rr in rows]

    def prep_b(m, i):
        def piece(j, c):
            top, bottom = raw_words(3 + m, i * KC + 32 * c, (j, j + NP))
            return store_rhs(wb, m, j, i * KC + 32 * c, *top, *bottom)

        return [lambda j=j, c=c: piece(j, c) for j in range(NP) for c in range(KC // 32)]

    def prep_a_cols(m, i):
        rows = 32
        st = {}

        def rotate(c):
            v = [jnp.concatenate(x, axis=0)
                 for x in zip(*raw_words(m, i * KC + c * rows, range(NT)))]
            st[c] = [x if t == 0 else pltpu.roll(x, 2 * t, 1) for t, x in enumerate(v)]
            return [x[24:] for x in st[c]]

        def shear(c):
            slot = (_iota((rows, 128), 1) >> 1) & 7
            v = [st[c][(-b) % NT] for b in range(NT)]
            for bit in (1, 2, 4):
                sel = (slot & bit) != 0
                v = [jnp.where(sel, v[(b - bit) % NT], v[b]) for b in range(NT)]
            st[c] = [x if b == 0 else pltpu.roll(x, 128 - 2 * b, 1) for b, x in enumerate(v)]
            return [x[16:] for x in v]

        def terms(c):
            v, half, outs = st[c], rows // 2, []
            for j in range(NP):
                outs += store_rhs(wa[m], 0, j, i * KC + c * rows, v[j][:half], v[j + NP][:half],
                                  v[j][half:], v[j + NP][half:])
            return outs

        order = [(f, k - lag) for k in range(6) for lag, f in enumerate((rotate, shear, terms))
                 if 0 <= k - lag < 4]
        return [lambda f=f, c=c: f(c) for f, c in order]

    def prep_a_rows(i):
        def stage(t):
            words = [pltpu.bitcast(wraw_o[i + h * NP, _tile(t), :], U32) for h in range(2)]
            for h in range(2):
                wtmp[h, pl.ds(65 * t, 64), :] = words[h]
            return words

        def rows(h, b, u):
            return jnp.concatenate(
                [wtmp[h, pl.ds(8 * (u + k) + b, 8, stride=65), :] for k in range(2)], axis=0)

        def piece(c, u):
            return store_rhs(wao, 0, i, 128 * c + 16 * u, rows(0, c, u), rows(1, c, u),
                             rows(0, c + NP, u), rows(1, c + NP, u))

        return ([lambda t=t: stage(t) for t in range(NT)]
                + [lambda c=c, u=u: piece(c, u) for c in range(4) for u in range(0, 8, 2)])

    def store_lhs(dst, t, r, a11, a12, a21, a22):
        words = [_words(v) for v in _lhs_terms(a11, a12, a21, a22)]
        dst[t, _rows(r >> 1, a11.shape[0] // 2), :] = jnp.concatenate(words, axis=1)
        return words

    def join(toks, slot, tok):
        if tok is not None:
            toks[slot] = tok if toks.get(slot) is None else toks[slot] | tok

    due = []

    def products(a_ref, w_ref, m, i, emit, only=None):
        st = {}

        def prod(k, toks, finish):
            toks = dict(toks or {})
            while due and due[0][0] < 16:
                slot, vals = due.pop(0)
                join(toks, slot, token(*vals))
            for entry in due:
                entry[0] -= 16
            if only is None:
                a = jnp.concatenate([after(a_ref[t, :, _tile(k)], toks if t == 0 else None)
                                     for t in range(NP)], axis=1)
                w = w_ref[m, i, :, _tile(k)]
            else:
                a = after(a_ref[only, :, _tile(k)], toks)
                w = w_ref[m, i, _rows(64 * only, 64), _tile(k)]
            r = _dot(_bf(a), _bf(w))
            finish(r)
            return r

        def p1(r):
            st["m1"] = r

        def p2(r):
            st["c21"], st["c22"] = r, st["m1"] - r

        def p3(r):
            st["c12"], st["c22"] = r, st["c22"] + r

        def p4(r):
            st["c11"] = st["m1"] + r
            emit(1, 0, st["c21"] + r)

        def p5(r):
            st["c11"] = st["c11"] - r
            emit(0, 1, st["c12"] + r)

        def p6(r):
            emit(1, 1, st["c22"] + r)

        def p7(r):
            emit(0, 0, st["c11"] + r)

        return [lambda toks, k=k, f=f: prod(k, toks, f)
                for k, f in enumerate((p1, p2, p3, p4, p5, p6, p7))]

    def ln_tasks(n, i, off, nr=16):
        src, dst = X[n % NSEG], XN[n % 2]
        st = {}

        def mean():
            x = jnp.concatenate(
                [src[_rows(i * RC + off + h * HL, nr), :].astype(F32) for h in range(2)], axis=0)
            st["x"] = [x[:, 128 * t:128 * (t + 1)] for t in range(NT)]
            part = _tree(jnp.add, st["x"])
            st["mean"] = jnp.sum(part, axis=1, keepdims=True) * (1.0 / D)
            return [part]

        def var():
            st["x"] = [x - st["mean"] for x in st["x"]]
            part = _tree(jnp.add, [x * x for x in st["x"]])
            st["var"] = jnp.sum(part, axis=1, keepdims=True) * (1.0 / D)
            return [part]

        def scale(t):
            if t == 0:
                st["inv"] = lax.rsqrt(st["var"] + 1e-5)
            y0, y1 = st["x"][t] * st["inv"], st["x"][t + NP] * st["inv"]
            return store_lhs(dst, t, i * RC + off, y0[:nr], y1[:nr], y0[nr:], y1[nr:])

        return [mean, var] + [lambda t=t: scale(t) for t in range(NP)]

    def proj_a(n, i, which, only=None):
        p = n % 2

        def emit(h, c, y):
            t = i + c * NP
            buf = (QA, KA, VA)[which]
            rows = pl.ds(h * HL + (HALO if which else 0), HL)
            if only:
                y = y + buf[p][t, rows, :]
            buf[p][t, rows, :] = y
            if which and h == 0 and n % NSEG == 0:
                buf[p][t, pl.ds(0, HALO), :] = jnp.zeros((HALO, 128), F32)
            elif which and h == 0:
                buf[p][t, pl.ds(0, HALO), :] = buf[1 - p][t, pl.ds(L, HALO), :]

        return products(XN[p], wa[which], 0, i, emit, only)

    def proj_b(n, i, which):
        p = n % 2

        def transposed(buf, h, c, y):
            words = pltpu.bitcast(y.astype(BF16).T, U32)
            buf[p][i + c * NP, :, pl.ds(h * HL, HL)] = words
            due.append([T_DUE, slabs(words[:, :128], 2) + slabs(words[:, 128:], 2)])

        def emit(h, c, y):
            wide = (i, pl.ds(h * HL // 2, HL // 2), _tile(c))
            if which == 0:
                if n % NSEG:
                    PQ[p][wide] = _words(_phi(y))
                y = y * QSCALE
                flip = jnp.concatenate([y[r ^ 96:(r ^ 96) + 32] for r in range(0, HL, 32)], axis=0)
                y = jnp.where((_iota(y.shape, 1) & 32) == 0, y, flip)
                transposed(QT, h, c, y)
            elif which == 1:
                KB[p][wide] = _words(y)
                if n % NSEG != NSEG - 1:
                    y = _phi(y)
                    PK[p][wide] = _words(y)
                    ZS[p][i + c * NP, pl.ds(8 * h, 8), :] = _fold(jnp.sum, y)
            else:
                transposed(VT, h, c, y)

        return products(XN[p], wb, which, i, emit)

    def out_stage(n, i):
        x = X[n % NSEG]

        def emit(h, c, y):
            where = (pl.ds(h * HL, HL), _tile(i + c * NP))
            x[where] = (x[where].astype(F32) + y).astype(BF16)

        if is_a(n):
            return products(O[n], wao, 0, i, emit)
        return products(O[n], wb, 3, i, emit)

    def att_a_tasks(n, i, off, times):
        p = n % 2
        base = pl.multiple_of(i * RC, RC) + off
        starts = [base + (u // 2) * HL + 8 * (u % 2) for u in range(4)]
        lg, mixed = [[] for _ in range(4)], {}

        def scores(u, ws):
            q = QA[p][:, pl.ds(starts[u], 8), :]
            for w in ws:
                k = KA[p][:, pl.ds(starts[u] + (HALO - DIL * w), 8), :]
                lg[u].append(jnp.sum(q * k, axis=0))
            return lg[u][-len(ws):]

        def exchange(u, bit):
            a = jnp.concatenate(lg[u], axis=0)
            low = (_iota(a.shape, 1) & bit) == 0
            lg[u] = [a + jnp.where(low, pltpu.roll(a, 128 - bit, 1), pltpu.roll(a, bit, 1))]
            return lg[u]

        def softmax(u):
            v = (lg[u][0] * QSCALE).reshape(WIN, 8, 128)
            if n % NSEG == 0 and off == 0 and u < 2:
                pos = _iota(v.shape, 1) + starts[u]
                v = jnp.where(pos >= DIL * _iota(v.shape, 0), v, MASKVAL)
            e = jnp.exp2(v - jnp.max(v, axis=0, keepdims=True))
            lg[u] = e * (1.0 / jnp.sum(e, axis=0, keepdims=True))
            return [lg[u].reshape(8 * WIN, 128)]

        def mix(t, h):
            rows = [pl.ds(starts[2 * h] + (HALO - DIL * w), 16) for w in range(WIN)]
            prob = jnp.concatenate([lg[2 * h], lg[2 * h + 1]], axis=1)
            for c in range(2):
                v = jnp.stack([VA[p][t + c * NP, r, :] for r in rows])
                mixed[t, h, c] = jnp.sum(prob * v, axis=0)
            return [mixed[t, h, c] for c in range(2)]

        def store(t):
            return store_lhs(O[n], t, i * RC + off,
                             *[mixed[t, h, c] for h in range(2) for c in range(2)])

        t_score, d_score, lag1, lag2, lag3, t_mix, d_mix, d_store = times
        tasks = []
        for u in range(4):
            t = t_score + d_score * (2 * u + 1)
            tasks += [(t - d_score, lambda u=u: scores(u, range(4))),
                      (t, lambda u=u: scores(u, range(4, 8))),
                      (t + lag1, lambda u=u: exchange(u, 1)),
                      (t + lag2, lambda u=u: exchange(u, 16)),
                      (t + lag3, lambda u=u: softmax(u))]
        for k in range(NP):
            t = t_mix + k * (d_mix + d_store)
            tasks += [(t, lambda k=k: mix(k, 0)), (t + d_mix, lambda k=k: mix(k, 1))]
            tasks += [(t + d_mix + d_store / 2, lambda k=k: store(k))]
        return tasks

    def att_b_piece(n, i, j, mem, tok):
        p = n % 2
        nk = 128 * j + 32
        shared = ((32, 1, 3), (64, 2, 2), (96, 3, 1))
        key, lane = _iota((32, 128), 0), _iota((32, 128), 1)
        causal = [jnp.where(key > q, MASKVAL, 0.0) for q in (lane, lane ^ 96)]
        even = [_iota((8, 128), 1) >= lo for lo, _, _ in shared]

        def place(parts):
            zero = jnp.zeros((16, 128), U32)
            return jnp.concatenate([parts.get(hh, zero) for hh in range(4)], axis=0)

        q = [[after(QT[p][i + h * NP, pl.ds(16 * hh, 16), _tile(j)], {0: tok}) for hh in range(4)]
             for h in range(2)]
        s = []
        for h in range(2):
            w = jnp.concatenate([place({hh: q[h][hh]}) for hh in range(4)], axis=1)
            st = _dot(_bf(KB[p][i, pl.ds(0, nk // 2), _tile(h)]), _bf(w))
            for hh in range(4):
                v = st[:, 128 * hh:128 * (hh + 1)]
                s.append([v[128 * c:128 * (c + 1)] for c in range(j)]
                         + [v[128 * j:] + causal[hh % 2]])
        sx = [[] for _ in range(4)]
        for lo, ce, co in shared:
            ahead = jnp.where(lane >= lo, key + 32 * ce - lane, key + 32 * co - (lane ^ 96))
            mask = jnp.where(ahead > 0, MASKVAL, 0.0)
            high = _iota((16, 128), 1) >= lo
            for h in range(2):
                ke, ko = (KB[p][i, pl.ds(64 * j + 16 * c, 16), _tile(h)] for c in (ce, co))
                k = ke if ce == co else jnp.where((_iota((16, 128), 1) & 32) == 0, ke, ko)
                w = jnp.concatenate(
                    [place({hh: jnp.where(high, q[h][hh], jnp.uint32(0)),
                            hh + 1: jnp.where(high, jnp.uint32(0), q[h][hh + 1])})
                     for hh in (0, 2)], axis=1)
                st = _dot(_bf(k), _bf(w))
                for u in range(2):
                    sx[2 * h + u].append(st[:, 128 * u:128 * (u + 1)] + mask)
        first = token(*[v[0][:8] for v in s])
        m = []
        for u in range(4):
            a = [_tree(jnp.maximum, [_fold(jnp.max, v) for v in s[2 * u + odd]]) for odd in range(2)]
            for sel, v in zip(even, sx[u]):
                mx = _fold(jnp.max, v)
                a = [jnp.where(sel, jnp.maximum(a[0], mx), a[0]),
                     jnp.where(sel, a[1], jnp.maximum(a[1], mx))]
            m += [jnp.broadcast_to(jnp.max(v, axis=0, keepdims=True), (8, 128)) for v in a]
        e = [[] for _ in range(8)]
        part = [[] for _ in range(8)]

        def exps(v, mh, tok):
            mh = mh + pltpu.bitcast(tok, F32)
            return jnp.exp2(v.reshape(-1, 8, 128) - mh[None]).reshape(v.shape)

        def collect(u, v):
            part[u] = [_tree(jnp.add, part[u] + [_fold(jnp.sum, v)])]
            e[u].append(v)

        def exp_tile(u, c, tok):
            collect(u, exps(s[u][c], m[u], tok))

        def exp_diag(u, tok):
            for odd in range(2):
                exp_tile(2 * u + odd, j, tok)
            v = [exps(a, jnp.where(sel, m[2 * u], m[2 * u + 1]), tok) for sel, a in zip(even, sx[u])]
            collect(2 * u, jnp.concatenate(
                [jnp.where(lane >= shared[c][0], v[c], 0.0) for c in (0, 1, 2)], axis=0))
            collect(2 * u + 1, jnp.concatenate(
                [jnp.where(lane >= shared[c][0], 0.0, v[c]) for c in (2, 1, 0)], axis=0))

        def finish(h, tok):
            g = i + h * NP
            ot = []
            for hh in range(4):
                u = 4 * h + hh
                vt = after(VT[p][g, pl.ds(16 * hh, 16), pl.ds(0, 128 * (j + 1))], {0: tok})
                acc = _dot(_bf(vt), jnp.concatenate(e[u], axis=0).astype(BF16))
                l = jnp.sum(part[u][0], axis=0, keepdims=True)
                gate = gtab[pl.ds(4 * g + hh, 1), :]
                acc = acc * ((1.0 - gate) / l)
                if hh % 2:
                    acc = jnp.where((lane & 32) == 0, pltpu.roll(acc, 32, 1), pltpu.roll(acc, 96, 1))
                if n % NSEG:
                    r = mem[h][:, 128 * j:128 * (j + 1)]
                    den = r[128 + 4 * hh:129 + 4 * hh] + 1e-6
                    acc = acc + r[32 * hh:32 * hh + 32] * (gate / den)
                ot.append(acc)
            return ot

        tasks = []
        for u in range(4):
            tasks += [lambda tok, u=2 * u + odd, c=c: exp_tile(u, c, tok)
                      for odd in range(2) for c in range(j)]
            tasks.append(lambda tok, u=u: exp_diag(u, tok))
        return first, tasks, finish

    def mem_load(n, g):
        if n % NSEG == 0:
            return jnp.zeros((MZ_ROWS, 128), F32)
        return mz[g]

    def mem_read(n, i, h, state, tok):
        pq = after(PQ[n % 2][i, :, _tile(h)], {8 * u: tok for u in range(4)})
        return _dot_nt(state.astype(BF16), _bf(pq))

    def mem_update(n, i, h, state, tok):
        p, g = n % 2, i + h * NP
        z = jnp.sum(ZS[p][g], axis=0, keepdims=True)
        new = jnp.concatenate([_dot(_bf(after(VT[p][g], {0: tok})), _bf(PK[p][i, :, _tile(h)])),
                               jnp.broadcast_to(z, (MZ_ROWS - 128, 128))], axis=0)
        row = _iota((MZ_ROWS, 128), 0)
        row_head = jnp.where(row < 128, row >> 5, (row - 128) >> 2)
        keep = row_head == (_iota((MZ_ROWS, 128), 1) >> 5)
        mz[g] = new = state + jnp.where(keep, new, 0.0)
        return new

    def is_a(n):
        return (n // NSEG) % 2 == 0

    def run_timed(mm, tasks):
        tasks = sorted(tasks, key=lambda x: x[0])
        for k, prod in enumerate(mm):
            toks = {}
            while tasks and tasks[0][0] < 16 * (k + 1):
                time, f = tasks.pop(0)
                join(toks, time - 16 * k, token(*f()))
            prod(toks)
        for _, f in tasks:
            f()

    def body_b(n, i, mm, ln):
        times = {LAST - 1: B_END1, LAST: B_END2}.get(
            n, (B_FIRST, B_PLAIN, B_PLAIN, B_THEN_A)[n % NSEG])
        share, (front, lag, tail, pitch) = times[:4], times[4:8]
        state = [mem_load(n, i + h * NP) for h in range(2)]
        late = [f for off in range(0, RC, 16) for f in ln_tasks(n + 2, i, off)] if ln else []
        mem, tiles, done = [], {}, []

        def values(j, finish, tok):
            posts = []
            for h in range(2):
                ot = finish(h, tok)

                def post(ot=ot, h=h):
                    tiles[j, h] = jnp.concatenate(ot, axis=0).T
                    return slabs(tiles[j, h], 4)

                posts.append(post)
            if j < 2:
                posts += [lambda r=r: store_lhs(
                    O[n], i, 128 * j + r,
                    *[tiles[j + u, h][r:r + B_STORE] for u in (0, 2) for h in range(2)])
                    for r in range(0, 128, B_STORE)]
            return posts

        tok, pending = token(mm.pop(0)(None)[:8]), None
        for k, j in enumerate((3, 1, 2, 0)):
            first, exps, finish = att_b_piece(n, i, j, mem, tok)
            done += values(*pending, first) if pending else []
            when = [int(32 * share[k] * front * u / len(exps)) for u in range(len(exps))]
            for c in range(share[k]):
                toks = {0: first} if c == 0 else {}
                for slot in times[8:10]:
                    if done and 16 * c + slot >= min(lag, 16 * share[k] - 1):
                        join(toks, slot, token(*done.pop(0)()))
                for slot in times[10:11 if len(late) % 6 in (0, 5) else 12]:
                    if late:
                        join(toks, slot, token(*late.pop(0)()))
                r = mm.pop(0)(toks)
                while exps and when[0] < 32 * (c + 1):
                    exps.pop(0)(token(r[8 * (when[0] - 32 * c):][:8]))
                    when.pop(0)
                tok = token(r[:8])
                if (k, c) == (0, 0) and n % NSEG:
                    mem.extend(mem_read(n, i, h, state[h], tok) for h in range(2))
                    done.append(lambda: [v[:8, 128 * u:128 * u + 128] for v in mem for u in range(4)])
                if (k, c) == (0, 0) and n % NSEG != NSEG - 1:
                    new = [mem_update(n, i, h, state[h], tok) for h in range(2)]
                    done.append(lambda: [v[:8] for v in new])
            pending = (j, finish)
        done += late + values(*pending, token(mm.pop(0)(None)[:8]))
        run_timed(mm, [(tail + pitch * u, f) for u, f in enumerate(done)])

    def step(n, ln=True, proj=(0, 1, 2), att=True, out=(1,), extra=None):
        @pl.loop(0, NP)
        def _(i):
            mm = []
            due.clear()
            for which in (B_MATS if att and not is_a(n) else A_MATS):
                if which in proj:
                    mm += (proj_a if is_a(n + 1) else proj_b)(n + 1, i, which)
                elif which == 3:
                    mm += [f for lag in out for f in out_stage(n - lag, i)]
            if att and not is_a(n):
                body_b(n, i, mm, ln)
                return
            times = A_FIRST if n == 0 else A_PLAIN if is_a(n + 1) else A_THEN_B
            fs = extra(i) if extra else []
            tasks = [(u % 4 + A_PREP_WHEN[u // 4] if att else 4 * (u + 1) / (len(fs) + 1), f)
                     for u, f in enumerate(fs)]
            for u, off in enumerate(range(0, RC, 16)):
                if att:
                    tasks += [(u + w, f) for w, f in att_a_tasks(n, i, off, times[:8])]
                if ln:
                    when = times[8:] if att else (.2, .6, 1.0, 1.15, 1.3, 1.45)
                    tasks += [(u + w, f) for w, f in zip(when, ln_tasks(n + 2, i, off))]
            run_timed(mm, [(int(4 * len(mm) * w), f) for w, f in tasks])

    for i in range(NP):
        start(x0_copies(i))
    start(slab_copies(0, 0))
    start([copy(beta_hbm, beta_ref.at[0], sem_b)])
    zero_ref[:8] = jnp.zeros((8, 128), U32)

    @pl.loop(0, NP)
    def _(i):
        pl.when(i == 2)(lambda: start(slab_copies(0, 1)))
        wait(x0_copies(i))
        for fs in zip(*[ln_tasks(0, i, off) for off in range(0, RC, 16)]):
            for f in fs:
                f()

    start(slab_copies(0, 2))
    wait(slab_copies(0, 0))
    for f in prep_a_cols(0, 0):
        f()

    plan = (([(0, 3), (1, 0)], [(0, 1)]), ([(1, 1), (1, 2)], [(0, 2), (0, 3)]),
            ([(1, 3), (2, 0)], [(1, 0), (1, 1)]), ([(2, 1), (2, 2)], [(1, 2), (1, 3)]))
    for t, (fetch, preps) in enumerate(plan):
        for mi in fetch:
            start(slab_copies(*mi))
        for mi in preps:
            wait(slab_copies(*mi))
        mm = [f for i in range(NP) for f in proj_a(0, i, 0, only=t)]
        fs = [f for group in zip(*[prep_a_cols(*mi) for mi in preps]) for f in group]
        run_timed(mm, [(16 * len(mm) * (u + 1) // (len(fs) + 1), f) for u, f in enumerate(fs)])

    def prep_wv(i):
        pl.when(i == 0)(lambda: start(x_copies(1) + wao_copies()))
        wait(slab_copies(2, i))
        return prep_a_cols(2, i)

    start(slab_copies(2, 3))
    step(-1, ln=False, proj=(1,), att=False, out=(), extra=prep_wv)
    start(x_copies(2))
    start(x_copies(3))
    wait(x_copies(1))
    wait(wao_copies())
    step(-1, proj=(2,), att=False, out=(), extra=prep_a_rows)
    for m in range(4):
        start(wb_copies(m))
    wait([copy(beta_hbm, beta_ref.at[0], sem_b)])
    gate = jax.nn.sigmoid(beta_ref[0].astype(F32))
    eye = _iota((H, H), 0) == _iota((H, H), 1)
    gcol = jnp.sum(jnp.where(eye, jnp.broadcast_to(gate, (H, H)), 0.0), axis=1, keepdims=True)
    gtab[...] = jnp.broadcast_to(gcol, (H, 128))
    wait(x_copies(2))
    step(0, out=())
    wait(x_copies(3))
    for m in range(4):
        wait(wb_copies(m))
    step(1, extra=lambda i: prep_b(0, i) + prep_b(1, i))
    step(2, extra=lambda i: prep_b(2, i) + prep_b(3, i))
    for n in range(3, 14):
        step(n)
    start(out_copies(0))
    step(14, ln=False, out=())
    step(15, ln=False, proj=(), out=(2, 1))
    start(out_copies(1))
    start(out_copies(2))
    due.clear()
    for i in range(NP):
        run_timed(out_stage(LAST, i), [])
        if i >= NP - 2:
            start(out_tile_copies(0, NP - 1) if i == NP - 2 else out_tile_copies(i, 1))
    for s in range(NSEG - 1):
        wait(out_copies(s))
    wait(out_tile_copies(0, NP - 1) + out_tile_copies(NP - 1, 1))


@jax.jit
def pallas_interleave_layers__sliding_local_dilated__memory_aug_infini_attn__prompt_kernel(
    A_x: jax.Array,
    A_wqkv: jax.Array,
    A_wo: jax.Array,
    B_x: jax.Array,
    B_wq: jax.Array,
    B_wk: jax.Array,
    B_wv: jax.Array,
    B_wo: jax.Array,
    B_beta: jax.Array,
):
    del B_x
    assert A_x.shape == (1, S, D)
    hbm = pl.BlockSpec(memory_space=pl.ANY)
    scratch = (
        [pltpu.VMEM((L, D), BF16)] * 4
        + [pltpu.VMEM((7, D, D), BF16), pltpu.VMEM((NT, D, 128), BF16),
           pltpu.VMEM((2, 576, 128), U32),
           *[pltpu.VMEM((1, NP, D // 4, 7 * 128), U32)] * 4,
           pltpu.VMEM((4, NP, D // 4, 7 * 128), U32)]
        + [pltpu.VMEM((NP, HL // 2, 7 * 128), U32)] * 5
        + [pltpu.VMEM((NT, L, 128), F32)] * 2
        + [pltpu.VMEM((NT, HALO + L, 128), F32)] * 4
        + [pltpu.VMEM((NP, L // 2, 2 * 128), U32)] * 6
        + [pltpu.VMEM((NT, 64, L), U32)] * 4
        + [pltpu.VMEM((NT, 16, 128), F32)] * 2
        + [pltpu.VMEM((NT, MZ_ROWS, 128), F32), pltpu.VMEM((8, 1, H), BF16),
           pltpu.VMEM((H, 128), F32),
           pltpu.VMEM((88, 128), U32),
           pltpu.SemaphoreType.DMA((NSEG,)), pltpu.SemaphoreType.DMA((5,)),
           pltpu.SemaphoreType.DMA((4, NP)),
           pltpu.SemaphoreType.DMA((NSEG,)), pltpu.SemaphoreType.DMA]
    )
    out = pl.pallas_call(
        _kernel,
        out_shape=jax.ShapeDtypeStruct((S, D), BF16),
        in_specs=[hbm] * 8,
        out_specs=hbm,
        scratch_shapes=scratch,
        compiler_params=pltpu.CompilerParams(vmem_limit_bytes=110 * 2**20),
        name="abab_stack",
    )(A_x.reshape(S, D), A_wqkv, A_wo, B_wq, B_wk, B_wv, B_wo, B_beta.reshape(1, H))
    return out.reshape(1, S, D)
```

```python
import jax
import jax.numpy as jnp
from jax import lax
import jax.experimental.pallas as pl
import jax.experimental.pallas.tpu as pltpu

S, D, H, DH = 2048, 1024, 32, 32
NSEG, L = 4, 512
HL = L // 2
NT = D // 128
NP = NT // 2
RC = HL // NP
KC = D // 2 // NP
LAST = 4 * NSEG - 1
WIN, DIL = 8, 2
HALO = 16
MZ_ROWS = 128 + 16
LOG2E = 1.4426950408889634
QSCALE = float(DH ** -0.5 * LOG2E)
MASKVAL = float(-1e9 * LOG2E)

A_MATS = (3, 0, 2, 1)
B_MATS = (2, 0, 1, 3)
B_PLAIN = (7, 6, 7, 4, 0.742, 26, 44, 2, 6, 13, 4, 8)
B_FIRST = (7, 7, 6, 4, 0.749, 26, 42, 0, 7, 15, 4, 9)
B_THEN_A = (7, 7, 6, 3, 0.794, 27, 42, 0, 8, 15, 6, 8)
B_END1 = (3, 2, 9, 3, 0.897, 30, 32, 1, 4, 15, 1, 8)
B_END2 = (4, 3, 2, 1, 0.835, 29, 28, 3, 7, 14, 5, 13)
B_STORE = 64
T_DUE = 36
A_PLAIN = (0.051, 0.047, 0.052, 0.179, 0.297, 0.638, 0.042, 0.039, 0.027, 0.292, 0.493, 0.512, 0.542, 0.553)
A_FIRST = (0.051, 0.036, 0.1, 0.227, 0.293, 0.607, 0.039, 0.04, 0.013, 0.316, 0.446, 0.473, 0.55, 0.56)
A_THEN_B = (0.055, 0.036, 0.081, 0.18, 0.246, 0.589, 0.021, 0.076, 0.062, 0.297, 0.447, 0.493, 0.503, 0.59)
A_PREP = (0.051, 0.047, 0.052, 0.179, 0.297, 0.65, 0.025, 0.039, 0.027, 0.292, 0.512, 0.519, 0.542, 0.553)
A_PREP_WHEN = (0.313, 0.283, 0.412, 0.447, 0.343, 0.481, 0.556, 0.582)

F32, BF16, U32 = jnp.float32, jnp.bfloat16, jnp.uint32
_NT_DIMS = (((1,), (1,)), ((), ()))


def _iota(shape, axis):
    return lax.broadcasted_iota(jnp.int32, shape, axis)


def _dot(a, b):
    return jnp.dot(a, b, preferred_element_type=F32)


def _dot_nt(a, b):
    return lax.dot_general(a, b, _NT_DIMS, preferred_element_type=F32)


def _rows(start, size):
    return pl.ds(start if isinstance(start, int) else pl.multiple_of(start, size), size)


def _tile(k):
    return _rows(128 * k, 128)


def _words(val):
    return pltpu.bitcast(val.astype(BF16), U32)


def _bf(words):
    return pltpu.bitcast(words, BF16)


def _phi(t):
    return jnp.where(t > 0, t + 1.0, jnp.exp(t))


def _tree(op, xs):
    xs = list(xs)
    while len(xs) > 1:
        xs = [op(xs[i], xs[i + 1]) if i + 1 < len(xs) else xs[i]
              for i in range(0, len(xs), 2)]
    return xs[0]


def _fold(reduce, val):
    return reduce(val.reshape(-1, 8, 128), axis=0)


def _lhs_terms(a11, a12, a21, a22):
    return (a11 + a22, a21 + a22, a11, a22, a11 + a12, a21 - a11, a12 - a22)


def _rhs_terms(b11, b12, b21, b22):
    return (b11 + b22, b11, b12 - b22, b21 - b11, b22, b11 + b12, b21 + b22)


def _kernel(x_hbm, wqkv_hbm, awo_hbm, wq_hbm, wk_hbm, wv_hbm, wo_hbm, beta_hbm,
            out_hbm,
            x0, x1, x2, x3, wraw, wraw_o, wtmp, waq, wak, wav, wao, wb,
            xn0, xn1, o0, o1, o2,
            qa0, qa1, ka0, ka1, va0, va1,
            pq0, pq1, kb0, kb1, pk0, pk1, qt0, qt1, vt0, vt1,
            zs0, zs1, mz, beta_ref, gtab, zero_ref, sem_x, sem_w, sem_s, sem_o, sem_b):
    X = (x0, x1, x2, x3)
    XN, wa = (xn0, xn1), (waq, wak, wav)
    O = [o2 if n == LAST else (o0, o1)[n % 2] for n in range(LAST + 1)]
    QA, KA, VA = (qa0, qa1), (ka0, ka1), (va0, va1)
    QT, PQ, KB, PK, VT = (qt0, qt1), (pq0, pq1), (kb0, kb1), (pk0, pk1), (vt0, vt1)
    ZS = (zs0, zs1)

    copy = pltpu.make_async_copy

    def x_copies(s):
        return [copy(x_hbm.at[pl.ds(s * L, L)], X[s], sem_x.at[s])]

    def out_copies(s):
        return [copy(X[s], out_hbm.at[pl.ds(s * L, L)], sem_o.at[s])]

    def out_tile_copies(t0, nt):
        cols = [pl.ds(128 * (t0 + c * NP), 128 * nt) for c in range(2)]
        return [copy(x3.at[:, c], out_hbm.at[pl.ds(S - L, L), c], sem_o.at[NSEG - 1]) for c in cols]

    def wao_copies():
        return [copy(awo_hbm.at[:, _tile(t)], wraw_o.at[t], sem_w.at[4]) for t in range(NT)]

    def wb_copies(m):
        return [copy((wq_hbm, wk_hbm, wv_hbm, wo_hbm)[m], wraw.at[3 + m], sem_w.at[m])]

    def slab_copies(m, i):
        return [copy(wqkv_hbm.at[r, _rows(m * D, D)], wraw.at[m, r], sem_s.at[m, i])
                for r in (_rows(h * (D // 2) + i * KC, KC) for h in range(2))]

    def x0_copies(i):
        return [copy(x_hbm.at[r], x0.at[r], sem_s.at[3, i])
                for r in (_rows(h * HL + i * RC, RC) for h in range(2))]

    def start(cs):
        for c in cs:
            c.start()

    def wait(cs):
        for c in cs:
            c.wait()

    def token(*vals):
        val = jnp.concatenate(vals, axis=0)
        val = _fold(jnp.max, val if val.dtype == F32 else pltpu.bitcast(val, F32))
        return pltpu.bitcast(val, U32) & zero_ref[:8]

    def slabs(val, every=1):
        return [val[u - 8:u] for u in range(val.shape[0], 0, -8 * every)]

    def after(words, toks):
        parts, done = [], 0
        for k in sorted(k for k, tok in (toks or {}).items() if tok is not None):
            tok = jnp.concatenate([toks[k]] * (words.shape[1] // 128), axis=1)
            parts += [words[done:8 * k]] * (done < 8 * k) + [words[8 * k:8 * k + 8] | tok]
            done = 8 * k + 8
        parts += [words[done:]] * (done < words.shape[0])
        return jnp.concatenate(parts, axis=0)

    def store_rhs(dst, m, i, r, b11, b12, b21, b22):
        terms = _rhs_terms(*[_bf(b).astype(F32) for b in (b11, b12, b21, b22)])
        words = [{1: b11, 4: b22}[k] if k in (1, 4) else _words(v) for k, v in enumerate(terms)]
        dst[m, i, _rows(r >> 1, b11.shape[0]), :] = jnp.concatenate(words, axis=1)
        return words

    def raw_words(m, r, tiles):
        rows = [_rows(r + h * (D // 2), 32) for h in range(2)]
        return [[pltpu.bitcast(wraw[m, rr, _tile(t)], U32) for t in tiles] for rr in rows]

    def prep_b(m, i):
        def piece(j, c):
            top, bottom = raw_words(3 + m, i * KC + 32 * c, (j, j + NP))
            return store_rhs(wb, m, j, i * KC + 32 * c, *top, *bottom)

        return [lambda j=j, c=c: piece(j, c) for j in range(NP) for c in range(KC // 32)]

    def prep_a_cols(m, i):
        rows = 32
        st = {}

        def rotate(c):
            v = [jnp.concatenate(x, axis=0)
                 for x in zip(*raw_words(m, i * KC + c * rows, range(NT)))]
            st[c] = [x if t == 0 else pltpu.roll(x, 2 * t, 1) for t, x in enumerate(v)]
            return [x[24:] for x in st[c]]

        def shear(c):
            slot = (_iota((rows, 128), 1) >> 1) & 7
            v = [st[c][(-b) % NT] for b in range(NT)]
            for bit in (1, 2, 4):
                sel = (slot & bit) != 0
                v = [jnp.where(sel, v[(b - bit) % NT], v[b]) for b in range(NT)]
            st[c] = [x if b == 0 else pltpu.roll(x, 128 - 2 * b, 1) for b, x in enumerate(v)]
            return [x[16:] for x in v]

        def terms(c):
            v, half, outs = st[c], rows // 2, []
            for j in range(NP):
                outs += store_rhs(wa[m], 0, j, i * KC + c * rows, v[j][:half], v[j + NP][:half],
                                  v[j][half:], v[j + NP][half:])
            return outs

        order = [(f, k - lag) for k in range(6) for lag, f in enumerate((rotate, shear, terms))
                 if 0 <= k - lag < 4]
        return [lambda f=f, c=c: f(c) for f, c in order]

    def prep_a_rows(i):
        def stage(t):
            words = [pltpu.bitcast(wraw_o[i + h * NP, _tile(t), :], U32) for h in range(2)]
            for h in range(2):
                wtmp[h, pl.ds(65 * t, 64), :] = words[h]
            return words

        def rows(h, b, u):
            return jnp.concatenate(
                [wtmp[h, pl.ds(8 * (u + k) + b, 8, stride=65), :] for k in range(2)], axis=0)

        def piece(c, u):
            return store_rhs(wao, 0, i, 128 * c + 16 * u, rows(0, c, u), rows(1, c, u),
                             rows(0, c + NP, u), rows(1, c + NP, u))

        return ([lambda t=t: stage(t) for t in range(NT)]
                + [lambda c=c, u=u: piece(c, u) for c in range(4) for u in range(0, 8, 2)])

    def store_lhs(dst, t, r, a11, a12, a21, a22):
        words = [_words(v) for v in _lhs_terms(a11, a12, a21, a22)]
        dst[t, _rows(r >> 1, a11.shape[0] // 2), :] = jnp.concatenate(words, axis=1)
        return words

    def join(toks, slot, tok):
        if tok is not None:
            toks[slot] = tok if toks.get(slot) is None else toks[slot] | tok

    due = []

    def products(a_ref, w_ref, m, i, emit, only=None):
        st = {}

        def prod(k, toks, finish):
            toks = dict(toks or {})
            while due and due[0][0] < 16:
                slot, vals = due.pop(0)
                join(toks, slot, token(*vals))
            for entry in due:
                entry[0] -= 16
            if only is None:
                a = jnp.concatenate([after(a_ref[t, :, _tile(k)], toks if t == 0 else None)
                                     for t in range(NP)], axis=1)
                w = w_ref[m, i, :, _tile(k)]
            else:
                a = after(a_ref[only, :, _tile(k)], toks)
                w = w_ref[m, i, _rows(64 * only, 64), _tile(k)]
            r = _dot(_bf(a), _bf(w))
            finish(r)
            return r

        def p1(r):
            st["m1"] = r

        def p2(r):
            st["c21"], st["c22"] = r, st["m1"] - r

        def p3(r):
            st["c12"], st["c22"] = r, st["c22"] + r

        def p4(r):
            st["c11"] = st["m1"] + r
            emit(1, 0, st["c21"] + r)

        def p5(r):
            st["c11"] = st["c11"] - r
            emit(0, 1, st["c12"] + r)

        def p6(r):
            emit(1, 1, st["c22"] + r)

        def p7(r):
            emit(0, 0, st["c11"] + r)

        return [lambda toks, k=k, f=f: prod(k, toks, f)
                for k, f in enumerate((p1, p2, p3, p4, p5, p6, p7))]

    def ln_tasks(n, i, off, nr=16):
        src, dst = X[n % NSEG], XN[n % 2]
        st = {}

        def mean():
            x = jnp.concatenate(
                [src[_rows(i * RC + off + h * HL, nr), :].astype(F32) for h in range(2)], axis=0)
            st["x"] = [x[:, 128 * t:128 * (t + 1)] for t in range(NT)]
            part = _tree(jnp.add, st["x"])
            st["mean"] = jnp.sum(part, axis=1, keepdims=True) * (1.0 / D)
            return [part]

        def var():
            st["x"] = [x - st["mean"] for x in st["x"]]
            part = _tree(jnp.add, [x * x for x in st["x"]])
            st["var"] = jnp.sum(part, axis=1, keepdims=True) * (1.0 / D)
            return [part]

        def scale(t):
            if t == 0:
                st["inv"] = lax.rsqrt(st["var"] + 1e-5)
            y0, y1 = st["x"][t] * st["inv"], st["x"][t + NP] * st["inv"]
            return store_lhs(dst, t, i * RC + off, y0[:nr], y1[:nr], y0[nr:], y1[nr:])

        return [mean, var] + [lambda t=t: scale(t) for t in range(NP)]

    def proj_a(n, i, which, only=None):
        p = n % 2

        def emit(h, c, y):
            t = i + c * NP
            buf = (QA, KA, VA)[which]
            rows = pl.ds(h * HL + (HALO if which else 0), HL)
            if only:
                y = y + buf[p][t, rows, :]
            buf[p][t, rows, :] = y
            if which and h == 0 and n % NSEG == 0:
                buf[p][t, pl.ds(0, HALO), :] = jnp.zeros((HALO, 128), F32)
            elif which and h == 0:
                buf[p][t, pl.ds(0, HALO), :] = buf[1 - p][t, pl.ds(L, HALO), :]

        return products(XN[p], wa[which], 0, i, emit, only)

    def proj_b(n, i, which):
        p = n % 2

        def transposed(buf, h, c, y):
            words = pltpu.bitcast(y.astype(BF16).T, U32)
            buf[p][i + c * NP, :, pl.ds(h * HL, HL)] = words
            due.append([T_DUE, slabs(words[:, :128], 2) + slabs(words[:, 128:], 2)])

        def emit(h, c, y):
            wide = (i, pl.ds(h * HL // 2, HL // 2), _tile(c))
            if which == 0:
                if n % NSEG:
                    PQ[p][wide] = _words(_phi(y))
                y = y * QSCALE
                flip = jnp.concatenate([y[r ^ 96:(r ^ 96) + 32] for r in range(0, HL, 32)], axis=0)
                y = jnp.where((_iota(y.shape, 1) & 32) == 0, y, flip)
                transposed(QT, h, c, y)
            elif which == 1:
                KB[p][wide] = _words(y)
                if n % NSEG != NSEG - 1:
                    y = _phi(y)
                    PK[p][wide] = _words(y)
                    ZS[p][i + c * NP, pl.ds(8 * h, 8), :] = _fold(jnp.sum, y)
            else:
                transposed(VT, h, c, y)

        return products(XN[p], wb, which, i, emit)

    def out_stage(n, i):
        x = X[n % NSEG]

        def emit(h, c, y):
            where = (pl.ds(h * HL, HL), _tile(i + c * NP))
            x[where] = (x[where].astype(F32) + y).astype(BF16)

        if is_a(n):
            return products(O[n], wao, 0, i, emit)
        return products(O[n], wb, 3, i, emit)

    def att_a_tasks(n, i, off, times):
        p = n % 2
        base = pl.multiple_of(i * RC, RC) + off
        starts = [base + (u // 2) * HL + 8 * (u % 2) for u in range(4)]
        lg, mixed = [[] for _ in range(4)], {}

        def scores(u, ws):
            q = QA[p][:, pl.ds(starts[u], 8), :]
            for w in ws:
                k = KA[p][:, pl.ds(starts[u] + (HALO - DIL * w), 8), :]
                lg[u].append(jnp.sum(q * k, axis=0))
            return lg[u][-len(ws):]

        def exchange(u, bit):
            a = jnp.concatenate(lg[u], axis=0)
            low = (_iota(a.shape, 1) & bit) == 0
            lg[u] = [a + jnp.where(low, pltpu.roll(a, 128 - bit, 1), pltpu.roll(a, bit, 1))]
            return lg[u]

        def softmax(u):
            v = (lg[u][0] * QSCALE).reshape(WIN, 8, 128)
            if n % NSEG == 0 and off == 0 and u < 2:
                pos = _iota(v.shape, 1) + starts[u]
                v = jnp.where(pos >= DIL * _iota(v.shape, 0), v, MASKVAL)
            e = jnp.exp2(v - jnp.max(v, axis=0, keepdims=True))
            lg[u] = e * (1.0 / jnp.sum(e, axis=0, keepdims=True))
            return [lg[u].reshape(8 * WIN, 128)]

        def mix(t, h):
            rows = [pl.ds(starts[2 * h] + (HALO - DIL * w), 16) for w in range(WIN)]
            prob = jnp.concatenate([lg[2 * h], lg[2 * h + 1]], axis=1)
            for c in range(2):
                v = jnp.stack([VA[p][t + c * NP, r, :] for r in rows])
                mixed[t, h, c] = jnp.sum(prob * v, axis=0)
            return [mixed[t, h, c] for c in range(2)]

        def store(t):
            return store_lhs(O[n], t, i * RC + off,
                             *[mixed[t, h, c] for h in range(2) for c in range(2)])

        t_score, d_score, lag1, lag2, lag3, t_mix, d_mix, d_store = times
        tasks = []
        for u in range(4):
            t = t_score + d_score * (2 * u + 1)
            tasks += [(t - d_score, lambda u=u: scores(u, range(4))),
                      (t, lambda u=u: scores(u, range(4, 8))),
                      (t + lag1, lambda u=u: exchange(u, 1)),
                      (t + lag2, lambda u=u: exchange(u, 16)),
                      (t + lag3, lambda u=u: softmax(u))]
        for k in range(NP):
            t = t_mix + k * (d_mix + d_store)
            tasks += [(t, lambda k=k: mix(k, 0)), (t + d_mix, lambda k=k: mix(k, 1))]
            tasks += [(t + d_mix + d_store / 2, lambda k=k: store(k))]
        return tasks

    def att_b_piece(n, i, j, mem, tok):
        p = n % 2
        nk = 128 * j + 32
        shared = ((32, 1, 3), (64, 2, 2), (96, 3, 1))
        key, lane = _iota((32, 128), 0), _iota((32, 128), 1)
        causal = [jnp.where(key > q, MASKVAL, 0.0) for q in (lane, lane ^ 96)]
        even = [_iota((8, 128), 1) >= lo for lo, _, _ in shared]

        def place(parts):
            zero = jnp.zeros((16, 128), U32)
            return jnp.concatenate([parts.get(hh, zero) for hh in range(4)], axis=0)

        q = [[after(QT[p][i + h * NP, pl.ds(16 * hh, 16), _tile(j)], {0: tok}) for hh in range(4)]
             for h in range(2)]
        s = []
        for h in range(2):
            w = jnp.concatenate([place({hh: q[h][hh]}) for hh in range(4)], axis=1)
            st = _dot(_bf(KB[p][i, pl.ds(0, nk // 2), _tile(h)]), _bf(w))
            for hh in range(4):
                v = st[:, 128 * hh:128 * (hh + 1)]
                s.append([v[128 * c:128 * (c + 1)] for c in range(j)]
                         + [v[128 * j:] + causal[hh % 2]])
        sx = [[] for _ in range(4)]
        for lo, ce, co in shared:
            ahead = jnp.where(lane >= lo, key + 32 * ce - lane, key + 32 * co - (lane ^ 96))
            mask = jnp.where(ahead > 0, MASKVAL, 0.0)
            high = _iota((16, 128), 1) >= lo
            for h in range(2):
                ke, ko = (KB[p][i, pl.ds(64 * j + 16 * c, 16), _tile(h)] for c in (ce, co))
                k = ke if ce == co else jnp.where((_iota((16, 128), 1) & 32) == 0, ke, ko)
                w = jnp.concatenate(
                    [place({hh: jnp.where(high, q[h][hh], jnp.uint32(0)),
                            hh + 1: jnp.where(high, jnp.uint32(0), q[h][hh + 1])})
                     for hh in (0, 2)], axis=1)
                st = _dot(_bf(k), _bf(w))
                for u in range(2):
                    sx[2 * h + u].append(st[:, 128 * u:128 * (u + 1)] + mask)
        first = token(*[v[0][:8] for v in s])
        m = []
        for u in range(4):
            a = [_tree(jnp.maximum, [_fold(jnp.max, v) for v in s[2 * u + odd]]) for odd in range(2)]
            for sel, v in zip(even, sx[u]):
                mx = _fold(jnp.max, v)
                a = [jnp.where(sel, jnp.maximum(a[0], mx), a[0]),
                     jnp.where(sel, a[1], jnp.maximum(a[1], mx))]
            m += [jnp.broadcast_to(jnp.max(v, axis=0, keepdims=True), (8, 128)) for v in a]
        e = [[] for _ in range(8)]
        part = [[] for _ in range(8)]

        def exps(v, mh, tok):
            mh = mh + pltpu.bitcast(tok, F32)
            return jnp.exp2(v.reshape(-1, 8, 128) - mh[None]).reshape(v.shape)

        def collect(u, v):
            part[u] = [_tree(jnp.add, part[u] + [_fold(jnp.sum, v)])]
            e[u].append(v)

        def exp_tile(u, c, tok):
            collect(u, exps(s[u][c], m[u], tok))

        def exp_diag(u, tok):
            for odd in range(2):
                exp_tile(2 * u + odd, j, tok)
            v = [exps(a, jnp.where(sel, m[2 * u], m[2 * u + 1]), tok) for sel, a in zip(even, sx[u])]
            collect(2 * u, jnp.concatenate(
                [jnp.where(lane >= shared[c][0], v[c], 0.0) for c in (0, 1, 2)], axis=0))
            collect(2 * u + 1, jnp.concatenate(
                [jnp.where(lane >= shared[c][0], 0.0, v[c]) for c in (2, 1, 0)], axis=0))

        def finish(h, tok):
            g = i + h * NP
            ot = []
            for hh in range(4):
                u = 4 * h + hh
                vt = after(VT[p][g, pl.ds(16 * hh, 16), pl.ds(0, 128 * (j + 1))], {0: tok})
                acc = _dot(_bf(vt), jnp.concatenate(e[u], axis=0).astype(BF16))
                l = jnp.sum(part[u][0], axis=0, keepdims=True)
                gate = gtab[pl.ds(4 * g + hh, 1), :]
                acc = acc * ((1.0 - gate) / l)
                if hh % 2:
                    acc = jnp.where((lane & 32) == 0, pltpu.roll(acc, 32, 1), pltpu.roll(acc, 96, 1))
                if n % NSEG:
                    r = mem[h][:, 128 * j:128 * (j + 1)]
                    den = r[128 + 4 * hh:129 + 4 * hh] + 1e-6
                    acc = acc + r[32 * hh:32 * hh + 32] * (gate / den)
                ot.append(acc)
            return ot

        tasks = []
        for u in range(4):
            tasks += [lambda tok, u=2 * u + odd, c=c: exp_tile(u, c, tok)
                      for odd in range(2) for c in range(j)]
            tasks.append(lambda tok, u=u: exp_diag(u, tok))
        return first, tasks, finish

    def mem_load(n, g):
        if n % NSEG == 0:
            return jnp.zeros((MZ_ROWS, 128), F32)
        return mz[g]

    def mem_read(n, i, h, state, tok):
        pq = after(PQ[n % 2][i, :, _tile(h)], {8 * u: tok for u in range(4)})
        return _dot_nt(state.astype(BF16), _bf(pq))

    def mem_update(n, i, h, state, tok):
        p, g = n % 2, i + h * NP
        z = jnp.sum(ZS[p][g], axis=0, keepdims=True)
        new = jnp.concatenate([_dot(_bf(after(VT[p][g], {0: tok})), _bf(PK[p][i, :, _tile(h)])),
                               jnp.broadcast_to(z, (MZ_ROWS - 128, 128))], axis=0)
        row = _iota((MZ_ROWS, 128), 0)
        row_head = jnp.where(row < 128, row >> 5, (row - 128) >> 2)
        keep = row_head == (_iota((MZ_ROWS, 128), 1) >> 5)
        mz[g] = new = state + jnp.where(keep, new, 0.0)
        return new

    def is_a(n):
        return (n // NSEG) % 2 == 0

    def run_timed(mm, tasks):
        tasks = sorted(tasks, key=lambda x: x[0])
        for k, prod in enumerate(mm):
            toks = {}
            while tasks and tasks[0][0] < 16 * (k + 1):
                time, f = tasks.pop(0)
                join(toks, time - 16 * k, token(*f()))
            prod(toks)
        for _, f in tasks:
            f()

    def body_b(n, i, mm, ln):
        times = {LAST - 1: B_END1, LAST: B_END2}.get(
            n, (B_FIRST, B_PLAIN, B_PLAIN, B_THEN_A)[n % NSEG])
        share, (front, lag, tail, pitch) = times[:4], times[4:8]
        state = [mem_load(n, i + h * NP) for h in range(2)]
        late = [f for off in range(0, RC, 16) for f in ln_tasks(n + 2, i, off)] if ln else []
        mem, tiles, done = [], {}, []

        def values(j, finish, tok):
            posts = []
            for h in range(2):
                ot = finish(h, tok)

                def post(ot=ot, h=h):
                    tiles[j, h] = jnp.concatenate(ot, axis=0).T
                    return slabs(tiles[j, h], 4)

                posts.append(post)
            if j < 2:
                posts += [lambda r=r: store_lhs(
                    O[n], i, 128 * j + r,
                    *[tiles[j + u, h][r:r + B_STORE] for u in (0, 2) for h in range(2)])
                    for r in range(0, 128, B_STORE)]
            return posts

        tok, pending = token(mm.pop(0)(None)[:8]), None
        for k, j in enumerate((3, 1, 2, 0)):
            first, exps, finish = att_b_piece(n, i, j, mem, tok)
            done += values(*pending, first) if pending else []
            when = [int(32 * share[k] * front * u / len(exps)) for u in range(len(exps))]
            for c in range(share[k]):
                toks = {0: first} if c == 0 else {}
                for slot in times[8:10]:
                    if done and 16 * c + slot >= min(lag, 16 * share[k] - 1):
                        join(toks, slot, token(*done.pop(0)()))
                for slot in times[10:11 if len(late) % 6 in (0, 5) else 12]:
                    if late:
                        join(toks, slot, token(*late.pop(0)()))
                r = mm.pop(0)(toks)
                while exps and when[0] < 32 * (c + 1):
                    exps.pop(0)(token(r[8 * (when[0] - 32 * c):][:8]))
                    when.pop(0)
                tok = token(r[:8])
                if (k, c) == (0, 0) and n % NSEG:
                    mem.extend(mem_read(n, i, h, state[h], tok) for h in range(2))
                    done.append(lambda: [v[:8, 128 * u:128 * u + 128] for v in mem for u in range(4)])
                if (k, c) == (0, 0) and n % NSEG != NSEG - 1:
                    new = [mem_update(n, i, h, state[h], tok) for h in range(2)]
                    done.append(lambda: [v[:8] for v in new])
            pending = (j, finish)
        done += late + values(*pending, token(mm.pop(0)(None)[:8]))
        run_timed(mm, [(tail + pitch * u, f) for u, f in enumerate(done)])

    def step(n, ln=True, proj=(0, 1, 2), att=True, out=(1,), extra=None):
        @pl.loop(0, NP)
        def _(i):
            mm = []
            due.clear()
            for which in (B_MATS if att and not is_a(n) else A_MATS):
                if which in proj:
                    mm += (proj_a if is_a(n + 1) else proj_b)(n + 1, i, which)
                elif which == 3:
                    mm += [f for lag in out for f in out_stage(n - lag, i)]
            if att and not is_a(n):
                body_b(n, i, mm, ln)
                return
            times = (A_PREP if extra else A_FIRST if n == 0 else
                     A_PLAIN if is_a(n + 1) else A_THEN_B)
            fs = extra(i) if extra else []
            tasks = [(u % 4 + A_PREP_WHEN[u // 4] if att else 4 * (u + 1) / (len(fs) + 1), f)
                     for u, f in enumerate(fs)]
            for u, off in enumerate(range(0, RC, 16)):
                if att:
                    tasks += [(u + w, f) for w, f in att_a_tasks(n, i, off, times[:8])]
                if ln:
                    when = times[8:] if att else (.15, .4, .7, .8, .9, 1.0)
                    tasks += [(u + w, f) for w, f in zip(when, ln_tasks(n + 2, i, off))]
            run_timed(mm, [(int(4 * len(mm) * w), f) for w, f in tasks])

    for i in range(NP):
        start(x0_copies(i))
    start(slab_copies(0, 0))
    start([copy(beta_hbm, beta_ref.at[0], sem_b)])
    zero_ref[:8] = jnp.zeros((8, 128), U32)

    @pl.loop(0, NP)
    def _(i):
        pl.when(i == 2)(lambda: start(slab_copies(0, 1)))
        wait(x0_copies(i))
        for fs in zip(*[ln_tasks(0, i, off) for off in range(0, RC, 16)]):
            for f in fs:
                f()

    start(slab_copies(0, 2))
    wait(slab_copies(0, 0))
    for f in prep_a_cols(0, 0):
        f()

    plan = (([(0, 3), (1, 0)], [(0, 1)]), ([(1, 1), (1, 2)], [(0, 2), (0, 3)]),
            ([(1, 3), (2, 0)], [(1, 0), (1, 1)]), ([(2, 1), (2, 2)], [(1, 2), (1, 3)]))
    for t, (fetch, preps) in enumerate(plan):
        for mi in fetch:
            start(slab_copies(*mi))
        for mi in preps:
            wait(slab_copies(*mi))
        mm = [f for i in range(NP) for f in proj_a(0, i, 0, only=t)]
        fs = [f for group in zip(*[prep_a_cols(*mi) for mi in preps]) for f in group]
        run_timed(mm, [(16 * len(mm) * (u + 1) // (len(fs) + 1), f) for u, f in enumerate(fs)])

    def prep_wv(i):
        pl.when(i == 0)(lambda: start(x_copies(1) + wao_copies()))
        wait(slab_copies(2, i))
        return prep_a_cols(2, i)

    start(slab_copies(2, 3))
    step(-1, ln=False, proj=(1,), att=False, out=(), extra=prep_wv)
    start(x_copies(2))
    start(x_copies(3))
    wait(x_copies(1))
    wait(wao_copies())
    step(-1, proj=(2,), att=False, out=(), extra=prep_a_rows)
    for m in range(4):
        start(wb_copies(m))
    wait([copy(beta_hbm, beta_ref.at[0], sem_b)])
    gate = jax.nn.sigmoid(beta_ref[0].astype(F32))
    eye = _iota((H, H), 0) == _iota((H, H), 1)
    gcol = jnp.sum(jnp.where(eye, jnp.broadcast_to(gate, (H, H)), 0.0), axis=1, keepdims=True)
    gtab[...] = jnp.broadcast_to(gcol, (H, 128))
    wait(x_copies(2))
    step(0, out=())
    wait(x_copies(3))
    for m in range(4):
        wait(wb_copies(m))
    step(1, extra=lambda i: prep_b(0, i) + prep_b(1, i))
    step(2, extra=lambda i: prep_b(2, i) + prep_b(3, i))
    for n in range(3, 14):
        step(n)
    start(out_copies(0))
    step(14, ln=False, out=())
    step(15, ln=False, proj=(), out=(2, 1))
    start(out_copies(1))
    start(out_copies(2))
    due.clear()
    for i in range(NP):
        run_timed(out_stage(LAST, i), [])
        if i >= NP - 2:
            start(out_tile_copies(0, NP - 1) if i == NP - 2 else out_tile_copies(i, 1))
    for s in range(NSEG - 1):
        wait(out_copies(s))
    wait(out_tile_copies(0, NP - 1) + out_tile_copies(NP - 1, 1))


@jax.jit
def pallas_interleave_layers__sliding_local_dilated__memory_aug_infini_attn__prompt_kernel(
    A_x: jax.Array,
    A_wqkv: jax.Array,
    A_wo: jax.Array,
    B_x: jax.Array,
    B_wq: jax.Array,
    B_wk: jax.Array,
    B_wv: jax.Array,
    B_wo: jax.Array,
    B_beta: jax.Array,
):
    del B_x
    assert A_x.shape == (1, S, D)
    hbm = pl.BlockSpec(memory_space=pl.ANY)
    scratch = (
        [pltpu.VMEM((L, D), BF16)] * 4
        + [pltpu.VMEM((7, D, D), BF16), pltpu.VMEM((NT, D, 128), BF16),
           pltpu.VMEM((2, 576, 128), U32),
           *[pltpu.VMEM((1, NP, D // 4, 7 * 128), U32)] * 4,
           pltpu.VMEM((4, NP, D // 4, 7 * 128), U32)]
        + [pltpu.VMEM((NP, HL // 2, 7 * 128), U32)] * 5
        + [pltpu.VMEM((NT, L, 128), F32)] * 2
        + [pltpu.VMEM((NT, HALO + L, 128), F32)] * 4
        + [pltpu.VMEM((NP, L // 2, 2 * 128), U32)] * 6
        + [pltpu.VMEM((NT, 64, L), U32)] * 4
        + [pltpu.VMEM((NT, 16, 128), F32)] * 2
        + [pltpu.VMEM((NT, MZ_ROWS, 128), F32), pltpu.VMEM((8, 1, H), BF16),
           pltpu.VMEM((H, 128), F32),
           pltpu.VMEM((88, 128), U32),
           pltpu.SemaphoreType.DMA((NSEG,)), pltpu.SemaphoreType.DMA((5,)),
           pltpu.SemaphoreType.DMA((4, NP)),
           pltpu.SemaphoreType.DMA((NSEG,)), pltpu.SemaphoreType.DMA]
    )
    out = pl.pallas_call(
        _kernel,
        out_shape=jax.ShapeDtypeStruct((S, D), BF16),
        in_specs=[hbm] * 8,
        out_specs=hbm,
        scratch_shapes=scratch,
        compiler_params=pltpu.CompilerParams(vmem_limit_bytes=110 * 2**20),
        name="abab_stack",
    )(A_x.reshape(S, D), A_wqkv, A_wo, B_wq, B_wk, B_wv, B_wo, B_beta.reshape(1, H))
    return out.reshape(1, S, D)
```

```python
import jax
import jax.numpy as jnp
from jax import lax
import jax.experimental.pallas as pl
import jax.experimental.pallas.tpu as pltpu

S, D, H, DH = 2048, 1024, 32, 32
NSEG, L = 4, 512
HL = L // 2
NT = D // 128
NP = NT // 2
RC = HL // NP
KC = D // 2 // NP
LAST = 4 * NSEG - 1
WIN, DIL = 8, 2
HALO = 16
MZ_ROWS = 128 + 16
LOG2E = 1.4426950408889634
QSCALE = float(DH ** -0.5 * LOG2E)
MASKVAL = float(-1e9 * LOG2E)

A_MATS = (3, 0, 2, 1)
B_MATS = (2, 0, 1, 3)
B_PLAIN = (7, 6, 7, 4, 0.742, 28, 44, 4, 6, 14, 4, 7)
B_FIRST = (7, 7, 6, 4, 0.749, 26, 42, 0, 7, 15, 4, 9)
B_THEN_A = (7, 7, 6, 3, 0.794, 27, 42, 0, 8, 15, 6, 7)
B_END1 = (3, 2, 9, 3, 0.897, 30, 32, 1, 4, 15, 1, 8)
B_END2 = (4, 3, 2, 1, 0.835, 29, 28, 3, 7, 14, 5, 13)
B_STORE = 64
T_DUE = 36
A_PLAIN = (0.051, 0.047, 0.045, 0.147, 0.306, 0.657, 0.032, 0.045, 0.027, 0.292, 0.473, 0.542, 0.553, 0.57)
A_FIRST = (0.046, 0.036, 0.117, 0.227, 0.285, 0.607, 0.039, 0.04, 0.013, 0.337, 0.462, 0.489, 0.55, 0.591)
A_THEN_B = (0.055, 0.036, 0.095, 0.18, 0.201, 0.589, 0.024, 0.089, 0.074, 0.297, 0.447, 0.493, 0.503, 0.69)
A_PREP = (0.073, 0.047, 0.083, 0.179, 0.2, 0.65, 0.025, 0.039, 0.031, 0.39, 0.455, 0.512, 0.519, 0.553)
A_PREP_WHEN = (0.33, 0.283, 0.412, 0.445, 0.343, 0.481, 0.556, 0.582)

F32, BF16, U32 = jnp.float32, jnp.bfloat16, jnp.uint32
_NT_DIMS = (((1,), (1,)), ((), ()))


def _iota(shape, axis):
    return lax.broadcasted_iota(jnp.int32, shape, axis)


def _dot(a, b):
    return jnp.dot(a, b, preferred_element_type=F32)


def _dot_nt(a, b):
    return lax.dot_general(a, b, _NT_DIMS, preferred_element_type=F32)


def _rows(start, size):
    return pl.ds(start if isinstance(start, int) else pl.multiple_of(start, size), size)


def _tile(k):
    return _rows(128 * k, 128)


def _words(val):
    return pltpu.bitcast(val.astype(BF16), U32)


def _bf(words):
    return pltpu.bitcast(words, BF16)


def _phi(t):
    return jnp.where(t > 0, t + 1.0, jnp.exp(t))


def _tree(op, xs):
    xs = list(xs)
    while len(xs) > 1:
        xs = [op(xs[i], xs[i + 1]) if i + 1 < len(xs) else xs[i]
              for i in range(0, len(xs), 2)]
    return xs[0]


def _fold(reduce, val):
    return reduce(val.reshape(-1, 8, 128), axis=0)


def _halve(op, val):
    while val.shape[0] > 1:
        val = op(val[:val.shape[0] // 2], val[val.shape[0] // 2:])
    return val


def _lhs_terms(a11, a12, a21, a22):
    return (a11 + a22, a21 + a22, a11, a22, a11 + a12, a21 - a11, a12 - a22)


def _rhs_terms(b11, b12, b21, b22):
    return (b11 + b22, b11, b12 - b22, b21 - b11, b22, b11 + b12, b21 + b22)


def _kernel(x_hbm, wqkv_hbm, awo_hbm, wq_hbm, wk_hbm, wv_hbm, wo_hbm, beta_hbm,
            out_hbm,
            x0, x1, x2, x3, wraw, wraw_o, wtmp, waq, wak, wav, wao, wb,
            xn0, xn1, o0, o1, o2,
            qa0, qa1, ka0, ka1, va0, va1,
            pq0, pq1, kb0, kb1, pk0, pk1, qt0, qt1, vt0, vt1,
            zs0, zs1, mz, beta_ref, gtab, zero_ref, sem_x, sem_w, sem_s, sem_o, sem_b):
    X = (x0, x1, x2, x3)
    XN, wa = (xn0, xn1), (waq, wak, wav)
    O = [o2 if n == LAST else (o0, o1)[n % 2] for n in range(LAST + 1)]
    QA, KA, VA = (qa0, qa1), (ka0, ka1), (va0, va1)
    QT, PQ, KB, PK, VT = (qt0, qt1), (pq0, pq1), (kb0, kb1), (pk0, pk1), (vt0, vt1)
    ZS = (zs0, zs1)

    copy = pltpu.make_async_copy

    def x_copies(s):
        return [copy(x_hbm.at[pl.ds(s * L, L)], X[s], sem_x.at[s])]

    def out_copies(s):
        return [copy(X[s], out_hbm.at[pl.ds(s * L, L)], sem_o.at[s])]

    def out_tile_copies(t0, nt):
        cols = [pl.ds(128 * (t0 + c * NP), 128 * nt) for c in range(2)]
        return [copy(x3.at[:, c], out_hbm.at[pl.ds(S - L, L), c], sem_o.at[NSEG - 1]) for c in cols]

    def wao_copies():
        return [copy(awo_hbm.at[:, _tile(t)], wraw_o.at[t], sem_w.at[4]) for t in range(NT)]

    def wb_copies(m):
        return [copy((wq_hbm, wk_hbm, wv_hbm, wo_hbm)[m], wraw.at[3 + m], sem_w.at[m])]

    def slab_copies(m, i):
        return [copy(wqkv_hbm.at[r, _rows(m * D, D)], wraw.at[m, r], sem_s.at[m, i])
                for r in (_rows(h * (D // 2) + i * KC, KC) for h in range(2))]

    def x0_copies(i):
        return [copy(x_hbm.at[r], x0.at[r], sem_s.at[3, i])
                for r in (_rows(h * HL + i * RC, RC) for h in range(2))]

    def start(cs):
        for c in cs:
            c.start()

    def wait(cs):
        for c in cs:
            c.wait()

    def token(*vals):
        val = jnp.concatenate(vals, axis=0)
        val = _fold(jnp.max, val if val.dtype == F32 else pltpu.bitcast(val, F32))
        return pltpu.bitcast(val, U32) & zero_ref[:8]

    def slabs(val, every=1):
        return [val[u - 8:u] for u in range(val.shape[0], 0, -8 * every)]

    def after(words, toks):
        parts, done = [], 0
        for k in sorted(k for k, tok in (toks or {}).items() if tok is not None):
            tok = jnp.concatenate([toks[k]] * (words.shape[1] // 128), axis=1)
            parts += [words[done:8 * k]] * (done < 8 * k) + [words[8 * k:8 * k + 8] | tok]
            done = 8 * k + 8
        parts += [words[done:]] * (done < words.shape[0])
        return jnp.concatenate(parts, axis=0)

    def store_rhs(dst, m, i, r, b11, b12, b21, b22):
        terms = _rhs_terms(*[_bf(b).astype(F32) for b in (b11, b12, b21, b22)])
        words = [{1: b11, 4: b22}[k] if k in (1, 4) else _words(v) for k, v in enumerate(terms)]
        dst[m, i, _rows(r >> 1, b11.shape[0]), :] = jnp.concatenate(words, axis=1)
        return words

    def raw_words(m, r, tiles):
        rows = [_rows(r + h * (D // 2), 32) for h in range(2)]
        return [[pltpu.bitcast(wraw[m, rr, _tile(t)], U32) for t in tiles] for rr in rows]

    def prep_b(m, i):
        def piece(j, c):
            top, bottom = raw_words(3 + m, i * KC + 32 * c, (j, j + NP))
            return store_rhs(wb, m, j, i * KC + 32 * c, *top, *bottom)

        return [lambda j=j, c=c: piece(j, c) for j in range(NP) for c in range(KC // 32)]

    def prep_a_cols(m, i):
        rows = 32
        st = {}

        def rotate(c):
            v = [jnp.concatenate(x, axis=0)
                 for x in zip(*raw_words(m, i * KC + c * rows, range(NT)))]
            st[c] = [x if t == 0 else pltpu.roll(x, 2 * t, 1) for t, x in enumerate(v)]
            return [x[24:] for x in st[c]]

        def shear(c):
            slot = (_iota((rows, 128), 1) >> 1) & 7
            v = [st[c][(-b) % NT] for b in range(NT)]
            for bit in (1, 2, 4):
                sel = (slot & bit) != 0
                v = [jnp.where(sel, v[(b - bit) % NT], v[b]) for b in range(NT)]
            st[c] = [x if b == 0 else pltpu.roll(x, 128 - 2 * b, 1) for b, x in enumerate(v)]
            return [x[16:] for x in v]

        def terms(c):
            v, half, outs = st[c], rows // 2, []
            for j in range(NP):
                outs += store_rhs(wa[m], 0, j, i * KC + c * rows, v[j][:half], v[j + NP][:half],
                                  v[j][half:], v[j + NP][half:])
            return outs

        order = [(f, k - lag) for k in range(6) for lag, f in enumerate((rotate, shear, terms))
                 if 0 <= k - lag < 4]
        return [lambda f=f, c=c: f(c) for f, c in order]

    def prep_a_rows(i):
        def stage(t):
            words = [pltpu.bitcast(wraw_o[i + h * NP, _tile(t), :], U32) for h in range(2)]
            for h in range(2):
                wtmp[h, pl.ds(65 * t, 64), :] = words[h]
            return words

        def rows(h, b, u):
            return jnp.concatenate(
                [wtmp[h, pl.ds(8 * (u + k) + b, 8, stride=65), :] for k in range(2)], axis=0)

        def piece(c, u):
            return store_rhs(wao, 0, i, 128 * c + 16 * u, rows(0, c, u), rows(1, c, u),
                             rows(0, c + NP, u), rows(1, c + NP, u))

        return ([lambda t=t: stage(t) for t in range(NT)]
                + [lambda c=c, u=u: piece(c, u) for c in range(4) for u in range(0, 8, 2)])

    def store_lhs(dst, t, r, a11, a12, a21, a22):
        words = [_words(v) for v in _lhs_terms(a11, a12, a21, a22)]
        dst[t, _rows(r >> 1, a11.shape[0] // 2), :] = jnp.concatenate(words, axis=1)
        return words

    def join(toks, slot, tok):
        if tok is not None:
            toks[slot] = tok if toks.get(slot) is None else toks[slot] | tok

    due = []

    def products(a_ref, w_ref, m, i, emit, only=None):
        st = {}

        def prod(k, toks, finish):
            toks = dict(toks or {})
            while due and due[0][0] < 16:
                slot, vals = due.pop(0)
                join(toks, slot, token(*vals))
            for entry in due:
                entry[0] -= 16
            if only is None:
                a = jnp.concatenate([after(a_ref[t, :, _tile(k)], toks if t == 0 else None)
                                     for t in range(NP)], axis=1)
                w = w_ref[m, i, :, _tile(k)]
            else:
                a = after(a_ref[only, :, _tile(k)], toks)
                w = w_ref[m, i, _rows(64 * only, 64), _tile(k)]
            r = _dot(_bf(a), _bf(w))
            finish(r)
            return r

        def p1(r):
            st["m1"] = r

        def p2(r):
            st["c21"], st["c22"] = r, st["m1"] - r

        def p3(r):
            st["c12"], st["c22"] = r, st["c22"] + r

        def p4(r):
            st["c11"] = st["m1"] + r
            emit(1, 0, st["c21"] + r)

        def p5(r):
            st["c11"] = st["c11"] - r
            emit(0, 1, st["c12"] + r)

        def p6(r):
            emit(1, 1, st["c22"] + r)

        def p7(r):
            emit(0, 0, st["c11"] + r)

        return [lambda toks, k=k, f=f: prod(k, toks, f)
                for k, f in enumerate((p1, p2, p3, p4, p5, p6, p7))]

    def ln_tasks(n, i, off, nr=16):
        src, dst = X[n % NSEG], XN[n % 2]
        st = {}

        def mean():
            x = jnp.concatenate(
                [src[_rows(i * RC + off + h * HL, nr), :].astype(F32) for h in range(2)], axis=0)
            st["x"] = [x[:, 128 * t:128 * (t + 1)] for t in range(NT)]
            part = _tree(jnp.add, st["x"])
            st["mean"] = jnp.sum(part, axis=1, keepdims=True) * (1.0 / D)
            return [part]

        def var():
            st["x"] = [x - st["mean"] for x in st["x"]]
            part = _tree(jnp.add, [x * x for x in st["x"]])
            st["var"] = jnp.sum(part, axis=1, keepdims=True) * (1.0 / D)
            return [part]

        def scale(t):
            if t == 0:
                st["inv"] = lax.rsqrt(st["var"] + 1e-5)
            y0, y1 = st["x"][t] * st["inv"], st["x"][t + NP] * st["inv"]
            return store_lhs(dst, t, i * RC + off, y0[:nr], y1[:nr], y0[nr:], y1[nr:])

        return [mean, var] + [lambda t=t: scale(t) for t in range(NP)]

    def proj_a(n, i, which, only=None):
        p = n % 2

        def emit(h, c, y):
            t = i + c * NP
            buf = (QA, KA, VA)[which]
            rows = pl.ds(h * HL + (HALO if which else 0), HL)
            if only:
                y = y + buf[p][t, rows, :]
            buf[p][t, rows, :] = y
            if which and h == 0 and n % NSEG == 0:
                buf[p][t, pl.ds(0, HALO), :] = jnp.zeros((HALO, 128), F32)
            elif which and h == 0:
                buf[p][t, pl.ds(0, HALO), :] = buf[1 - p][t, pl.ds(L, HALO), :]

        return products(XN[p], wa[which], 0, i, emit, only)

    def proj_b(n, i, which):
        p = n % 2

        def transposed(buf, h, c, y):
            words = pltpu.bitcast(y.astype(BF16).T, U32)
            buf[p][i + c * NP, :, pl.ds(h * HL, HL)] = words
            due.append([T_DUE, slabs(words[:, :128], 2) + slabs(words[:, 128:], 2)])

        def emit(h, c, y):
            wide = (i, pl.ds(h * HL // 2, HL // 2), _tile(c))
            if which == 0:
                if n % NSEG:
                    PQ[p][wide] = _words(_phi(y))
                y = y * QSCALE
                flip = jnp.concatenate([y[r ^ 96:(r ^ 96) + 32] for r in range(0, HL, 32)], axis=0)
                y = jnp.where((_iota(y.shape, 1) & 32) == 0, y, flip)
                transposed(QT, h, c, y)
            elif which == 1:
                KB[p][wide] = _words(y)
                if n % NSEG != NSEG - 1:
                    y = _phi(y)
                    PK[p][wide] = _words(y)
                    ZS[p][i + c * NP, pl.ds(8 * h, 8), :] = _fold(jnp.sum, y)
            else:
                transposed(VT, h, c, y)

        return products(XN[p], wb, which, i, emit)

    def out_stage(n, i):
        x = X[n % NSEG]

        def emit(h, c, y):
            where = (pl.ds(h * HL, HL), _tile(i + c * NP))
            x[where] = (x[where].astype(F32) + y).astype(BF16)

        if is_a(n):
            return products(O[n], wao, 0, i, emit)
        return products(O[n], wb, 3, i, emit)

    def att_a_tasks(n, i, off, times):
        p = n % 2
        base = pl.multiple_of(i * RC, RC) + off
        starts = [base + (u // 2) * HL + 8 * (u % 2) for u in range(4)]
        lg, mixed = [[] for _ in range(4)], {}

        def scores(u, ws):
            q = QA[p][:, pl.ds(starts[u], 8), :]
            for w in ws:
                k = KA[p][:, pl.ds(starts[u] + (HALO - DIL * w), 8), :]
                lg[u].append(_halve(jnp.add, q * k)[0])
            return lg[u][-len(ws):]

        def exchange(u, bit):
            a = jnp.concatenate(lg[u], axis=0)
            low = (_iota(a.shape, 1) & bit) == 0
            lg[u] = [a + jnp.where(low, pltpu.roll(a, 128 - bit, 1), pltpu.roll(a, bit, 1))]
            return lg[u]

        def softmax(u):
            v = (lg[u][0] * QSCALE).reshape(WIN, 8, 128)
            if n % NSEG == 0 and off == 0 and u < 2:
                pos = _iota(v.shape, 1) + starts[u]
                v = jnp.where(pos >= DIL * _iota(v.shape, 0), v, MASKVAL)
            e = jnp.exp2(v - _halve(jnp.maximum, v))
            lg[u] = e * (1.0 / _halve(jnp.add, e))
            return [lg[u].reshape(8 * WIN, 128)]

        def mix(t, h):
            rows = [pl.ds(starts[2 * h] + (HALO - DIL * w), 16) for w in range(WIN)]
            prob = jnp.concatenate([lg[2 * h], lg[2 * h + 1]], axis=1)
            for c in range(2):
                v = jnp.stack([VA[p][t + c * NP, r, :] for r in rows])
                mixed[t, h, c] = _halve(jnp.add, prob * v)[0]
            return [mixed[t, h, c] for c in range(2)]

        def store(t):
            return store_lhs(O[n], t, i * RC + off,
                             *[mixed[t, h, c] for h in range(2) for c in range(2)])

        t_score, d_score, lag1, lag2, lag3, t_mix, d_mix, d_store = times
        tasks = []
        for u in range(4):
            t = t_score + d_score * (2 * u + 1)
            tasks += [(t - d_score, lambda u=u: scores(u, range(4))),
                      (t, lambda u=u: scores(u, range(4, 8))),
                      (t + lag1, lambda u=u: exchange(u, 1)),
                      (t + lag2, lambda u=u: exchange(u, 16)),
                      (t + lag3, lambda u=u: softmax(u))]
        for k in range(NP):
            t = t_mix + k * (d_mix + d_store)
            tasks += [(t, lambda k=k: mix(k, 0)), (t + d_mix, lambda k=k: mix(k, 1))]
            tasks += [(t + d_mix + d_store / 2, lambda k=k: store(k))]
        return tasks

    def att_b_piece(n, i, j, mem, tok):
        p = n % 2
        nk = 128 * j + 32
        shared = ((32, 1, 3), (64, 2, 2), (96, 3, 1))
        key, lane = _iota((32, 128), 0), _iota((32, 128), 1)
        causal = [jnp.where(key > q, MASKVAL, 0.0) for q in (lane, lane ^ 96)]
        even = [_iota((8, 128), 1) >= lo for lo, _, _ in shared]

        def place(parts):
            zero = jnp.zeros((16, 128), U32)
            return jnp.concatenate([parts.get(hh, zero) for hh in range(4)], axis=0)

        q = [[after(QT[p][i + h * NP, pl.ds(16 * hh, 16), _tile(j)], {0: tok}) for hh in range(4)]
             for h in range(2)]
        s = []
        for h in range(2):
            w = jnp.concatenate([place({hh: q[h][hh]}) for hh in range(4)], axis=1)
            st = _dot(_bf(KB[p][i, pl.ds(0, nk // 2), _tile(h)]), _bf(w))
            for hh in range(4):
                v = st[:, 128 * hh:128 * (hh + 1)]
                s.append([v[128 * c:128 * (c + 1)] for c in range(j)]
                         + [v[128 * j:] + causal[hh % 2]])
        sx = [[] for _ in range(4)]
        for lo, ce, co in shared:
            ahead = jnp.where(lane >= lo, key + 32 * ce - lane, key + 32 * co - (lane ^ 96))
            mask = jnp.where(ahead > 0, MASKVAL, 0.0)
            high = _iota((16, 128), 1) >= lo
            for h in range(2):
                ke, ko = (KB[p][i, pl.ds(64 * j + 16 * c, 16), _tile(h)] for c in (ce, co))
                k = ke if ce == co else jnp.where((_iota((16, 128), 1) & 32) == 0, ke, ko)
                w = jnp.concatenate(
                    [place({hh: jnp.where(high, q[h][hh], jnp.uint32(0)),
                            hh + 1: jnp.where(high, jnp.uint32(0), q[h][hh + 1])})
                     for hh in (0, 2)], axis=1)
                st = _dot(_bf(k), _bf(w))
                for u in range(2):
                    sx[2 * h + u].append(st[:, 128 * u:128 * (u + 1)] + mask)
        first = token(*[v[0][:8] for v in s])
        m = []
        for u in range(4):
            a = [_tree(jnp.maximum, [_fold(jnp.max, v) for v in s[2 * u + odd]]) for odd in range(2)]
            for sel, v in zip(even, sx[u]):
                mx = _fold(jnp.max, v)
                a = [jnp.where(sel, jnp.maximum(a[0], mx), a[0]),
                     jnp.where(sel, a[1], jnp.maximum(a[1], mx))]
            m += [jnp.broadcast_to(jnp.max(v, axis=0, keepdims=True), (8, 128)) for v in a]
        e = [[] for _ in range(8)]
        part = [[] for _ in range(8)]

        def exps(v, mh, tok):
            mh = mh + pltpu.bitcast(tok, F32)
            return jnp.exp2(v.reshape(-1, 8, 128) - mh[None]).reshape(v.shape)

        def collect(u, v):
            part[u] = [_tree(jnp.add, part[u] + [_fold(jnp.sum, v)])]
            e[u].append(v)

        def exp_tile(u, c, tok):
            collect(u, exps(s[u][c], m[u], tok))

        def exp_diag(u, tok):
            for odd in range(2):
                exp_tile(2 * u + odd, j, tok)
            v = [exps(a, jnp.where(sel, m[2 * u], m[2 * u + 1]), tok) for sel, a in zip(even, sx[u])]
            collect(2 * u, jnp.concatenate(
                [jnp.where(lane >= shared[c][0], v[c], 0.0) for c in (0, 1, 2)], axis=0))
            collect(2 * u + 1, jnp.concatenate(
                [jnp.where(lane >= shared[c][0], 0.0, v[c]) for c in (2, 1, 0)], axis=0))

        def finish(h, tok):
            g = i + h * NP
            ot = []
            for hh in range(4):
                u = 4 * h + hh
                vt = after(VT[p][g, pl.ds(16 * hh, 16), pl.ds(0, 128 * (j + 1))], {0: tok})
                acc = _dot(_bf(vt), jnp.concatenate(e[u], axis=0).astype(BF16))
                l = jnp.sum(part[u][0], axis=0, keepdims=True)
                gate = gtab[pl.ds(4 * g + hh, 1), :]
                acc = acc * ((1.0 - gate) / l)
                if hh % 2:
                    acc = jnp.where((lane & 32) == 0, pltpu.roll(acc, 32, 1), pltpu.roll(acc, 96, 1))
                if n % NSEG:
                    r = mem[h][:, 128 * j:128 * (j + 1)]
                    den = r[128 + 4 * hh:129 + 4 * hh] + 1e-6
                    acc = acc + r[32 * hh:32 * hh + 32] * (gate / den)
                ot.append(acc)
            return ot

        tasks = []
        for u in range(4):
            tasks += [lambda tok, u=2 * u + odd, c=c: exp_tile(u, c, tok)
                      for odd in range(2) for c in range(j)]
            tasks.append(lambda tok, u=u: exp_diag(u, tok))
        return first, tasks, finish

    def mem_load(n, g):
        if n % NSEG == 0:
            return jnp.zeros((MZ_ROWS, 128), F32)
        return mz[g]

    def mem_read(n, i, h, state, tok):
        pq = after(PQ[n % 2][i, :, _tile(h)], {8 * u: tok for u in range(4)})
        return _dot_nt(state.astype(BF16), _bf(pq))

    def mem_update(n, i, h, state, tok):
        p, g = n % 2, i + h * NP
        z = jnp.sum(ZS[p][g], axis=0, keepdims=True)
        new = jnp.concatenate([_dot(_bf(after(VT[p][g], {0: tok})), _bf(PK[p][i, :, _tile(h)])),
                               jnp.broadcast_to(z, (MZ_ROWS - 128, 128))], axis=0)
        row = _iota((MZ_ROWS, 128), 0)
        row_head = jnp.where(row < 128, row >> 5, (row - 128) >> 2)
        keep = row_head == (_iota((MZ_ROWS, 128), 1) >> 5)
        mz[g] = new = state + jnp.where(keep, new, 0.0)
        return new

    def is_a(n):
        return (n // NSEG) % 2 == 0

    def run_timed(mm, tasks):
        tasks = sorted(tasks, key=lambda x: x[0])
        for k, prod in enumerate(mm):
            toks = {}
            while tasks and tasks[0][0] < 16 * (k + 1):
                time, f = tasks.pop(0)
                join(toks, time - 16 * k, token(*f()))
            prod(toks)
        for _, f in tasks:
            f()

    def body_b(n, i, mm, ln):
        times = {LAST - 1: B_END1, LAST: B_END2}.get(
            n, (B_FIRST, B_PLAIN, B_PLAIN, B_THEN_A)[n % NSEG])
        share, (front, lag, tail, pitch) = times[:4], times[4:8]
        state = [mem_load(n, i + h * NP) for h in range(2)]
        late = [f for off in range(0, RC, 16) for f in ln_tasks(n + 2, i, off)] if ln else []
        mem, tiles, done = [], {}, []

        def values(j, finish, tok):
            posts = []
            for h in range(2):
                ot = finish(h, tok)

                def post(ot=ot, h=h):
                    tiles[j, h] = jnp.concatenate(ot, axis=0).T
                    return slabs(tiles[j, h], 4)

                posts.append(post)
            if j < 2:
                posts += [lambda r=r: store_lhs(
                    O[n], i, 128 * j + r,
                    *[tiles[j + u, h][r:r + B_STORE] for u in (0, 2) for h in range(2)])
                    for r in range(0, 128, B_STORE)]
            return posts

        tok, pending = token(mm.pop(0)(None)[:8]), None
        for k, j in enumerate((3, 1, 2, 0)):
            first, exps, finish = att_b_piece(n, i, j, mem, tok)
            done += values(*pending, first) if pending else []
            when = [int(32 * share[k] * front * u / len(exps)) for u in range(len(exps))]
            for c in range(share[k]):
                toks = {0: first} if c == 0 else {}
                for slot in times[8:10]:
                    if done and 16 * c + slot >= min(lag, 16 * share[k] - 1):
                        join(toks, slot, token(*done.pop(0)()))
                for slot in times[10:11 if len(late) % 6 in (0, 5) else 12]:
                    if late:
                        join(toks, slot, token(*late.pop(0)()))
                r = mm.pop(0)(toks)
                while exps and when[0] < 32 * (c + 1):
                    exps.pop(0)(token(r[8 * (when[0] - 32 * c):][:8]))
                    when.pop(0)
                tok = token(r[:8])
                if (k, c) == (0, 0) and n % NSEG:
                    mem.extend(mem_read(n, i, h, state[h], tok) for h in range(2))
                    done.append(lambda: [v[:8, 128 * u:128 * u + 128] for v in mem for u in range(4)])
                if (k, c) == (0, 0) and n % NSEG != NSEG - 1:
                    new = [mem_update(n, i, h, state[h], tok) for h in range(2)]
                    done.append(lambda: [v[:8] for v in new])
            pending = (j, finish)
        done += late + values(*pending, token(mm.pop(0)(None)[:8]))
        run_timed(mm, [(tail + pitch * u, f) for u, f in enumerate(done)])

    def step(n, ln=True, proj=(0, 1, 2), att=True, out=(1,), extra=None):
        @pl.loop(0, NP)
        def _(i):
            mm = []
            due.clear()
            for which in (B_MATS if att and not is_a(n) else A_MATS):
                if which in proj:
                    mm += (proj_a if is_a(n + 1) else proj_b)(n + 1, i, which)
                elif which == 3:
                    mm += [f for lag in out for f in out_stage(n - lag, i)]
            if att and not is_a(n):
                body_b(n, i, mm, ln)
                return
            times = (A_PREP if extra else A_FIRST if n == 0 else
                     A_PLAIN if is_a(n + 1) else A_THEN_B)
            fs = extra(i) if extra else []
            tasks = [(u % 4 + A_PREP_WHEN[u // 4] if att else 4 * (u + 1) / (len(fs) + 1), f)
                     for u, f in enumerate(fs)]
            for u, off in enumerate(range(0, RC, 16)):
                if att:
                    tasks += [(u + w, f) for w, f in att_a_tasks(n, i, off, times[:8])]
                if ln:
                    when = times[8:] if att else (.15, .4, .7, .8, .9, 1.0)
                    tasks += [(u + w, f) for w, f in zip(when, ln_tasks(n + 2, i, off))]
            run_timed(mm, [(int(4 * len(mm) * w), f) for w, f in tasks])

    for i in range(NP):
        start(x0_copies(i))
    start(slab_copies(0, 0))
    start([copy(beta_hbm, beta_ref.at[0], sem_b)])
    zero_ref[:8] = jnp.zeros((8, 128), U32)

    @pl.loop(0, NP)
    def _(i):
        pl.when(i == 2)(lambda: start(slab_copies(0, 1)))
        wait(x0_copies(i))
        for fs in zip(*[ln_tasks(0, i, off) for off in range(0, RC, 16)]):
            for f in fs:
                f()

    start(slab_copies(0, 2))
    wait(slab_copies(0, 0))
    for f in prep_a_cols(0, 0):
        f()

    plan = (([(0, 3), (1, 0)], [(0, 1)]), ([(1, 1), (1, 2)], [(0, 2), (0, 3)]),
            ([(1, 3), (2, 0)], [(1, 0), (1, 1)]), ([(2, 1), (2, 2)], [(1, 2), (1, 3)]))
    for t, (fetch, preps) in enumerate(plan):
        for mi in fetch:
            start(slab_copies(*mi))
        for mi in preps:
            wait(slab_copies(*mi))
        mm = [f for i in range(NP) for f in proj_a(0, i, 0, only=t)]
        fs = [f for group in zip(*[prep_a_cols(*mi) for mi in preps]) for f in group]
        run_timed(mm, [(16 * len(mm) * (u + 1) // (len(fs) + 1), f) for u, f in enumerate(fs)])

    def prep_wv(i):
        pl.when(i == 0)(lambda: start(x_copies(1) + wao_copies()))
        wait(slab_copies(2, i))
        return prep_a_cols(2, i)

    start(slab_copies(2, 3))
    step(-1, ln=False, proj=(1,), att=False, out=(), extra=prep_wv)
    start(x_copies(2))
    start(x_copies(3))
    wait(x_copies(1))
    wait(wao_copies())
    step(-1, proj=(2,), att=False, out=(), extra=prep_a_rows)
    for m in range(4):
        start(wb_copies(m))
    wait([copy(beta_hbm, beta_ref.at[0], sem_b)])
    gate = jax.nn.sigmoid(beta_ref[0].astype(F32))
    eye = _iota((H, H), 0) == _iota((H, H), 1)
    gcol = jnp.sum(jnp.where(eye, jnp.broadcast_to(gate, (H, H)), 0.0), axis=1, keepdims=True)
    gtab[...] = jnp.broadcast_to(gcol, (H, 128))
    wait(x_copies(2))
    step(0, out=())
    wait(x_copies(3))
    for m in range(4):
        wait(wb_copies(m))
    step(1, extra=lambda i: prep_b(0, i) + prep_b(1, i))
    step(2, extra=lambda i: prep_b(2, i) + prep_b(3, i))
    for n in range(3, 14):
        step(n)
    start(out_copies(0))
    step(14, ln=False, out=())
    step(15, ln=False, proj=(), out=(2, 1))
    start(out_copies(1))
    start(out_copies(2))
    due.clear()
    for i in range(NP):
        run_timed(out_stage(LAST, i), [])
        if i >= NP - 2:
            start(out_tile_copies(0, NP - 1) if i == NP - 2 else out_tile_copies(i, 1))
    for s in range(NSEG - 1):
        wait(out_copies(s))
    wait(out_tile_copies(0, NP - 1) + out_tile_copies(NP - 1, 1))


@jax.jit
def pallas_interleave_layers__sliding_local_dilated__memory_aug_infini_attn__prompt_kernel(
    A_x: jax.Array,
    A_wqkv: jax.Array,
    A_wo: jax.Array,
    B_x: jax.Array,
    B_wq: jax.Array,
    B_wk: jax.Array,
    B_wv: jax.Array,
    B_wo: jax.Array,
    B_beta: jax.Array,
):
    del B_x
    assert A_x.shape == (1, S, D)
    hbm = pl.BlockSpec(memory_space=pl.ANY)
    scratch = (
        [pltpu.VMEM((L, D), BF16)] * 4
        + [pltpu.VMEM((7, D, D), BF16), pltpu.VMEM((NT, D, 128), BF16),
           pltpu.VMEM((2, 576, 128), U32),
           *[pltpu.VMEM((1, NP, D // 4, 7 * 128), U32)] * 4,
           pltpu.VMEM((4, NP, D // 4, 7 * 128), U32)]
        + [pltpu.VMEM((NP, HL // 2, 7 * 128), U32)] * 5
        + [pltpu.VMEM((NT, L, 128), F32)] * 2
        + [pltpu.VMEM((NT, HALO + L, 128), F32)] * 4
        + [pltpu.VMEM((NP, L // 2, 2 * 128), U32)] * 6
        + [pltpu.VMEM((NT, 64, L), U32)] * 4
        + [pltpu.VMEM((NT, 16, 128), F32)] * 2
        + [pltpu.VMEM((NT, MZ_ROWS, 128), F32), pltpu.VMEM((8, 1, H), BF16),
           pltpu.VMEM((H, 128), F32),
           pltpu.VMEM((88, 128), U32),
           pltpu.SemaphoreType.DMA((NSEG,)), pltpu.SemaphoreType.DMA((5,)),
           pltpu.SemaphoreType.DMA((4, NP)),
           pltpu.SemaphoreType.DMA((NSEG,)), pltpu.SemaphoreType.DMA]
    )
    out = pl.pallas_call(
        _kernel,
        out_shape=jax.ShapeDtypeStruct((S, D), BF16),
        in_specs=[hbm] * 8,
        out_specs=hbm,
        scratch_shapes=scratch,
        compiler_params=pltpu.CompilerParams(vmem_limit_bytes=110 * 2**20),
        name="abab_stack",
    )(A_x.reshape(S, D), A_wqkv, A_wo, B_wq, B_wk, B_wv, B_wo, B_beta.reshape(1, H))
    return out.reshape(1, S, D)
```
